```python
import jax
import jax.numpy as jnp

def _softmax(x, axis=-1):
    return jax.nn.softmax(x, axis=axis)

def _gelu(x):
    return jax.nn.gelu(x, approximate=True)

def _silu(x):
    return jax.nn.silu(x)

def _sigmoid(x):
    return jax.nn.sigmoid(x)

def _layernorm(x, axis=-1, eps=1e-05):
    m = jnp.mean(x, axis=axis, keepdims=True)
    v = jnp.var(x, axis=axis, keepdims=True)
    return (x - m) / jnp.sqrt(v + eps)

def _scatter_add(tgt, idx, src, axis=0):
    return tgt.at[idx].add(src)

def _segment_sum(src, seg, n):
    return jax.ops.segment_sum(src, seg, n)

class _Rng:

    def __init__(self, key):
        self._k = key

    def _next(self):
        self._k, sub = jax.random.split(self._k)
        return sub

    def normal(self, shape):
        return jax.random.normal(self._next(), shape, dtype=jnp.bfloat16)

    def randint(self, lo, hi, shape):
        return jax.random.randint(self._next(), shape, lo, hi, dtype=jnp.int32)

    def uniform(self, shape, lo=0.0, hi=1.0):
        return jax.random.uniform(self._next(), shape, jnp.bfloat16, lo, hi)

    def permutation(self, n):
        return jax.random.permutation(self._next(), n)
kernel_name = 'sequential_preLN__memory_aug_recurrent_mem_tr__mixer_s_mlp__prompt'

def setup_inputs():
    _rng = _Rng(jax.random.key(int.from_bytes(__import__("os").urandom(4), "little")))
    _w = lambda a: (lambda t: t.astype(jnp.bfloat16) if jnp.issubdtype(t.dtype, jnp.floating) else t)(jnp.asarray(a))

    def _A_setup():
        B, S, Dm = (1, 2048, 1024)
        H, Dh = (32, 128)
        M, seg = (8, 32)
        seg = min(seg, S)
        S = S // seg * seg
        return {'x': _w((lambda *s: _rng.normal(s) * 0.05)(B, S, Dm)), 'mem0': _w((lambda *s: _rng.normal(s) * 0.05)(B, M, Dm)), 'Wq': _w((lambda *s: _rng.normal(s) * 0.05)(Dm, H, Dh) * Dm ** (-0.5)), 'Wk': _w((lambda *s: _rng.normal(s) * 0.05)(Dm, H, Dh) * Dm ** (-0.5)), 'Wv': _w((lambda *s: _rng.normal(s) * 0.05)(Dm, H, Dh) * Dm ** (-0.5)), 'Wo': _w((lambda *s: _rng.normal(s) * 0.05)(H, Dh, Dm) * (H * Dh) ** (-0.5)), 'seg_len': seg}
    _A_in = _A_setup()

    def _B_setup():
        B, S, D, F = (1, 2048, 1024, 3584)
        return {'x': _w((lambda *s: _rng.normal(s) * 0.05)(B, S, D)), 'w1': _w((lambda *s: _rng.normal(s) * 0.05)(D, D) * D ** (-0.5)), 'w2': _w((lambda *s: _rng.normal(s) * 0.05)(D, D) * D ** (-0.5)), 'w3': _w((lambda *s: _rng.normal(s) * 0.05)(D, F) * D ** (-0.5)), 'w4': _w((lambda *s: _rng.normal(s) * 0.05)(F, D) * F ** (-0.5))}
    _B_in = _B_setup()
    return {'A_x': _A_in['x'], 'A_mem0': _A_in['mem0'], 'A_Wq': _A_in['Wq'], 'A_Wk': _A_in['Wk'], 'A_Wv': _A_in['Wv'], 'A_Wo': _A_in['Wo'], 'A_seg_len': _A_in['seg_len'], 'B_x': _B_in['x'], 'B_w1': _B_in['w1'], 'B_w2': _B_in['w2'], 'B_w3': _B_in['w3'], 'B_w4': _B_in['w4']}

def reference(A_x, A_mem0, A_Wq, A_Wk, A_Wv, A_Wo, A_seg_len, B_x, B_w1, B_w2, B_w3, B_w4):

    def _A_ref(x, mem0, Wq, Wk, Wv, Wo, seg_len):
        B, S, Dm = x.shape
        H, Dh = (Wq.shape[1], Wq.shape[2])
        M = mem0.shape[1]
        scale = Dh ** (-0.5)
        n_seg = S // seg_len
        L = M + seg_len
        idx = jnp.arange(L)
        mask = (idx[:, None] < M) | (idx[:, None] >= idx[None, :])
        mem = mem0
        outs = []
        for s in range(n_seg):
            xs = x[:, s * seg_len:(s + 1) * seg_len, :].copy()
            h = jnp.concatenate([mem, xs], axis=1)
            q = jnp.einsum('btd,dhe->bhte', h, Wq)
            k = jnp.einsum('btd,dhe->bhte', h, Wk)
            v = jnp.einsum('btd,dhe->bhte', h, Wv)
            scores = jnp.einsum('bhqe,bhke->bhqk', q, k) * scale
            scores = jnp.where(mask[None, None], scores, -1000000000.0)
            p = _softmax(scores, axis=-1)
            o = jnp.einsum('bhqk,bhke->bhqe', p, v)
            o = jnp.einsum('bhte,hed->btd', o, Wo)
            mem = o[:, :M, :].copy()
            outs.append(o[:, M:, :])
        return jnp.concatenate(outs, axis=1)

    def _B_ref(x, w1, w2, w3, w4):
        B, S, D = x.shape
        h = _gelu(_layernorm(x, axis=-1) @ w1)
        c = D // 4
        g0 = jnp.pad(h[:, :, 0 * c:1 * c], ((0, 0), (1, 0), (0, 0)))[:, :S, :]
        g1 = jnp.pad(h[:, :, 1 * c:2 * c], ((0, 0), (0, 1), (0, 0)))[:, 1:, :]
        g2 = jnp.pad(h[:, :, 2 * c:3 * c], ((0, 0), (2, 0), (0, 0)))[:, :S, :]
        g3 = jnp.pad(h[:, :, 3 * c:], ((0, 0), (0, 2), (0, 0)))[:, 2:, :]
        hs = jnp.concatenate([g0, g1, g2, g3], axis=-1) @ w2
        x1 = x + hs
        h2 = _gelu(_layernorm(x1, axis=-1) @ w3) @ w4
        return x1 + h2
    x = A_x
    h = x + _A_ref(_layernorm(x, axis=-1), A_mem0, A_Wq, A_Wk, A_Wv, A_Wo, A_seg_len)
    h2 = h + _B_ref(_layernorm(h, axis=-1), B_w1, B_w2, B_w3, B_w4)
    return h2
```

```python
import functools
import itertools
import os

import jax
import jax.numpy as jnp
from jax import lax
import jax.experimental.pallas as pl
import jax.experimental.pallas.tpu as pltpu

S = 2048
D = 1024
H = 32
DH = 128
MEM = 8
SEG = 32
F = 3584
NSEG = S // SEG
L = MEM + SEG
TOK = 24
P0 = S - TOK * NSEG
RING = 576
XP = (S - P0) // 12
C4 = D // 4
HALO = 8
RB = 256
R = 128
NB = S // (4 * R)
NJ = F // 512
HD = D // 2
E_ = lambda k, d: int(os.environ.get(k, d))
EPS = 1e-5
NEG = -1000000000.0

LAG_QK, LAG_PV, LAG_WO = E_('LQ', 2), E_('LP', 4), E_('LW', 6)
FILL_AT = E_('FA', 18)
UNROLL = 2

bf16 = jnp.bfloat16
f32 = jnp.float32
u32 = jnp.uint32

SEM_X0, SEM_X, SEM_WO, SEM_W1, SEM_W2, SEM_OUT, SEM_W, SEM_W4, SEM_W3 = (
    0, 2, 10, 14, 18, 20, 28, 40, 47)
NSEM = SEM_W3 + 4 * NJ

ENC_A = (((0, 0, 1), (1, 1, 1)), ((1, 0, 1), (1, 1, 1)), ((0, 0, 1),), ((1, 1, 1),),
         ((0, 0, 1), (0, 1, 1)), ((1, 0, 1), (0, 0, -1)), ((0, 1, 1), (1, 1, -1)))
ENC_B = (((0, 0, 1), (1, 1, 1)), ((0, 0, 1),), ((0, 1, 1), (1, 1, -1)),
         ((1, 0, 1), (0, 0, -1)), ((1, 1, 1),), ((0, 0, 1), (0, 1, 1)),
         ((1, 0, 1), (1, 1, 1)))
DEC = (((0, 0, 1), (1, 1, 1)), ((1, 0, 1), (1, 1, -1)), ((0, 1, 1), (1, 1, 1)),
       ((0, 0, 1), (1, 0, 1)), ((0, 1, 1), (0, 0, -1)), ((1, 1, 1),), ((0, 0, 1),))
ORDER = (0, 1, 3, 2, 4, 5, 6)
LAST = {(1, 0): 3, (0, 1): 4, (1, 1): 5, (0, 0): 6}


def _enc(terms, get):
    v = get(*terms[0][:2])
    for i, j, sign in terms[1:]:
        v = v + get(i, j) if sign > 0 else v - get(i, j)
    return v


def _enc2(table, get, emit):
    for g in range(7):
        y = [[_enc(table[g], lambda i1, j1: get(2 * i1 + i0, 2 * j1 + j0))
              for j0 in range(2)] for i0 in range(2)]
        for k in range(7):
            emit(7 * g + k, _enc(table[k], lambda i0, j0: y[i0][j0]))
        yield


def _accumulate(c, key, m, sign):
    c[key] = m if key not in c else (c[key] + m if sign > 0 else c[key] - m)


def _dec(get):
    c = {}
    for k in range(7):
        m = get(k)
        for i, j, sign in DEC[k]:
            _accumulate(c, (i, j), m, sign)
    return c


def _pace(ref, lead, row, result):
    n = 32 // ref.dtype.itemsize
    ref[(*lead, pl.ds(pl.multiple_of(row, n), n), pl.ds(0, 128))] = (
        result[-n:, :128].astype(ref.dtype))


def _run(gen):
    for _ in gen:
        pass


def _mult(i, n):
    return i if isinstance(i, int) else pl.multiple_of(i, n)


def _ln(x):
    m = jnp.mean(x, axis=-1, keepdims=True)
    d = x - m
    v = jnp.mean(d * d, axis=-1, keepdims=True)
    return d * lax.rsqrt(v + EPS)


def _gelu(x):
    c = 0.7978845608028654
    hx = 0.5 * x
    return hx + hx * jnp.tanh(x * (c + (c * 0.044715) * (x * x)))


def _unpack(x):
    return pltpu.bitcast(x, bf16)


def _operand(ref, blocks, rows=slice(None)):
    words = ref.bitcast(u32)
    return _unpack(jnp.concatenate([words[b, rows, :] for b in blocks], axis=1))


def _set_blocks(ref, rows, v):
    for c in range(v.shape[1] // 128):
        ref[c, rows, :] = v[:, 128 * c:128 * c + 128].astype(bf16)


def _dot(a, b):
    return jnp.dot(a, b, preferred_element_type=f32)


def _rows(ref, rows):
    return jnp.concatenate([ref[0, rows, :], ref[1, rows, :]], axis=1)


def _set_rows(ref, rows, v):
    ref[0, rows, :] = v[:, :HD]
    ref[1, rows, :] = v[:, HD:]


def _kernel(*refs):
    out_hbm, wa, xs, hbuf, w4t, yt, sems = refs[10:]
    zero = pl.run_scoped(
        functools.partial(_attention_and_mixer, *refs),
        pltpu.VMEM((H * DH // 2, D), u32),
        pltpu.VMEM((4, S + 3 * HALO, C4), f32),
        pltpu.VMEM((8, 4 * TOK, 128), bf16),
        pltpu.VMEM((4, D // 2, C4), u32),
        pltpu.VMEM((D // 2, D), u32),
        *[pltpu.VMEM((H // 8, RING, DH), f32)] * 8)
    if E_("SKIP_MLP", 0):
        for b in (w4t, yt, wa):
            pltpu.sync_copy(b.at[0, pl.ds(0, 128)], out_hbm.at[pl.ds(0, 128), pl.ds(0, 128)])
        return
    with jax.named_scope('s_mlp'): pl.run_scoped(
        functools.partial(_mlp, zero, out_hbm, wa, xs, hbuf, w4t, yt, sems),
        *[pltpu.VMEM((49 * NJ + 1, R, 128), bf16)] * 2,
        *[pltpu.VMEM((50, R // 2 + 8, 128), f32)] * 2,
        pltpu.VMEM((14, R, C4), f32))


def _attention_and_mixer(x_hbm, mem0_ref, wq_hbm, wk_hbm, wv_hbm, wo_hbm, w1_hbm, w2_hbm,
                         w3_hbm, w4_hbm, out_hbm, wa, xs, hbuf, w4t, yt, sems,
                         wo_b, xg, ubuf, w1b, w2b, *q_rings):
    w2_copy = pltpu.make_async_copy(w2_hbm.bitcast(u32), w2b, sems.at[SEM_W2])

    def w3_copy(c):
        return pltpu.make_async_copy(w3_hbm.at[:, :, pl.ds(_mult(c * 128, 128), 128)],
                                     yt.at[pl.ds(8 * c, 8), pl.ds(0, R)], sems.at[SEM_W3 + c])

    zero = pl.run_scoped(
        functools.partial(_attention, x_hbm, mem0_ref, (wq_hbm, wk_hbm, wv_hbm), wo_hbm,
                          w1_hbm, w2_copy, w3_copy,
                          w4_hbm, w4t, yt, wa, xs, hbuf, sems, wo_b, xg, ubuf, w1b, q_rings),
        *[pltpu.VMEM((H // 8, RING, DH), f32)] * 16)
    w2_copy.wait()
    for c in range(4 * NJ):
        w3_copy(c).wait()
    if E_("SKIP_POST", 0): return zero
    with jax.named_scope('s_mix'): pl.run_scoped(
        functools.partial(_mixer, zero, wa, hbuf, yt, wo_b, xg, w1b, w2b, q_rings),
        pltpu.VMEM((8, P0 + 4 * TOK + 16, 128), bf16),
        *[pltpu.VMEM((8, P0, 128), bf16)] * 2, *[pltpu.VMEM((RB, D), f32)] * 2,
        *[pltpu.VMEM((RB + 8, D), f32)] * 2)
    return zero


def _attention(x_hbm, mem0_ref, w_hbm, wo_hbm, w1_hbm, w2_copy, w3_copy,
               w4_hbm, w4t, yt, wa, xs, hbuf, sems, wo_b, xg, ubuf, w1b, q_rings, *kv_rings):
    rings = q_rings + kv_rings
    ring = [[rings[m * 8 + h % 8].at[h // 8] for h in range(H)] for m in range(3)]
    q_r, k_r, v_r = ring

    class x_rows:
        def __init__(self, rows, sem):
            self.copies = [
                pltpu.make_async_copy(x_hbm.at[rows, pl.ds(n * HD, HD)], xs.at[n, rows],
                                      sems.at[sem + n]) for n in range(2)]

        def start(self):
            for c in self.copies:
                c.start()

        def wait(self):
            for c in self.copies:
                c.wait()

    x0_copy = x_rows(pl.ds(0, P0), SEM_X0)

    def x_copy(g):
        return x_rows(pl.ds(_mult(P0 + g * 3 * XP, XP), 3 * XP), SEM_X + 2 * g)

    def wo_copy(i):
        rows = pl.ds(_mult(i * 512, 512), 512)
        return pltpu.make_async_copy(wo_hbm.bitcast(u32).at[rows], wo_b.at[rows],
                                     sems.at[SEM_WO + i])

    def w1_copy(i):
        cols = pl.ds(_mult(i * C4, C4), C4)
        return pltpu.make_async_copy(w1_hbm.bitcast(u32).at[:, cols], w1b.at[i],
                                     sems.at[SEM_W1 + i])

    def prologue(*stg):

        def start_chunk(g, m):
            src = w_hbm[m].bitcast(u32)
            dst = stg[m].reshape(D // 2, 8, DH)
            for par in range(2):
                pltpu.make_async_copy(
                    src.at[:, pl.ds(_mult(16 * par + 4 * g, 4), 4), :],
                    dst.at[:, pl.ds(4 * par, 4), :],
                    sems.at[SEM_W + 3 * g + m]).start()

        def wait_chunk(g, m):
            pltpu.make_async_copy(stg[m], stg[m], sems.at[SEM_W + 3 * g + m]).wait()

        def relayout(g, m, pair, i0, n):
            ev = stg[m][pl.ds(8 * i0 + pair, n, stride=8), :]
            od = stg[m][pl.ds(8 * i0 + 4 + pair, n, stride=8), :]
            h = 8 * g + 2 * pair
            words = wa.bitcast(u32)
            words[m * H + h, pl.ds(i0, n), :] = (ev & jnp.uint32(0xFFFF)) | (od << 16)
            words[m * H + h + 1, pl.ds(i0, n), :] = (ev >> 16) | (od & jnp.uint32(0xFFFF0000))

        def weights(g, m, pair):
            h = m * H + 8 * g + 2 * pair
            for t in range(D // 32 + 1):
                if t < D // 32:
                    for k in range(2):
                        relayout(g, m, pair, D // 4 * k + 8 * t, 8)
                if t > 0:
                    r = 16 * (t - 1)
                    b = [[wa[h + n, pl.ds(HD * k + r, 16), :].astype(f32) for n in range(2)]
                         for k in range(2)]
                    for p in range(7):
                        w4t[28 * m + 7 * pair + p, pl.ds(r, 16), :] = _enc(
                            ENC_B[p], lambda k, n: b[k][n]).astype(bf16)
                yield

        def norm_rows(r0, n):
            xv = _rows(xs, pl.ds(r0, n)).astype(f32)
            _set_rows(hbuf, pl.ds(r0, n), xv)
            return _ln(xv)

        def later_rows(r0):
            for r in range(0, XP, 16):
                xn = norm_rows(pl.multiple_of(r0 + r, 16), 16)
                for c in range(4):
                    xg[c, pl.ds(pl.multiple_of(HALO + r0 + r, 8), 16), :] = (
                        xn[:, c * C4:(c + 1) * C4])
                yield

        x0_copy.start()
        start_chunk(0, 0)
        start_chunk(0, 1)
        x_copy(0).start()
        start_chunk(0, 2)
        zero = jnp.zeros((HALO, C4), f32)
        for c in range(4):
            xg[c, pl.ds(0, HALO), :] = zero
            xg[c, pl.ds(HALO + S, HALO), :] = zero
        x0_copy.wait()

        @pl.loop(0, P0 // 64)
        def _(i):
            a = [norm_rows(pl.multiple_of(P0 // 2 * k + 32 * i, 32), 32) for k in range(2)]
            for p in range(7):
                v = _enc(ENC_A[p], lambda k, n: a[k][:, HD * n:HD * n + HD])
                for c in range(4):
                    yt[8 * p + 4 * (i // 4) + c, pl.ds(pl.multiple_of(i % 4 * 32, 32), 32), :] = (
                        v[:, 128 * c:128 * c + 128].astype(bf16))

        wait_chunk(0, 0)
        pl.loop(0, 4)(lambda pair: _run(weights(0, 0, pair)))

        def stage(g, m):
            c = 3 * g + m
            m1 = (m + 1) % 3
            g1 = jnp.minimum(g + (1 if m == 2 else 0), 3)
            pl.when(c < 11)(functools.partial(wait_chunk, g1, m1))
            if m == 0:
                x_copy(g).wait()

            @pl.when(g < 3)
            def _():
                start_chunk(g + 1, m)
                if m == 1:
                    x_copy(g + 1).start()
            if m == 0:
                wo_copy(g).start()
            if m == 2:
                w1_copy(g).start()
            n = E_("PR", 64)
            acc = {}

            def dot(pair, r, p):
                res = _dot(
                    _operand(yt, [8 * p + 4 * (r // R) + k for k in range(4)],
                             pl.ds(r % R // 2, n // 2)),
                    _operand(w4t, [28 * m + 7 * pair + p], pl.ds(0, HD // 2)))
                for i, j, sign in DEC[p]:
                    _accumulate(acc, (i, j), res, sign)
                    if LAST[i, j] == p:
                        rings[m * 8 + 2 * pair + j][g, pl.ds(P0 // 2 * i + r, n), :] = (
                            acc.pop((i, j)))
                return res

            _interleave(
                [functools.partial(dot, pair, r, p) for pair in range(4)
                 for r in range(0, P0 // 2, n) for p in ORDER],
                lambda res: [_pace(wa, (3 * H,), 16 * (g >> 10), res),
                             _pace(xg, (0,), S + 2 * HALO + 8 * (g >> 10), res)],
                (itertools.chain(*[weights(g1, m1, pair) for pair in range(4)]),
                 4 * (D // 32 + 1)),
                (later_rows(P0 + c * XP), XP // 16), pieces=E_("PQ", 1))

        @pl.loop(0, 4)
        def _(g):
            for m in range(3):
                stage(g, m)

    if not E_('SKIP_PRO', 0):
     with jax.named_scope('s_pro'): pl.run_scoped(
        prologue,
        pltpu.VMEM((8 * D // 2, DH), u32),
        pltpu.VMEM((8 * D // 2, DH), u32),
        pltpu.VMEM((8 * D // 2, DH), u32),
    )
    for i in range(4):
        wo_copy(i).wait()
    for i in range(4):
        w1_copy(i).wait()

    def wrap(r):
        return jnp.where(r >= RING, r - RING, r)

    def load_tok(s):
        rows = pl.ds(pl.multiple_of(HALO + P0 + TOK * s, 8), TOK)
        return jnp.concatenate([xg[c, rows, :] for c in range(4)], axis=1)

    def step(s, carry, tok, first_of_group, side_work, pace):
        mem, rp, ra, rw = carry
        ri = lax.broadcasted_iota(jnp.int32, (2 * L, 2 * L), 0)
        ci = lax.broadcasted_iota(jnp.int32, (2 * L, 2 * L), 1)
        same = (ri >= L) == (ci >= L)
        ri, ci = (jnp.where(v >= L, v - L, v) for v in (ri, ci))
        mask = same & ((ri < MEM) | (ri >= ci))
        fill = jnp.where(same, NEG, -jnp.inf)

        lhs = jnp.concatenate([mem, tok], axis=0).astype(bf16)
        rps = [pl.multiple_of(wrap(rp + 8 * i), 8) for i in range(3)]
        ra_ = pl.multiple_of(ra, SEG)
        rw_ = pl.multiple_of(rw, 8)

        col = s & 3
        rb = pl.multiple_of(jnp.maximum((s >> 2) - 1, 0) * (4 * TOK), 8)
        if first_of_group:
            _set_blocks(ubuf, slice(None), _ln(_ln(_rows(hbuf, pl.ds(rb, 4 * TOK)))))

        def filler(j):
            r = _dot(_operand(ubuf, range(8)), _unpack(w1b[col, :, pl.ds(j * 128, 128)]))
            xg[col, pl.ds(HALO + rb, 4 * TOK), pl.ds(j * 128, 128)] = _gelu(r)

        mem_qkv = {}
        scores = {}
        o_mem = {}
        total = [None]

        def qkv(h):
            res = []
            for m in range(3):
                r = _dot(lhs, _operand(wa, [m * H + h]))
                for i in range(3):
                    ring[m][h][pl.ds(rps[i], 8), :] = r[8 + 8 * i:16 + 8 * i]
                res.append(r[:MEM])
                if (3 * h + m) % E_('SM', 3) == E_('SO', 0) and h >= E_('S0', 2):
                    pace(r)
                    next(side_work, None)
            mem_qkv[h] = res

        def both(m, a):
            return jnp.concatenate(
                [v for h in (2 * a, 2 * a + 1)
                 for v in (mem_qkv[h][m], ring[m][h][pl.ds(ra_, SEG), :])],
                axis=0).astype(bf16)

        def qk(a):
            scores[a] = lax.dot_general(both(0, a), both(1, a), (((1,), (1,)), ((), ())),
                                        preferred_element_type=f32)

        def pv(a):
            sc = jnp.where(mask, scores.pop(a) * (DH ** -0.5), fill)
            mx = jnp.max(sc, axis=1, keepdims=True)
            e = jnp.exp(sc - mx)
            den = jnp.sum(e, axis=1, keepdims=True)
            inv = pl.reciprocal(den, approx=True)
            inv = inv * (2.0 - den * inv)
            o = _dot(e.astype(bf16), both(2, a)) * inv
            for i, h in enumerate((2 * a, 2 * a + 1)):
                q_r[h][pl.ds(ra_, SEG), :] = o[i * L + MEM:(i + 1) * L]
                o_mem[h] = o[i * L:i * L + MEM]

        def wo(h):
            lo = jnp.concatenate([o_mem.pop(h), q_r[h][pl.ds(rw_, TOK), :]],
                                 axis=0).astype(bf16)
            r = _dot(lo, _unpack(wo_b[pl.ds(h * DH // 2, DH // 2), :]))
            total[0] = r if total[0] is None else total[0] + r

        npair = H // 2
        for t in range(npair + LAG_WO):
            def attend():
                if E_("AM", 1) == 1:
                    for f, lag in ((qk, LAG_QK), (pv, LAG_PV)):
                        if 0 <= t - lag < npair:
                            f(t - lag)
                elif t % 2 == E_("PH", 0):
                    for f, lag in ((qk, LAG_QK), (pv, LAG_PV))[::E_("REV", 1)]:
                        for a in (t - lag, t - lag + 1):
                            if 0 <= a < npair:
                                f(a)
            if E_("AP", 0) == 0: attend()
            if t < npair:
                qkv(2 * t)
            if E_("AP", 0) == 1: attend()
            if t < npair:
                qkv(2 * t + 1)
            if E_("AP", 0) == 2: attend()
            if t == FILL_AT:
                filler(0)
            if 0 <= t - LAG_WO < npair:
                wo(2 * (t - LAG_WO))
                wo(2 * (t - LAG_WO) + 1)
            if E_("AP", 0) == 3: attend()
        filler(1)

        a = total[0]
        rows = pl.ds(pl.multiple_of(TOK * s, 8), TOK)
        _set_rows(hbuf, rows, _rows(hbuf, rows) + a[MEM:])
        return a[:MEM], wrap(rp + TOK), wrap(ra + SEG), wrap(rw + TOK)

    def recurrence(w4b):
        def w4_copy(j):
            rows = pl.ds(_mult(512 * j, 512), 512)
            return pltpu.make_async_copy(w4_hbm.at[rows], w4b.at[rows], sems.at[SEM_W4 + j])

        w4_copy(0).start()
        for k in range(4):
            w4b[pl.ds(F - 128 * k - 32, 32), :] = jnp.zeros((32, D), bf16)

        def encode_w4(i):
            for t, c in itertools.product(range(2), range(2)):
                r = pl.multiple_of(32 * (i & 3) + 16 * t, 16)

                def get(k, n):
                    return w4b[pl.ds(512 * (i >> 2) + 128 * k + r, 16),
                               pl.ds(C4 * n + 128 * c, 128)].astype(f32)

                def emit(p, v):
                    w4t[2 * p + c, pl.ds(128 * (i >> 2) + r, 16), :] = v.astype(bf16)

                yield from _enc2(ENC_B, get, emit)

        def steps(i, carry):
            @pl.when(i < 4 * NJ)
            def _():
                w3_copy(i).start()

                @pl.when(i & 3 == 1)
                def _():
                    w4_copy(i >> 2).wait()
                    pl.when(i < 4 * (NJ - 1))(lambda: w4_copy((i >> 2) + 1).start())

            pl.when(i == 4 * NJ)(w2_copy.start)
            side_work = encode_w4(jnp.where((i == 0) | (i > 4 * NJ), 4 * NJ, i) - 1)
            toks = [load_tok(i * UNROLL + k) for k in range(UNROLL)]
            for k in range(UNROLL):
                carry = step(i * UNROLL + k, carry, toks[k], k == 0,
                             itertools.islice(side_work, 28 // UNROLL),
                             lambda r: [_pace(*p, r) for p in (
                                 (w4b, (), F + 16 * (i >> 10)),
                                 (w4t, (98,), 16 * (i >> 10)))[E_("L0", 0):E_("L1", 2)]])
            _run(side_work)
            return carry

        return lax.fori_loop(
            0, NSEG // UNROLL, steps,
            (mem0_ref[...].astype(f32), jnp.int32(P0), jnp.int32(0), jnp.int32(0)))[3]

    if E_('SKIP_LOOP', 0): return lax.fori_loop(0, 64, lambda i, c: wrap(c + TOK), jnp.int32(0)) - TOK * NSEG % RING
    with jax.named_scope('s_loop'): return pl.run_scoped(recurrence, pltpu.VMEM((F + 16, D), bf16)) - TOK * NSEG % RING


def _interleave(dots, pace, *work, pieces=8):
    for i, dot in enumerate(dots):
        res = dot()
        k = min(pieces, res.shape[0] // 16)
        for j in range(k):
            pace(res[:res.shape[0] // 16 * (j + 1) // k * 16])
            for gen, n in work:
                for _ in range(n * (i * k + j) // (k * len(dots)),
                               n * (i * k + j + 1) // (k * len(dots))):
                    next(gen)
    for gen, _ in work:
        _run(gen)


def _mixer(zero, wa, hbuf, yt, wo_b, xg, w1b, w2b, q_rings, ulast, lhs0, lhs1, hs0, hs1, *ybuf):
    lhs, hs = (lhs0, lhs1), (hs0, hs1)

    def encode_w3(j, t):
        def get(k, n):
            r = C4 * k + 16 * t
            return yt[32 * j + 8 * n + r // 128, pl.ds(r % 128, 16), :].astype(f32)

        def emit(p, v):
            wa[13 * j + p // 4, pl.ds(C4 * (p % 4) + 16 * t, 16), :] = v.astype(bf16)

        return _enc2(ENC_B, get, emit)

    done = TOK * NSEG
    first = 4 * TOK * (NSEG // 4 - 1)

    @jax.named_scope('q1')
    def q1(g):
        n = E_("WR", 128)
        for k, q in enumerate(q_rings):
            for r in range(0, P0, 64):
                lhs0[k, pl.ds(r, 64), :] = q[g, pl.ds((done + r) % RING, 64), :].astype(bf16)

        def dot(r, c):
            w = wo_b[pl.ds(pl.multiple_of(g * 4 * DH, 4 * DH), 4 * DH), pl.ds(128 * c, 128)]
            res = _dot(_operand(lhs0, range(8), pl.ds(r // 2, n // 2)), _unpack(w))
            hbuf[c // 4, pl.ds(done + r, n), pl.ds(128 * (c % 4), 128)] += res
            return res

        _interleave(
            [functools.partial(dot, r, c) for r in range(0, P0, n) for c in range(8)],
            functools.partial(_pace, yt, (98 * NB - 1,), zero),
            (itertools.chain(*[encode_w3(jnp.minimum(2 * g + k, NJ - 1), t)
                               for k in range(2) for t in range(16)]), 7 * 32))

    pl.loop(0, H // 8)(q1)

    def mixer_norm(r0, n):
        for r in range(r0, r0 + n, 16):
            _set_blocks(ulast, pl.ds(r, 16), _ln(_ln(_rows(hbuf, pl.ds(first + r, 16)))))
            yield

    def mixer_in(c):
        n = (S - first) // 2
        for r, k in itertools.product((0, n), range(2)):
            cols = pl.ds(128 * k, 128)
            xg[c, pl.ds(HALO + first + r, n), cols] = _gelu(_dot(
                _operand(ulast, range(8), pl.ds(r // 2, n // 2)), _unpack(w1b[c, :, cols])))

    def shift(i, dst):
        for r in range(0, RB, 64):
            for c, off in enumerate((-1, 1, -2, 2)):
                win = xg[c, pl.ds(_mult(i * RB + r, 64), 64 + 2 * HALO), :]
                g = win[HALO + off:HALO + off + 64].astype(bf16)
                for k in range(2):
                    dst[2 * c + k, pl.ds(r, 64), :] = g[:, 128 * k:128 * k + 128]
                yield

    def mixer_out(src, dst):
        n = E_("MR", 128)

        def dot(r, c):
            cols = pl.ds(128 * c, 128)
            res = _dot(_operand(src, range(8), pl.ds(r // 2, n // 2)), _unpack(w2b[:, cols]))
            dst[pl.ds(r, n), cols] = res
            return res

        return [functools.partial(dot, r, c) for r in range(0, RB, n) for c in range(8)]

    def residual(i, src, dst):
        late = []
        for t in range(0, RB, 8):
            rows = pl.ds(_mult(i * RB + t, 8), 8)
            hv = _rows(hbuf, rows)
            x1 = _ln(hv) + src[pl.ds(t, 8), :]
            late.append((rows, hv + x1, t, _ln(x1)))
            if len(late) > E_("LT", 2) or t == RB - 8:
                for rows, v, t0, y in late[:None if t == RB - 8 else 1]:
                    _set_rows(hbuf, rows, v)
                    dst[pl.ds(t0, 8), :] = y
                del late[0]
            yield

    def up_operands(i, src):
        per = 4 * R // RB
        for t, c in itertools.product(range(0, RB, 64), range(2)):
            def emit(p, v):
                yt[98 * (i // per) + 2 * p + c,
                   pl.ds(_mult(i % per * (RB // 4) + t // 4, 16), 16), :] = v.astype(bf16)

            yield from _enc2(ENC_A, lambda q, k: src[
                pl.ds(t + 16 * q, 16), pl.ds(C4 * k + 128 * c, 128)], emit)

    def job(i, par, extra=None):
        work = [(shift(jnp.minimum(i + 1, S // RB - 1), lhs[1 - par]), RB // 16)]
        paced = [(lhs[1 - par], (0,), P0 - 16 + zero)]
        if extra is None:
            work.append((up_operands(i - 2, ybuf[par]), 14 * RB // 64))
            paced.append((yt, (98 * NB,), zero))
        else:
            work.append((mixer_norm(*extra), extra[1] // 16))
            paced.append((ulast, (0,), S - first + zero))
        if extra is None or i > 0:
            work.append((residual(i - 1, hs[1 - par], ybuf[1 - par]), RB // 8))
            paced.append((ybuf[1 - par], (), RB + zero))
        pl.loop(zero, 1)(lambda _: _interleave(
            mixer_out(lhs[par], hs[par]), lambda res: [_pace(*p, res) for p in paced], *work))

    cut = E_("CUT", 416)
    _run(shift(0, lhs[0]))
    with jax.named_scope('j01'):
        job(0, 0, (0, cut))
        job(1, 1, (cut, S - first - cut))
    with jax.named_scope('in'): pl.loop(0, 4)(mixer_in)

    @pl.loop(1, S // RB // 2)
    @jax.named_scope('jobs')
    def _(i):
        job(2 * i, 0)
        job(2 * i + 1, 1)

    last = S // RB - 1
    _run(up_operands(last - 1, ybuf[0]))
    _run(residual(last, hs[1], ybuf[1]))
    _run(up_operands(last, ybuf[1]))


def _mlp(zero, out_hbm, wa, xs, hbuf, w4t, yt, sems, tt0, tt1, mu0, mu1, md):
    tts, mu = (tt0, tt1), (mu0, mu1)
    hr = R // 2
    lag = E_("LAG", 14)

    def out_copy(b, n):
        rows = pl.ds(_mult(b * 4 * R, 4 * R), 4 * R)
        return pltpu.make_async_copy(xs.at[n, rows], out_hbm.at[rows, pl.ds(n * HD, HD)],
                                     sems.at[SEM_OUT + 2 * b + n])

    def up_dot(b, j, half, p):
        res = _dot(
            _operand(yt, [98 * b + 2 * p, 98 * b + 2 * p + 1], pl.ds(half * hr // 2, hr // 2)),
            _operand(wa, [13 * j + p // 4], pl.ds(128 * (p % 4), 128)))
        mu[half][p, pl.ds(0, hr), :] = res
        return res

    def up_sums(act):
        for half, t in itertools.product(range(2), range(hr // 8)):
            c = {}
            for g in ORDER:
                y = _dec(lambda k: mu[half][7 * g + k, pl.ds(8 * t, 8), :])
                for i1, n1, sign in DEC[g]:
                    for (i0, n0), m in y.items():
                        key = (2 * i1 + i0, 2 * n1 + n0)
                        _accumulate(c, key, m, sign)
                        if LAST[i1, n1] == g:
                            act[half, t, key] = _gelu(c.pop(key))
                yield

    def down_operands(act, tt, j):
        for half, t in itertools.product(range(2), range(hr // 16)):
            def emit(p, v):
                tt[NJ * p + j, pl.ds(half * hr + 16 * t, 16), :] = v.astype(bf16)

            yield from _enc2(ENC_A, lambda q, k: jnp.concatenate(
                [act[half, 2 * t, (q, k)], act[half, 2 * t + 1, (q, k)]], axis=0), emit)

    n_sums = 7 * 2 * (hr // 8)

    def up_vector_work(tt, j):
        act = {}
        a, b = up_sums(act), down_operands(act, tt, j)
        for i in range(n_sums + lag):
            if i < n_sums:
                next(a)
            if i >= lag and (i - lag) % 2 == 1:
                next(b)
            yield

    def down_dot(tt, g, slot, i):
        p = 7 * g + i // 2
        res = _dot(
            _operand(tt, [NJ * p + q for q in range(NJ)], pl.ds(0, R // 2)), _operand(w4t, [14 * g + i], pl.ds(0, F // 8)))
        md[7 * slot + i // 2, pl.ds(0, R), pl.ds(128 * (i % 2), 128)] = res
        return res

    def down_sums(b, g, slot):
        dst = []
        for w in range(2):
            i1 = n1 = sign = 0
            for q in range(7):
                e = DEC[q][w] if w < len(DEC[q]) else DEC[q][0][:2] + (0,)
                i1, n1, sign = (jnp.where(g == q, new, old)
                                for new, old in zip(e, (i1, n1, sign)))
            dst.append((b * 4 * R + 32 * i1, n1, sign.astype(f32)))
        for t in range(R // 16):
            c = _dec(lambda k: md[7 * slot + k, pl.ds(16 * t, 16), :])
            m = jnp.concatenate(
                [jnp.concatenate([c[i0, 0], c[i0, 1]], axis=1) for i0 in range(2)], axis=0)
            rows = [pl.ds(pl.multiple_of(d[0] + 64 * t, 32), 32) for d in dst]
            new = [hbuf[dst[0][1], rows[0], :] + m,
                   hbuf[dst[1][1], rows[1], :] + dst[1][2] * m]
            for w in (1, 0):
                hbuf[dst[w][1], rows[w], :] = new[w]
                xs[dst[w][1], rows[w], :] = new[w].astype(bf16)
            yield

    def step(b, par, up, down, j):
        slot = (7 * b + j) & 1
        dots = []
        if up:
            nb = jnp.minimum(b + (j + 1) // NJ, NB - 1)
            nj = jnp.where(j == NJ - 1, 0, j + 1)
            dots = ([(1, functools.partial(up_dot, b, j, 1, p)) for p in range(49)]
                    + [(1, functools.partial(up_dot, nb, nj, 0, p)) for p in range(49)])
            up_work = up_vector_work(tts[par], j)
        if down:
            for i in range(14):
                dots.insert((8 * i + E_('D0', 7) if not E_('DM', 0) else [int(v) for v in os.environ['AT'].split(',')][i // E_('DM', 0)] + i) if up else i,
                            (7, functools.partial(down_dot, tts[1 - par], j, slot, i)))
            down_work = down_sums(jnp.maximum(b - 1 - (j == 0), 0),
                                  jnp.where(j == 0, 6, j - 1), 1 - slot)
        total = sum(w for w, _ in dots)
        pos = n_up = done_up = done_down = 0
        for w, dot in dots:
            if down:
                goal = (pos + E_("AD", 14)) * (R // 16) * 100 // (E_("DE", 100) * total)
                for _ in range(done_down, goal):
                    next(down_work, None)
                done_down = max(done_down, goal)
            res = dot()
            k = E_("PD", 4) if w > 1 else 1
            for i in range(k * up):
                if E_('PM', 2) and (w > 1 or n_up % E_('PM', 2) == 0):
                    _pace(mu[done_up >= n_sums // 2], (49,), zero, res[:res.shape[0] * (i + 1) // k])
                if E_('PN', 2) and (w > 1 or n_up % E_('PN', 2) == 0):
                    _pace(tts[par], (49 * NJ,), zero, res[:res.shape[0] * (i + 1) // k])
                goal = (pos * k + w * (i + 1) + E_("AH", 4) * k) * (n_sums + lag) // (total * k)
                goal = (min(goal, n_sums // 2) if n_up + (w == 1) < 49
                        else max(goal, n_sums // 2))
                for _ in range(done_up, goal):
                    next(up_work, None)
                done_up = max(done_up, goal)
            pos += w
            n_up += w == 1
        if up:
            _run(up_work)
        if down:
            _run(down_work)
        if down:
            @pl.when((j == 0) & (b > 1))
            def _():
                for n in range(2):
                    out_copy(b - 2, n).start()

    md[pl.ds(0, 7), pl.ds(0, R), :] = jnp.zeros((7, R, C4), f32)
    for p in range(49):
        up_dot(0, 0, 0, p)
    with jax.named_scope('b0'): pl.loop(0, NJ)(functools.partial(step, 0, 0, True, False))

    @pl.loop(0, NB // 2)
    @jax.named_scope('bmid')
    def _(i):
        pl.loop(0, NJ)(functools.partial(step, 2 * i + 1, 1, True, True))
        pl.loop(0, jnp.where(2 * i + 2 < NB, NJ, 0))(
            functools.partial(step, 2 * i + 2, 0, True, True))

    with jax.named_scope('b4'): pl.loop(0, NJ)(functools.partial(step, NB, 0, False, True))
    _run(down_sums(NB - 1, jnp.int32(6), (7 * NB + 6) & 1))
    for n in range(2):
        out_copy(NB - 1, n).start()
    for b in range(NB):
        for n in range(2):
            out_copy(b, n).wait()


@jax.jit
def pallas_sequential_preLN__memory_aug_recurrent_mem_tr__mixer_s_mlp__prompt_kernel(
    A_x: jax.Array,
    A_mem0: jax.Array,
    A_Wq: jax.Array,
    A_Wk: jax.Array,
    A_Wv: jax.Array,
    A_Wo: jax.Array,
    A_seg_len: jax.Array,
    B_x: jax.Array,
    B_w1: jax.Array,
    B_w2: jax.Array,
    B_w3: jax.Array,
    B_w4: jax.Array,
):
    del A_seg_len, B_x
    hbm = pl.BlockSpec(memory_space=pl.ANY)
    vmem = pl.BlockSpec(memory_space=pltpu.VMEM)
    scratch = [
        pltpu.VMEM((3 * H + 1, D, DH), bf16),
        pltpu.VMEM((2, S, HD), bf16),
        pltpu.VMEM((2, S, HD), f32),
        pltpu.VMEM((99, F // 4, 128), bf16),
        pltpu.VMEM((98 * NB + 1, R, 128), bf16),
        pltpu.SemaphoreType.DMA((NSEM,)),
    ]
    out = pl.pallas_call(
        _kernel,
        out_shape=jax.ShapeDtypeStruct((S, D), A_x.dtype),
        in_specs=[hbm, vmem] + [hbm] * 8,
        out_specs=hbm,
        scratch_shapes=scratch,
        compiler_params=pltpu.CompilerParams(vmem_limit_bytes=127 * 1024 * 1024),
    )(A_x.reshape(S, D), A_mem0.reshape(MEM, D),
      A_Wq.reshape(D // 2, 2 * H, DH), A_Wk.reshape(D // 2, 2 * H, DH),
      A_Wv.reshape(D // 2, 2 * H, DH),
      A_Wo.reshape(H * DH, D), B_w1, B_w2, B_w3.reshape(D // R, R, F), B_w4)
    return out.reshape(A_x.shape)
```

```python
import functools
import itertools
import os

import jax
import jax.numpy as jnp
from jax import lax
import jax.experimental.pallas as pl
import jax.experimental.pallas.tpu as pltpu

S = 2048
D = 1024
H = 32
DH = 128
MEM = 8
SEG = 32
F = 3584
NSEG = S // SEG
L = MEM + SEG
TOK = 24
P0 = S - TOK * NSEG
RING = 576
XP = (S - P0) // 12
C4 = D // 4
HALO = 8
RB = 256
R = 128
NB = S // (4 * R)
NJ = F // 512
HD = D // 2
W4T = (F - S) // R
E_ = lambda k, d: int(os.environ.get(k, d))
EPS = 1e-5
NEG = -1000000000.0

LAG_QK, LAG_PV, LAG_WO = E_('LQ', 2), E_('LP', 4), E_('LW', 5)
FILL_AT = E_('FA', 17)
UNROLL = 2

bf16 = jnp.bfloat16
f32 = jnp.float32
u32 = jnp.uint32

SEM_X0, SEM_X, SEM_WO, SEM_W1, SEM_W2, SEM_OUT, SEM_W, SEM_W4, SEM_W3 = (
    0, 2, 10, 14, 18, 20, 28, 40, 50)
NSEM = SEM_W3 + 4 * NJ

ENC_A = (((0, 0, 1), (1, 1, 1)), ((1, 0, 1), (1, 1, 1)), ((0, 0, 1),), ((1, 1, 1),),
         ((0, 0, 1), (0, 1, 1)), ((1, 0, 1), (0, 0, -1)), ((0, 1, 1), (1, 1, -1)))
ENC_B = (((0, 0, 1), (1, 1, 1)), ((0, 0, 1),), ((0, 1, 1), (1, 1, -1)),
         ((1, 0, 1), (0, 0, -1)), ((1, 1, 1),), ((0, 0, 1), (0, 1, 1)),
         ((1, 0, 1), (1, 1, 1)))
DEC = (((0, 0, 1), (1, 1, 1)), ((1, 0, 1), (1, 1, -1)), ((0, 1, 1), (1, 1, 1)),
       ((0, 0, 1), (1, 0, 1)), ((0, 1, 1), (0, 0, -1)), ((1, 1, 1),), ((0, 0, 1),))
ORDER = (0, 1, 3, 2, 4, 5, 6)
LAST = {(1, 0): 3, (0, 1): 4, (1, 1): 5, (0, 0): 6}


def _enc(terms, get):
    v = get(*terms[0][:2])
    for i, j, sign in terms[1:]:
        v = v + get(i, j) if sign > 0 else v - get(i, j)
    return v


def _enc2(table, get, emit):
    for g in range(7):
        y = [[_enc(table[g], lambda i1, j1: get(2 * i1 + i0, 2 * j1 + j0))
              for j0 in range(2)] for i0 in range(2)]
        for k in range(7):
            emit(7 * g + k, _enc(table[k], lambda i0, j0: y[i0][j0]))
        yield


def _accumulate(c, key, m, sign):
    c[key] = m if key not in c else (c[key] + m if sign > 0 else c[key] - m)


def _dec(get):
    c = {}
    for k in range(7):
        m = get(k)
        for i, j, sign in DEC[k]:
            _accumulate(c, (i, j), m, sign)
    return c


def _pace(ref, lead, row, result):
    n = 32 // ref.dtype.itemsize
    ref[(*lead, pl.ds(pl.multiple_of(row, n), n), pl.ds(0, 128))] = (
        result[-n:, :128].astype(ref.dtype))


def _run(gen):
    for _ in gen:
        pass


def _mult(i, n):
    return i if isinstance(i, int) else pl.multiple_of(i, n)


def _ln(x):
    m = jnp.mean(x, axis=-1, keepdims=True)
    d = x - m
    v = jnp.mean(d * d, axis=-1, keepdims=True)
    return d * lax.rsqrt(v + EPS)


def _gelu(x):
    c = 0.7978845608028654
    hx = 0.5 * x
    return hx + hx * jnp.tanh(x * (c + (c * 0.044715) * (x * x)))


def _unpack(x):
    return pltpu.bitcast(x, bf16)


def _operand(ref, blocks, rows=slice(None)):
    words = ref.bitcast(u32)
    return _unpack(jnp.concatenate([words[b, rows, :] for b in blocks], axis=1))


def _set_blocks(ref, rows, v):
    for c in range(v.shape[1] // 128):
        ref[c, rows, :] = v[:, 128 * c:128 * c + 128].astype(bf16)


def _dot(a, b):
    return jnp.dot(a, b, preferred_element_type=f32)


def _rows(ref, rows):
    return jnp.concatenate([ref[0, rows, :], ref[1, rows, :]], axis=1)


def _set_rows(ref, rows, v):
    ref[0, rows, :] = v[:, :HD]
    ref[1, rows, :] = v[:, HD:]


def _kernel(*refs):
    out_hbm, wa, xs, hbuf, w4t, yt, mu0, sems = refs[11:]
    zero = pl.run_scoped(
        functools.partial(_attention_and_mixer, *refs),
        pltpu.VMEM((H * DH // 2, D), u32),
        pltpu.VMEM((8, S + 4 * HALO, 128), f32),
        pltpu.VMEM((8, 4 * TOK, 128), bf16),
        pltpu.VMEM((4, D // 2, C4), u32),
        pltpu.VMEM((D // 2, D), u32),
        *[pltpu.VMEM((H // 8, RING, DH), f32)] * 8)
    if E_("SKIP_MLP", 0):
        for b in (w4t, yt, wa):
            pltpu.sync_copy(b.at[0, pl.ds(0, 128)], out_hbm.at[pl.ds(0, 128), pl.ds(0, 128)])
        return
    with jax.named_scope('s_mlp'): pl.run_scoped(
        functools.partial(_mlp, zero, out_hbm, wa, xs, hbuf, w4t, yt, sems, mu0),
        *[pltpu.VMEM((49 * NJ + 1, R, 128), bf16)] * 2,
        pltpu.VMEM(mu0.shape, f32),
        pltpu.VMEM((14, R, C4), f32))


def _attention_and_mixer(x_hbm, mem0_ref, wq_hbm, wk_hbm, wv_hbm, wo_hbm, w1_hbm, w2_hbm,
                         w3_hbm, w4_hbm, w4a_hbm, out_hbm, wa, xs, hbuf, w4t, yt, mu0, sems,
                         wo_b, xg, ubuf, w1b, w2b, *q_rings):
    w2_copy = pltpu.make_async_copy(w2_hbm.bitcast(u32), w2b, sems.at[SEM_W2])

    def w3_copy(c):
        return pltpu.make_async_copy(
            w3_hbm.at[:, :, pl.ds(_mult(c * 128, 128), 128)], yt.at[pl.ds(8 * c, 8)],
            sems.at[SEM_W3 + c])

    def w4_head_copy(n):
        return pltpu.make_async_copy(
            w4a_hbm.at[pl.ds(0, S), pl.ds(n * HD, HD)], xs.at[n, pl.ds(0, S)], sems.at[SEM_W4 + n])

    def w4_tail_copy(c):
        return pltpu.make_async_copy(
            w4_hbm.at[pl.ds(S // R, W4T), :, pl.ds(c * 128, 128)],
            yt.at[pl.ds(32 * NJ + W4T * c, W4T)], sems.at[SEM_W4 + 2 + c])

    others = [[w2_copy], [w4_head_copy(0)], [w4_head_copy(1)],
              [w4_tail_copy(c) for c in range(8)]]

    def fetch(i):
        pl.when(i >= 4)(lambda: w3_copy(i - 4).start())
        for k, copies in enumerate(others):
            @pl.when(i == k)
            def _():
                for c in copies:
                    c.start()

    zero = pl.run_scoped(
        functools.partial(_attention, x_hbm, mem0_ref, (wq_hbm, wk_hbm, wv_hbm), wo_hbm,
                          w1_hbm, fetch, w4t, yt, wa, xs, hbuf, sems, wo_b, xg, ubuf, w1b, q_rings),
        *[pltpu.VMEM((H // 8, RING, DH), f32)] * 16)
    for c in sum(others, []):
        c.wait()
    for c in range(4 * NJ):
        w3_copy(c).wait()
    if E_("SKIP_POST", 0): return zero
    with jax.named_scope('s_mix'): pl.run_scoped(
        functools.partial(_mixer, zero, mu0, wa, xs, w4t, hbuf, yt, wo_b, xg, w1b, w2b, q_rings),
        pltpu.VMEM((8, P0 + 4 * TOK + 16, 128), bf16),
        *[pltpu.VMEM((8, P0, 128), bf16)] * 2, *[pltpu.VMEM((RB, D), f32)] * 2,
        *[pltpu.VMEM((RB + 8, D), f32)] * 2)
    return zero


def _attention(x_hbm, mem0_ref, w_hbm, wo_hbm, w1_hbm, fetch,
               w4t, yt, wa, xs, hbuf, sems, wo_b, xg, ubuf, w1b, q_rings, *kv_rings):
    rings = q_rings + kv_rings
    ring = [[rings[m * 8 + h % 8].at[h // 8] for h in range(H)] for m in range(3)]
    q_r, k_r, v_r = ring

    class x_rows:
        def __init__(self, rows, sem):
            self.copies = [
                pltpu.make_async_copy(x_hbm.at[rows, pl.ds(n * HD, HD)], xs.at[n, rows],
                                      sems.at[sem + n]) for n in range(2)]

        def start(self):
            for c in self.copies:
                c.start()

        def wait(self):
            for c in self.copies:
                c.wait()

    x0_copy = x_rows(pl.ds(0, P0), SEM_X0)

    def x_copy(g):
        return x_rows(pl.ds(_mult(P0 + g * 3 * XP, XP), 3 * XP), SEM_X + 2 * g)

    def wo_copy(i):
        rows = pl.ds(_mult(i * 512, 512), 512)
        return pltpu.make_async_copy(wo_hbm.bitcast(u32).at[rows], wo_b.at[rows],
                                     sems.at[SEM_WO + i])

    def w1_copy(i):
        cols = pl.ds(_mult(i * C4, C4), C4)
        return pltpu.make_async_copy(w1_hbm.bitcast(u32).at[:, cols], w1b.at[i],
                                     sems.at[SEM_W1 + i])

    def prologue(*stg):

        def start_chunk(g, m):
            src = w_hbm[m].bitcast(u32)
            dst = stg[m].reshape(D // 2, 8, DH)
            for par in range(2):
                pltpu.make_async_copy(
                    src.at[:, pl.ds(_mult(16 * par + 4 * g, 4), 4), :],
                    dst.at[:, pl.ds(4 * par, 4), :],
                    sems.at[SEM_W + 3 * g + m]).start()

        def wait_chunk(g, m):
            pltpu.make_async_copy(stg[m], stg[m], sems.at[SEM_W + 3 * g + m]).wait()

        def relayout(g, m, pair, i0, n):
            ev = stg[m][pl.ds(8 * i0 + pair, n, stride=8), :]
            od = stg[m][pl.ds(8 * i0 + 4 + pair, n, stride=8), :]
            h = 8 * g + 2 * pair
            words = wa.bitcast(u32)
            words[m * H + h, pl.ds(i0, n), :] = (ev & jnp.uint32(0xFFFF)) | (od << 16)
            words[m * H + h + 1, pl.ds(i0, n), :] = (ev >> 16) | (od & jnp.uint32(0xFFFF0000))

        def weights(g, m, pair):
            h = m * H + 8 * g + 2 * pair
            for t in range(D // 32 + 1):
                if t < D // 32:
                    for k in range(2):
                        relayout(g, m, pair, D // 4 * k + 8 * t, 8)
                if t > 0:
                    r = 16 * (t - 1)
                    b = [[wa[h + n, pl.ds(HD * k + r, 16), :].astype(f32) for n in range(2)]
                         for k in range(2)]
                    for p in range(7):
                        w4t[28 * m + 7 * pair + p, pl.ds(r, 16), :] = _enc(
                            ENC_B[p], lambda k, n: b[k][n]).astype(bf16)
                yield

        def norm_rows(r0, n):
            xv = _rows(xs, pl.ds(r0, n)).astype(f32)
            _set_rows(hbuf, pl.ds(r0, n), xv)
            return _ln(xv)

        def later_rows(r0):
            for r in range(0, XP, 16):
                xn = norm_rows(pl.multiple_of(r0 + r, 16), 16)
                for c in range(8):
                    xg[c, pl.ds(pl.multiple_of(HALO + r0 + r, 8), 16), :] = (
                        xn[:, 128 * c:128 * c + 128])
                yield

        x0_copy.start()
        start_chunk(0, 0)
        start_chunk(0, 1)
        x_copy(0).start()
        start_chunk(0, 2)
        zero = jnp.zeros((HALO, 128), f32)
        for c in range(8):
            xg[c, pl.ds(0, HALO), :] = zero
            xg[c, pl.ds(HALO + S, HALO), :] = zero
        with jax.named_scope('wx'): x0_copy.wait()

        @pl.loop(0, P0 // 64)
        def _(i):
            a = [norm_rows(pl.multiple_of(P0 // 2 * k + 32 * i, 32), 32) for k in range(2)]
            for p in range(7):
                v = _enc(ENC_A[p], lambda k, n: a[k][:, HD * n:HD * n + HD])
                for c in range(4):
                    yt[8 * p + 4 * (i // 4) + c, pl.ds(pl.multiple_of(i % 4 * 32, 32), 32), :] = (
                        v[:, 128 * c:128 * c + 128].astype(bf16))

        with jax.named_scope('w0'): wait_chunk(0, 0)
        pl.loop(0, 4)(lambda pair: _run(weights(0, 0, pair)))

        def stage(g, m):
            c = 3 * g + m
            m1 = (m + 1) % 3
            g1 = jnp.minimum(g + (1 if m == 2 else 0), 3)
            pl.when(c < 11)(functools.partial(wait_chunk, g1, m1))
            if m == 0:
                x_copy(g).wait()

            @pl.when(g < 3)
            def _():
                start_chunk(g + 1, m)
                if m == 1:
                    x_copy(g + 1).start()
            if m == 0:
                wo_copy(g).start()
            if m == 2:
                w1_copy(g).start()
            n = E_("PR", 64)
            acc = {}

            def dot(pair, r, p):
                res = _dot(
                    _operand(yt, [8 * p + 4 * (r // R) + k for k in range(4)],
                             pl.ds(r % R // 2, n // 2)),
                    _operand(w4t, [28 * m + 7 * pair + p], pl.ds(0, HD // 2)))
                for i, j, sign in DEC[p]:
                    _accumulate(acc, (i, j), res, sign)
                    if LAST[i, j] == p:
                        rings[m * 8 + 2 * pair + j][g, pl.ds(P0 // 2 * i + r, n), :] = (
                            acc.pop((i, j)))
                return res

            _interleave(
                [functools.partial(dot, pair, r, p) for pair in range(4)
                 for r in range(0, P0 // 2, n) for p in ORDER],
                lambda res: [_pace(wa, (3 * H,), 16 * (g >> 10), res),
                             _pace(xg, (0,), S + 2 * HALO + 8 * (g >> 10), res)],
                (itertools.chain(*[weights(g1, m1, pair) for pair in range(4)]),
                 4 * (D // 32 + 1)),
                (later_rows(P0 + c * XP), XP // 16), pieces=E_("PQ", 1))

        @pl.loop(0, 4)
        def _(g):
            for m in range(3):
                stage(g, m)

    if not E_('SKIP_PRO', 0):
     with jax.named_scope('s_pro'): pl.run_scoped(
        prologue,
        pltpu.VMEM((8 * D // 2, DH), u32),
        pltpu.VMEM((8 * D // 2, DH), u32),
        pltpu.VMEM((8 * D // 2, DH), u32),
    )
    for i in range(4):
        with jax.named_scope('wwo'): wo_copy(i).wait()
    for i in range(4):
        w1_copy(i).wait()

    def wrap(r):
        return jnp.where(r >= RING, r - RING, r)

    def load_tok(s):
        rows = pl.ds(pl.multiple_of(HALO + P0 + TOK * s, 8), TOK)
        return jnp.concatenate([xg[c, rows, :] for c in range(8)], axis=1)

    def step(s, carry, tok, first_of_group):
        mem, rp, ra, rw = carry
        ri = lax.broadcasted_iota(jnp.int32, (2 * L, 2 * L), 0)
        ci = lax.broadcasted_iota(jnp.int32, (2 * L, 2 * L), 1)
        same = (ri >= L) == (ci >= L)
        ri, ci = (jnp.where(v >= L, v - L, v) for v in (ri, ci))
        mask = same & ((ri < MEM) | (ri >= ci))
        fill = jnp.where(same, NEG, -jnp.inf)

        lhs = jnp.concatenate([mem, tok], axis=0).astype(bf16)
        rps = [pl.multiple_of(wrap(rp + 8 * i), 8) for i in range(3)]
        ra_ = pl.multiple_of(ra, SEG)
        rw_ = pl.multiple_of(rw, 8)

        col = s & 3
        rb = pl.multiple_of(jnp.maximum((s >> 2) - 1, 0) * (4 * TOK), 8)
        if first_of_group:
            _set_blocks(ubuf, slice(None), _ln(_ln(_rows(hbuf, pl.ds(rb, 4 * TOK)))))

        def filler(j):
            r = _dot(_operand(ubuf, range(8)), _unpack(w1b[col, :, pl.ds(j * 128, 128)]))
            xg[2 * col + j, pl.ds(HALO + rb, 4 * TOK), :] = _gelu(r)

        mem_qkv = {}
        scores = {}
        o_mem = {}
        total = [None]

        def qkv(h):
            res = []
            for m in range(3):
                r = _dot(lhs, _operand(wa, [m * H + h]))
                for i in range(3):
                    ring[m][h][pl.ds(rps[i], 8), :] = r[8 + 8 * i:16 + 8 * i]
                res.append(r[:MEM])
            mem_qkv[h] = res

        def both(m, a):
            return jnp.concatenate(
                [v for h in (2 * a, 2 * a + 1)
                 for v in (mem_qkv[h][m], ring[m][h][pl.ds(ra_, SEG), :])],
                axis=0).astype(bf16)

        def qk(a):
            scores[a] = lax.dot_general(both(0, a), both(1, a), (((1,), (1,)), ((), ())),
                                        preferred_element_type=f32)

        def pv(a):
            sc = jnp.where(mask, scores.pop(a) * (DH ** -0.5), fill)
            mx = jnp.max(sc, axis=1, keepdims=True)
            e = jnp.exp(sc - mx)
            den = jnp.sum(e, axis=1, keepdims=True)
            inv = pl.reciprocal(den, approx=True)
            inv = inv * (2.0 - den * inv)
            o = _dot(e.astype(bf16), both(2, a)) * inv
            for i, h in enumerate((2 * a, 2 * a + 1)):
                q_r[h][pl.ds(ra_, SEG), :] = o[i * L + MEM:(i + 1) * L]
                o_mem[h] = o[i * L:i * L + MEM]

        def wo(h):
            lo = jnp.concatenate([o_mem.pop(h), q_r[h][pl.ds(rw_, TOK), :]],
                                 axis=0).astype(bf16)
            r = _dot(lo, _unpack(wo_b[pl.ds(h * DH // 2, DH // 2), :]))
            total[0] = r if total[0] is None else total[0] + r

        npair = H // 2
        for t in range(npair + LAG_WO):
            def attend():
                if E_("AM", 1) == 1:
                    for f, lag in ((qk, LAG_QK), (pv, LAG_PV))[::E_("REV", 1)]:
                        if 0 <= t - lag < npair:
                            f(t - lag)
                elif t % 2 == E_("PH", 0):
                    for f, lag in ((qk, LAG_QK), (pv, LAG_PV))[::E_("REV", 1)]:
                        for a in (t - lag, t - lag + 1):
                            if 0 <= a < npair:
                                f(a)
            if E_("WF", 0) and 0 <= t - LAG_WO < npair:
                wo(2 * (t - LAG_WO))
                wo(2 * (t - LAG_WO) + 1)
            if E_("AP", 0) == 0: attend()
            if t < npair:
                qkv(2 * t)
            if E_("AP", 0) == 1: attend()
            if t < npair:
                qkv(2 * t + 1)
            if E_("AP", 0) == 2: attend()
            if t == FILL_AT:
                filler(0)
            if not E_("WF", 0) and 0 <= t - LAG_WO < npair:
                wo(2 * (t - LAG_WO))
                wo(2 * (t - LAG_WO) + 1)
            if E_("AP", 0) == 3: attend()
        filler(1)

        a = total[0]
        rows = pl.ds(pl.multiple_of(TOK * s, 8), TOK)
        _set_rows(hbuf, rows, _rows(hbuf, rows) + a[MEM:])
        return a[:MEM], wrap(rp + TOK), wrap(ra + SEG), wrap(rw + TOK)

    def steps(i, carry):
        fetch(i)
        toks = [load_tok(i * UNROLL + k) for k in range(UNROLL)]
        for k in range(UNROLL):
            carry = step(i * UNROLL + k, carry, toks[k], k == 0)
        return carry

    if E_('SKIP_LOOP', 0): return lax.fori_loop(0, 64, lambda i, c: wrap(c + TOK), jnp.int32(0)) - TOK * NSEG % RING
    with jax.named_scope('s_loop'): carry = lax.fori_loop(
        0, NSEG // UNROLL, steps,
        (mem0_ref[...].astype(f32), jnp.int32(P0), jnp.int32(0), jnp.int32(0)))
    return carry[3] - TOK * NSEG % RING


def _interleave(dots, pace, *work, pieces=8):
    for i, dot in enumerate(dots):
        res = dot()
        k = min(pieces, res.shape[0] // 16)
        for j in range(k):
            pace(res[:res.shape[0] // 16 * (j + 1) // k * 16])
            for gen, n in work:
                for _ in range(n * (i * k + j) // (k * len(dots)),
                               n * (i * k + j + 1) // (k * len(dots))):
                    next(gen)
    for gen, _ in work:
        _run(gen)


def _up_dot(yt, wa, mu, b, j, half, p):
    res = _dot(
        _operand(yt, [98 * b + 2 * p, 98 * b + 2 * p + 1], pl.ds(half * R // 4, R // 4)),
        _operand(wa, [13 * j + p // 4], pl.ds(128 * (p % 4), 128)))
    mu[p, pl.ds(0, R // 2), :] = res
    return res


def _mixer(zero, mu0, wa, xs, w4t, hbuf, yt, wo_b, xg, w1b, w2b, q_rings, ulast, lhs0, lhs1, hs0, hs1, *ybuf):
    lhs, hs = (lhs0, lhs1), (hs0, hs1)

    def encode_w3(j, t):
        def get(k, n):
            r = C4 * k + 16 * t
            return yt[32 * j + 8 * n + r // 128, pl.ds(r % 128, 16), :].astype(f32)

        def emit(p, v):
            wa[13 * j + p // 4, pl.ds(C4 * (p % 4) + 16 * t, 16), :] = v.astype(bf16)

        return _enc2(ENC_B, get, emit)

    def encode_w4(j, t, c, head):
        def get(k, n):
            if head:
                return xs[n // 2, pl.ds(pl.multiple_of(512 * j + 128 * k + 16 * t, 16), 16),
                          pl.ds(C4 * (n % 2) + 128 * c, 128)].astype(f32)
            return yt[32 * NJ + W4T * (2 * n + c) + 4 * j - S // R + k,
                      pl.ds(16 * t, 16), :].astype(f32)

        def emit(p, v):
            w4t[2 * p + c, pl.ds(pl.multiple_of(128 * j + 16 * t, 16), 16), :] = v.astype(bf16)

        return _enc2(ENC_B, get, emit)

    done = TOK * NSEG
    first = 4 * TOK * (NSEG // 4 - 1)

    @jax.named_scope('q1')
    def q1(g):
        n = 128
        for k, q in enumerate(q_rings):
            for r in range(0, P0, 64):
                lhs0[k, pl.ds(r, 64), :] = q[g, pl.ds((done + r) % RING, 64), :].astype(bf16)

        part = []

        def dot(r, c, k):
            w = wo_b[pl.ds(pl.multiple_of((2 * g + k) * 2 * DH, 2 * DH), 2 * DH),
                     pl.ds(128 * c, 128)]
            res = _dot(_operand(lhs0, range(4 * k, 4 * k + 4), pl.ds(r // 2, n // 2)), _unpack(w))
            if k == 0:
                part.append(res)
            else:
                hbuf[c // 4, pl.ds(done + r, n), pl.ds(128 * (c % 4), 128)] += part.pop() + res
            return res

        _interleave(
            [functools.partial(dot, r, c, k)
             for r in range(0, P0, n) for c in range(8) for k in range(2)],
            lambda res: [_pace(yt, (98 * NB,), zero, res), _pace(xs, (0,), S + zero, res)] + ([_pace(w4t, (98,), zero, res)] if E_('P4', 0) else []),
            (itertools.chain(*[
                encode_w4(j, t, c, head) for t in range(8) for c in range(2)
                for j, head in ((g, True), (jnp.minimum(S // 512 + g, NJ - 1), False))]), 7 * 32),
            (itertools.chain(*[encode_w3(jnp.minimum(2 * g + k, NJ - 1), t)
                               for k in range(2) for t in range(16)]), 7 * 32), pieces=E_('QP', 4))

    pl.loop(0, H // 8)(q1)

    def mixer_norm(r0, n):
        for r in range(r0, r0 + n, 16):
            _set_blocks(ulast, pl.ds(r, 16), _ln(_ln(_rows(hbuf, pl.ds(first + r, 16)))))
            yield

    def mixer_in(c):
        n = (S - first) // 2
        for r, k in itertools.product((0, n), range(2)):
            cols = pl.ds(128 * k, 128)
            xg[2 * c + k, pl.ds(HALO + first + r, n), :] = _gelu(_dot(
                _operand(ulast, range(8), pl.ds(r // 2, n // 2)), _unpack(w1b[c, :, cols])))

    def shift(i, dst):
        for r in range(0, RB, 64):
            for c, off in enumerate((-1, 1, -2, 2)):
                for k in (2 * c, 2 * c + 1):
                    dst[k, pl.ds(r, 64), :] = xg[
                        k, pl.ds(HALO + off + i * RB + r, 64), :].astype(bf16)
                yield

    def mixer_out(src, dst):
        n = E_("MR", 128)

        part = []

        def dot(r, c, k):
            cols = pl.ds(128 * c, 128)
            res = _dot(_operand(src, range(4 * k, 4 * k + 4), pl.ds(r // 2, n // 2)),
                       _unpack(w2b[pl.ds(C4 * k, C4), cols]))
            if k == 0:
                part.append(res)
            else:
                dst[pl.ds(r, n), cols] = part.pop() + res
            return res

        return [functools.partial(dot, r, c, k)
                for r in range(0, RB, n) for c in range(8) for k in range(2)]

    def residual(i, src, dst):
        late = []
        for t in range(0, RB, 8):
            rows = pl.ds(_mult(i * RB + t, 8), 8)
            hv = _rows(hbuf, rows)
            x1 = _ln(hv) + src[pl.ds(t, 8), :]
            late.append((rows, hv + x1, t, _ln(x1)))
            if len(late) > E_("LT", 0) or t == RB - 8:
                for rows, v, t0, y in late[:None if t == RB - 8 else 1]:
                    _set_rows(hbuf, rows, v)
                    dst[pl.ds(t0, 8), :] = y
                del late[0]
            yield

    def up_operands(i, src):
        per = 4 * R // RB
        for t, c in itertools.product(range(0, RB, 64), range(2)):
            def emit(p, v):
                yt[98 * (i // per) + 2 * p + c,
                   pl.ds(_mult(i % per * (RB // 4) + t // 4, 16), 16), :] = v.astype(bf16)

            yield from _enc2(ENC_A, lambda q, k: src[
                pl.ds(t + 16 * q, 16), pl.ds(C4 * k + 128 * c, 128)], emit)

    def job(i, par, extra=None):
        work, paced = [], []
        if i + 1 < S // RB:
            work.append((shift(i + 1, lhs[1 - par]), RB // 16))
            paced.append((lhs[1 - par], (0,), P0 - 16 + zero))
        if extra is None:
            work.append((up_operands(i - 2, ybuf[par]), 14 * RB // 64))
            paced.append((yt, (98 * NB,), zero))
        else:
            work.append((mixer_norm(*extra), extra[1] // 16))
            paced.append((ulast, (0,), S - first + zero))
        if extra is None or i > 0:
            work.append((residual(i - 1, hs[1 - par], ybuf[1 - par]), RB // 8))
            paced.append((ybuf[1 - par], (), RB + zero))
        pl.loop(zero, 1)(lambda _: _interleave(
            mixer_out(lhs[par], hs[par]), lambda res: [_pace(*p, res) for p in paced], *work,
            pieces=8))

    cut = E_("CUT", 416)
    _run(shift(0, lhs[0]))
    with jax.named_scope('j01'):
        job(0, 0, (0, cut))
        job(1, 1, (cut, S - first - cut))
    with jax.named_scope('in'): pl.loop(0, 4)(mixer_in)

    with jax.named_scope('jobs'):
        for i in range(2, S // RB):
            job(i, i % 2)

    last = S // RB - 1
    _interleave(
        [functools.partial(_up_dot, yt, wa, mu0, 0, 0, 0, p) for p in range(49)],
        lambda res: [_pace(y, (), RB + zero, res) for y in ybuf],
        (up_operands(last - 1, ybuf[0]), 14 * RB // 64),
        (residual(last, hs[1], ybuf[1]), RB // 8), pieces=1)
    _run(up_operands(last, ybuf[1]))


def _mlp(zero, out_hbm, wa, xs, hbuf, w4t, yt, sems, mu0, tt0, tt1, mu1, md):
    tts, mu = (tt0, tt1), (mu0, mu1)
    hr = R // 2
    lag = E_("LAG", 14)

    def out_copy(b, n):
        rows = pl.ds(_mult(b * 4 * R, 4 * R), 4 * R)
        return pltpu.make_async_copy(xs.at[n, rows], out_hbm.at[rows, pl.ds(n * HD, HD)],
                                     sems.at[SEM_OUT + 2 * b + n])

    def up_dot(b, j, half, p):
        return _up_dot(yt, wa, mu[half], b, j, half, p)

    def up_sums(act):
        for half, t in itertools.product(range(2), range(hr // 8)):
            c = {}
            for g in ORDER:
                y = _dec(lambda k: mu[half][7 * g + k, pl.ds(8 * t, 8), :])
                for i1, n1, sign in DEC[g]:
                    for (i0, n0), m in y.items():
                        key = (2 * i1 + i0, 2 * n1 + n0)
                        _accumulate(c, key, m, sign)
                        if LAST[i1, n1] == g:
                            act[half, t, key] = _gelu(c.pop(key))
                yield

    def down_operands(act, tt, j):
        for half, t in itertools.product(range(2), range(hr // 16)):
            def emit(p, v):
                tt[NJ * p + j, pl.ds(half * hr + 16 * t, 16), :] = v.astype(bf16)

            yield from _enc2(ENC_A, lambda q, k: jnp.concatenate(
                [act[half, 2 * t, (q, k)], act[half, 2 * t + 1, (q, k)]], axis=0), emit)

    n_sums = 7 * 2 * (hr // 8)

    def up_vector_work(tt, j):
        act = {}
        a, b = up_sums(act), down_operands(act, tt, j)
        for i in range(n_sums + lag):
            if i < n_sums:
                next(a)
            if i >= lag and (i - lag) % 2 == 1:
                next(b)
            yield

    def down_dot(tt, g, slot, i):
        p = 7 * g + i // 2
        res = _dot(
            _operand(tt, [NJ * p + q for q in range(NJ)], pl.ds(0, R // 2)), _operand(w4t, [14 * g + i], pl.ds(0, F // 8)))
        md[7 * slot + i // 2, pl.ds(0, R), pl.ds(128 * (i % 2), 128)] = res
        return res

    def down_block(slot, t):
        c = _dec(lambda k: md[7 * slot + k, pl.ds(16 * t, 16), :])
        return jnp.concatenate(
            [jnp.concatenate([c[i0, 0], c[i0, 1]], axis=1) for i0 in range(2)], axis=0)

    def down_sums(b, g, slot):
        dst = []
        for w in range(2):
            i1 = n1 = sign = 0
            for q in range(7):
                e = DEC[q][w] if w < len(DEC[q]) else DEC[q][0][:2] + (0,)
                i1, n1, sign = (jnp.where(g == q, new, old)
                                for new, old in zip(e, (i1, n1, sign)))
            dst.append((b * 4 * R + 32 * i1, n1, sign.astype(f32)))
        for t in range(R // 16):
            m = down_block(slot, t)
            rows = [pl.ds(pl.multiple_of(d[0] + 64 * t, 32), 32) for d in dst]
            new = [hbuf[dst[0][1], rows[0], :] + m,
                   hbuf[dst[1][1], rows[1], :] + dst[1][2] * m]
            for w in (1, 0):
                hbuf[dst[w][1], rows[w], :] = new[w]
                xs[dst[w][1], rows[w], :] = new[w].astype(bf16)
            yield

    def step(b, par, up, down, j):
        slot = (7 * b + j) & 1
        dots = []
        if up:
            nb = jnp.minimum(b + (j + 1) // NJ, NB - 1)
            nj = jnp.where(j == NJ - 1, 0, j + 1)
            dots = ([(1, functools.partial(up_dot, b, j, 1, p)) for p in range(49)]
                    + [(1, functools.partial(up_dot, nb, nj, 0, p)) for p in range(49)])
            up_work = up_vector_work(tts[par], j)
        if down:
            for i in range(14):
                dots.insert((8 * i + E_('D0', 7) if not E_('DM', 0) else [int(v) for v in os.environ['AT'].split(',')][i // E_('DM', 0)] + i) if up else i,
                            (7, functools.partial(down_dot, tts[1 - par], j, slot, i)))
            down_work = down_sums(jnp.maximum(b - 1 - (j == 0), 0),
                                  jnp.where(j == 0, 6, j - 1), 1 - slot)
        total = sum(w for w, _ in dots)
        pos = n_up = done_up = done_down = 0
        for w, dot in dots:
            if down:
                goal = (pos + E_("AD", 14)) * (R // 16) * 100 // (E_("DE", 100) * total)
                for _ in range(done_down, goal):
                    next(down_work, None)
                done_down = max(done_down, goal)
            res = dot()
            k = E_("PD", 4) if w > 1 else 1
            for i in range(k * up):
                if E_('PM', 2) and (w > 1 or n_up % E_('PM', 2) == 0):
                    _pace(mu[done_up >= n_sums // 2], (49,), zero, res[:res.shape[0] * (i + 1) // k])
                if E_('PN', 2) and (w > 1 or n_up % E_('PN', 2) == 0):
                    _pace(tts[par], (49 * NJ,), zero, res[:res.shape[0] * (i + 1) // k])
                goal = (pos * k + w * (i + 1) + E_("AH", 4) * k) * (n_sums + lag) // (total * k)
                goal = (min(goal, n_sums // 2) if n_up + (w == 1) < 49
                        else max(goal, n_sums // 2))
                for _ in range(done_up, goal):
                    next(up_work, None)
                done_up = max(done_up, goal)
            pos += w
            n_up += w == 1
        if up:
            _run(up_work)
        if down:
            _run(down_work)
        if down:
            @pl.when((j == 0) & (b > 1))
            def _():
                for n in range(2):
                    out_copy(b - 2, n).start()

    md[pl.ds(0, 7), pl.ds(0, R), :] = jnp.zeros((7, R, C4), f32)
    with jax.named_scope('b0'): pl.loop(0, NJ)(functools.partial(step, 0, 0, True, False))

    @pl.loop(0, NB // 2)
    @jax.named_scope('bmid')
    def _(i):
        pl.loop(0, NJ)(functools.partial(step, 2 * i + 1, 1, True, True))
        pl.loop(0, jnp.where(2 * i + 2 < NB, NJ, 0))(
            functools.partial(step, 2 * i + 2, 0, True, True))

    with jax.named_scope('b4'): pl.loop(0, NJ)(functools.partial(step, NB, 0, False, True))
    out_copy(NB - 1, 1).start()
    pieces = []
    for t in range(R // 16):
        rows = pl.ds(S - 4 * R + 64 * t, 32)
        xs[0, rows, :] = (hbuf[0, rows, :] + down_block((7 * NB + 6) & 1, t)).astype(bf16)
        if t % 2:
            rows = pl.ds(S - 4 * R + 64 * (t - 1), 128)
            pieces.append(pltpu.make_async_copy(
                xs.at[0, rows], out_hbm.at[rows, pl.ds(0, HD)], sems.at[t // 2]))
            pieces[-1].start()
    for b, n in itertools.product(range(NB), range(2)):
        if (b, n) != (NB - 1, 0):
            out_copy(b, n).wait()
    for c in pieces:
        c.wait()


@jax.jit
def pallas_sequential_preLN__memory_aug_recurrent_mem_tr__mixer_s_mlp__prompt_kernel(
    A_x: jax.Array,
    A_mem0: jax.Array,
    A_Wq: jax.Array,
    A_Wk: jax.Array,
    A_Wv: jax.Array,
    A_Wo: jax.Array,
    A_seg_len: jax.Array,
    B_x: jax.Array,
    B_w1: jax.Array,
    B_w2: jax.Array,
    B_w3: jax.Array,
    B_w4: jax.Array,
):
    del A_seg_len, B_x
    hbm = pl.BlockSpec(memory_space=pl.ANY)
    vmem = pl.BlockSpec(memory_space=pltpu.VMEM)
    scratch = [
        pltpu.VMEM((3 * H + 1, D, DH), bf16),
        pltpu.VMEM((2, S + 32, HD), bf16),
        pltpu.VMEM((2, S, HD), f32),
        pltpu.VMEM((99, F // 4, 128), bf16),
        pltpu.VMEM((98 * NB + 1, R, 128), bf16),
        pltpu.VMEM((52, R // 2 + 8, 128), f32),
        pltpu.SemaphoreType.DMA((NSEM,)),
    ]
    out = pl.pallas_call(
        _kernel,
        out_shape=jax.ShapeDtypeStruct((S, D), A_x.dtype),
        in_specs=[hbm, vmem] + [hbm] * 9,
        out_specs=hbm,
        scratch_shapes=scratch,
        compiler_params=pltpu.CompilerParams(vmem_limit_bytes=127 * 1024 * 1024),
    )(A_x.reshape(S, D), A_mem0.reshape(MEM, D),
      A_Wq.reshape(D // 2, 2 * H, DH), A_Wk.reshape(D // 2, 2 * H, DH),
      A_Wv.reshape(D // 2, 2 * H, DH),
      A_Wo.reshape(H * DH, D), B_w1, B_w2, B_w3.reshape(D // R, R, F),
      B_w4.reshape(F // R, R, D), B_w4)
    return out.reshape(A_x.shape)
```

```python
import functools
import itertools
import os

import jax
import jax.numpy as jnp
from jax import lax
import jax.experimental.pallas as pl
import jax.experimental.pallas.tpu as pltpu

S = 2048
D = 1024
H = 32
DH = 128
MEM = 8
SEG = 32
F = 3584
NSEG = S // SEG
L = MEM + SEG
TOK = 24
P0 = S - TOK * NSEG
RING = 576
XP = (S - P0) // 8
C4 = D // 4
HALO = 8
RB = 256
R = 128
NB = S // (4 * R)
NJ = F // 512
HD = D // 2
W4T = (F - S) // R
E_ = lambda k, d: int(os.environ.get(k, d))
EPS = 1e-5
NEG = -1000000000.0

LAG_QK, LAG_PV, LAG_WO = E_('LQ', 2), E_('LP', 4), E_('LW', 5)
FILL_AT = E_('FA', 17)
UNROLL = 2

bf16 = jnp.bfloat16
f32 = jnp.float32
u32 = jnp.uint32

SEM_X0, SEM_X, SEM_WO, SEM_W1, SEM_W2, SEM_OUT, SEM_W, SEM_W4, SEM_W3 = (
    0, 2, 10, 14, 18, 20, 28, 40, 50)
NSEM = SEM_W3 + 4 * NJ

ENC_A = (((0, 0, 1), (1, 1, 1)), ((1, 0, 1), (1, 1, 1)), ((0, 0, 1),), ((1, 1, 1),),
         ((0, 0, 1), (0, 1, 1)), ((1, 0, 1), (0, 0, -1)), ((0, 1, 1), (1, 1, -1)))
ENC_B = (((0, 0, 1), (1, 1, 1)), ((0, 0, 1),), ((0, 1, 1), (1, 1, -1)),
         ((1, 0, 1), (0, 0, -1)), ((1, 1, 1),), ((0, 0, 1), (0, 1, 1)),
         ((1, 0, 1), (1, 1, 1)))
DEC = (((0, 0, 1), (1, 1, 1)), ((1, 0, 1), (1, 1, -1)), ((0, 1, 1), (1, 1, 1)),
       ((0, 0, 1), (1, 0, 1)), ((0, 1, 1), (0, 0, -1)), ((1, 1, 1),), ((0, 0, 1),))
ORDER = (0, 1, 3, 2, 4, 5, 6)
LAST = {(1, 0): 3, (0, 1): 4, (1, 1): 5, (0, 0): 6}


def _enc(terms, get):
    v = get(*terms[0][:2])
    for i, j, sign in terms[1:]:
        v = v + get(i, j) if sign > 0 else v - get(i, j)
    return v


def _enc2(table, get, emit):
    for g in range(7):
        y = [[_enc(table[g], lambda i1, j1: get(2 * i1 + i0, 2 * j1 + j0))
              for j0 in range(2)] for i0 in range(2)]
        for k in range(7):
            emit(7 * g + k, _enc(table[k], lambda i0, j0: y[i0][j0]))
        yield


def _accumulate(c, key, m, sign):
    c[key] = m if key not in c else (c[key] + m if sign > 0 else c[key] - m)


def _dec(get):
    c = {}
    for k in range(7):
        m = get(k)
        for i, j, sign in DEC[k]:
            _accumulate(c, (i, j), m, sign)
    return c


def _pace(ref, lead, row, result):
    n = 32 // ref.dtype.itemsize
    ref[(*lead, pl.ds(pl.multiple_of(row, n), n), pl.ds(0, 128))] = (
        result[-n:, :128].astype(ref.dtype))


def _run(gen):
    for _ in gen:
        pass


def _mult(i, n):
    return i if isinstance(i, int) else pl.multiple_of(i, n)


def _ln(x):
    m = jnp.mean(x, axis=-1, keepdims=True)
    d = x - m
    v = jnp.mean(d * d, axis=-1, keepdims=True)
    return d * lax.rsqrt(v + EPS)


def _gelu(x):
    c = 0.7978845608028654
    hx = 0.5 * x
    return hx + hx * jnp.tanh(x * (c + (c * 0.044715) * (x * x)))


def _unpack(x):
    return pltpu.bitcast(x, bf16)


def _operand(ref, blocks, rows=slice(None)):
    words = ref.bitcast(u32)
    return _unpack(jnp.concatenate([words[b, rows, :] for b in blocks], axis=1))


def _set_blocks(ref, rows, v):
    for c in range(v.shape[1] // 128):
        ref[c, rows, :] = v[:, 128 * c:128 * c + 128].astype(bf16)


def _dot(a, b):
    return jnp.dot(a, b, preferred_element_type=f32)


def _rows(ref, rows):
    return jnp.concatenate([ref[0, rows, :], ref[1, rows, :]], axis=1)


def _set_rows(ref, rows, v):
    ref[0, rows, :] = v[:, :HD]
    ref[1, rows, :] = v[:, HD:]


def _kernel(*refs):
    out_hbm, wa, xs, hbuf, w4t, yt, mu0, sems = refs[11:]
    zero = pl.run_scoped(
        functools.partial(_attention_and_mixer, *refs),
        pltpu.VMEM((H * DH // 2, D), u32),
        pltpu.VMEM((8, S + 4 * HALO, 128), f32),
        pltpu.VMEM((8, 4 * TOK, 128), bf16),
        pltpu.VMEM((4, D // 2, C4), u32),
        pltpu.VMEM((D, D), bf16),
        *[pltpu.VMEM((H // 8, RING, DH), f32)] * 8)
    if E_("SKIP_MLP", 0):
        for b in (w4t, yt, wa):
            pltpu.sync_copy(b.at[0, pl.ds(0, 128)], out_hbm.at[pl.ds(0, 128), pl.ds(0, 128)])
        return
    with jax.named_scope('s_mlp'): pl.run_scoped(
        functools.partial(_mlp, zero, out_hbm, wa, xs, hbuf, w4t, yt, sems, mu0),
        *[pltpu.VMEM((49 * NJ + 1, R, 128), bf16)] * 2,
        pltpu.VMEM(mu0.shape, f32),
        pltpu.VMEM((14, R, C4), f32))


def _attention_and_mixer(x_hbm, mem0_ref, wq_hbm, wk_hbm, wv_hbm, wo_hbm, w1_hbm, w2_hbm,
                         w3_hbm, w4_hbm, w4a_hbm, out_hbm, wa, xs, hbuf, w4t, yt, mu0, sems,
                         wo_b, xg, ubuf, w1b, w2b, *q_rings):
    w2_copy = pltpu.make_async_copy(w2_hbm, w2b, sems.at[SEM_W2])

    def w3_copy(c):
        return pltpu.make_async_copy(
            w3_hbm.at[:, :, pl.ds(_mult(c * 128, 128), 128)], yt.at[pl.ds(8 * c, 8)],
            sems.at[SEM_W3 + c])

    def w4_head_copy(n):
        return pltpu.make_async_copy(
            w4a_hbm.at[pl.ds(0, S), pl.ds(n * HD, HD)], xs.at[n, pl.ds(0, S)], sems.at[SEM_W4 + n])

    def w4_tail_copy(c):
        return pltpu.make_async_copy(
            w4_hbm.at[pl.ds(S // R, W4T), :, pl.ds(c * 128, 128)],
            yt.at[pl.ds(32 * NJ + W4T * c, W4T)], sems.at[SEM_W4 + 2 + c])

    others = [[w2_copy], [w4_head_copy(0)], [w4_head_copy(1)],
              [w4_tail_copy(c) for c in range(8)]]

    def fetch(i):
        for c in range(NJ):
            w3_copy(NJ * i + c).start()
        for k, copies in enumerate(others):
            @pl.when(i == k)
            def _():
                for c in copies:
                    c.start()

    zero = pl.run_scoped(
        functools.partial(_attention, x_hbm, mem0_ref, (wq_hbm, wk_hbm, wv_hbm), wo_hbm,
                          w1_hbm, fetch, w4t, yt, wa, xs, hbuf, sems, wo_b, xg, ubuf, w1b, q_rings),
        *[pltpu.VMEM((H // 8, RING, DH), f32)] * 16)
    for c in sum(others, []):
        c.wait()
    for c in range(4 * NJ):
        w3_copy(c).wait()
    if E_("SKIP_POST", 0): return zero
    with jax.named_scope('s_mix'): pl.run_scoped(
        functools.partial(_mixer, zero, mu0, wa, xs, w4t, hbuf, yt, wo_b, xg, w1b, w2b, q_rings),
        pltpu.VMEM((29, HD, 128), bf16),
        pltpu.VMEM((8, P0 + 4 * TOK + 16, 128), bf16),
        *[pltpu.VMEM((8, P0, 128), bf16)] * 2, *[pltpu.VMEM((RB, D), f32)] * 2,
        *[pltpu.VMEM((RB + 8, D), f32)] * 2)
    return zero


def _attention(x_hbm, mem0_ref, w_hbm, wo_hbm, w1_hbm, fetch,
               w4t, yt, wa, xs, hbuf, sems, wo_b, xg, ubuf, w1b, q_rings, *kv_rings):
    rings = q_rings + kv_rings
    ring = [[rings[m * 8 + h % 8].at[h // 8] for h in range(H)] for m in range(3)]
    q_r, k_r, v_r = ring

    class x_rows:
        def __init__(self, rows, sem):
            self.copies = [
                pltpu.make_async_copy(x_hbm.at[rows, pl.ds(n * HD, HD)], xs.at[n, rows],
                                      sems.at[sem + n]) for n in range(2)]

        def start(self):
            for c in self.copies:
                c.start()

        def wait(self):
            for c in self.copies:
                c.wait()

    x0_copy = x_rows(pl.ds(0, P0), SEM_X0)

    def x_copy(g):
        return x_rows(pl.ds(_mult(P0 + g * 2 * XP, XP), 2 * XP), SEM_X + 2 * g)

    def wo_copy(i):
        rows = pl.ds(_mult(i * 512, 512), 512)
        return pltpu.make_async_copy(wo_hbm.bitcast(u32).at[rows], wo_b.at[rows],
                                     sems.at[SEM_WO + i])

    def w1_copy(i):
        cols = pl.ds(_mult(i * C4, C4), C4)
        return pltpu.make_async_copy(w1_hbm.bitcast(u32).at[:, cols], w1b.at[i],
                                     sems.at[SEM_W1 + i])

    def prologue(*stg):

        def start_chunk(g, m):
            src = w_hbm[m].bitcast(u32)
            dst = stg[m].reshape(D // 2, 8, DH)
            for q in range(8 * E_("DS", 1)):
                pltpu.make_async_copy(
                    src.at[:, 16 * (q // 4) + 4 * g + q % 4, :],
                    stg[m].at[pl.ds(q * HD, HD)], sems.at[SEM_W + 3 * g + m]).start()
            for par in range(2 - 2 * E_("DS", 1)):
                pltpu.make_async_copy(
                    src.at[:, pl.ds(_mult(16 * par + 4 * g, 4), 4), :],
                    dst.at[:, pl.ds(4 * par, 4), :],
                    sems.at[SEM_W + 3 * g + m]).start()

        def wait_chunk(g, m):
            pltpu.make_async_copy(stg[m], stg[m], sems.at[SEM_W + 3 * g + m]).wait()

        def relayout(g, m, pair, i0, n):
            ev = stg[m][pl.ds(8 * i0 + pair, n, stride=8), :]
            od = stg[m][pl.ds(8 * i0 + 4 + pair, n, stride=8), :]
            if E_("DS", 1):
                ev = stg[m][pl.ds(_mult(pair * HD + i0, 8), n), :]
                od = stg[m][pl.ds(_mult((4 + pair) * HD + i0, 8), n), :]
            h = 8 * g + 2 * pair
            words = wa.bitcast(u32)
            words[m * H + h, pl.ds(i0, n), :] = (ev & jnp.uint32(0xFFFF)) | (od << 16)
            words[m * H + h + 1, pl.ds(i0, n), :] = (ev >> 16) | (od & jnp.uint32(0xFFFF0000))

        def weights(g, m, pair):
            h = m * H + 8 * g + 2 * pair
            for t in range(D // 32 + 1):
                if t < D // 32:
                    for k in range(2):
                        relayout(g, m, pair, D // 4 * k + 8 * t, 8)
                if t > 0:
                    r = 16 * (t - 1)
                    b = [[wa[h + n, pl.ds(HD * k + r, 16), :].astype(f32) for n in range(2)]
                         for k in range(2)]
                    for p in range(7):
                        w4t[28 * m + 7 * pair + p, pl.ds(r, 16), :] = _enc(
                            ENC_B[p], lambda k, n: b[k][n]).astype(bf16)
                yield

        def norm_rows(r0, n):
            xv = _rows(xs, pl.ds(r0, n)).astype(f32)
            _set_rows(hbuf, pl.ds(r0, n), xv)
            return _ln(xv)

        def later_rows(r0):
            for r in range(0, XP, 16):
                xn = norm_rows(pl.multiple_of(r0 + r, 16), 16)
                for c in range(8):
                    xg[c, pl.ds(pl.multiple_of(HALO + r0 + r, 8), 16), :] = (
                        xn[:, 128 * c:128 * c + 128])
                yield

        x0_copy.start()
        start_chunk(0, 0)
        start_chunk(0, 1)
        start_chunk(0, 2)
        x_copy(0).start()
        zero = jnp.zeros((HALO, 128), f32)
        for c in range(8):
            xg[c, pl.ds(0, HALO), :] = zero
            xg[c, pl.ds(HALO + S, HALO), :] = zero
        with jax.named_scope('wx'): x0_copy.wait()

        @pl.loop(0, P0 // 64)
        def _(i):
            a = [norm_rows(pl.multiple_of(P0 // 2 * k + 32 * i, 32), 32) for k in range(2)]
            for p in range(7):
                v = _enc(ENC_A[p], lambda k, n: a[k][:, HD * n:HD * n + HD])
                for c in range(4):
                    yt[8 * p + 4 * (i // 4) + c, pl.ds(pl.multiple_of(i % 4 * 32, 32), 32), :] = (
                        v[:, 128 * c:128 * c + 128].astype(bf16))

        with jax.named_scope('w0'): wait_chunk(0, 0)
        pl.loop(0, 4)(lambda pair: _run(weights(0, 0, pair)))

        def stage(g, m):
            m1 = (m + 1) % 3
            g1 = jnp.minimum(g + (1 if m == 2 else 0), 3)
            if m > 0:
                pl.when(3 * g + m < 11)(functools.partial(wait_chunk, g1, m1))
            if m == 1:
                x_copy(g).wait()

            @pl.when(g < 3)
            def _():
                start_chunk(g + 1, m)
                if m == 1:
                    x_copy(g + 1).start()
            if m == E_('WM', 1):
                wo_copy(g).start()
            if m == 2:
                w1_copy(g).start()
            n = E_("PR", 64)
            acc = {}

            def dot(pair, r, p):
                res = _dot(
                    _operand(yt, [8 * p + 4 * (r // R) + k for k in range(4)],
                             pl.ds(r % R // 2, n // 2)),
                    _operand(w4t, [28 * m + 7 * pair + p], pl.ds(0, HD // 2)))
                for i, j, sign in DEC[p]:
                    _accumulate(acc, (i, j), res, sign)
                    if LAST[i, j] == p:
                        rings[m * 8 + 2 * pair + j][g, pl.ds(P0 // 2 * i + r, n), :] = (
                            acc.pop((i, j)))
                return res

            dots = [functools.partial(dot, pair, r, p) for pair in range(4)
                    for r in range(0, P0 // 2, n) for p in ORDER]
            work = [(itertools.chain(*[weights(g1, m1, pair) for pair in range(4)]),
                     4 * (D // 32 + 1))]
            paced = [(wa, (3 * H,), 16 * (g >> 10))]
            if m == 0:
                early = E_("EA", 49)
                for d in dots[:early]:
                    d()
                dots = dots[early:]
                wait_chunk(g1, m1)
            else:
                work.append((later_rows(P0 + (2 * g + m - 1) * XP), XP // 16))
                paced.append((xg, (0,), S + 2 * HALO + 8 * (g >> 10)))
            _interleave(dots, lambda res: [_pace(*p, res) for p in paced], *work,
                        pieces=1 if m else E_("PQ", 2))

        @pl.loop(0, 4)
        def _(g):
            for m in range(3):
                stage(g, m)

    if not E_('SKIP_PRO', 0):
     with jax.named_scope('s_pro'): pl.run_scoped(
        prologue,
        pltpu.VMEM((8 * D // 2, DH), u32),
        pltpu.VMEM((8 * D // 2, DH), u32),
        pltpu.VMEM((8 * D // 2, DH), u32),
    )
    for i in range(4):
        if E_('WM', 1) > 2: wo_copy(i).start()
        with jax.named_scope('wwo'): wo_copy(i).wait()
    for i in range(4):
        w1_copy(i).wait()

    def wrap(r):
        return jnp.where(r >= RING, r - RING, r)

    def load_tok(s):
        rows = pl.ds(pl.multiple_of(HALO + P0 + TOK * s, 8), TOK)
        return jnp.concatenate([xg[c, rows, :] for c in range(8)], axis=1)

    def step(s, carry, tok, first_of_group):
        mem, rp, ra, rw = carry
        ri = lax.broadcasted_iota(jnp.int32, (2 * L, 2 * L), 0)
        ci = lax.broadcasted_iota(jnp.int32, (2 * L, 2 * L), 1)
        same = (ri >= L) == (ci >= L)
        ri, ci = (jnp.where(v >= L, v - L, v) for v in (ri, ci))
        mask = same & ((ri < MEM) | (ri >= ci))
        fill = jnp.where(same, NEG, -jnp.inf)

        lhs = jnp.concatenate([mem, tok], axis=0).astype(bf16)
        rps = [pl.multiple_of(wrap(rp + 8 * i), 8) for i in range(3)]
        ra_ = pl.multiple_of(ra, SEG)
        rw_ = pl.multiple_of(rw, 8)

        col = s & 3
        rb = pl.multiple_of(jnp.maximum((s >> 2) - 1, 0) * (4 * TOK), 8)
        if first_of_group:
            _set_blocks(ubuf, slice(None), _ln(_ln(_rows(hbuf, pl.ds(rb, 4 * TOK)))))

        def filler(j):
            r = _dot(_operand(ubuf, range(8)), _unpack(w1b[col, :, pl.ds(j * 128, 128)]))
            xg[2 * col + j, pl.ds(HALO + rb, 4 * TOK), :] = _gelu(r)

        mem_qkv = {}
        scores = {}
        o_mem = {}
        total = [None]

        def qkv(h):
            res = []
            for m in range(3):
                r = _dot(lhs, _operand(wa, [m * H + h]))
                for i in range(3):
                    ring[m][h][pl.ds(rps[i], 8), :] = r[8 + 8 * i:16 + 8 * i]
                res.append(r[:MEM])
            mem_qkv[h] = res

        def both(m, a):
            return jnp.concatenate(
                [v for h in (2 * a, 2 * a + 1)
                 for v in (mem_qkv[h][m], ring[m][h][pl.ds(ra_, SEG), :])],
                axis=0).astype(bf16)

        def qk(a):
            scores[a] = lax.dot_general(both(0, a), both(1, a), (((1,), (1,)), ((), ())),
                                        preferred_element_type=f32)

        def pv(a):
            sc = jnp.where(mask, scores.pop(a) * (DH ** -0.5), fill)
            mx = jnp.max(sc, axis=1, keepdims=True)
            e = jnp.exp(sc - mx)
            den = jnp.sum(e, axis=1, keepdims=True)
            inv = pl.reciprocal(den, approx=True)
            inv = inv * (2.0 - den * inv)
            o = _dot(e.astype(bf16), both(2, a)) * inv
            for i, h in enumerate((2 * a, 2 * a + 1)):
                q_r[h][pl.ds(ra_, SEG), :] = o[i * L + MEM:(i + 1) * L]
                o_mem[h] = o[i * L:i * L + MEM]

        def wo(h):
            lo = jnp.concatenate([o_mem.pop(h), q_r[h][pl.ds(rw_, TOK), :]],
                                 axis=0).astype(bf16)
            r = _dot(lo, _unpack(wo_b[pl.ds(h * DH // 2, DH // 2), :]))
            total[0] = r if total[0] is None else total[0] + r

        npair = H // 2
        for t in range(npair + LAG_WO):
            def attend():
                if E_("AM", 1) == 1:
                    for f, lag in ((qk, LAG_QK), (pv, LAG_PV))[::E_("REV", 1)]:
                        if 0 <= t - lag < npair:
                            f(t - lag)
                elif t % 2 == E_("PH", 0):
                    for f, lag in ((qk, LAG_QK), (pv, LAG_PV))[::E_("REV", 1)]:
                        for a in (t - lag, t - lag + 1):
                            if 0 <= a < npair:
                                f(a)
            if E_("WF", 0) and 0 <= t - LAG_WO < npair:
                wo(2 * (t - LAG_WO))
                wo(2 * (t - LAG_WO) + 1)
            if E_("AP", 0) == 0: attend()
            if t < npair:
                qkv(2 * t)
            if E_("AP", 0) == 1: attend()
            if t < npair:
                qkv(2 * t + 1)
            if E_("AP", 0) == 2: attend()
            if t == FILL_AT:
                filler(0)
            if not E_("WF", 0) and 0 <= t - LAG_WO < npair:
                wo(2 * (t - LAG_WO))
                wo(2 * (t - LAG_WO) + 1)
            if E_("AP", 0) == 3: attend()
        filler(1)

        a = total[0]
        rows = pl.ds(pl.multiple_of(TOK * s, 8), TOK)
        _set_rows(hbuf, rows, _rows(hbuf, rows) + a[MEM:])
        return a[:MEM], wrap(rp + TOK), wrap(ra + SEG), wrap(rw + TOK)

    def steps(i, carry):
        toks = [load_tok(i * UNROLL + k) for k in range(UNROLL)]
        for k in range(UNROLL):
            carry = step(i * UNROLL + k, carry, toks[k], k == 0)
        return carry

    def quarter(k, carry):
        fetch(k)
        n = NSEG // UNROLL // 4
        return lax.fori_loop(k * n, (k + 1) * n, steps, carry)

    if E_('SKIP_LOOP', 0): return lax.fori_loop(0, 64, lambda i, c: wrap(c + TOK), jnp.int32(0)) - TOK * NSEG % RING
    with jax.named_scope('s_loop'): carry = lax.fori_loop(
        0, 4, quarter,
        (mem0_ref[...].astype(f32), jnp.int32(P0), jnp.int32(0), jnp.int32(0)))
    return carry[3] - TOK * NSEG % RING


def _interleave(dots, pace, *work, pieces=8):
    for i, dot in enumerate(dots):
        res = dot()
        k = min(pieces, res.shape[0] // 16)
        for j in range(k):
            pace(res[:res.shape[0] // 16 * (j + 1) // k * 16])
            for gen, n in work:
                for _ in range(n * (i * k + j) // (k * len(dots)),
                               n * (i * k + j + 1) // (k * len(dots))):
                    next(gen)
    for gen, _ in work:
        _run(gen)


def _up_dot(yt, wa, mu, b, j, half, p):
    res = _dot(
        _operand(yt, [98 * b + 2 * p, 98 * b + 2 * p + 1], pl.ds(half * R // 4, R // 4)),
        _operand(wa, [13 * j + p // 4], pl.ds(128 * (p % 4), 128)))
    mu[p, pl.ds(0, R // 2), :] = res
    return res


def _mixer(zero, mu0, wa, xs, w4t, hbuf, yt, wo_b, xg, w1b, w2b, q_rings, w2t, ulast, lhs0, lhs1, hs0, hs1, *ybuf):
    lhs, hs = (lhs0, lhs1), (hs0, hs1)

    def encode_w3(g):
        for j, t in itertools.product(range(NJ), range(4)):
            def get(k, n):
                return yt[32 * j + 8 * n + 2 * k + (g >> 1),
                          pl.ds(pl.multiple_of(64 * (g & 1) + 16 * t, 16), 16), :].astype(f32)

            def emit(p, v):
                wa[13 * j + p // 4, pl.ds(pl.multiple_of(C4 * (p % 4) + 64 * g + 16 * t, 16), 16),
                   :] = v.astype(bf16)

            yield from _enc2(ENC_B, get, emit)

    def encode_w4(g):
        for j, t, c in itertools.product(range(NJ), range(2), range(2)):
            r = pl.multiple_of(32 * g + 16 * t, 16)

            def get(k, n):
                if 512 * j < S:
                    return xs[n // 2, pl.ds(512 * j + 128 * k + r, 16),
                              pl.ds(C4 * (n % 2) + 128 * c, 128)].astype(f32)
                return yt[32 * NJ + W4T * (2 * n + c) + 4 * j - S // R + k,
                          pl.ds(r, 16), :].astype(f32)

            def emit(p, v):
                w4t[2 * p + c, pl.ds(128 * j + r, 16), :] = v.astype(bf16)

            yield from _enc2(ENC_B, get, emit)

    def encode_w2(g):
        for t, c in itertools.product(range(8), range(4)):
            r = pl.multiple_of(128 * g + 16 * t, 16)
            b = [[w2b[pl.ds(HD * k + r, 16), pl.ds(HD * n + 128 * c, 128)].astype(f32)
                  for n in range(2)] for k in range(2)]
            for p in range(7):
                w2t[4 * p + c, pl.ds(r, 16), :] = _enc(
                    ENC_B[p], lambda k, n: b[k][n]).astype(bf16)
            yield

    done = TOK * NSEG
    first = 4 * TOK * (NSEG // 4 - 1)

    @jax.named_scope('q1')
    def q1(g):
        n = 128
        for k, q in enumerate(q_rings):
            for r in range(0, P0, 64):
                lhs0[k, pl.ds(r, 64), :] = q[g, pl.ds((done + r) % RING, 64), :].astype(bf16)

        part = []

        def dot(r, c, k):
            w = wo_b[pl.ds(pl.multiple_of((2 * g + k) * 2 * DH, 2 * DH), 2 * DH),
                     pl.ds(128 * c, 128)]
            res = _dot(_operand(lhs0, range(4 * k, 4 * k + 4), pl.ds(r // 2, n // 2)), _unpack(w))
            if k == 0:
                part.append(res)
            else:
                hbuf[c // 4, pl.ds(done + r, n), pl.ds(128 * (c % 4), 128)] += part.pop() + res
            return res

        _interleave(
            [functools.partial(dot, r, c, k)
             for r in range(0, P0, n) for c in range(8) for k in range(2)],
            lambda res: [_pace(yt, (98 * NB,), zero, res), _pace(xs, (0,), S + zero, res),
                         _pace(w2t, (28,), zero, res)],
            (encode_w2(g), 32),
            (encode_w4(g), 28 * NJ), (encode_w3(g), 28 * NJ), pieces=8)

    pl.loop(0, H // 8)(q1)

    def mixer_norm(r0, n):
        for r in range(r0, r0 + n, 16):
            _set_blocks(ulast, pl.ds(r, 16), _ln(_ln(_rows(hbuf, pl.ds(first + r, 16)))))
            yield

    def mixer_in(c):
        n = (S - first) // 2
        for r, k in itertools.product((0, n), range(2)):
            cols = pl.ds(128 * k, 128)
            xg[2 * c + k, pl.ds(HALO + first + r, n), :] = _gelu(_dot(
                _operand(ulast, range(8), pl.ds(r // 2, n // 2)), _unpack(w1b[c, :, cols])))

    def shift(i, dst):
        for r, c in itertools.product(range(0, RB // 2, 16), range(4)):
            a = [[xg[4 * k + c, pl.ds(HALO + (-1, 1, -2, 2)[2 * k + c // 2]
                                      + i * RB + RB // 2 * q + r, 16), :]
                  for k in range(2)] for q in range(2)]
            for p in range(7):
                dst[p, pl.ds(RB // 2 * c + r, 16), :] = _enc(
                    ENC_A[p], lambda q, k: a[q][k]).astype(bf16)
            yield

    def mixer_out(src, dst):
        n = 128
        acc = {}

        def dot(r, c, p):
            words = src.bitcast(u32)
            a = jnp.concatenate([words[p, pl.ds((RB // 2 * k + r) // 2, n // 2), :]
                                 for k in range(4)], axis=1)
            res = _dot(_unpack(a), _operand(w2t, [4 * p + c]))
            for i, j, sign in DEC[p]:
                _accumulate(acc, (i, j), res, sign)
                if LAST[i, j] == p:
                    dst[pl.ds(RB // 2 * i + r, n), pl.ds(HD * j + 128 * c, 128)] = acc.pop((i, j))
            return res

        return [functools.partial(dot, r, c, p)
                for r in range(0, RB // 2, n) for c in range(4) for p in ORDER]

    def residual(i, src, dst):
        late = []
        for t in range(0, RB, 8):
            rows = pl.ds(_mult(i * RB + t, 8), 8)
            hv = _rows(hbuf, rows)
            x1 = _ln(hv) + src[pl.ds(t, 8), :]
            late.append((rows, hv + x1, t, _ln(x1)))
            if len(late) > E_("LT", 0) or t == RB - 8:
                for rows, v, t0, y in late[:None if t == RB - 8 else 1]:
                    _set_rows(hbuf, rows, v)
                    dst[pl.ds(t0, 8), :] = y
                del late[0]
            yield

    def up_operands(i, src):
        per = 4 * R // RB
        for t, c in itertools.product(range(0, RB, 64), range(2)):
            def emit(p, v):
                yt[98 * (i // per) + 2 * p + c,
                   pl.ds(_mult(i % per * (RB // 4) + t // 4, 16), 16), :] = v.astype(bf16)

            yield from _enc2(ENC_A, lambda q, k: src[
                pl.ds(t + 16 * q, 16), pl.ds(C4 * k + 128 * c, 128)], emit)

    def job(i, par, extra=None):
        work, paced = [], []
        if i + 1 < S // RB:
            work.append((shift(i + 1, lhs[1 - par]), RB // 8))
            paced.append((lhs[1 - par], (7,), zero))
        if extra is None:
            work.append((up_operands(i - 2, ybuf[par]), 14 * RB // 64))
            paced.append((yt, (98 * NB,), zero))
        else:
            work.append((mixer_norm(*extra), extra[1] // 16))
            paced.append((ulast, (0,), S - first + zero))
        if extra is None or i > 0:
            work.append((residual(i - 1, hs[1 - par], ybuf[1 - par]), RB // 8))
            paced.append((ybuf[1 - par], (), RB + zero))
        pl.loop(zero, 1)(lambda _: _interleave(
            mixer_out(lhs[par], hs[par]), lambda res: [_pace(*p, res) for p in paced], *work,
            pieces=8))

    cut = E_('CUT', 496)
    _run(shift(0, lhs[0]))
    with jax.named_scope('j01'):
        job(0, 0, (0, cut))
        job(1, 1, (cut, S - first - cut))
    with jax.named_scope('in'): pl.loop(0, 4)(mixer_in)

    with jax.named_scope('jobs'):
        for i in range(2, S // RB):
            job(i, i % 2)

    last = S // RB - 1
    _interleave(
        [functools.partial(_up_dot, yt, wa, mu0, 0, 0, 0, p) for p in range(49)],
        lambda res: [_pace(y, (), RB + zero, res) for y in ybuf],
        (up_operands(last - 1, ybuf[0]), 14 * RB // 64),
        (residual(last, hs[1], ybuf[1]), RB // 8), pieces=1)
    _run(up_operands(last, ybuf[1]))


def _mlp(zero, out_hbm, wa, xs, hbuf, w4t, yt, sems, mu0, tt0, tt1, mu1, md):
    tts, mu = (tt0, tt1), (mu0, mu1)
    hr = R // 2
    lag = E_("LAG", 14)

    def out_copy(b, n):
        rows = pl.ds(_mult(b * 4 * R, 4 * R), 4 * R)
        return pltpu.make_async_copy(xs.at[n, rows], out_hbm.at[rows, pl.ds(n * HD, HD)],
                                     sems.at[SEM_OUT + 2 * b + n])

    def up_dot(b, j, half, p):
        return _up_dot(yt, wa, mu[half], b, j, half, p)

    def up_sums(act):
        for half, t in itertools.product(range(2), range(hr // 8)):
            c = {}
            for g in ORDER:
                y = _dec(lambda k: mu[half][7 * g + k, pl.ds(8 * t, 8), :])
                for i1, n1, sign in DEC[g]:
                    for (i0, n0), m in y.items():
                        key = (2 * i1 + i0, 2 * n1 + n0)
                        _accumulate(c, key, m, sign)
                        if LAST[i1, n1] == g:
                            act[half, t, key] = _gelu(c.pop(key))
                yield

    def down_operands(act, tt, j):
        for half, t in itertools.product(range(2), range(hr // 16)):
            def emit(p, v):
                tt[NJ * p + j, pl.ds(half * hr + 16 * t, 16), :] = v.astype(bf16)

            yield from _enc2(ENC_A, lambda q, k: jnp.concatenate(
                [act[half, 2 * t, (q, k)], act[half, 2 * t + 1, (q, k)]], axis=0), emit)

    n_sums = 7 * 2 * (hr // 8)

    def up_vector_work(tt, j):
        act = {}
        a, b = up_sums(act), down_operands(act, tt, j)
        for i in range(n_sums + lag):
            if i < n_sums:
                next(a)
            if i >= lag and (i - lag) % 2 == 1:
                next(b)
            yield

    part = []

    def down_dot(tt, g, slot, i, lo, hi):
        p = 7 * g + i // 2
        res = _dot(_operand(tt, [NJ * p + q for q in range(lo, hi)]),
                   _operand(w4t, [14 * g + i], pl.ds(64 * lo, 64 * (hi - lo))))
        if hi < NJ:
            part.append(res)
        else:
            md[7 * slot + i // 2, :, pl.ds(128 * (i % 2), 128)] = part.pop() + res if lo else res
        return res

    def down_block(slot, t):
        c = _dec(lambda k: md[7 * slot + k, pl.ds(16 * t, 16), :])
        return jnp.concatenate(
            [jnp.concatenate([c[i0, 0], c[i0, 1]], axis=1) for i0 in range(2)], axis=0)

    def down_sums(b, g, slot):
        dst = []
        for w in range(2):
            i1 = n1 = sign = 0
            for q in range(7):
                e = DEC[q][w] if w < len(DEC[q]) else DEC[q][0][:2] + (0,)
                i1, n1, sign = (jnp.where(g == q, new, old)
                                for new, old in zip(e, (i1, n1, sign)))
            dst.append((b * 4 * R + 32 * i1, n1, sign.astype(f32)))
        for t in range(R // 16):
            m = down_block(slot, t)
            rows = [pl.ds(pl.multiple_of(d[0] + 64 * t, 32), 32) for d in dst]
            new = [hbuf[dst[0][1], rows[0], :] + m,
                   hbuf[dst[1][1], rows[1], :] + dst[1][2] * m]
            for w in (1, 0):
                hbuf[dst[w][1], rows[w], :] = new[w]
                xs[dst[w][1], rows[w], :] = new[w].astype(bf16)
            yield

    def step(b, par, up, down, j):
        slot = (7 * b + j) & 1
        dots = []
        if up:
            nb = jnp.minimum(b + (j + 1) // NJ, NB - 1)
            nj = jnp.where(j == NJ - 1, 0, j + 1)
            dots = ([(1, functools.partial(up_dot, b, j, 1, p)) for p in range(49)]
                    + [(1, functools.partial(up_dot, nb, nj, 0, p)) for p in range(49)])
            up_work = up_vector_work(tts[par], j)
        if down:
            cuts = (0, E_("KS", 4), NJ) if E_("KS", 4) and up else (0, NJ)
            for i in reversed(range(14)):
                dots[7 * i + E_('D0', 6):7 * i + E_('D0', 6)] = [
                    (hi - lo, functools.partial(down_dot, tts[1 - par], j, slot, i, lo, hi))
                    for lo, hi in zip(cuts, cuts[1:])]
            down_work = down_sums(jnp.maximum(b - 1 - (j == 0), 0),
                                  jnp.where(j == 0, 6, j - 1), 1 - slot)
        total = sum(w for w, _ in dots)
        pos = n_up = done_up = done_down = 0
        for w, dot in dots:
            if down:
                goal = (pos + E_('AD', 8)) * (R // 16) * 100 // (E_("DE", 100) * total)
                for _ in range(done_down, goal):
                    next(down_work, None)
                done_down = max(done_down, goal)
            res = dot()
            k = min(w, E_('PD', 7))
            for i in range(k * up):
                if E_('PM', 2) and (w > 1 or n_up % E_('PM', 2) == 0):
                    _pace(mu[done_up >= n_sums // 2], (49,), zero, res[:res.shape[0] * (i + 1) // k])
                if E_('PN', 1) and (w > 1 or n_up % E_('PN', 1) == 0):
                    _pace(tts[par], (49 * NJ,), zero, res[:res.shape[0] * (i + 1) // k])
                goal = (pos * k + w * (i + 1) + E_('AH', 3) * k) * (n_sums + lag) // (total * k)
                goal = (min(goal, n_sums // 2) if n_up + (w == 1) < 49
                        else max(goal, n_sums // 2))
                for _ in range(done_up, goal):
                    next(up_work, None)
                done_up = max(done_up, goal)
            pos += w
            n_up += w == 1
        if up:
            _run(up_work)
        if down:
            _run(down_work)
        if down:
            @pl.when((j == 0) & (b > 1))
            def _():
                for n in range(2):
                    out_copy(b - 2, n).start()

    md[pl.ds(0, 7)] = jnp.zeros((7, R, C4), f32)
    with jax.named_scope('b0'): pl.loop(0, NJ)(functools.partial(step, 0, 0, True, False))

    @pl.loop(0, NB // 2)
    @jax.named_scope('bmid')
    def _(i):
        pl.loop(0, NJ)(functools.partial(step, 2 * i + 1, 1, True, True))
        pl.loop(0, jnp.where(2 * i + 2 < NB, NJ, 0))(
            functools.partial(step, 2 * i + 2, 0, True, True))

    with jax.named_scope('b4'): pl.loop(0, NJ)(functools.partial(step, NB, 0, False, True))
    out_copy(NB - 1, 1).start()
    pieces = []
    for t in range(R // 16):
        rows = pl.ds(S - 4 * R + 64 * t, 32)
        xs[0, rows, :] = (hbuf[0, rows, :] + down_block((7 * NB + 6) & 1, t)).astype(bf16)
        if t % 2:
            rows = pl.ds(S - 4 * R + 64 * (t - 1), 128)
            pieces.append(pltpu.make_async_copy(
                xs.at[0, rows], out_hbm.at[rows, pl.ds(0, HD)], sems.at[t // 2]))
            pieces[-1].start()
    for b, n in itertools.product(range(NB), range(2)):
        if (b, n) != (NB - 1, 0):
            out_copy(b, n).wait()
    for c in pieces:
        c.wait()


@jax.jit
def pallas_sequential_preLN__memory_aug_recurrent_mem_tr__mixer_s_mlp__prompt_kernel(
    A_x: jax.Array,
    A_mem0: jax.Array,
    A_Wq: jax.Array,
    A_Wk: jax.Array,
    A_Wv: jax.Array,
    A_Wo: jax.Array,
    A_seg_len: jax.Array,
    B_x: jax.Array,
    B_w1: jax.Array,
    B_w2: jax.Array,
    B_w3: jax.Array,
    B_w4: jax.Array,
):
    del A_seg_len, B_x
    hbm = pl.BlockSpec(memory_space=pl.ANY)
    vmem = pl.BlockSpec(memory_space=pltpu.VMEM)
    scratch = [
        pltpu.VMEM((3 * H + 1, D, DH), bf16),
        pltpu.VMEM((2, S + 32, HD), bf16),
        pltpu.VMEM((2, S, HD), f32),
        pltpu.VMEM((98, F // 4, 128), bf16),
        pltpu.VMEM((98 * NB + 1, R, 128), bf16),
        pltpu.VMEM((52, R // 2 + 8, 128), f32),
        pltpu.SemaphoreType.DMA((NSEM,)),
    ]
    out = pl.pallas_call(
        _kernel,
        out_shape=jax.ShapeDtypeStruct((S, D), A_x.dtype),
        in_specs=[hbm, vmem] + [hbm] * 9,
        out_specs=hbm,
        scratch_shapes=scratch,
        compiler_params=pltpu.CompilerParams(vmem_limit_bytes=127 * 1024 * 1024),
    )(A_x.reshape(S, D), A_mem0.reshape(MEM, D),
      A_Wq.reshape(D // 2, 2 * H, DH), A_Wk.reshape(D // 2, 2 * H, DH),
      A_Wv.reshape(D // 2, 2 * H, DH),
      A_Wo.reshape(H * DH, D), B_w1, B_w2, B_w3.reshape(D // R, R, F),
      B_w4.reshape(F // R, R, D), B_w4)
    return out.reshape(A_x.shape)
```

```python
import functools
import itertools
import os

import jax
import jax.numpy as jnp
from jax import lax
import jax.experimental.pallas as pl
import jax.experimental.pallas.tpu as pltpu

S = 2048
D = 1024
H = 32
DH = 128
MEM = 8
SEG = 32
F = 3584
NSEG = S // SEG
L = MEM + SEG
TOK = 24
P0 = S - TOK * NSEG
RING = 576
XP = (S - P0) // 8
C4 = D // 4
HALO = 8
RB = 256
R = 128
NB = S // (4 * R)
NJ = F // 512
HD = D // 2
W1_AT, W2_AT = 64, 320
W4T = (F - S) // R
E_ = lambda k, d: int(os.environ.get(k, d))
EPS = 1e-5
NEG = -1000000000.0

LAG_QK, LAG_PV, LAG_WO = E_('LQ', 1), E_('LP', 3), E_('LW', 4)
FILL_AT = E_('FA', 17)
UNROLL = 2

bf16 = jnp.bfloat16
f32 = jnp.float32
u32 = jnp.uint32

SEM_X0, SEM_X, SEM_WO, SEM_W1, SEM_W2, SEM_OUT, SEM_W, SEM_W4, SEM_W3 = (
    0, 2, 10, 14, 22, 30, 38, 50, 66)
NSEM = SEM_W3 + 4 * NJ

ENC_A = (((0, 0, 1), (1, 1, 1)), ((1, 0, 1), (1, 1, 1)), ((0, 0, 1),), ((1, 1, 1),),
         ((0, 0, 1), (0, 1, 1)), ((1, 0, 1), (0, 0, -1)), ((0, 1, 1), (1, 1, -1)))
ENC_B = (((0, 0, 1), (1, 1, 1)), ((0, 0, 1),), ((0, 1, 1), (1, 1, -1)),
         ((1, 0, 1), (0, 0, -1)), ((1, 1, 1),), ((0, 0, 1), (0, 1, 1)),
         ((1, 0, 1), (1, 1, 1)))
DEC = (((0, 0, 1), (1, 1, 1)), ((1, 0, 1), (1, 1, -1)), ((0, 1, 1), (1, 1, 1)),
       ((0, 0, 1), (1, 0, 1)), ((0, 1, 1), (0, 0, -1)), ((1, 1, 1),), ((0, 0, 1),))
ORDER = (0, 1, 3, 2, 4, 5, 6)
LAST = {(1, 0): 3, (0, 1): 4, (1, 1): 5, (0, 0): 6}


def _enc(terms, get):
    v = get(*terms[0][:2])
    for i, j, sign in terms[1:]:
        v = v + get(i, j) if sign > 0 else v - get(i, j)
    return v


def _enc2(table, get, emit):
    for g in range(7):
        y = [[_enc(table[g], lambda i1, j1: get(2 * i1 + i0, 2 * j1 + j0))
              for j0 in range(2)] for i0 in range(2)]
        for k in range(7):
            emit(7 * g + k, _enc(table[k], lambda i0, j0: y[i0][j0]))
        yield


def _right_operands(get, dst, first, row):
    b = [[get(i, j).astype(f32) for j in range(2)] for i in range(2)]
    for p in range(7):
        dst[first + p, pl.ds(row, 16), :] = _enc(ENC_B[p], lambda i, j: b[i][j]).astype(bf16)


def _left_operands(halves, dst, rows):
    for p in range(7):
        v = _enc(ENC_A[p], lambda i, j: halves[i][:, HD * j:HD * j + HD])
        for c in range(4):
            dst[4 * p + c, rows, :] = v[:, 128 * c:128 * c + 128].astype(bf16)


def _collect(acc, p, res, emit):
    for i, j, sign in DEC[p]:
        _accumulate(acc, (i, j), res, sign)
        if LAST[i, j] == p:
            emit(i, j, acc.pop((i, j)))
    return res


def _accumulate(c, key, m, sign):
    c[key] = m if key not in c else (c[key] + m if sign > 0 else c[key] - m)


def _dec(get):
    c = {}
    for k in range(7):
        m = get(k)
        for i, j, sign in DEC[k]:
            _accumulate(c, (i, j), m, sign)
    return c


def _pace(ref, lead, row, result):
    n = 32 // ref.dtype.itemsize
    ref[(*lead, pl.ds(pl.multiple_of(row, n), n), pl.ds(0, 128))] = (
        result[-n:, :128].astype(ref.dtype))


def _run(gen):
    for _ in gen:
        pass


def _mult(i, n):
    return i if isinstance(i, int) else pl.multiple_of(i, n)


def _ln(x):
    m = jnp.mean(x, axis=-1, keepdims=True)
    d = x - m
    v = jnp.mean(d * d, axis=-1, keepdims=True)
    return d * lax.rsqrt(v + EPS)


def _gelu(x):
    c = 0.7978845608028654
    hx = 0.5 * x
    return hx + hx * jnp.tanh(x * (c + (c * 0.044715) * (x * x)))


def _unpack(x):
    return pltpu.bitcast(x, bf16)


def _operand(ref, blocks, rows=slice(None)):
    words = ref.bitcast(u32)
    return _unpack(jnp.concatenate([words[b, rows, :] for b in blocks], axis=1))


def _dot(a, b):
    return jnp.dot(a, b, preferred_element_type=f32)


def _rows(ref, rows):
    return jnp.concatenate([ref[0, rows, :], ref[1, rows, :]], axis=1)


def _set_rows(ref, rows, v):
    ref[0, rows, :] = v[:, :HD]
    ref[1, rows, :] = v[:, HD:]


def _kernel(*refs):
    out_hbm, wa, xs, hbuf, w4t, yt, mu0, sems = refs[11:]
    zero = pl.run_scoped(
        functools.partial(_attention_and_mixer, *refs),
        pltpu.VMEM((H * DH // 2, D), u32),
        pltpu.VMEM((8, S + 4 * HALO, 128), f32),
        pltpu.VMEM((28, 2 * TOK, 128), bf16),
        pltpu.VMEM((28, HD, 128), bf16),
        *[pltpu.VMEM((H // 8, RING, DH), f32)] * 8)
    if E_("SKIP_MLP", 0):
        for b in (w4t, yt, wa):
            pltpu.sync_copy(b.at[0, pl.ds(0, 128)], out_hbm.at[pl.ds(0, 128), pl.ds(0, 128)])
        return
    with jax.named_scope('s_mlp'): pl.run_scoped(
        functools.partial(_mlp, zero, out_hbm, wa, xs, hbuf, w4t, yt, sems, mu0),
        *[pltpu.VMEM((49 * NJ + 1, R, 128), bf16)] * 2,
        pltpu.VMEM(mu0.shape, f32),
        pltpu.VMEM((14, R, C4), f32))


def _attention_and_mixer(x_hbm, mem0_ref, wq_hbm, wk_hbm, wv_hbm, wo_hbm, w1_hbm, w2_hbm,
                         w3_hbm, w4_hbm, w4a_hbm, out_hbm, wa, xs, hbuf, w4t, yt, mu0, sems,
                         wo_b, xg, ubuf, w1t, *q_rings):
    def w3_copy(c):
        return pltpu.make_async_copy(
            w3_hbm.at[:, :, pl.ds(_mult(c * 128, 128), 128)], yt.at[pl.ds(8 * c, 8)],
            sems.at[SEM_W3 + c])

    def w4_head_copy(c):
        return pltpu.make_async_copy(
            w4a_hbm.at[pl.ds(0, S), pl.ds(c * 128, 128)],
            xs.at[c % 2, pl.ds(0, S), pl.ds(c // 2 * 128, 128)], sems.at[SEM_W4 + c])

    def w4_tail_copy(c):
        return pltpu.make_async_copy(
            w4_hbm.at[pl.ds(S // R, W4T), :, pl.ds(c * 128, 128)],
            yt.at[pl.ds(32 * NJ + W4T * c, W4T)], sems.at[SEM_W4 + 8 + c])

    def w2_copy(c):
        return pltpu.make_async_copy(
            w2_hbm.at[:, :, pl.ds(c * 128, 128)], yt.at[pl.ds(W2_AT + 8 * c, 8)],
            sems.at[SEM_W2 + c])

    others = [[w2_copy(c) for c in range(8)], [w4_head_copy(c) for c in range(4)],
              [w4_head_copy(c) for c in range(4, 8)], [w4_tail_copy(c) for c in range(8)]]

    def fetch(i):
        for c in range(NJ):
            w3_copy(NJ * i + c).start()
        for k, copies in enumerate(others):
            @pl.when(i == k)
            def _():
                for c in copies:
                    c.start()

    zero = pl.run_scoped(
        functools.partial(_attention, x_hbm, mem0_ref, (wq_hbm, wk_hbm, wv_hbm), wo_hbm,
                          w1_hbm, fetch, w4t, yt, wa, xs, hbuf, sems, wo_b, xg, ubuf, w1t, q_rings),
        *[pltpu.VMEM((H // 8, RING, DH), f32)] * 16)
    for c in sum(others, []):
        c.wait()
    for c in range(4 * NJ):
        w3_copy(c).wait()
    if E_("SKIP_POST", 0): return zero
    with jax.named_scope('s_mix'): pl.run_scoped(
        functools.partial(_mixer, zero, mu0, wa, xs, w4t, hbuf, yt, wo_b, xg, w1t, q_rings),
        pltpu.VMEM((28, HD, 128), bf16),
        pltpu.VMEM((28, P0 // 2 + 2 * TOK + 16, 128), bf16),
        *[pltpu.VMEM((8, P0, 128), bf16)] * 2, *[pltpu.VMEM((RB, D), f32)] * 2,
        *[pltpu.VMEM((RB + 8, D), f32)] * 2)
    return zero


def _attention(x_hbm, mem0_ref, w_hbm, wo_hbm, w1_hbm, fetch,
               w4t, yt, wa, xs, hbuf, sems, wo_b, xg, ubuf, w1t, q_rings, *kv_rings):
    rings = q_rings + kv_rings
    ring = [[rings[m * 8 + h % 8].at[h // 8] for h in range(H)] for m in range(3)]
    q_r, k_r, v_r = ring

    class x_rows:
        def __init__(self, rows, sem):
            self.copies = [
                pltpu.make_async_copy(x_hbm.at[rows, pl.ds(n * HD, HD)], xs.at[n, rows],
                                      sems.at[sem + n]) for n in range(2)]

        def start(self):
            for c in self.copies:
                c.start()

        def wait(self):
            for c in self.copies:
                c.wait()

    x0_copy = x_rows(pl.ds(0, P0), SEM_X0)

    def x_copy(g):
        return x_rows(pl.ds(_mult(P0 + g * 2 * XP, XP), 2 * XP), SEM_X + 2 * g)

    def wo_copy(i):
        rows = pl.ds(_mult(i * 512, 512), 512)
        return pltpu.make_async_copy(wo_hbm.bitcast(u32).at[rows], wo_b.at[rows],
                                     sems.at[SEM_WO + i])

    def w1_copy(c):
        return pltpu.make_async_copy(
            w1_hbm.at[:, :, pl.ds(_mult(c * 128, 128), 128)], yt.at[pl.ds(W1_AT + 8 * c, 8)],
            sems.at[SEM_W1 + c])

    def prologue(*stg):

        def start_chunk(g, m):
            src = w_hbm[m].bitcast(u32)
            dst = stg[m].reshape(D // 2, 8, DH)
            for q in range(8 * E_("DS", 1)):
                pltpu.make_async_copy(
                    src.at[:, 16 * (q // 4) + 4 * g + q % 4, :],
                    stg[m].at[pl.ds(q * HD, HD)], sems.at[SEM_W + 3 * g + m]).start()
            for par in range(2 - 2 * E_("DS", 1)):
                pltpu.make_async_copy(
                    src.at[:, pl.ds(_mult(16 * par + 4 * g, 4), 4), :],
                    dst.at[:, pl.ds(4 * par, 4), :],
                    sems.at[SEM_W + 3 * g + m]).start()

        def wait_chunk(g, m):
            pltpu.make_async_copy(stg[m], stg[m], sems.at[SEM_W + 3 * g + m]).wait()

        def relayout(g, m, pair, i0, n):
            ev = stg[m][pl.ds(8 * i0 + pair, n, stride=8), :]
            od = stg[m][pl.ds(8 * i0 + 4 + pair, n, stride=8), :]
            if E_("DS", 1):
                ev = stg[m][pl.ds(_mult(pair * HD + i0, 8), n), :]
                od = stg[m][pl.ds(_mult((4 + pair) * HD + i0, 8), n), :]
            h = 8 * g + 2 * pair
            words = wa.bitcast(u32)
            words[m * H + h, pl.ds(i0, n), :] = (ev & jnp.uint32(0xFFFF)) | (od << 16)
            words[m * H + h + 1, pl.ds(i0, n), :] = (ev >> 16) | (od & jnp.uint32(0xFFFF0000))

        def weights(g, m, pair):
            h = m * H + 8 * g + 2 * pair
            for t in range(D // 32 + 1):
                if t < D // 32:
                    for k in range(2):
                        relayout(g, m, pair, D // 4 * k + 8 * t, 8)
                if t > 0:
                    r = 16 * (t - 1)
                    _right_operands(lambda k, n: wa[h + n, pl.ds(HD * k + r, 16), :],
                                    w4t, 28 * m + 7 * pair, r)
                yield

        def norm_rows(r0, n):
            xv = _rows(xs, pl.ds(r0, n)).astype(f32)
            _set_rows(hbuf, pl.ds(r0, n), xv)
            return _ln(xv)

        def later_rows(r0):
            for r in range(0, XP, 16):
                xn = norm_rows(pl.multiple_of(r0 + r, 16), 16)
                for c in range(8):
                    xg[c, pl.ds(pl.multiple_of(HALO + r0 + r, 8), 16), :] = (
                        xn[:, 128 * c:128 * c + 128])
                yield

        x0_copy.start()
        start_chunk(0, 0)
        start_chunk(0, 1)
        start_chunk(0, 2)
        x_copy(0).start()
        zero = jnp.zeros((HALO, 128), f32)
        for c in range(8):
            xg[c, pl.ds(0, HALO), :] = zero
            xg[c, pl.ds(HALO + S, HALO), :] = zero
        with jax.named_scope('wx'): x0_copy.wait()

        @pl.loop(0, P0 // 64)
        def _(i):
            a = [norm_rows(pl.multiple_of(P0 // 2 * k + 32 * i, 32), 32) for k in range(2)]
            for p in range(7):
                v = _enc(ENC_A[p], lambda k, n: a[k][:, HD * n:HD * n + HD])
                for c in range(4):
                    yt[8 * p + 4 * (i // 4) + c, pl.ds(pl.multiple_of(i % 4 * 32, 32), 32), :] = (
                        v[:, 128 * c:128 * c + 128].astype(bf16))

        with jax.named_scope('w0'): wait_chunk(0, 0)
        pl.loop(0, 4)(lambda pair: _run(weights(0, 0, pair)))

        def stage(g, m):
            m1 = (m + 1) % 3
            g1 = jnp.minimum(g + (1 if m == 2 else 0), 3)
            if m > 0:
                pl.when(3 * g + m < 11)(functools.partial(wait_chunk, g1, m1))
            if m == 1:
                x_copy(g).wait()

            @pl.when(g < 3)
            def _():
                start_chunk(g + 1, m)
                if m == 1:
                    x_copy(g + 1).start()
            if m == E_('WM', 1):
                wo_copy(g).start()
            if m == 2:
                w1_copy(2 * g).start()
                w1_copy(2 * g + 1).start()
            n = E_("PR", 64)
            acc = {}

            def dot(pair, r, p):
                res = _dot(
                    _operand(yt, [8 * p + 4 * (r // R) + k for k in range(4)],
                             pl.ds(r % R // 2, n // 2)),
                    _operand(w4t, [28 * m + 7 * pair + p], pl.ds(0, HD // 2)))
                for i, j, sign in DEC[p]:
                    _accumulate(acc, (i, j), res, sign)
                    if LAST[i, j] == p:
                        rings[m * 8 + 2 * pair + j][g, pl.ds(P0 // 2 * i + r, n), :] = (
                            acc.pop((i, j)))
                return res

            dots = [functools.partial(dot, pair, r, p) for pair in range(4)
                    for r in range(0, P0 // 2, n) for p in ORDER]
            work = [(itertools.chain(*[weights(g1, m1, pair) for pair in range(4)]),
                     4 * (D // 32 + 1))]
            paced = [(wa, (3 * H,), 16 * (g >> 10))]
            if m == 0:
                early = E_("EA", 49)
                for d in dots[:early]:
                    d()
                dots = dots[early:]
                wait_chunk(g1, m1)
            else:
                work.append((later_rows(P0 + (2 * g + m - 1) * XP), XP // 16))
                paced.append((xg, (0,), S + 2 * HALO + 8 * (g >> 10)))
            _interleave(dots, lambda res: [_pace(*p, res) for p in paced], *work,
                        pieces=1 if m else E_("PQ", 2))

        @pl.loop(0, 4)
        def _(g):
            for m in range(3):
                stage(g, m)

    if not E_('SKIP_PRO', 0):
     with jax.named_scope('s_pro'): pl.run_scoped(
        prologue,
        pltpu.VMEM((8 * D // 2, DH), u32),
        pltpu.VMEM((8 * D // 2, DH), u32),
        pltpu.VMEM((8 * D // 2, DH), u32),
    )
    for i in range(4):
        if E_('WM', 1) > 2: wo_copy(i).start()
        with jax.named_scope('wwo'): wo_copy(i).wait()
    for c in range(8):
        w1_copy(c).wait()

    @pl.loop(0, 16)
    def _(i):
        c, q = i >> 2, i & 3
        for r in range(0, 128, 16):
            _right_operands(lambda k, n: yt[W1_AT + 16 * c + 8 * n + 4 * k + q, pl.ds(r, 16), :],
                            w1t, 7 * c, pl.multiple_of(128 * q + r, 16))

    def wrap(r):
        return jnp.where(r >= RING, r - RING, r)

    def load_tok(s):
        rows = pl.ds(pl.multiple_of(HALO + P0 + TOK * s, 8), TOK)
        return jnp.concatenate([xg[c, rows, :] for c in range(8)], axis=1)

    def step(s, carry, tok, first_of_group):
        mem, rp, ra, rw = carry
        ri = lax.broadcasted_iota(jnp.int32, (2 * L, 2 * L), 0)
        ci = lax.broadcasted_iota(jnp.int32, (2 * L, 2 * L), 1)
        same = (ri >= L) == (ci >= L)
        ri, ci = (jnp.where(v >= L, v - L, v) for v in (ri, ci))
        mask = same & ((ri < MEM) | (ri >= ci))
        fill = jnp.where(same, NEG, -jnp.inf)

        lhs = jnp.concatenate([mem, tok], axis=0).astype(bf16)
        rps = [pl.multiple_of(wrap(rp + 8 * i), 8) for i in range(3)]
        ra_ = pl.multiple_of(ra, SEG)
        rw_ = pl.multiple_of(rw, 8)

        col = s & 3
        rb = pl.multiple_of(jnp.maximum((s >> 2) - 1, 0) * (4 * TOK), 8)
        if first_of_group:
            _left_operands([_ln(_ln(_rows(hbuf, pl.ds(rb + 2 * TOK * i, 2 * TOK))))
                            for i in range(2)], ubuf, slice(None))
        filled = {}

        def filler(products):
            def emit(i, j, v):
                xg[2 * col + j, pl.ds(HALO + rb + 2 * TOK * i, 2 * TOK), :] = _gelu(v)

            for p in products:
                _collect(filled, p, _dot(_operand(ubuf, range(4 * p, 4 * p + 4)),
                                         _operand(w1t, [7 * col + p])), emit)

        mem_qkv = {}
        scores = {}
        o_mem = {}
        total = [None]

        def qkv(h):
            res = {}
            for m in ((0, 1, 2), (1, 0, 2), (2, 0, 1), (2, 1, 0))[E_('MO', 0)]:
                r = _dot(lhs, _operand(wa, [m * H + h]))
                for i in range(3):
                    ring[m][h][pl.ds(rps[i], 8), :] = r[8 + 8 * i:16 + 8 * i]
                res[m] = r[:MEM]
            mem_qkv[h] = res

        def both(m, a):
            return jnp.concatenate(
                [v for h in (2 * a, 2 * a + 1)
                 for v in (mem_qkv[h][m], ring[m][h][pl.ds(ra_, SEG), :])],
                axis=0).astype(bf16)

        def qk(a):
            scores[a] = lax.dot_general(both(0, a), both(1, a), (((1,), (1,)), ((), ())),
                                        preferred_element_type=f32)

        def pv(a):
            sc = jnp.where(mask, scores.pop(a) * (DH ** -0.5), fill)
            mx = jnp.max(sc, axis=1, keepdims=True)
            e = jnp.exp(sc - mx)
            den = jnp.sum(e, axis=1, keepdims=True)
            inv = pl.reciprocal(den, approx=True)
            inv = inv * (2.0 - den * inv)
            o = _dot(e.astype(bf16), both(2, a)) * inv
            for i, h in enumerate((2 * a, 2 * a + 1)):
                q_r[h][pl.ds(ra_, SEG), :] = o[i * L + MEM:(i + 1) * L]
                o_mem[h] = o[i * L:i * L + MEM]

        def wo(h):
            lo = jnp.concatenate([o_mem.pop(h), q_r[h][pl.ds(rw_, TOK), :]],
                                 axis=0).astype(bf16)
            r = _dot(lo, _unpack(wo_b[pl.ds(h * DH // 2, DH // 2), :]))
            total[0] = r if total[0] is None else total[0] + r

        npair = H // 2
        for t in range(npair + LAG_WO):
            heads = (2 * t, 2 * t + 1) if t < npair else ()
            late = (2 * (t - LAG_WO), 2 * (t - LAG_WO) + 1) if t >= LAG_WO else ()
            cuts = [0, E_('FS', 2), E_('FS', 2) + E_('F2', 0)]
            for op in os.environ.get("SEQ", "abqpfcd"):
                if op in "ab" and heads: qkv(heads[op == "b"])
                if op in "cd" and late: wo(late[op == "d"])
                if op == "q" and 0 <= t - LAG_QK < npair: qk(t - LAG_QK)
                if op == "p" and 0 <= t - LAG_PV < npair: pv(t - LAG_PV)
                if op == "f" and 0 <= t - FILL_AT < 2: filler(ORDER[cuts[t - FILL_AT]:cuts[t - FILL_AT + 1]])
        filler(ORDER[cuts[2]:])

        a = total[0]
        rows = pl.ds(pl.multiple_of(TOK * s, 8), TOK)
        _set_rows(hbuf, rows, _rows(hbuf, rows) + a[MEM:])
        return a[:MEM], wrap(rp + TOK), wrap(ra + SEG), wrap(rw + TOK)

    def steps(i, carry):
        toks = [load_tok(i * UNROLL + k) for k in range(UNROLL)]
        for k in range(UNROLL):
            carry = step(i * UNROLL + k, carry, toks[k], k == 0)
        return carry

    def quarter(k, carry):
        fetch(k)
        n = NSEG // UNROLL // 4
        return lax.fori_loop(k * n, (k + 1) * n, steps, carry)

    if E_('SKIP_LOOP', 0): return lax.fori_loop(0, 64, lambda i, c: wrap(c + TOK), jnp.int32(0)) - TOK * NSEG % RING
    with jax.named_scope('s_loop'): carry = lax.fori_loop(
        0, 4, quarter,
        (mem0_ref[...].astype(f32), jnp.int32(P0), jnp.int32(0), jnp.int32(0)))
    return carry[3] - TOK * NSEG % RING


def _interleave(dots, pace, *work, pieces=8):
    for i, dot in enumerate(dots):
        res = dot()
        k = min(pieces, res.shape[0] // 16)
        for j in range(k):
            pace(res[:res.shape[0] // 16 * (j + 1) // k * 16])
            for gen, n in work:
                for _ in range(n * (i * k + j) // (k * len(dots)),
                               n * (i * k + j + 1) // (k * len(dots))):
                    next(gen)
    for gen, _ in work:
        _run(gen)


def _up_dot(yt, wa, mu, b, j, half, p):
    res = _dot(
        _operand(yt, [98 * b + 2 * p, 98 * b + 2 * p + 1], pl.ds(half * R // 4, R // 4)),
        _operand(wa, [13 * j + p // 4], pl.ds(128 * (p % 4), 128)))
    mu[p, pl.ds(0, R // 2), :] = res
    return res


def _mixer(zero, mu0, wa, xs, w4t, hbuf, yt, wo_b, xg, w1t, q_rings, w2t, ulast, lhs0, lhs1, hs0, hs1, *ybuf):
    lhs, hs = (lhs0, lhs1), (hs0, hs1)

    def encode_w3(g):
        for j, t in itertools.product(range(NJ), range(4)):
            def get(k, n):
                return yt[32 * j + 8 * n + 2 * k + (g >> 1),
                          pl.ds(pl.multiple_of(64 * (g & 1) + 16 * t, 16), 16), :].astype(f32)

            def emit(p, v):
                wa[13 * j + p // 4, pl.ds(pl.multiple_of(C4 * (p % 4) + 64 * g + 16 * t, 16), 16),
                   :] = v.astype(bf16)

            yield from _enc2(ENC_B, get, emit)

    def encode_w4(g):
        c = g >> 1
        for j, t in itertools.product(range(NJ), range(4)):
            r = pl.multiple_of(64 * (g & 1) + 16 * t, 16)

            def get(k, n):
                if 512 * j < S:
                    return xs[c, pl.ds(512 * j + 128 * k + r, 16), pl.ds(128 * n, 128)].astype(f32)
                return yt[32 * NJ + W4T * (2 * n + c) + 4 * j - S // R + k,
                          pl.ds(r, 16), :].astype(f32)

            def emit(p, v):
                w4t[2 * p + c, pl.ds(128 * j + r, 16), :] = v.astype(bf16)

            yield from _enc2(ENC_B, get, emit)

    def encode_w2(g):
        for t, c in itertools.product(range(8), range(4)):
            _right_operands(
                lambda k, n: yt[W2_AT + 8 * (4 * n + c) + 4 * k + g, pl.ds(16 * t, 16), :],
                w2t, 7 * c, pl.multiple_of(128 * g + 16 * t, 16))
            yield

    done = TOK * NSEG
    first = 4 * TOK * (NSEG // 4 - 1)

    @jax.named_scope('q1')
    def q1(g):
        n = 128
        for k, q in enumerate(q_rings):
            for r in range(0, P0, 64):
                lhs0[k, pl.ds(r, 64), :] = q[g, pl.ds((done + r) % RING, 64), :].astype(bf16)

        part = []

        def dot(r, c, k):
            w = wo_b[pl.ds(pl.multiple_of((2 * g + k) * 2 * DH, 2 * DH), 2 * DH),
                     pl.ds(128 * c, 128)]
            res = _dot(_operand(lhs0, range(4 * k, 4 * k + 4), pl.ds(r // 2, n // 2)), _unpack(w))
            if k == 0:
                part.append(res)
            else:
                hbuf[c // 4, pl.ds(done + r, n), pl.ds(128 * (c % 4), 128)] += part.pop() + res
            return res

        _interleave(
            [functools.partial(dot, r, c, k)
             for r in range(0, P0, n) for c in range(8) for k in range(2)],
            lambda res: [_pace(yt, (98 * NB,), zero, res), _pace(xs, (0,), S + zero, res)],
            (encode_w2(g), 32),
            (encode_w4(g), 28 * NJ), (encode_w3(g), 28 * NJ), pieces=8)

    pl.loop(0, H // 8)(q1)

    half = (S - first) // 2

    def mixer_norm(r0, n):
        for r in range(r0, r0 + n, 16):
            _left_operands([_ln(_ln(_rows(hbuf, pl.ds(first + half * i + r, 16))))
                            for i in range(2)], ulast, pl.ds(r, 16))
            yield

    def mixer_in(c):
        step = E_("IR", 64)
        for r in range(0, half, step):
            n = min(step, half - r)
            acc = {}

            def emit(i, j, v):
                xg[2 * c + j, pl.ds(HALO + first + half * i + r, n), :] = _gelu(v)

            for p in ORDER:
                _collect(acc, p, _dot(
                    _operand(ulast, range(4 * p, 4 * p + 4), pl.ds(r // 2, n // 2)),
                    _operand(w1t, [7 * c + p])), emit)

    def shift(i, dst):
        for r, c in itertools.product(range(0, RB // 2, 16), range(4)):
            a = [[xg[4 * k + c, pl.ds(HALO + (-1, 1, -2, 2)[2 * k + c // 2]
                                      + i * RB + RB // 2 * q + r, 16), :]
                  for k in range(2)] for q in range(2)]
            for p in range(7):
                dst[p, pl.ds(RB // 2 * c + r, 16), :] = _enc(
                    ENC_A[p], lambda q, k: a[q][k]).astype(bf16)
            yield

    def mixer_out(src, dst):
        n = 128
        acc = {}

        def dot(r, c, p):
            words = src.bitcast(u32)
            a = jnp.concatenate([words[p, pl.ds((RB // 2 * k + r) // 2, n // 2), :]
                                 for k in range(4)], axis=1)
            res = _dot(_unpack(a), _operand(w2t, [7 * c + p]))
            for i, j, sign in DEC[p]:
                _accumulate(acc, (i, j), res, sign)
                if LAST[i, j] == p:
                    dst[pl.ds(RB // 2 * i + r, n), pl.ds(HD * j + 128 * c, 128)] = acc.pop((i, j))
            return res

        return [functools.partial(dot, r, c, p)
                for r in range(0, RB // 2, n) for c in range(4) for p in ORDER]

    def residual(i, src, dst):
        late = []
        for t in range(0, RB, 8):
            rows = pl.ds(_mult(i * RB + t, 8), 8)
            hv = _rows(hbuf, rows)
            x1 = _ln(hv) + src[pl.ds(t, 8), :]
            late.append((rows, hv + x1, t, _ln(x1)))
            if len(late) > E_("LT", 0) or t == RB - 8:
                for rows, v, t0, y in late[:None if t == RB - 8 else 1]:
                    _set_rows(hbuf, rows, v)
                    dst[pl.ds(t0, 8), :] = y
                del late[0]
            yield

    def up_operands(i, src):
        per = 4 * R // RB
        for t, c in itertools.product(range(0, RB, 64), range(2)):
            def emit(p, v):
                yt[98 * (i // per) + 2 * p + c,
                   pl.ds(_mult(i % per * (RB // 4) + t // 4, 16), 16), :] = v.astype(bf16)

            yield from _enc2(ENC_A, lambda q, k: src[
                pl.ds(t + 16 * q, 16), pl.ds(C4 * k + 128 * c, 128)], emit)

    def job(i, par, extra=None):
        work, paced = [], []
        if i + 1 < S // RB:
            work.append((shift(i + 1, lhs[1 - par]), RB // 8))
            paced.append((lhs[1 - par], (7,), zero))
        if extra is None:
            work.append((up_operands(i - 2, ybuf[par]), 14 * RB // 64))
            paced.append((yt, (98 * NB,), zero))
        else:
            work.append((mixer_norm(*extra), extra[1] // 16))
            paced.append((ulast, (0,), half + zero))
        if extra is None or i > 0:
            work.append((residual(i - 1, hs[1 - par], ybuf[1 - par]), RB // 8))
            paced.append((ybuf[1 - par], (), RB + zero))
        pl.loop(zero, 1)(lambda _: _interleave(
            mixer_out(lhs[par], hs[par]), lambda res: [_pace(*p, res) for p in paced], *work,
            pieces=8))

    cut = E_('CUT', 240)
    _run(shift(0, lhs[0]))
    with jax.named_scope('j01'):
        job(0, 0, (0, cut))
        job(1, 1, (cut, half - cut))
    with jax.named_scope('in'): pl.loop(0, 4)(mixer_in)

    with jax.named_scope('jobs'):
        for i in range(2, S // RB):
            job(i, i % 2)

    last = S // RB - 1
    _interleave(
        [functools.partial(_up_dot, yt, wa, mu0, 0, 0, 0, p) for p in range(49)],
        lambda res: [_pace(y, (), RB + zero, res) for y in ybuf],
        (up_operands(last - 1, ybuf[0]), 14 * RB // 64),
        (residual(last, hs[1], ybuf[1]), RB // 8), pieces=1)
    _run(up_operands(last, ybuf[1]))


def _mlp(zero, out_hbm, wa, xs, hbuf, w4t, yt, sems, mu0, tt0, tt1, mu1, md):
    tts, mu = (tt0, tt1), (mu0, mu1)
    hr = R // 2
    lag = E_("LAG", 14)

    def out_copy(b, n):
        rows = pl.ds(_mult(b * 4 * R, 4 * R), 4 * R)
        return pltpu.make_async_copy(xs.at[n, rows], out_hbm.at[rows, pl.ds(n * HD, HD)],
                                     sems.at[SEM_OUT + 2 * b + n])

    def up_dot(b, j, half, p):
        return _up_dot(yt, wa, mu[half], b, j, half, p)

    def up_sums(act):
        for half, t in itertools.product(range(2), range(hr // 8)):
            c = {}
            for g in ORDER:
                y = _dec(lambda k: mu[half][7 * g + k, pl.ds(8 * t, 8), :])
                for i1, n1, sign in DEC[g]:
                    for (i0, n0), m in y.items():
                        key = (2 * i1 + i0, 2 * n1 + n0)
                        _accumulate(c, key, m, sign)
                        if LAST[i1, n1] == g:
                            act[half, t, key] = _gelu(c.pop(key))
                yield

    def down_operands(act, tt, j):
        for half, t in itertools.product(range(2), range(hr // 16)):
            def emit(p, v):
                tt[NJ * p + j, pl.ds(half * hr + 16 * t, 16), :] = v.astype(bf16)

            yield from _enc2(ENC_A, lambda q, k: jnp.concatenate(
                [act[half, 2 * t, (q, k)], act[half, 2 * t + 1, (q, k)]], axis=0), emit)

    n_sums = 7 * 2 * (hr // 8)

    def up_vector_work(tt, j):
        act = {}
        a, b = up_sums(act), down_operands(act, tt, j)
        for i in range(n_sums + lag):
            if i < n_sums:
                next(a)
            if i >= lag and (i - lag) % 2 == 1:
                next(b)
            yield

    part = []

    def down_dot(tt, g, slot, i, lo, hi):
        p = 7 * g + i // 2
        res = _dot(_operand(tt, [NJ * p + q for q in range(lo, hi)]),
                   _operand(w4t, [14 * g + i], pl.ds(64 * lo, 64 * (hi - lo))))
        if hi < NJ:
            part.append(res)
        else:
            md[7 * slot + i // 2, :, pl.ds(128 * (i % 2), 128)] = part.pop() + res if lo else res
        return res

    def down_block(slot, t):
        c = _dec(lambda k: md[7 * slot + k, pl.ds(16 * t, 16), :])
        return jnp.concatenate(
            [jnp.concatenate([c[i0, 0], c[i0, 1]], axis=1) for i0 in range(2)], axis=0)

    def down_sums(b, g, slot):
        dst = []
        for w in range(2):
            i1 = n1 = sign = 0
            for q in range(7):
                e = DEC[q][w] if w < len(DEC[q]) else DEC[q][0][:2] + (0,)
                i1, n1, sign = (jnp.where(g == q, new, old)
                                for new, old in zip(e, (i1, n1, sign)))
            dst.append((b * 4 * R + 32 * i1, n1, sign.astype(f32)))
        for t in range(R // 16):
            m = down_block(slot, t)
            rows = [pl.ds(pl.multiple_of(d[0] + 64 * t, 32), 32) for d in dst]
            new = [hbuf[dst[0][1], rows[0], :] + m,
                   hbuf[dst[1][1], rows[1], :] + dst[1][2] * m]
            for w in (1, 0):
                hbuf[dst[w][1], rows[w], :] = new[w]
                xs[dst[w][1], rows[w], :] = new[w].astype(bf16)
            yield

    def step(b, par, up, down, j):
        slot = (7 * b + j) & 1
        dots = []
        if up:
            nb = jnp.minimum(b + (j + 1) // NJ, NB - 1)
            nj = jnp.where(j == NJ - 1, 0, j + 1)
            dots = ([(1, functools.partial(up_dot, b, j, 1, p)) for p in range(49)]
                    + [(1, functools.partial(up_dot, nb, nj, 0, p)) for p in range(49)])
            up_work = up_vector_work(tts[par], j)
        if down:
            cuts = (0, E_("KS", 4), NJ) if E_("KS", 4) and up else (0, NJ)
            for i in reversed(range(14)):
                dots[7 * i + E_('D0', 6):7 * i + E_('D0', 6)] = [
                    (hi - lo, functools.partial(down_dot, tts[1 - par], j, slot, i, lo, hi))
                    for lo, hi in zip(cuts, cuts[1:])]
            down_work = down_sums(jnp.maximum(b - 1 - (j == 0), 0),
                                  jnp.where(j == 0, 6, j - 1), 1 - slot)
        total = sum(w for w, _ in dots)
        pos = n_up = done_up = done_down = 0
        for w, dot in dots:
            if down:
                goal = (pos + E_('AD', 8)) * (R // 16) * 100 // (E_("DE", 100) * total)
                for _ in range(done_down, goal):
                    next(down_work, None)
                done_down = max(done_down, goal)
            res = dot()
            k = min(w, E_('PD', 2))
            for i in range(k * up):
                if E_('PM', 1) and (w > 1 or n_up % E_('PM', 1) == 0):
                    _pace(mu[done_up >= n_sums // 2], (49,), zero, res[:res.shape[0] * (i + 1) // k])
                if E_('PN', 1) and (w > 1 or n_up % E_('PN', 1) == 0):
                    _pace(tts[par], (49 * NJ,), zero, res[:res.shape[0] * (i + 1) // k])
                goal = (pos * k + w * (i + 1) + E_('AH', 1) * k) * (n_sums + lag) // (total * k)
                goal = (min(goal, n_sums // 2) if n_up + (w == 1) < 49
                        else max(goal, n_sums // 2))
                for _ in range(done_up, goal):
                    next(up_work, None)
                done_up = max(done_up, goal)
            pos += w
            n_up += w == 1
        if up:
            _run(up_work)
        if down:
            _run(down_work)
        if down:
            @pl.when((j == 0) & (b > 1))
            def _():
                for n in range(2):
                    out_copy(b - 2, n).start()

    md[pl.ds(0, 7)] = jnp.zeros((7, R, C4), f32)
    with jax.named_scope('b0'): pl.loop(0, NJ)(functools.partial(step, 0, 0, True, False))

    @pl.loop(0, NB // 2)
    @jax.named_scope('bmid')
    def _(i):
        pl.loop(0, NJ)(functools.partial(step, 2 * i + 1, 1, True, True))
        pl.loop(0, jnp.where(2 * i + 2 < NB, NJ, 0))(
            functools.partial(step, 2 * i + 2, 0, True, True))

    with jax.named_scope('b4'): pl.loop(0, NJ)(functools.partial(step, NB, 0, False, True))
    out_copy(NB - 1, 1).start()
    pieces = []
    for t in range(R // 16):
        rows = pl.ds(S - 4 * R + 64 * t, 32)
        xs[0, rows, :] = (hbuf[0, rows, :] + down_block((7 * NB + 6) & 1, t)).astype(bf16)
        if t % 2:
            rows = pl.ds(S - 4 * R + 64 * (t - 1), 128)
            pieces.append(pltpu.make_async_copy(
                xs.at[0, rows], out_hbm.at[rows, pl.ds(0, HD)], sems.at[t // 2]))
            pieces[-1].start()
    for b, n in itertools.product(range(NB), range(2)):
        if (b, n) != (NB - 1, 0):
            out_copy(b, n).wait()
    for c in pieces:
        c.wait()


@jax.jit
def pallas_sequential_preLN__memory_aug_recurrent_mem_tr__mixer_s_mlp__prompt_kernel(
    A_x: jax.Array,
    A_mem0: jax.Array,
    A_Wq: jax.Array,
    A_Wk: jax.Array,
    A_Wv: jax.Array,
    A_Wo: jax.Array,
    A_seg_len: jax.Array,
    B_x: jax.Array,
    B_w1: jax.Array,
    B_w2: jax.Array,
    B_w3: jax.Array,
    B_w4: jax.Array,
):
    del A_seg_len, B_x
    hbm = pl.BlockSpec(memory_space=pl.ANY)
    vmem = pl.BlockSpec(memory_space=pltpu.VMEM)
    scratch = [
        pltpu.VMEM((3 * H + 1, D, DH), bf16),
        pltpu.VMEM((2, S + 32, HD), bf16),
        pltpu.VMEM((2, S, HD), f32),
        pltpu.VMEM((98, F // 4, 128), bf16),
        pltpu.VMEM((98 * NB + 1, R, 128), bf16),
        pltpu.VMEM((52, R // 2 + 8, 128), f32),
        pltpu.SemaphoreType.DMA((NSEM,)),
    ]
    out = pl.pallas_call(
        _kernel,
        out_shape=jax.ShapeDtypeStruct((S, D), A_x.dtype),
        in_specs=[hbm, vmem] + [hbm] * 9,
        out_specs=hbm,
        scratch_shapes=scratch,
        compiler_params=pltpu.CompilerParams(vmem_limit_bytes=127 * 1024 * 1024),
    )(A_x.reshape(S, D), A_mem0.reshape(MEM, D),
      A_Wq.reshape(D // 2, 2 * H, DH), A_Wk.reshape(D // 2, 2 * H, DH),
      A_Wv.reshape(D // 2, 2 * H, DH),
      A_Wo.reshape(H * DH, D), B_w1.reshape(D // R, R, D), B_w2.reshape(D // R, R, D),
      B_w3.reshape(D // R, R, F),
      B_w4.reshape(F // R, R, D), B_w4)
    return out.reshape(A_x.shape)
```

```python
import functools
import itertools
import os

import jax
import jax.numpy as jnp
from jax import lax
import jax.experimental.pallas as pl
import jax.experimental.pallas.tpu as pltpu

S = 2048
D = 1024
H = 32
DH = 128
MEM = 8
SEG = 32
F = 3584
NSEG = S // SEG
L = MEM + SEG
TOK = 24
P0 = S - TOK * NSEG
RING = 576
XP = (S - P0) // 8
C4 = D // 4
HALO = 32
RB = 256
R = 128
NB = S // (4 * R)
NJ = F // 512
HD = D // 2
W1_AT, W2_AT = 64, 320
W4T = (F - S) // R
E_ = lambda k, d: int(os.environ.get(k, d))
EPS = 1e-5
NEG = -1000000000.0

LAG_QK, LAG_PV, LAG_WO = E_('LQ', 1), E_('LP', 3), E_('LW', 4)
FILL_AT = E_('FA', 17)
UNROLL = 4

bf16 = jnp.bfloat16
f32 = jnp.float32
u32 = jnp.uint32

SEM_X0, SEM_X, SEM_WO, SEM_W1, SEM_W2, SEM_OUT, SEM_W, SEM_W4, SEM_W3 = (
    0, 2, 10, 14, 22, 30, 38, 50, 66)
NSEM = SEM_W3 + 4 * NJ

ENC_A = (((0, 0, 1), (1, 1, 1)), ((1, 0, 1), (1, 1, 1)), ((0, 0, 1),), ((1, 1, 1),),
         ((0, 0, 1), (0, 1, 1)), ((1, 0, 1), (0, 0, -1)), ((0, 1, 1), (1, 1, -1)))
ENC_B = (((0, 0, 1), (1, 1, 1)), ((0, 0, 1),), ((0, 1, 1), (1, 1, -1)),
         ((1, 0, 1), (0, 0, -1)), ((1, 1, 1),), ((0, 0, 1), (0, 1, 1)),
         ((1, 0, 1), (1, 1, 1)))
DEC = (((0, 0, 1), (1, 1, 1)), ((1, 0, 1), (1, 1, -1)), ((0, 1, 1), (1, 1, 1)),
       ((0, 0, 1), (1, 0, 1)), ((0, 1, 1), (0, 0, -1)), ((1, 1, 1),), ((0, 0, 1),))
ORDER = (0, 1, 3, 2, 4, 5, 6)
LAST = {(1, 0): 3, (0, 1): 4, (1, 1): 5, (0, 0): 6}


def _enc(terms, get):
    v = get(*terms[0][:2])
    for i, j, sign in terms[1:]:
        v = v + get(i, j) if sign > 0 else v - get(i, j)
    return v


def _enc2(table, get, emit):
    for g in range(7):
        y = [[_enc(table[g], lambda i1, j1: get(2 * i1 + i0, 2 * j1 + j0))
              for j0 in range(2)] for i0 in range(2)]
        for k in range(7):
            emit(7 * g + k, _enc(table[k], lambda i0, j0: y[i0][j0]))
        yield


def _right_operands(get, dst, first, row):
    b = [[get(i, j).astype(f32) for j in range(2)] for i in range(2)]
    for p in range(7):
        dst[first + p, pl.ds(row, 16), :] = _enc(ENC_B[p], lambda i, j: b[i][j]).astype(bf16)


def _left_operands(halves, dst, rows):
    for p in range(7):
        v = _enc(ENC_A[p], lambda i, j: halves[i][:, HD * j:HD * j + HD])
        for c in range(4):
            dst[4 * p + c, rows, :] = v[:, 128 * c:128 * c + 128].astype(bf16)


def _collect(acc, p, res, emit):
    for i, j, sign in DEC[p]:
        _accumulate(acc, (i, j), res, sign)
        if LAST[i, j] == p:
            emit(i, j, acc.pop((i, j)))
    return res


def _accumulate(c, key, m, sign):
    c[key] = m if key not in c else (c[key] + m if sign > 0 else c[key] - m)


def _dec(get):
    c = {}
    for k in range(7):
        m = get(k)
        for i, j, sign in DEC[k]:
            _accumulate(c, (i, j), m, sign)
    return c


def _pace(ref, lead, row, result):
    n = 32 // ref.dtype.itemsize
    ref[(*lead, pl.ds(pl.multiple_of(row, n), n), pl.ds(0, 128))] = (
        result[-n:, :128].astype(ref.dtype))


def _run(gen):
    for _ in gen:
        pass


def _mult(i, n):
    return i if isinstance(i, int) else pl.multiple_of(i, n)


def _ln(x):
    m = jnp.mean(x, axis=-1, keepdims=True)
    d = x - m
    v = jnp.mean(d * d, axis=-1, keepdims=True)
    return d * lax.rsqrt(v + EPS)


def _gelu(x):
    c = 0.7978845608028654
    hx = 0.5 * x
    return hx + hx * jnp.tanh(x * (c + (c * 0.044715) * (x * x)))


def _unpack(x):
    return pltpu.bitcast(x, bf16)


def _operand(ref, blocks, rows=slice(None)):
    words = ref.bitcast(u32)
    return _unpack(jnp.concatenate([words[b, rows, :] for b in blocks], axis=1))


def _dot(a, b):
    return jnp.dot(a, b, preferred_element_type=f32)


def _rows(ref, rows):
    return jnp.concatenate([ref[0, rows, :], ref[1, rows, :]], axis=1)


def _set_rows(ref, rows, v):
    ref[0, rows, :] = v[:, :HD]
    ref[1, rows, :] = v[:, HD:]


def _kernel(*refs):
    out_hbm, wa, xs, hbuf, w4t, yt, mu0, sems = refs[11:]
    zero = pl.run_scoped(
        functools.partial(_attention_and_mixer, *refs),
        pltpu.VMEM((H * DH // 2, D), u32),
        pltpu.VMEM((8, S + 2 * HALO, 128), f32),
        pltpu.VMEM((28, 2 * TOK, 128), bf16),
        pltpu.VMEM((28, HD, 128), bf16),
        *[pltpu.VMEM((H // 8, RING, DH), f32)] * 8)
    if E_("SKIP_MLP", 0):
        for b in (w4t, yt, wa):
            pltpu.sync_copy(b.at[0, pl.ds(0, 128)], out_hbm.at[pl.ds(0, 128), pl.ds(0, 128)])
        return
    with jax.named_scope('s_mlp'): pl.run_scoped(
        functools.partial(_mlp, zero, out_hbm, wa, xs, hbuf, w4t, yt, sems, mu0),
        *[pltpu.VMEM((49 * NJ + 1, R, 128), bf16)] * 2,
        pltpu.VMEM(mu0.shape, f32),
        pltpu.VMEM((14, R, C4), f32))


def _attention_and_mixer(x_hbm, mem0_ref, wq_hbm, wk_hbm, wv_hbm, wo_hbm, w1_hbm, w2_hbm,
                         w3_hbm, w4_hbm, w4a_hbm, out_hbm, wa, xs, hbuf, w4t, yt, mu0, sems,
                         wo_b, xg, ubuf, w1t, *q_rings):
    def w3_copy(c):
        return pltpu.make_async_copy(
            w3_hbm.at[:, :, pl.ds(_mult(c * 128, 128), 128)], yt.at[pl.ds(8 * c, 8)],
            sems.at[SEM_W3 + c])

    def w4_head_copy(c):
        return pltpu.make_async_copy(
            w4a_hbm.at[pl.ds(0, S), pl.ds(_mult(c * 128, 128), 128)],
            xs.at[c % 2, pl.ds(0, S), pl.ds(_mult(c // 2 * 128, 128), 128)], sems.at[SEM_W4 + c])

    def w4_tail_copy(c):
        return pltpu.make_async_copy(
            w4_hbm.at[pl.ds(S // R, W4T), :, pl.ds(_mult(c * 128, 128), 128)],
            yt.at[pl.ds(32 * NJ + W4T * c, W4T)], sems.at[SEM_W4 + 8 + c])

    def w2_copy(c):
        return pltpu.make_async_copy(
            w2_hbm.at[:, :, pl.ds(_mult(c * 128, 128), 128)], yt.at[pl.ds(W2_AT + 8 * c, 8)],
            sems.at[SEM_W2 + c])

    others = [f(c) for f in (w2_copy, w4_head_copy, w4_tail_copy) for c in range(8)]

    def fetch(i):
        @pl.loop(i, jnp.where(i < 8, i + 1, i))
        def _(c):
            for f in (w2_copy, w4_head_copy, w4_tail_copy):
                f(c).start()

            @pl.when(c < NJ)
            def _():
                for k in range(4):
                    w3_copy(4 * c + k).start()

    zero = pl.run_scoped(
        functools.partial(_attention, x_hbm, mem0_ref, (wq_hbm, wk_hbm, wv_hbm), wo_hbm,
                          w1_hbm, fetch, w4t, yt, wa, xs, hbuf, sems, wo_b, xg, ubuf, w1t, q_rings),
        *[pltpu.VMEM((H // 8, RING, DH), f32)] * 16)
    for c in others:
        c.wait()
    for c in range(4 * NJ):
        w3_copy(c).wait()
    if E_("SKIP_POST", 0): return zero
    with jax.named_scope('s_mix'): pl.run_scoped(
        functools.partial(_mixer, zero, mu0, wa, xs, w4t, hbuf, yt, wo_b, xg, w1t, q_rings),
        pltpu.VMEM((28, HD, 128), bf16),
        pltpu.VMEM((28, P0 // 2 + 2 * TOK + 16, 128), bf16),
        *[pltpu.VMEM((8, P0, 128), bf16)] * 2, *[pltpu.VMEM((RB, D), f32)] * 2,
        *[pltpu.VMEM((RB + 8, D), f32)] * 2)
    return zero


def _attention(x_hbm, mem0_ref, w_hbm, wo_hbm, w1_hbm, fetch,
               w4t, yt, wa, xs, hbuf, sems, wo_b, xg, ubuf, w1t, q_rings, *kv_rings):
    rings = q_rings + kv_rings
    ring = [[rings[m * 8 + h % 8].at[h // 8] for h in range(H)] for m in range(3)]
    q_r, k_r, v_r = ring

    class x_rows:
        def __init__(self, rows, sem):
            self.copies = [
                pltpu.make_async_copy(x_hbm.at[rows, pl.ds(n * HD, HD)], xs.at[n, rows],
                                      sems.at[sem + n]) for n in range(2)]

        def start(self):
            for c in self.copies:
                c.start()

        def wait(self):
            for c in self.copies:
                c.wait()

    x0_copy = x_rows(pl.ds(0, P0), SEM_X0)

    def x_copy(g):
        return x_rows(pl.ds(_mult(P0 + g * 2 * XP, XP), 2 * XP), SEM_X + 2 * g)

    def wo_copy(i):
        rows = pl.ds(_mult(i * 512, 512), 512)
        return pltpu.make_async_copy(wo_hbm.bitcast(u32).at[rows], wo_b.at[rows],
                                     sems.at[SEM_WO + i])

    def w1_copy(c):
        return pltpu.make_async_copy(
            w1_hbm.at[:, :, pl.ds(_mult(c * 128, 128), 128)], yt.at[pl.ds(W1_AT + 8 * c, 8)],
            sems.at[SEM_W1 + c])

    def prologue(*stg):

        def start_chunk(g, m, first=False):
            src = w_hbm[m].bitcast(u32)
            for pair, par in itertools.product(range(4), range(2)):
                pltpu.make_async_copy(
                    src.at[:, 16 * par + 4 * g + pair, :],
                    stg[m].at[pl.ds((2 * pair + par) * HD, HD)],
                    sems.at[SEM_OUT + pair if first else SEM_W + 3 * g + m]).start()

        def wait_chunk(g, m):
            pltpu.make_async_copy(stg[m], stg[m], sems.at[SEM_W + 3 * g + m]).wait()

        def relayout(g, m, pair, i0, n):
            ev, od = (stg[m][pl.ds(_mult((2 * pair + par) * HD + i0, 8), n), :]
                      for par in range(2))
            h = 8 * g + 2 * pair
            words = wa.bitcast(u32)
            words[m * H + h, pl.ds(i0, n), :] = (ev & jnp.uint32(0xFFFF)) | (od << 16)
            words[m * H + h + 1, pl.ds(i0, n), :] = (ev >> 16) | (od & jnp.uint32(0xFFFF0000))

        def weights(g, m, pair):
            h = m * H + 8 * g + 2 * pair
            for t in range(D // 32 + 1):
                if t < D // 32:
                    for k in range(2):
                        relayout(g, m, pair, D // 4 * k + 8 * t, 8)
                if t > 0:
                    r = 16 * (t - 1)
                    _right_operands(lambda k, n: wa[h + n, pl.ds(HD * k + r, 16), :],
                                    w4t, 28 * m + 7 * pair, r)
                yield

        def norm_rows(r0, n):
            xv = _rows(xs, pl.ds(r0, n)).astype(f32)
            _set_rows(hbuf, pl.ds(r0, n), xv)
            return _ln(xv)

        def later_rows(r0):
            for r in range(0, XP, 16):
                xn = norm_rows(pl.multiple_of(r0 + r, 16), 16)
                for c in range(8):
                    xg[c, pl.ds(pl.multiple_of(HALO + r0 + r, 8), 16), :] = (
                        xn[:, 128 * c:128 * c + 128])
                yield

        x0_copy.start()
        start_chunk(0, 0, first=True)
        start_chunk(0, 1)
        start_chunk(0, 2)
        x_copy(0).start()
        zero = jnp.zeros((HALO, 128), f32)
        for c in range(8):
            xg[c, pl.ds(0, HALO), :] = zero
            xg[c, pl.ds(HALO + S, HALO), :] = zero
        with jax.named_scope('wx'): x0_copy.wait()

        @pl.loop(0, P0 // 64)
        def _(i):
            a = [norm_rows(pl.multiple_of(P0 // 2 * k + 32 * i, 32), 32) for k in range(2)]
            for p in range(7):
                v = _enc(ENC_A[p], lambda k, n: a[k][:, HD * n:HD * n + HD])
                for c in range(4):
                    yt[8 * p + 4 * (i // 4) + c, pl.ds(pl.multiple_of(i % 4 * 32, 32), 32), :] = (
                        v[:, 128 * c:128 * c + 128].astype(bf16))

        @pl.loop(0, 4)
        def _(pair):
            both = stg[0].at[pl.ds(pl.multiple_of(pair * D, D), D)]
            pltpu.make_async_copy(both, both, sems.at[SEM_OUT + pair]).wait()
            _run(weights(0, 0, pair))

        def stage(g, m):
            m1 = (m + 1) % 3
            g1 = jnp.minimum(g + (1 if m == 2 else 0), 3)
            if m > 0:
                pl.when(3 * g + m < 11)(functools.partial(wait_chunk, g1, m1))
            if m == 1:
                x_copy(g).wait()

            @pl.when(g < 3)
            def _():
                start_chunk(g + 1, m)
                if m == 1:
                    x_copy(g + 1).start()
            if m == E_('WM', 1):
                wo_copy(g).start()
            if m == 2:
                w1_copy(2 * g).start()
                w1_copy(2 * g + 1).start()
            n = E_("PR", 64)
            acc = {}

            def dot(pair, r, p):
                res = _dot(
                    _operand(yt, [8 * p + 4 * (r // R) + k for k in range(4)],
                             pl.ds(r % R // 2, n // 2)),
                    _operand(w4t, [28 * m + 7 * pair + p], pl.ds(0, HD // 2)))
                for i, j, sign in DEC[p]:
                    _accumulate(acc, (i, j), res, sign)
                    if LAST[i, j] == p:
                        rings[m * 8 + 2 * pair + j][g, pl.ds(P0 // 2 * i + r, n), :] = (
                            acc.pop((i, j)))
                return res

            dots = [functools.partial(dot, pair, r, p) for pair in range(4)
                    for r in range(0, P0 // 2, n) for p in ORDER]
            work = [(itertools.chain(*[weights(g1, m1, pair) for pair in range(4)]),
                     4 * (D // 32 + 1))]
            paced = [(wa, (3 * H,), 16 * (g >> 10))]
            if m == 0:
                early = E_("EA", 49)
                for d in dots[:early]:
                    d()
                dots = dots[early:]
                wait_chunk(g1, m1)
            else:
                work.append((later_rows(P0 + (2 * g + m - 1) * XP), XP // 16))
                paced.append((xg, (0,), 8 * (g >> 10)))
            _interleave(dots, lambda res: [_pace(*p, res) for p in paced], *work,
                        pieces=1 if m else E_("PQ", 2))

        @pl.loop(0, 4)
        def _(g):
            for m in range(3):
                with jax.named_scope(f'st{m}'): stage(g, m)

    if not E_('SKIP_PRO', 0):
     with jax.named_scope('s_pro'): pl.run_scoped(
        prologue,
        pltpu.VMEM((8 * D // 2, DH), u32),
        pltpu.VMEM((8 * D // 2, DH), u32),
        pltpu.VMEM((8 * D // 2, DH), u32),
    )
    for i in range(4):
        if E_('WM', 1) > 2: wo_copy(i).start()
        with jax.named_scope('wwo'): wo_copy(i).wait()
    for c in range(8):
        w1_copy(c).wait()

    @pl.loop(0, 16)
    def _(i):
        c, q = i >> 2, i & 3
        for r in range(0, 128, 16):
            _right_operands(lambda k, n: yt[W1_AT + 16 * c + 8 * n + 4 * k + q, pl.ds(r, 16), :],
                            w1t, 7 * c, pl.multiple_of(128 * q + r, 16))

    def wrap(r):
        return jnp.where(r >= RING, r - RING, r)

    group = UNROLL * TOK

    def step(i, k, mem, tok, rp, ra, rw):
        ri = lax.broadcasted_iota(jnp.int32, (2 * L, 2 * L), 0)
        ci = lax.broadcasted_iota(jnp.int32, (2 * L, 2 * L), 1)
        same = (ri >= L) == (ci >= L)
        ri, ci = (jnp.where(v >= L, v - L, v) for v in (ri, ci))
        mask = same & ((ri < MEM) | (ri >= ci))
        fill = jnp.where(same, NEG, -jnp.inf)

        lhs = jnp.concatenate([mem, tok], axis=0).astype(bf16)
        rps = [pl.multiple_of(wrap(rp + r // SEG * SEG), SEG) + r % SEG
               for r in range(TOK * k, TOK * (k + 1), 8)]
        ra_ = pl.multiple_of(wrap(ra + SEG * k), SEG)
        rw_ = pl.multiple_of(rw, SEG) + TOK * k

        rb = pl.multiple_of(jnp.maximum(i - 1, 0) * group, SEG)
        if k == 0:
            _left_operands([_ln(_ln(_rows(hbuf, pl.ds(rb + group // 2 * q, group // 2))))
                            for q in range(2)], ubuf, slice(None))
        filled = {}

        def filler(products):
            def emit(q, j, v):
                xg[2 * k + j, pl.ds(HALO + rb + group // 2 * q, group // 2), :] = _gelu(v)

            for p in products:
                _collect(filled, p, _dot(_operand(ubuf, range(4 * p, 4 * p + 4)),
                                         _operand(w1t, [7 * k + p])), emit)

        mem_qkv = {}
        scores = {}
        o_mem = {}
        total = [None]

        def qkv(h):
            res = {}
            for m in ((0, 1, 2), (1, 0, 2), (2, 0, 1), (2, 1, 0))[E_('MO', 0)]:
                r = _dot(lhs, _operand(wa, [m * H + h]))
                for q in range(3):
                    ring[m][h][pl.ds(rps[q], 8), :] = r[8 + 8 * q:16 + 8 * q]
                res[m] = r[:MEM]
            mem_qkv[h] = res

        def both(m, a):
            return jnp.concatenate(
                [v for h in (2 * a, 2 * a + 1)
                 for v in (mem_qkv[h][m], ring[m][h][pl.ds(ra_, SEG), :])],
                axis=0).astype(bf16)

        def qk(a):
            scores[a] = lax.dot_general(both(0, a), both(1, a), (((1,), (1,)), ((), ())),
                                        preferred_element_type=f32)

        def pv(a):
            sc = jnp.where(mask, scores.pop(a) * (DH ** -0.5), fill)
            mx = jnp.max(sc, axis=1, keepdims=True)
            e = jnp.exp(sc - mx)
            den = jnp.sum(e, axis=1, keepdims=True)
            inv = pl.reciprocal(den, approx=True)
            inv = inv * (2.0 - den * inv)
            o = _dot(e.astype(bf16), both(2, a)) * inv
            for q, h in enumerate((2 * a, 2 * a + 1)):
                q_r[h][pl.ds(ra_, SEG), :] = o[q * L + MEM:(q + 1) * L]
                o_mem[h] = o[q * L:q * L + MEM]

        def wo(h):
            lo = jnp.concatenate([o_mem.pop(h), q_r[h][pl.ds(rw_, TOK), :]],
                                 axis=0).astype(bf16)
            r = _dot(lo, _unpack(wo_b[pl.ds(h * DH // 2, DH // 2), :]))
            total[0] = r if total[0] is None else total[0] + r

        npair = H // 2
        for t in range(npair + LAG_WO):
            heads = (2 * t, 2 * t + 1) if t < npair else ()
            late = (2 * (t - LAG_WO), 2 * (t - LAG_WO) + 1) if t >= LAG_WO else ()
            cuts = [0, E_('FS', 2), E_('FS', 2) + E_('F2', 0)]
            for op in os.environ.get("SEQ", "abqpfcd"):
                if op in "ab" and heads: qkv(heads[op == "b"])
                if op in "cd" and late: wo(late[op == "d"])
                if op == "q" and 0 <= t - LAG_QK < npair: qk(t - LAG_QK)
                if op == "p" and 0 <= t - LAG_PV < npair: pv(t - LAG_PV)
                if op == "f" and 0 <= t - FILL_AT < 2: filler(ORDER[cuts[t - FILL_AT]:cuts[t - FILL_AT + 1]])
        filler(ORDER[cuts[2]:])

        a = total[0]
        rows = pl.ds(pl.multiple_of(group * i, SEG) + TOK * k, TOK)
        _set_rows(hbuf, rows, _rows(hbuf, rows) + a[MEM:])
        return a[:MEM]

    def steps(i, carry):
        mem, rp, ra, rw = carry
        fetch(i)
        r0 = pl.multiple_of(HALO + P0 + group * i, SEG)
        toks = [jnp.concatenate([xg[c, pl.ds(r0 + TOK * k, TOK), :] for c in range(8)], axis=1)
                for k in range(UNROLL)]
        for k in range(UNROLL):
            mem = step(i, k, mem, toks[k], rp, ra, rw)
        return mem, wrap(rp + group), wrap(ra + UNROLL * SEG), wrap(rw + group)

    if E_('SKIP_LOOP', 0): return lax.fori_loop(0, 64, lambda i, c: wrap(c + TOK), jnp.int32(0)) - TOK * NSEG % RING
    with jax.named_scope('s_loop'): carry = lax.fori_loop(
        0, NSEG // UNROLL, steps,
        (mem0_ref[...].astype(f32), jnp.int32(P0), jnp.int32(0), jnp.int32(0)))
    return carry[3] - TOK * NSEG % RING


def _interleave(dots, pace, *work, pieces=8):
    for i, dot in enumerate(dots):
        res = dot()
        k = min(pieces, res.shape[0] // 16)
        for j in range(k):
            pace(res[:res.shape[0] // 16 * (j + 1) // k * 16])
            for gen, n in work:
                for _ in range(n * (i * k + j) // (k * len(dots)),
                               n * (i * k + j + 1) // (k * len(dots))):
                    next(gen)
    for gen, _ in work:
        _run(gen)


def _up_dot(yt, wa, mu, b, j, half, p):
    res = _dot(
        _operand(yt, [98 * b + 2 * p, 98 * b + 2 * p + 1], pl.ds(half * R // 4, R // 4)),
        _operand(wa, [13 * j + p // 4], pl.ds(128 * (p % 4), 128)))
    mu[p, pl.ds(0, R // 2), :] = res
    return res


def _mixer(zero, mu0, wa, xs, w4t, hbuf, yt, wo_b, xg, w1t, q_rings, w2t, ulast, lhs0, lhs1, hs0, hs1, *ybuf):
    lhs, hs = (lhs0, lhs1), (hs0, hs1)

    def encode_w3(g):
        for j, t in itertools.product(range(NJ), range(4)):
            def get(k, n):
                return yt[32 * j + 8 * n + 2 * k + (g >> 1),
                          pl.ds(pl.multiple_of(64 * (g & 1) + 16 * t, 16), 16), :].astype(f32)

            def emit(p, v):
                wa[13 * j + p // 4, pl.ds(pl.multiple_of(C4 * (p % 4) + 64 * g + 16 * t, 16), 16),
                   :] = v.astype(bf16)

            yield from _enc2(ENC_B, get, emit)

    def encode_w4(g):
        c = g >> 1
        for j, t in itertools.product(range(NJ), range(4)):
            r = pl.multiple_of(64 * (g & 1) + 16 * t, 16)

            def get(k, n):
                if 512 * j < S:
                    return xs[c, pl.ds(512 * j + 128 * k + r, 16), pl.ds(128 * n, 128)].astype(f32)
                return yt[32 * NJ + W4T * (2 * n + c) + 4 * j - S // R + k,
                          pl.ds(r, 16), :].astype(f32)

            def emit(p, v):
                w4t[2 * p + c, pl.ds(128 * j + r, 16), :] = v.astype(bf16)

            yield from _enc2(ENC_B, get, emit)

    def encode_w2(g):
        for t, c in itertools.product(range(8), range(4)):
            _right_operands(
                lambda k, n: yt[W2_AT + 8 * (4 * n + c) + 4 * k + g, pl.ds(16 * t, 16), :],
                w2t, 7 * c, pl.multiple_of(128 * g + 16 * t, 16))
            yield

    done = TOK * NSEG
    first = 4 * TOK * (NSEG // 4 - 1)

    @jax.named_scope('q1')
    def q1(g):
        n = 128
        for k, q in enumerate(q_rings):
            for r in range(0, P0, 64):
                lhs0[k, pl.ds(r, 64), :] = q[g, pl.ds((done + r) % RING, 64), :].astype(bf16)

        part = []

        def dot(r, c, k):
            w = wo_b[pl.ds(pl.multiple_of((2 * g + k) * 2 * DH, 2 * DH), 2 * DH),
                     pl.ds(128 * c, 128)]
            res = _dot(_operand(lhs0, range(4 * k, 4 * k + 4), pl.ds(r // 2, n // 2)), _unpack(w))
            if k == 0:
                part.append(res)
            else:
                hbuf[c // 4, pl.ds(done + r, n), pl.ds(128 * (c % 4), 128)] += part.pop() + res
            return res

        _interleave(
            [functools.partial(dot, r, c, k)
             for r in range(0, P0, n) for c in range(8) for k in range(2)],
            lambda res: [_pace(yt, (98 * NB,), zero, res), _pace(xs, (0,), S + zero, res)],
            (encode_w2(g), 32),
            (encode_w4(g), 28 * NJ), (encode_w3(g), 28 * NJ), pieces=8)

    pl.loop(0, H // 8)(q1)

    half = (S - first) // 2

    def mixer_norm(r0, n):
        for r in range(r0, r0 + n, 16):
            _left_operands([_ln(_ln(_rows(hbuf, pl.ds(first + half * i + r, 16))))
                            for i in range(2)], ulast, pl.ds(r, 16))
            yield

    def mixer_in(c):
        step = E_("IR", 64)
        for r in range(0, half, step):
            n = min(step, half - r)
            acc = {}

            def emit(i, j, v):
                xg[2 * c + j, pl.ds(HALO + first + half * i + r, n), :] = _gelu(v)

            for p in ORDER:
                _collect(acc, p, _dot(
                    _operand(ulast, range(4 * p, 4 * p + 4), pl.ds(r // 2, n // 2)),
                    _operand(w1t, [7 * c + p])), emit)

    def shift(i, dst):
        for r, c in itertools.product(range(0, RB // 2, 16), range(4)):
            a = [[xg[4 * k + c, pl.ds(HALO + (-1, 1, -2, 2)[2 * k + c // 2]
                                      + i * RB + RB // 2 * q + r, 16), :]
                  for k in range(2)] for q in range(2)]
            for p in range(7):
                dst[p, pl.ds(RB // 2 * c + r, 16), :] = _enc(
                    ENC_A[p], lambda q, k: a[q][k]).astype(bf16)
            yield

    def mixer_out(src, dst):
        n = 128
        acc = {}

        def dot(r, c, p):
            words = src.bitcast(u32)
            a = jnp.concatenate([words[p, pl.ds((RB // 2 * k + r) // 2, n // 2), :]
                                 for k in range(4)], axis=1)
            res = _dot(_unpack(a), _operand(w2t, [7 * c + p]))
            for i, j, sign in DEC[p]:
                _accumulate(acc, (i, j), res, sign)
                if LAST[i, j] == p:
                    dst[pl.ds(RB // 2 * i + r, n), pl.ds(HD * j + 128 * c, 128)] = acc.pop((i, j))
            return res

        return [functools.partial(dot, r, c, p)
                for r in range(0, RB // 2, n) for c in range(4) for p in ORDER]

    def residual(i, src, dst):
        late = []
        for t in range(0, RB, 8):
            rows = pl.ds(_mult(i * RB + t, 8), 8)
            hv = _rows(hbuf, rows)
            x1 = _ln(hv) + src[pl.ds(t, 8), :]
            late.append((rows, hv + x1, t, _ln(x1)))
            if len(late) > E_("LT", 0) or t == RB - 8:
                for rows, v, t0, y in late[:None if t == RB - 8 else 1]:
                    _set_rows(hbuf, rows, v)
                    dst[pl.ds(t0, 8), :] = y
                del late[0]
            yield

    def up_operands(i, src):
        per = 4 * R // RB
        for t, c in itertools.product(range(0, RB, 64), range(2)):
            def emit(p, v):
                yt[98 * (i // per) + 2 * p + c,
                   pl.ds(_mult(i % per * (RB // 4) + t // 4, 16), 16), :] = v.astype(bf16)

            yield from _enc2(ENC_A, lambda q, k: src[
                pl.ds(t + 16 * q, 16), pl.ds(C4 * k + 128 * c, 128)], emit)

    def job(i, par, extra=None):
        work, paced = [], []
        if i + 1 < S // RB:
            work.append((shift(i + 1, lhs[1 - par]), RB // 8))
            paced.append((lhs[1 - par], (7,), zero))
        if extra is None:
            work.append((up_operands(i - 2, ybuf[par]), 14 * RB // 64))
            paced.append((yt, (98 * NB,), zero))
        else:
            work.append((mixer_norm(*extra), extra[1] // 16))
            paced.append((ulast, (0,), half + zero))
        if extra is None or i > 0:
            work.append((residual(i - 1, hs[1 - par], ybuf[1 - par]), RB // 8))
            paced.append((ybuf[1 - par], (), RB + zero))
        pl.loop(zero, 1)(lambda _: _interleave(
            mixer_out(lhs[par], hs[par]), lambda res: [_pace(*p, res) for p in paced], *work,
            pieces=8))

    cut = E_('CUT', 240)
    _run(shift(0, lhs[0]))
    with jax.named_scope('j01'):
        job(0, 0, (0, cut))
        job(1, 1, (cut, half - cut))
    with jax.named_scope('in'): pl.loop(0, 4)(mixer_in)

    with jax.named_scope('jobs'):
        for i in range(2, S // RB):
            job(i, i % 2)

    last = S // RB - 1
    _interleave(
        [functools.partial(_up_dot, yt, wa, mu0, 0, 0, 0, p) for p in range(49)],
        lambda res: [_pace(y, (), RB + zero, res) for y in ybuf],
        (up_operands(last - 1, ybuf[0]), 14 * RB // 64),
        (residual(last, hs[1], ybuf[1]), RB // 8), pieces=1)
    _run(up_operands(last, ybuf[1]))


def _mlp(zero, out_hbm, wa, xs, hbuf, w4t, yt, sems, mu0, tt0, tt1, mu1, md):
    tts, mu = (tt0, tt1), (mu0, mu1)
    hr = R // 2
    lag = E_("LAG", 14)

    def out_copy(b, n):
        rows = pl.ds(_mult(b * 4 * R, 4 * R), 4 * R)
        return pltpu.make_async_copy(xs.at[n, rows], out_hbm.at[rows, pl.ds(n * HD, HD)],
                                     sems.at[SEM_OUT + 2 * b + n])

    def up_dot(b, j, half, p):
        return _up_dot(yt, wa, mu[half], b, j, half, p)

    def up_sums(act):
        for half, t in itertools.product(range(2), range(hr // 8)):
            c = {}
            for g in ORDER:
                y = _dec(lambda k: mu[half][7 * g + k, pl.ds(8 * t, 8), :])
                for i1, n1, sign in DEC[g]:
                    for (i0, n0), m in y.items():
                        key = (2 * i1 + i0, 2 * n1 + n0)
                        _accumulate(c, key, m, sign)
                        if LAST[i1, n1] == g:
                            act[half, t, key] = _gelu(c.pop(key))
                yield

    def down_operands(act, tt, j):
        for half, t in itertools.product(range(2), range(hr // 16)):
            def emit(p, v):
                tt[NJ * p + j, pl.ds(half * hr + 16 * t, 16), :] = v.astype(bf16)

            yield from _enc2(ENC_A, lambda q, k: jnp.concatenate(
                [act[half, 2 * t, (q, k)], act[half, 2 * t + 1, (q, k)]], axis=0), emit)

    n_sums = 7 * 2 * (hr // 8)

    def up_vector_work(tt, j):
        act = {}
        a, b = up_sums(act), down_operands(act, tt, j)
        for i in range(n_sums + lag):
            if i < n_sums:
                next(a)
            if i >= lag and (i - lag) % 2 == 1:
                next(b)
            yield

    part = []

    def down_dot(tt, g, slot, i, lo, hi):
        p = 7 * g + i // 2
        res = _dot(_operand(tt, [NJ * p + q for q in range(lo, hi)]),
                   _operand(w4t, [14 * g + i], pl.ds(64 * lo, 64 * (hi - lo))))
        if hi < NJ:
            part.append(res)
        else:
            md[7 * slot + i // 2, :, pl.ds(128 * (i % 2), 128)] = part.pop() + res if lo else res
        return res

    def down_block(slot, t):
        c = _dec(lambda k: md[7 * slot + k, pl.ds(16 * t, 16), :])
        return jnp.concatenate(
            [jnp.concatenate([c[i0, 0], c[i0, 1]], axis=1) for i0 in range(2)], axis=0)

    def down_sums(b, g, slot):
        dst = []
        for w in range(2):
            i1 = n1 = sign = 0
            for q in range(7):
                e = DEC[q][w] if w < len(DEC[q]) else DEC[q][0][:2] + (0,)
                i1, n1, sign = (jnp.where(g == q, new, old)
                                for new, old in zip(e, (i1, n1, sign)))
            dst.append((b * 4 * R + 32 * i1, n1, sign.astype(f32)))
        for t in range(R // 16):
            m = down_block(slot, t)
            rows = [pl.ds(pl.multiple_of(d[0] + 64 * t, 32), 32) for d in dst]
            new = [hbuf[dst[0][1], rows[0], :] + m,
                   hbuf[dst[1][1], rows[1], :] + dst[1][2] * m]
            for w in (1, 0):
                hbuf[dst[w][1], rows[w], :] = new[w]
                xs[dst[w][1], rows[w], :] = new[w].astype(bf16)
            yield

    def step(b, par, up, down, j):
        slot = (7 * b + j) & 1
        dots = []
        if up:
            nb = jnp.minimum(b + (j + 1) // NJ, NB - 1)
            nj = jnp.where(j == NJ - 1, 0, j + 1)
            dots = ([(1, functools.partial(up_dot, b, j, 1, p)) for p in range(49)]
                    + [(1, functools.partial(up_dot, nb, nj, 0, p)) for p in range(49)])
            up_work = up_vector_work(tts[par], j)
        if down:
            cuts = (0, E_("KS", 4), NJ) if E_("KS", 4) and up else (0, NJ)
            for i in reversed(range(14)):
                dots[7 * i + E_('D0', 6):7 * i + E_('D0', 6)] = [
                    (hi - lo, functools.partial(down_dot, tts[1 - par], j, slot, i, lo, hi))
                    for lo, hi in zip(cuts, cuts[1:])]
            down_work = down_sums(jnp.maximum(b - 1 - (j == 0), 0),
                                  jnp.where(j == 0, 6, j - 1), 1 - slot)
        total = sum(w for w, _ in dots)
        pos = n_up = done_up = done_down = 0
        for w, dot in dots:
            if down:
                goal = (pos + E_('AD', 8)) * (R // 16) * 100 // (E_("DE", 100) * total)
                for _ in range(done_down, goal):
                    next(down_work, None)
                done_down = max(done_down, goal)
            res = dot()
            k = min(w, E_('PD', 2))
            for i in range(k * up):
                if E_('PM', 1) and (w > 1 or n_up % E_('PM', 1) == 0):
                    _pace(mu[done_up >= n_sums // 2], (49,), zero, res[:res.shape[0] * (i + 1) // k])
                if E_('PN', 1) and (w > 1 or n_up % E_('PN', 1) == 0):
                    _pace(tts[par], (49 * NJ,), zero, res[:res.shape[0] * (i + 1) // k])
                goal = (pos * k + w * (i + 1) + E_('AH', 1) * k) * (n_sums + lag) // (total * k)
                goal = (min(goal, n_sums // 2) if n_up + (w == 1) < 49
                        else max(goal, n_sums // 2))
                for _ in range(done_up, goal):
                    next(up_work, None)
                done_up = max(done_up, goal)
            pos += w
            n_up += w == 1
        if up:
            _run(up_work)
        if down:
            _run(down_work)
        if down:
            @pl.when((j == 0) & (b > 1))
            def _():
                for n in range(2):
                    out_copy(b - 2, n).start()

    md[pl.ds(0, 7)] = jnp.zeros((7, R, C4), f32)
    with jax.named_scope('b0'): pl.loop(0, NJ)(functools.partial(step, 0, 0, True, False))

    @pl.loop(0, NB // 2)
    @jax.named_scope('bmid')
    def _(i):
        pl.loop(0, NJ)(functools.partial(step, 2 * i + 1, 1, True, True))
        pl.loop(0, jnp.where(2 * i + 2 < NB, NJ, 0))(
            functools.partial(step, 2 * i + 2, 0, True, True))

    with jax.named_scope('b4'): pl.loop(0, NJ)(functools.partial(step, NB, 0, False, True))
    out_copy(NB - 1, 1).start()
    pieces = []
    for t in range(R // 16):
        rows = pl.ds(S - 4 * R + 64 * t, 32)
        xs[0, rows, :] = (hbuf[0, rows, :] + down_block((7 * NB + 6) & 1, t)).astype(bf16)
        if t % 2:
            rows = pl.ds(S - 4 * R + 64 * (t - 1), 128)
            pieces.append(pltpu.make_async_copy(
                xs.at[0, rows], out_hbm.at[rows, pl.ds(0, HD)], sems.at[t // 2]))
            pieces[-1].start()
    for b, n in itertools.product(range(NB), range(2)):
        if (b, n) != (NB - 1, 0):
            out_copy(b, n).wait()
    for c in pieces:
        c.wait()


@jax.jit
def pallas_sequential_preLN__memory_aug_recurrent_mem_tr__mixer_s_mlp__prompt_kernel(
    A_x: jax.Array,
    A_mem0: jax.Array,
    A_Wq: jax.Array,
    A_Wk: jax.Array,
    A_Wv: jax.Array,
    A_Wo: jax.Array,
    A_seg_len: jax.Array,
    B_x: jax.Array,
    B_w1: jax.Array,
    B_w2: jax.Array,
    B_w3: jax.Array,
    B_w4: jax.Array,
):
    del A_seg_len, B_x
    hbm = pl.BlockSpec(memory_space=pl.ANY)
    vmem = pl.BlockSpec(memory_space=pltpu.VMEM)
    scratch = [
        pltpu.VMEM((3 * H + 1, D, DH), bf16),
        pltpu.VMEM((2, S + 32, HD), bf16),
        pltpu.VMEM((2, S, HD), f32),
        pltpu.VMEM((98, F // 4, 128), bf16),
        pltpu.VMEM((98 * NB + 1, R, 128), bf16),
        pltpu.VMEM((52, R // 2 + 8, 128), f32),
        pltpu.SemaphoreType.DMA((NSEM,)),
    ]
    out = pl.pallas_call(
        _kernel,
        out_shape=jax.ShapeDtypeStruct((S, D), A_x.dtype),
        in_specs=[hbm, vmem] + [hbm] * 9,
        out_specs=hbm,
        scratch_shapes=scratch,
        compiler_params=pltpu.CompilerParams(vmem_limit_bytes=127 * 1024 * 1024),
    )(A_x.reshape(S, D), A_mem0.reshape(MEM, D),
      A_Wq.reshape(D // 2, 2 * H, DH), A_Wk.reshape(D // 2, 2 * H, DH),
      A_Wv.reshape(D // 2, 2 * H, DH),
      A_Wo.reshape(H * DH, D), B_w1.reshape(D // R, R, D), B_w2.reshape(D // R, R, D),
      B_w3.reshape(D // R, R, F),
      B_w4.reshape(F // R, R, D), B_w4)
    return out.reshape(A_x.shape)
```

```python
import functools
import itertools
import os

import jax
import jax.numpy as jnp
from jax import lax
import jax.experimental.pallas as pl
import jax.experimental.pallas.tpu as pltpu

S = 2048
D = 1024
H = 32
DH = 128
MEM = 8
SEG = 32
F = 3584
NSEG = S // SEG
L = MEM + SEG
TOK = 24
P0 = S - TOK * NSEG
RING = 576
XP = (S - P0) // 8
C4 = D // 4
HALO = 32
RB = 256
R = 128
NB = S // (4 * R)
NJ = F // 512
HD = D // 2
W1_AT, W2_AT = 64, 320
W4T = (F - S) // R
E_ = lambda k, d: int(os.environ.get(k, d))
EPS = 1e-5
NEG = -1000000000.0

LAG_QK, LAG_PV, LAG_WO = E_('LQ', 1), E_('LP', 3), E_('LW', 4)
FILL_AT = E_('FA', 17)
UNROLL = 4

bf16 = jnp.bfloat16
f32 = jnp.float32
u32 = jnp.uint32

SEM_X0, SEM_X, SEM_WO, SEM_W1, SEM_W2, SEM_OUT, SEM_W, SEM_W4, SEM_W3 = (
    0, 2, 10, 14, 22, 30, 38, 50, 66)
NSEM = SEM_W3 + 4 * NJ

ENC_A = (((0, 0, 1), (1, 1, 1)), ((1, 0, 1), (1, 1, 1)), ((0, 0, 1),), ((1, 1, 1),),
         ((0, 0, 1), (0, 1, 1)), ((1, 0, 1), (0, 0, -1)), ((0, 1, 1), (1, 1, -1)))
ENC_B = (((0, 0, 1), (1, 1, 1)), ((0, 0, 1),), ((0, 1, 1), (1, 1, -1)),
         ((1, 0, 1), (0, 0, -1)), ((1, 1, 1),), ((0, 0, 1), (0, 1, 1)),
         ((1, 0, 1), (1, 1, 1)))
DEC = (((0, 0, 1), (1, 1, 1)), ((1, 0, 1), (1, 1, -1)), ((0, 1, 1), (1, 1, 1)),
       ((0, 0, 1), (1, 0, 1)), ((0, 1, 1), (0, 0, -1)), ((1, 1, 1),), ((0, 0, 1),))
ORDER = (0, 1, 3, 2, 4, 5, 6)
LAST = {(1, 0): 3, (0, 1): 4, (1, 1): 5, (0, 0): 6}


def _enc(terms, get):
    v = get(*terms[0][:2])
    for i, j, sign in terms[1:]:
        v = v + get(i, j) if sign > 0 else v - get(i, j)
    return v


def _enc2(table, get, emit):
    for g in range(7):
        y = [[_enc(table[g], lambda i1, j1: get(2 * i1 + i0, 2 * j1 + j0))
              for j0 in range(2)] for i0 in range(2)]
        for k in range(7):
            emit(7 * g + k, _enc(table[k], lambda i0, j0: y[i0][j0]))
        yield


def _right_operands(get, dst, first, row):
    b = [[get(i, j).astype(f32) for j in range(2)] for i in range(2)]
    for p in range(7):
        dst[first + p, pl.ds(row, 16), :] = _enc(ENC_B[p], lambda i, j: b[i][j]).astype(bf16)


def _left_operands(halves, dst, rows):
    for p in range(7):
        v = _enc(ENC_A[p], lambda i, j: halves[i][:, HD * j:HD * j + HD])
        for c in range(4):
            dst[4 * p + c, rows, :] = v[:, 128 * c:128 * c + 128].astype(bf16)


def _collect(acc, p, res, emit):
    for i, j, sign in DEC[p]:
        _accumulate(acc, (i, j), res, sign)
        if LAST[i, j] == p:
            emit(i, j, acc.pop((i, j)))
    return res


def _accumulate(c, key, m, sign):
    c[key] = m if key not in c else (c[key] + m if sign > 0 else c[key] - m)


def _dec(get):
    c = {}
    for k in range(7):
        m = get(k)
        for i, j, sign in DEC[k]:
            _accumulate(c, (i, j), m, sign)
    return c


def _pace(ref, lead, row, result):
    n = 32 // ref.dtype.itemsize
    ref[(*lead, pl.ds(pl.multiple_of(row, n), n), pl.ds(0, 128))] = (
        result[-n:, :128].astype(ref.dtype))


def _run(gen):
    for _ in gen:
        pass


def _mult(i, n):
    return i if isinstance(i, int) else pl.multiple_of(i, n)


def _ln(x):
    m = jnp.mean(x, axis=-1, keepdims=True)
    d = x - m
    v = jnp.mean(d * d, axis=-1, keepdims=True)
    return d * lax.rsqrt(v + EPS)


def _gelu(x):
    c = 0.7978845608028654
    hx = 0.5 * x
    return hx + hx * jnp.tanh(x * (c + (c * 0.044715) * (x * x)))


def _unpack(x):
    return pltpu.bitcast(x, bf16)


def _operand(ref, blocks, rows=slice(None)):
    words = ref.bitcast(u32)
    return _unpack(jnp.concatenate([words[b, rows, :] for b in blocks], axis=1))


def _dot(a, b):
    return jnp.dot(a, b, preferred_element_type=f32)


def _rows(ref, rows):
    return jnp.concatenate([ref[0, rows, :], ref[1, rows, :]], axis=1)


def _set_rows(ref, rows, v):
    ref[0, rows, :] = v[:, :HD]
    ref[1, rows, :] = v[:, HD:]


def _kernel(*refs):
    out_hbm, wa, xs, hbuf, w4t, yt, mu0, sems = refs[11:]
    zero = pl.run_scoped(
        functools.partial(_attention_and_mixer, *refs),
        pltpu.VMEM((H * DH // 2, D), u32),
        pltpu.VMEM((8, S + 2 * HALO, 128), f32),
        pltpu.VMEM((28, 2 * TOK, 128), bf16),
        pltpu.VMEM((28, HD, 128), bf16),
        *[pltpu.VMEM((H // 8, RING, DH), f32)] * 8)
    if E_("SKIP_MLP", 0):
        for b in (w4t, yt, wa):
            pltpu.sync_copy(b.at[0, pl.ds(0, 128)], out_hbm.at[pl.ds(0, 128), pl.ds(0, 128)])
        return
    with jax.named_scope('s_mlp'): pl.run_scoped(
        functools.partial(_mlp, zero, out_hbm, wa, xs, hbuf, w4t, yt, sems, mu0),
        *[pltpu.VMEM((49 * NJ + 1, R, 128), bf16)] * 2,
        pltpu.VMEM(mu0.shape, f32),
        pltpu.VMEM((14, R, C4), f32))


def _attention_and_mixer(x_hbm, mem0_ref, wq_hbm, wk_hbm, wv_hbm, wo_hbm, w1_hbm, w2_hbm,
                         w3_hbm, w4_hbm, w4a_hbm, out_hbm, wa, xs, hbuf, w4t, yt, mu0, sems,
                         wo_b, xg, ubuf, w1t, *q_rings):
    def w3_copy(c):
        return pltpu.make_async_copy(
            w3_hbm.at[:, :, pl.ds(_mult(c * 128, 128), 128)], yt.at[pl.ds(8 * c, 8)],
            sems.at[SEM_W3 + c])

    def w4_head_copy(c):
        return pltpu.make_async_copy(
            w4a_hbm.at[pl.ds(0, S), pl.ds(_mult(c * 128, 128), 128)],
            xs.at[c % 2, pl.ds(0, S), pl.ds(_mult(c // 2 * 128, 128), 128)], sems.at[SEM_W4 + c])

    def w4_tail_copy(c):
        return pltpu.make_async_copy(
            w4_hbm.at[pl.ds(S // R, W4T), :, pl.ds(_mult(c * 128, 128), 128)],
            yt.at[pl.ds(32 * NJ + W4T * c, W4T)], sems.at[SEM_W4 + 8 + c])

    def w2_copy(c):
        return pltpu.make_async_copy(
            w2_hbm.at[:, :, pl.ds(_mult(c * 128, 128), 128)], yt.at[pl.ds(W2_AT + 8 * c, 8)],
            sems.at[SEM_W2 + c])

    others = [f(c) for f in (w2_copy, w4_head_copy, w4_tail_copy) for c in range(8)]

    def fetch(i):
        @pl.loop(i, jnp.where(i < 8, i + 1, i))
        def _(c):
            for f in (w2_copy, w4_head_copy, w4_tail_copy):
                f(c).start()

            @pl.when(c < NJ)
            def _():
                for k in range(4):
                    w3_copy(4 * c + k).start()

    zero = pl.run_scoped(
        functools.partial(_attention, x_hbm, mem0_ref, (wq_hbm, wk_hbm, wv_hbm), wo_hbm,
                          w1_hbm, fetch, w4t, yt, wa, xs, hbuf, sems, wo_b, xg, ubuf, w1t, q_rings),
        *[pltpu.VMEM((H // 8, RING, DH), f32)] * 16)
    for c in others:
        c.wait()
    for c in range(4 * NJ):
        w3_copy(c).wait()
    if E_("SKIP_POST", 0): return zero
    with jax.named_scope('s_mix'): pl.run_scoped(
        functools.partial(_mixer, zero, mu0, wa, xs, w4t, hbuf, yt, wo_b, xg, w1t, q_rings),
        pltpu.VMEM((28, HD, 128), bf16),
        pltpu.VMEM((28, P0 // 2 + 2 * TOK + 16, 128), bf16),
        *[pltpu.VMEM((8, P0, 128), bf16)] * 2, *[pltpu.VMEM((RB, D), f32)] * 2,
        *[pltpu.VMEM((RB + 8, D), f32)] * 2)
    return zero


def _attention(x_hbm, mem0_ref, w_hbm, wo_hbm, w1_hbm, fetch,
               w4t, yt, wa, xs, hbuf, sems, wo_b, xg, ubuf, w1t, q_rings, *kv_rings):
    rings = q_rings + kv_rings
    ring = [[rings[m * 8 + h % 8].at[h // 8] for h in range(H)] for m in range(3)]
    q_r, k_r, v_r = ring

    class x_rows:
        def __init__(self, rows, sem):
            self.copies = [
                pltpu.make_async_copy(x_hbm.at[rows, pl.ds(n * HD, HD)], xs.at[n, rows],
                                      sems.at[sem + n]) for n in range(2)]

        def start(self):
            for c in self.copies:
                c.start()

        def wait(self):
            for c in self.copies:
                c.wait()

    x0_copy = x_rows(pl.ds(0, P0), SEM_X0)

    def x_copy(g):
        return x_rows(pl.ds(_mult(P0 + g * 2 * XP, XP), 2 * XP), SEM_X + 2 * g)

    def wo_copy(i):
        rows = pl.ds(_mult(i * 512, 512), 512)
        return pltpu.make_async_copy(wo_hbm.bitcast(u32).at[rows], wo_b.at[rows],
                                     sems.at[SEM_WO + i])

    def w1_copy(c):
        return pltpu.make_async_copy(
            w1_hbm.at[:, :, pl.ds(_mult(c * 128, 128), 128)], yt.at[pl.ds(W1_AT + 8 * c, 8)],
            sems.at[SEM_W1 + c])

    def prologue(*stg):

        def start_chunk(g, m, first=False):
            src = w_hbm[m].bitcast(u32)
            for pair, par in itertools.product(range(4), range(2)):
                pltpu.make_async_copy(
                    src.at[:, 16 * par + 4 * g + pair, :],
                    stg[m].at[pl.ds((2 * pair + par) * HD, HD)],
                    sems.at[SEM_OUT + pair if first else SEM_W + 3 * g + m]).start()

        def wait_chunk(g, m):
            pltpu.make_async_copy(stg[m], stg[m], sems.at[SEM_W + 3 * g + m]).wait()

        def relayout(g, m, pair, i0, n):
            ev, od = (stg[m][pl.ds(_mult((2 * pair + par) * HD + i0, 8), n), :]
                      for par in range(2))
            h = 8 * g + 2 * pair
            words = wa.bitcast(u32)
            words[m * H + h, pl.ds(i0, n), :] = (ev & jnp.uint32(0xFFFF)) | (od << 16)
            words[m * H + h + 1, pl.ds(i0, n), :] = (ev >> 16) | (od & jnp.uint32(0xFFFF0000))

        def weights(g, m, pair):
            h = m * H + 8 * g + 2 * pair
            for t in range(D // 32 + 1):
                if t < D // 32:
                    for k in range(2):
                        relayout(g, m, pair, D // 4 * k + 8 * t, 8)
                if t > 0:
                    r = 16 * (t - 1)
                    _right_operands(lambda k, n: wa[h + n, pl.ds(HD * k + r, 16), :],
                                    w4t, 28 * m + 7 * pair, r)
                yield

        def norm_rows(r0, n):
            xv = _rows(xs, pl.ds(r0, n)).astype(f32)
            _set_rows(hbuf, pl.ds(r0, n), xv)
            return _ln(xv)

        def later_rows(r0):
            for r in range(0, XP, 16):
                xn = norm_rows(pl.multiple_of(r0 + r, 16), 16)
                for c in range(8):
                    xg[c, pl.ds(pl.multiple_of(HALO + r0 + r, 8), 16), :] = (
                        xn[:, 128 * c:128 * c + 128])
                yield

        x0_copy.start()
        start_chunk(0, 0, first=True)
        start_chunk(0, 1)
        start_chunk(0, 2)
        x_copy(0).start()
        zero = jnp.zeros((HALO, 128), f32)
        for c in range(8):
            xg[c, pl.ds(0, HALO), :] = zero
            xg[c, pl.ds(HALO + S, HALO), :] = zero
        with jax.named_scope('wx'): x0_copy.wait()

        @pl.loop(0, P0 // 64)
        def _(i):
            a = [norm_rows(pl.multiple_of(P0 // 2 * k + 32 * i, 32), 32) for k in range(2)]
            for p in range(7):
                v = _enc(ENC_A[p], lambda k, n: a[k][:, HD * n:HD * n + HD])
                for c in range(4):
                    yt[8 * p + 4 * (i // 4) + c, pl.ds(pl.multiple_of(i % 4 * 32, 32), 32), :] = (
                        v[:, 128 * c:128 * c + 128].astype(bf16))

        @pl.loop(0, 4)
        def _(pair):
            both = stg[0].at[pl.ds(pl.multiple_of(pair * D, D), D)]
            pltpu.make_async_copy(both, both, sems.at[SEM_OUT + pair]).wait()
            _run(weights(0, 0, pair))

        def stage(g, m):
            m1 = (m + 1) % 3
            g1 = jnp.minimum(g + (1 if m == 2 else 0), 3)
            if m > 0:
                pl.when(3 * g + m < 11)(functools.partial(wait_chunk, g1, m1))
            if m == 1:
                x_copy(g).wait()

            @pl.when(g < 3)
            def _():
                start_chunk(g + 1, m)
                if m == 1:
                    x_copy(g + 1).start()
            if m == E_('WM', 1):
                wo_copy(g).start()
            if m == 2:
                w1_copy(2 * g).start()
                w1_copy(2 * g + 1).start()
            n = E_("PR", 64)
            acc = {}

            def dot(pair, r, p):
                res = _dot(
                    _operand(yt, [8 * p + 4 * (r // R) + k for k in range(4)],
                             pl.ds(r % R // 2, n // 2)),
                    _operand(w4t, [28 * m + 7 * pair + p], pl.ds(0, HD // 2)))
                for i, j, sign in DEC[p]:
                    _accumulate(acc, (i, j), res, sign)
                    if LAST[i, j] == p:
                        rings[m * 8 + 2 * pair + j][g, pl.ds(P0 // 2 * i + r, n), :] = (
                            acc.pop((i, j)))
                return res

            dots = [functools.partial(dot, pair, r, p) for pair in range(4)
                    for r in range(0, P0 // 2, n) for p in ORDER]
            work = [(itertools.chain(*[weights(g1, m1, pair) for pair in range(4)]),
                     4 * (D // 32 + 1))]
            paced = [(wa, (3 * H,), 16 * (g >> 10))]
            if m == 0:
                early = E_("EA", 49)
                for d in dots[:early]:
                    d()
                dots = dots[early:]
                wait_chunk(g1, m1)
            else:
                work.append((later_rows(P0 + (2 * g + m - 1) * XP), XP // 16))
                paced.append((xg, (0,), 8 * (g >> 10)))
            _interleave(dots, lambda res: [_pace(*p, res) for p in paced], *work,
                        pieces=1 if m else E_("PQ", 2))

        @pl.loop(0, 4)
        def _(g):
            for m in range(3):
                with jax.named_scope(f'st{m}'): stage(g, m)

    if not E_('SKIP_PRO', 0):
     with jax.named_scope('s_pro'): pl.run_scoped(
        prologue,
        pltpu.VMEM((8 * D // 2, DH), u32),
        pltpu.VMEM((8 * D // 2, DH), u32),
        pltpu.VMEM((8 * D // 2, DH), u32),
    )
    for i in range(4):
        if E_('WM', 1) > 2: wo_copy(i).start()
        with jax.named_scope('wwo'): wo_copy(i).wait()
    for c in range(8):
        w1_copy(c).wait()

    @pl.loop(0, 16)
    def _(i):
        c, q = i >> 2, i & 3
        for r in range(0, 128, 16):
            _right_operands(lambda k, n: yt[W1_AT + 16 * c + 8 * n + 4 * k + q, pl.ds(r, 16), :],
                            w1t, 7 * c, pl.multiple_of(128 * q + r, 16))

    def wrap(r):
        return jnp.where(r >= RING, r - RING, r)

    group = UNROLL * TOK

    def step(i, k, mem, tok, rp, ra, rw):
        ri = lax.broadcasted_iota(jnp.int32, (2 * L, 2 * L), 0)
        ci = lax.broadcasted_iota(jnp.int32, (2 * L, 2 * L), 1)
        same = (ri >= L) == (ci >= L)
        ri, ci = (jnp.where(v >= L, v - L, v) for v in (ri, ci))
        mask = same & ((ri < MEM) | (ri >= ci))
        fill = jnp.where(same, NEG, -jnp.inf)

        lhs = jnp.concatenate([mem, tok], axis=0).astype(bf16)
        rps = [pl.multiple_of(wrap(rp + r // SEG * SEG), SEG) + r % SEG
               for r in range(TOK * k, TOK * (k + 1), 8)]
        ra_ = pl.multiple_of(wrap(ra + SEG * k), SEG)
        rw_ = pl.multiple_of(rw, SEG) + TOK * k

        rb = pl.multiple_of(jnp.maximum(i - 1, 0) * group, SEG)
        if k == 0:
            _left_operands([_ln(_ln(_rows(hbuf, pl.ds(rb + group // 2 * q, group // 2))))
                            for q in range(2)], ubuf, slice(None))
        filled = {}

        def filler(products):
            def emit(q, j, v):
                xg[2 * k + j, pl.ds(HALO + rb + group // 2 * q, group // 2), :] = _gelu(v)

            for p in products:
                _collect(filled, p, _dot(_operand(ubuf, range(4 * p, 4 * p + 4)),
                                         _operand(w1t, [7 * k + p])), emit)

        mem_qkv = {}
        scores = {}
        o_mem = {}
        total = [None]

        def qkv(h):
            res = {}
            for m in ((0, 1, 2), (1, 0, 2), (2, 0, 1), (2, 1, 0))[E_('MO', 0)]:
                r = _dot(lhs, _operand(wa, [m * H + h]))
                for q in range(3):
                    ring[m][h][pl.ds(rps[q], 8), :] = r[8 + 8 * q:16 + 8 * q]
                res[m] = r[:MEM]
            mem_qkv[h] = res

        def both(m, a):
            return jnp.concatenate(
                [v for h in (2 * a, 2 * a + 1)
                 for v in (mem_qkv[h][m], ring[m][h][pl.ds(ra_, SEG), :])],
                axis=0).astype(bf16)

        def qk(a):
            scores[a] = lax.dot_general(both(0, a), both(1, a), (((1,), (1,)), ((), ())),
                                        preferred_element_type=f32)

        def pv(a):
            sc = jnp.where(mask, scores.pop(a) * (DH ** -0.5), fill)
            mx = jnp.max(sc, axis=1, keepdims=True)
            e = jnp.exp(sc - mx)
            den = jnp.sum(e, axis=1, keepdims=True)
            inv = pl.reciprocal(den, approx=True)
            inv = inv * (2.0 - den * inv)
            o = _dot(e.astype(bf16), both(2, a)) * inv
            for q, h in enumerate((2 * a, 2 * a + 1)):
                q_r[h][pl.ds(ra_, SEG), :] = o[q * L + MEM:(q + 1) * L]
                o_mem[h] = o[q * L:q * L + MEM]

        def wo(h):
            lo = jnp.concatenate([o_mem.pop(h), q_r[h][pl.ds(rw_, TOK), :]],
                                 axis=0).astype(bf16)
            r = _dot(lo, _unpack(wo_b[pl.ds(h * DH // 2, DH // 2), :]))
            total[0] = r if total[0] is None else total[0] + r

        npair = H // 2
        for t in range(npair + LAG_WO):
            heads = (2 * t, 2 * t + 1) if t < npair else ()
            late = (2 * (t - LAG_WO), 2 * (t - LAG_WO) + 1) if t >= LAG_WO else ()
            cuts = [0, E_('FS', 2), E_('FS', 2) + E_('F2', 0)]
            for op in os.environ.get("SEQ", "abqpfcd"):
                if op in "ab" and heads: qkv(heads[op == "b"])
                if op in "cd" and late: wo(late[op == "d"])
                if op == "q" and 0 <= t - LAG_QK < npair: qk(t - LAG_QK)
                if op == "p" and 0 <= t - LAG_PV < npair: pv(t - LAG_PV)
                if op == "f" and 0 <= t - FILL_AT < 2: filler(ORDER[cuts[t - FILL_AT]:cuts[t - FILL_AT + 1]])
        filler(ORDER[cuts[2]:])

        a = total[0]
        rows = pl.ds(pl.multiple_of(group * i, SEG) + TOK * k, TOK)
        _set_rows(hbuf, rows, _rows(hbuf, rows) + a[MEM:])
        return a[:MEM]

    def steps(i, carry):
        mem, rp, ra, rw = carry
        fetch(i)
        r0 = pl.multiple_of(HALO + P0 + group * i, SEG)
        toks = [jnp.concatenate([xg[c, pl.ds(r0 + TOK * k, TOK), :] for c in range(8)], axis=1)
                for k in range(UNROLL)]
        for k in range(UNROLL):
            mem = step(i, k, mem, toks[k], rp, ra, rw)
        return mem, wrap(rp + group), wrap(ra + UNROLL * SEG), wrap(rw + group)

    if E_('SKIP_LOOP', 0): return lax.fori_loop(0, 64, lambda i, c: wrap(c + TOK), jnp.int32(0)) - TOK * NSEG % RING
    with jax.named_scope('s_loop'): carry = lax.fori_loop(
        0, NSEG // UNROLL, steps,
        (mem0_ref[...].astype(f32), jnp.int32(P0), jnp.int32(0), jnp.int32(0)))
    return carry[3] - TOK * NSEG % RING


def _interleave(dots, pace, *work, pieces=8):
    for i, dot in enumerate(dots):
        res = dot()
        k = min(pieces, res.shape[0] // 16)
        for j in range(k):
            pace(res[:res.shape[0] // 16 * (j + 1) // k * 16])
            for gen, n in work:
                for _ in range(n * (i * k + j) // (k * len(dots)),
                               n * (i * k + j + 1) // (k * len(dots))):
                    next(gen)
    for gen, _ in work:
        _run(gen)


def _up_dot(yt, wa, mu, b, j, half, p):
    res = _dot(
        _operand(yt, [98 * b + 2 * p, 98 * b + 2 * p + 1], pl.ds(half * R // 4, R // 4)),
        _operand(wa, [13 * j + p // 4], pl.ds(128 * (p % 4), 128)))
    mu[p, pl.ds(0, R // 2), :] = res
    return res


def _mixer(zero, mu0, wa, xs, w4t, hbuf, yt, wo_b, xg, w1t, q_rings, w2t, ulast, lhs0, lhs1, hs0, hs1, *ybuf):
    lhs, hs = (lhs0, lhs1), (hs0, hs1)

    def encode_w3(g):
        for j, t in itertools.product(range(NJ), range(4)):
            def get(k, n):
                return yt[32 * j + 8 * n + 2 * k + (g >> 1),
                          pl.ds(pl.multiple_of(64 * (g & 1) + 16 * t, 16), 16), :].astype(f32)

            def emit(p, v):
                wa[13 * j + p // 4, pl.ds(pl.multiple_of(C4 * (p % 4) + 64 * g + 16 * t, 16), 16),
                   :] = v.astype(bf16)

            yield from _enc2(ENC_B, get, emit)

    def encode_w4(g):
        c = g >> 1
        for j, t in itertools.product(range(NJ), range(4)):
            r = pl.multiple_of(64 * (g & 1) + 16 * t, 16)

            def get(k, n):
                if 512 * j < S:
                    return xs[c, pl.ds(512 * j + 128 * k + r, 16), pl.ds(128 * n, 128)].astype(f32)
                return yt[32 * NJ + W4T * (2 * n + c) + 4 * j - S // R + k,
                          pl.ds(r, 16), :].astype(f32)

            def emit(p, v):
                w4t[2 * p + c, pl.ds(128 * j + r, 16), :] = v.astype(bf16)

            yield from _enc2(ENC_B, get, emit)

    def encode_w2(g):
        for t, c in itertools.product(range(8), range(4)):
            _right_operands(
                lambda k, n: yt[W2_AT + 8 * (4 * n + c) + 4 * k + g, pl.ds(16 * t, 16), :],
                w2t, 7 * c, pl.multiple_of(128 * g + 16 * t, 16))
            yield

    done = TOK * NSEG
    first = 4 * TOK * (NSEG // 4 - 1)

    @jax.named_scope('q1')
    def q1(g):
        n = 128
        for k, q in enumerate(q_rings):
            for r in range(0, P0, 64):
                lhs0[k, pl.ds(r, 64), :] = q[g, pl.ds((done + r) % RING, 64), :].astype(bf16)

        part = []

        def dot(r, c, k):
            w = wo_b[pl.ds(pl.multiple_of((2 * g + k) * 2 * DH, 2 * DH), 2 * DH),
                     pl.ds(128 * c, 128)]
            res = _dot(_operand(lhs0, range(4 * k, 4 * k + 4), pl.ds(r // 2, n // 2)), _unpack(w))
            if k == 0:
                part.append(res)
            else:
                hbuf[c // 4, pl.ds(done + r, n), pl.ds(128 * (c % 4), 128)] += part.pop() + res
            return res

        _interleave(
            [functools.partial(dot, r, c, k)
             for r in range(0, P0, n) for c in range(8) for k in range(2)],
            lambda res: [_pace(yt, (98 * NB,), zero, res), _pace(xs, (0,), S + zero, res)],
            (encode_w2(g), 32),
            (encode_w4(g), 28 * NJ), (encode_w3(g), 28 * NJ), pieces=8)

    pl.loop(0, H // 8)(q1)

    half = (S - first) // 2

    def mixer_norm(r0, n):
        for r in range(r0, r0 + n, 16):
            _left_operands([_ln(_ln(_rows(hbuf, pl.ds(first + half * i + r, 16))))
                            for i in range(2)], ulast, pl.ds(r, 16))
            yield

    def mixer_in(c):
        step = E_("IR", 64)
        for r in range(0, half, step):
            n = min(step, half - r)
            acc = {}

            def emit(i, j, v):
                xg[2 * c + j, pl.ds(HALO + first + half * i + r, n), :] = _gelu(v)

            for p in ORDER:
                _collect(acc, p, _dot(
                    _operand(ulast, range(4 * p, 4 * p + 4), pl.ds(r // 2, n // 2)),
                    _operand(w1t, [7 * c + p])), emit)

    def shift(i, dst):
        for r, c in itertools.product(range(0, RB // 2, 16), range(4)):
            a = [[xg[4 * k + c, pl.ds(HALO + (-1, 1, -2, 2)[2 * k + c // 2]
                                      + i * RB + RB // 2 * q + r, 16), :]
                  for k in range(2)] for q in range(2)]
            for p in range(7):
                dst[p, pl.ds(RB // 2 * c + r, 16), :] = _enc(
                    ENC_A[p], lambda q, k: a[q][k]).astype(bf16)
            yield

    def mixer_out(src, dst):
        n = 128
        acc = {}

        def dot(r, c, p):
            words = src.bitcast(u32)
            a = jnp.concatenate([words[p, pl.ds((RB // 2 * k + r) // 2, n // 2), :]
                                 for k in range(4)], axis=1)
            res = _dot(_unpack(a), _operand(w2t, [7 * c + p]))
            for i, j, sign in DEC[p]:
                _accumulate(acc, (i, j), res, sign)
                if LAST[i, j] == p:
                    dst[pl.ds(RB // 2 * i + r, n), pl.ds(HD * j + 128 * c, 128)] = acc.pop((i, j))
            return res

        return [functools.partial(dot, r, c, p)
                for r in range(0, RB // 2, n) for c in range(4) for p in ORDER]

    def residual(i, src, dst):
        late = []
        for t in range(0, RB, 8):
            rows = pl.ds(_mult(i * RB + t, 8), 8)
            hv = _rows(hbuf, rows)
            x1 = _ln(hv) + src[pl.ds(t, 8), :]
            late.append((rows, hv + x1, t, _ln(x1)))
            if len(late) > E_("LT", 2) or t == RB - 8:
                for rows, v, t0, y in late[:None if t == RB - 8 else 1]:
                    _set_rows(hbuf, rows, v)
                    dst[pl.ds(t0, 8), :] = y
                del late[0]
            yield

    def up_operands(i, src):
        per = 4 * R // RB
        for t, c in itertools.product(range(0, RB, 64), range(2)):
            def emit(p, v):
                yt[98 * (i // per) + 2 * p + c,
                   pl.ds(_mult(i % per * (RB // 4) + t // 4, 16), 16), :] = v.astype(bf16)

            yield from _enc2(ENC_A, lambda q, k: src[
                pl.ds(t + 16 * q, 16), pl.ds(C4 * k + 128 * c, 128)], emit)

    def job(i, par, extra=None):
        work, paced = [], []
        if not isinstance(i, int) or i + 1 < S // RB:
            work.append((shift(i + 1, lhs[1 - par]), RB // 8))
            paced.append((lhs[1 - par], (7,), zero))
        if extra is None:
            work.append((up_operands(i - 2, ybuf[par]), 14 * RB // 64))
            paced.append((yt, (98 * NB,), zero))
        else:
            work.append((mixer_norm(*extra), extra[1] // 16))
            paced.append((ulast, (0,), half + zero))
        if extra is None or i > 0:
            work.append((residual(i - 1, hs[1 - par], ybuf[1 - par]), RB // 8))
            paced.append((ybuf[1 - par], (), RB + zero))
        (pl.loop(zero, 1) if par in [int(c) for c in os.environ.get('BB', '01')] else lambda f: f(0))(lambda _: _interleave(
            mixer_out(lhs[par], hs[par]), lambda res: [_pace(*p, res) for p in paced], *work,
            pieces=8))

    cut = E_('CUT', 240)
    _run(shift(0, lhs[0]))
    with jax.named_scope('j01'):
        job(0, 0, (0, cut))
        job(1, 1, (cut, half - cut))
    with jax.named_scope('in'): pl.loop(0, 4)(mixer_in)

    with jax.named_scope('jobs'):
        if E_("JL", 1):
            @pl.loop(1, 3)
            def _(i):
                job(2 * i, 0)
                job(2 * i + 1, 1)
        for i in range(2 + 4 * E_("JL", 1), S // RB):
            job(i, i % 2)

    last = S // RB - 1
    _interleave(
        [functools.partial(_up_dot, yt, wa, mu0, 0, 0, 0, p) for p in range(49)],
        lambda res: [_pace(y, (), RB + zero, res) for y in ybuf],
        (up_operands(last - 1, ybuf[0]), 14 * RB // 64),
        (residual(last, hs[1], ybuf[1]), RB // 8), pieces=1)
    _run(up_operands(last, ybuf[1]))


def _mlp(zero, out_hbm, wa, xs, hbuf, w4t, yt, sems, mu0, tt0, tt1, mu1, md):
    tts, mu = (tt0, tt1), (mu0, mu1)
    hr = R // 2
    lag = E_("LAG", 15)

    def out_copy(b, n):
        rows = pl.ds(_mult(b * 4 * R, 4 * R), 4 * R)
        return pltpu.make_async_copy(xs.at[n, rows], out_hbm.at[rows, pl.ds(n * HD, HD)],
                                     sems.at[SEM_OUT + 2 * b + n])

    def up_dot(b, j, half, p):
        return _up_dot(yt, wa, mu[half], b, j, half, p)

    def up_sums(act):
        for half, t in itertools.product(range(2), range(hr // 8)):
            c = {}
            for g in ORDER:
                y = _dec(lambda k: mu[half][7 * g + k, pl.ds(8 * t, 8), :])
                for i1, n1, sign in DEC[g]:
                    for (i0, n0), m in y.items():
                        key = (2 * i1 + i0, 2 * n1 + n0)
                        _accumulate(c, key, m, sign)
                        if LAST[i1, n1] == g:
                            act[half, t, key] = _gelu(c.pop(key))
                yield

    def down_operands(act, tt, j):
        for half, t in itertools.product(range(2), range(hr // 16)):
            def emit(p, v):
                tt[NJ * p + j, pl.ds(half * hr + 16 * t, 16), :] = v.astype(bf16)

            yield from _enc2(ENC_A, lambda q, k: jnp.concatenate(
                [act[half, 2 * t, (q, k)], act[half, 2 * t + 1, (q, k)]], axis=0), emit)

    n_sums = 7 * 2 * (hr // 8)

    def up_vector_work(tt, j):
        act = {}
        a, b = up_sums(act), down_operands(act, tt, j)
        for i in range(n_sums + lag):
            if i < n_sums:
                next(a)
            if i >= lag and (i - lag) % 2 == 1:
                next(b)
            yield

    part = []

    def down_dot(tt, g, slot, i, lo, hi):
        p = 7 * g + i // 2
        res = _dot(_operand(tt, [NJ * p + q for q in range(lo, hi)]),
                   _operand(w4t, [14 * g + i], pl.ds(64 * lo, 64 * (hi - lo))))
        if hi < NJ:
            part.append(res)
        else:
            md[7 * slot + i // 2, :, pl.ds(128 * (i % 2), 128)] = part.pop() + res if lo else res
        return res

    def down_block(slot, t):
        c = _dec(lambda k: md[7 * slot + k, pl.ds(16 * t, 16), :])
        return jnp.concatenate(
            [jnp.concatenate([c[i0, 0], c[i0, 1]], axis=1) for i0 in range(2)], axis=0)

    def down_sums(b, g, slot):
        dst = []
        for w in range(2):
            i1 = n1 = sign = 0
            for q in range(7):
                e = DEC[q][w] if w < len(DEC[q]) else DEC[q][0][:2] + (0,)
                i1, n1, sign = (jnp.where(g == q, new, old)
                                for new, old in zip(e, (i1, n1, sign)))
            dst.append((b * 4 * R + 32 * i1, n1, sign.astype(f32)))
        for t in range(R // 16):
            m = down_block(slot, t)
            rows = [pl.ds(pl.multiple_of(d[0] + 64 * t, 32), 32) for d in dst]
            new = [hbuf[dst[0][1], rows[0], :] + m,
                   hbuf[dst[1][1], rows[1], :] + dst[1][2] * m]
            for w in (1, 0):
                hbuf[dst[w][1], rows[w], :] = new[w]
                xs[dst[w][1], rows[w], :] = new[w].astype(bf16)
            yield

    def step(b, par, up, down, j):
        slot = (7 * b + j) & 1
        dots = []
        if up:
            nb = jnp.minimum(b + (j + 1) // NJ, NB - 1)
            nj = jnp.where(j == NJ - 1, 0, j + 1)
            dots = ([(1, functools.partial(up_dot, b, j, 1, p)) for p in range(49)]
                    + [(1, functools.partial(up_dot, nb, nj, 0, p)) for p in range(49)])
            up_work = up_vector_work(tts[par], j)
        if down:
            cuts = (0, E_("KS", 4), NJ) if E_("KS", 4) and up else (0, NJ)
            for i in reversed(range(14)):
                dots[7 * i + E_('D0', 6):7 * i + E_('D0', 6)] = [
                    (hi - lo, functools.partial(down_dot, tts[1 - par], j, slot, i, lo, hi))
                    for lo, hi in zip(cuts, cuts[1:])]
            down_work = down_sums(jnp.maximum(b - 1 - (j == 0), 0),
                                  jnp.where(j == 0, 6, j - 1), 1 - slot)
        total = sum(w for w, _ in dots)
        pos = n_up = done_up = done_down = 0
        for w, dot in dots:
            if down:
                goal = (pos + E_('AD', 14)) * (R // 16) * 100 // (E_("DE", 105) * total)
                for _ in range(done_down, goal):
                    next(down_work, None)
                done_down = max(done_down, goal)
            res = dot()
            k = min(w, E_('PD', 3))
            for i in range(k * up):
                if E_('PM', 1) and (w > 1 or n_up % E_('PM', 1) == 0):
                    _pace(mu[done_up >= n_sums // 2], (49,), zero, res[:res.shape[0] * (i + 1) // k])
                if E_('PN', 1) and (w > 1 or n_up % E_('PN', 1) == 0):
                    _pace(tts[par], (49 * NJ,), zero, res[:res.shape[0] * (i + 1) // k])
                goal = (pos * k + w * (i + 1) + E_('AH', 4) * k) * (n_sums + lag) // (total * k)
                goal = (min(goal, n_sums // 2) if n_up + (w == 1) < 49
                        else max(goal, n_sums // 2))
                for _ in range(done_up, goal):
                    next(up_work, None)
                done_up = max(done_up, goal)
            pos += w
            n_up += w == 1
        if up:
            _run(up_work)
        if down:
            _run(down_work)
        if down:
            @pl.when((j == 0) & (b > 1))
            def _():
                for n in range(2):
                    out_copy(b - 2, n).start()

    md[pl.ds(0, 7)] = jnp.zeros((7, R, C4), f32)
    with jax.named_scope('b0'): pl.loop(0, NJ)(functools.partial(step, 0, 0, True, False))

    @pl.loop(0, NB // 2)
    @jax.named_scope('bmid')
    def _(i):
        pl.loop(0, NJ)(functools.partial(step, 2 * i + 1, 1, True, True))
        pl.loop(0, jnp.where(2 * i + 2 < NB, NJ, 0))(
            functools.partial(step, 2 * i + 2, 0, True, True))

    with jax.named_scope('b4'): pl.loop(0, NJ)(functools.partial(step, NB, 0, False, True))
    out_copy(NB - 1, 1).start()
    pieces = []
    for t in range(R // 16):
        rows = pl.ds(S - 4 * R + 64 * t, 32)
        xs[0, rows, :] = (hbuf[0, rows, :] + down_block((7 * NB + 6) & 1, t)).astype(bf16)
        if t % 2:
            rows = pl.ds(S - 4 * R + 64 * (t - 1), 128)
            pieces.append(pltpu.make_async_copy(
                xs.at[0, rows], out_hbm.at[rows, pl.ds(0, HD)], sems.at[t // 2]))
            pieces[-1].start()
    for b, n in itertools.product(range(NB), range(2)):
        if (b, n) != (NB - 1, 0):
            out_copy(b, n).wait()
    for c in pieces:
        c.wait()


@jax.jit
def pallas_sequential_preLN__memory_aug_recurrent_mem_tr__mixer_s_mlp__prompt_kernel(
    A_x: jax.Array,
    A_mem0: jax.Array,
    A_Wq: jax.Array,
    A_Wk: jax.Array,
    A_Wv: jax.Array,
    A_Wo: jax.Array,
    A_seg_len: jax.Array,
    B_x: jax.Array,
    B_w1: jax.Array,
    B_w2: jax.Array,
    B_w3: jax.Array,
    B_w4: jax.Array,
):
    del A_seg_len, B_x
    hbm = pl.BlockSpec(memory_space=pl.ANY)
    vmem = pl.BlockSpec(memory_space=pltpu.VMEM)
    scratch = [
        pltpu.VMEM((3 * H + 1, D, DH), bf16),
        pltpu.VMEM((2, S + 32, HD), bf16),
        pltpu.VMEM((2, S, HD), f32),
        pltpu.VMEM((98, F // 4, 128), bf16),
        pltpu.VMEM((98 * NB + 1, R, 128), bf16),
        pltpu.VMEM((52, R // 2 + 8, 128), f32),
        pltpu.SemaphoreType.DMA((NSEM,)),
    ]
    out = pl.pallas_call(
        _kernel,
        out_shape=jax.ShapeDtypeStruct((S, D), A_x.dtype),
        in_specs=[hbm, vmem] + [hbm] * 9,
        out_specs=hbm,
        scratch_shapes=scratch,
        compiler_params=pltpu.CompilerParams(vmem_limit_bytes=127 * 1024 * 1024, flags={k: True for k in os.environ.get('FL', 'XLA_TPU_EVENLY_DISTRIBUTE_CRITICAL_NODES').split(',') if k}),
    )(A_x.reshape(S, D), A_mem0.reshape(MEM, D),
      A_Wq.reshape(D // 2, 2 * H, DH), A_Wk.reshape(D // 2, 2 * H, DH),
      A_Wv.reshape(D // 2, 2 * H, DH),
      A_Wo.reshape(H * DH, D), B_w1.reshape(D // R, R, D), B_w2.reshape(D // R, R, D),
      B_w3.reshape(D // R, R, F),
      B_w4.reshape(F // R, R, D), B_w4)
    return out.reshape(A_x.shape)
```

```python
import functools
import itertools

import jax
import jax.numpy as jnp
from jax import lax
import jax.experimental.pallas as pl
import jax.experimental.pallas.tpu as pltpu

S = 2048
D = 1024
H = 32
DH = 128
MEM = 8
SEG = 32
F = 3584
NSEG = S // SEG
L = MEM + SEG
TOK = 24
P0 = S - TOK * NSEG
RING = 576
XP = (S - P0) // 4
C4 = D // 4
HALO = 32
RB = 256
R = 128
NB = S // (4 * R)
NJ = F // 512
HD = D // 2
W1_AT, W2_AT = 64, 320
W4T = (F - S) // R
EPS = 1e-5
NEG = -1000000000.0

LAG_QK, LAG_PV, LAG_WO = 1, 3, 4
FILL_AT = 17
UNROLL = 4

bf16 = jnp.bfloat16
f32 = jnp.float32
u32 = jnp.uint32

SEM_X0, SEM_X, SEM_WO, SEM_W1, SEM_W2, SEM_OUT, SEM_W, SEM_W4, SEM_W3 = (
    0, 2, 10, 14, 22, 30, 38, 50, 66)
NSEM = SEM_W3 + 4 * NJ

ENC_A = (((0, 0, 1), (1, 1, 1)), ((1, 0, 1), (1, 1, 1)), ((0, 0, 1),), ((1, 1, 1),),
         ((0, 0, 1), (0, 1, 1)), ((1, 0, 1), (0, 0, -1)), ((0, 1, 1), (1, 1, -1)))
ENC_B = (((0, 0, 1), (1, 1, 1)), ((0, 0, 1),), ((0, 1, 1), (1, 1, -1)),
         ((1, 0, 1), (0, 0, -1)), ((1, 1, 1),), ((0, 0, 1), (0, 1, 1)),
         ((1, 0, 1), (1, 1, 1)))
DEC = (((0, 0, 1), (1, 1, 1)), ((1, 0, 1), (1, 1, -1)), ((0, 1, 1), (1, 1, 1)),
       ((0, 0, 1), (1, 0, 1)), ((0, 1, 1), (0, 0, -1)), ((1, 1, 1),), ((0, 0, 1),))
ORDER = (0, 1, 3, 2, 4, 5, 6)
LAST = {(1, 0): 3, (0, 1): 4, (1, 1): 5, (0, 0): 6}


def _enc(terms, get):
    v = get(*terms[0][:2])
    for i, j, sign in terms[1:]:
        v = v + get(i, j) if sign > 0 else v - get(i, j)
    return v


def _enc2(table, get, emit):
    for g in range(7):
        y = [[_enc(table[g], lambda i1, j1: get(2 * i1 + i0, 2 * j1 + j0))
              for j0 in range(2)] for i0 in range(2)]
        for k in range(7):
            emit(7 * g + k, _enc(table[k], lambda i0, j0: y[i0][j0]))
        yield


def _right_operands(get, dst, first, row):
    b = [[get(i, j).astype(f32) for j in range(2)] for i in range(2)]
    for p in range(7):
        dst[first + p, pl.ds(row, 16), :] = _enc(ENC_B[p], lambda i, j: b[i][j]).astype(bf16)


def _left_operands(halves, dst, rows):
    for p in range(7):
        v = _enc(ENC_A[p], lambda i, j: halves[i][:, HD * j:HD * j + HD])
        for c in range(4):
            dst[4 * p + c, rows, :] = v[:, 128 * c:128 * c + 128].astype(bf16)


def _collect(acc, p, res, emit):
    for i, j, sign in DEC[p]:
        _accumulate(acc, (i, j), res, sign)
        if LAST[i, j] == p:
            emit(i, j, acc.pop((i, j)))
    return res


def _accumulate(c, key, m, sign):
    c[key] = m if key not in c else (c[key] + m if sign > 0 else c[key] - m)


def _dec(get):
    c = {}
    for k in range(7):
        m = get(k)
        for i, j, sign in DEC[k]:
            _accumulate(c, (i, j), m, sign)
    return c


def _pace(ref, lead, row, result):
    n = 32 // ref.dtype.itemsize
    ref[(*lead, pl.ds(pl.multiple_of(row, n), n), pl.ds(0, 128))] = (
        result[-n:, :128].astype(ref.dtype))


def _run(gen):
    for _ in gen:
        pass


def _mult(i, n):
    return i if isinstance(i, int) else pl.multiple_of(i, n)


def _ln(x):
    m = jnp.mean(x, axis=-1, keepdims=True)
    d = x - m
    v = jnp.mean(d * d, axis=-1, keepdims=True)
    return d * lax.rsqrt(v + EPS)


def _gelu(x):
    c = 0.7978845608028654
    hx = 0.5 * x
    return hx + hx * jnp.tanh(x * (c + (c * 0.044715) * (x * x)))


def _unpack(x):
    return pltpu.bitcast(x, bf16)


def _operand(ref, blocks, rows=slice(None)):
    words = ref.bitcast(u32)
    return _unpack(jnp.concatenate([words[b, rows, :] for b in blocks], axis=1))


def _dot(a, b):
    return jnp.dot(a, b, preferred_element_type=f32)


def _rows(ref, rows):
    return jnp.concatenate([ref[0, rows, :], ref[1, rows, :]], axis=1)


def _set_rows(ref, rows, v):
    ref[0, rows, :] = v[:, :HD]
    ref[1, rows, :] = v[:, HD:]


def _kernel(*refs):
    out_hbm, wa, xs, hbuf, w4t, yt, mu0, sems = refs[11:]
    zero = pl.run_scoped(
        functools.partial(_attention_and_mixer, *refs),
        pltpu.VMEM((H * DH // 2, D), u32),
        pltpu.VMEM((8, S + 2 * HALO, 128), f32),
        pltpu.VMEM((28, 2 * TOK, 128), bf16),
        pltpu.VMEM((28, HD, 128), bf16),
        *[pltpu.VMEM((H // 8, RING, DH), f32)] * 8)
    pl.run_scoped(
        functools.partial(_mlp, zero, out_hbm, wa, xs, hbuf, w4t, yt, sems, mu0),
        *[pltpu.VMEM((49 * NJ + 1, R, 128), bf16)] * 2,
        pltpu.VMEM(mu0.shape, f32),
        pltpu.VMEM((14, R, C4), f32))


def _attention_and_mixer(x_hbm, mem0_ref, wq_hbm, wk_hbm, wv_hbm, wo_hbm, w1_hbm, w2_hbm,
                         w3_hbm, w4_hbm, w4a_hbm, out_hbm, wa, xs, hbuf, w4t, yt, mu0, sems,
                         wo_b, xg, ubuf, w1t, *q_rings):
    def w3_copy(c):
        return pltpu.make_async_copy(
            w3_hbm.at[:, :, pl.ds(_mult(c * 128, 128), 128)], yt.at[pl.ds(8 * c, 8)],
            sems.at[SEM_W3 + c])

    def w4_head_copy(c):
        return pltpu.make_async_copy(
            w4a_hbm.at[pl.ds(0, S), pl.ds(_mult(c * 128, 128), 128)],
            xs.at[c % 2, pl.ds(0, S), pl.ds(_mult(c // 2 * 128, 128), 128)], sems.at[SEM_W4 + c])

    def w4_tail_copy(c):
        return pltpu.make_async_copy(
            w4_hbm.at[pl.ds(S // R, W4T), :, pl.ds(_mult(c * 128, 128), 128)],
            yt.at[pl.ds(32 * NJ + W4T * c, W4T)], sems.at[SEM_W4 + 8 + c])

    def w2_copy(c):
        return pltpu.make_async_copy(
            w2_hbm.at[:, :, pl.ds(_mult(c * 128, 128), 128)], yt.at[pl.ds(W2_AT + 8 * c, 8)],
            sems.at[SEM_W2 + c])

    others = [f(c) for f in (w2_copy, w4_head_copy, w4_tail_copy) for c in range(8)]

    def fetch(i):
        @pl.loop(i, jnp.where(i < 8, i + 1, i))
        def _(c):
            for f in (w2_copy, w4_head_copy, w4_tail_copy):
                f(c).start()

            @pl.when(c < NJ)
            def _():
                for k in range(4):
                    w3_copy(4 * c + k).start()

    zero = pl.run_scoped(
        functools.partial(_attention, x_hbm, mem0_ref, (wq_hbm, wk_hbm, wv_hbm), wo_hbm,
                          w1_hbm, fetch, w4t, yt, wa, xs, hbuf, sems, wo_b, xg, ubuf, w1t, q_rings),
        *[pltpu.VMEM((H // 8, RING, DH), f32)] * 16)
    for c in others:
        c.wait()
    for c in range(4 * NJ):
        w3_copy(c).wait()
    pl.run_scoped(
        functools.partial(_mixer, zero, mu0, wa, xs, w4t, hbuf, yt, wo_b, xg, w1t, q_rings),
        pltpu.VMEM((28, HD, 128), bf16),
        pltpu.VMEM((28, P0 // 2 + 2 * TOK + 16, 128), bf16),
        *[pltpu.VMEM((8, P0, 128), bf16)] * 2, *[pltpu.VMEM((RB, D), f32)] * 2,
        *[pltpu.VMEM((RB + 8, D), f32)] * 2)
    return zero


def _attention(x_hbm, mem0_ref, w_hbm, wo_hbm, w1_hbm, fetch,
               w4t, yt, wa, xs, hbuf, sems, wo_b, xg, ubuf, w1t, q_rings, *kv_rings):
    rings = q_rings + kv_rings
    ring = [[rings[m * 8 + h % 8].at[h // 8] for h in range(H)] for m in range(3)]
    q_r, k_r, v_r = ring

    class x_rows:
        def __init__(self, rows, sem):
            self.copies = [
                pltpu.make_async_copy(x_hbm.at[rows, pl.ds(n * HD, HD)], xs.at[n, rows],
                                      sems.at[sem + n]) for n in range(2)]

        def start(self):
            for c in self.copies:
                c.start()

        def wait(self):
            for c in self.copies:
                c.wait()

    x0_copy = x_rows(pl.ds(0, P0), SEM_X0)

    def x_copy(g):
        return x_rows(pl.ds(_mult(P0 + g * XP, 128), XP), SEM_X + 2 * g)

    def wo_copy(i):
        rows = pl.ds(_mult(i * 512, 512), 512)
        return pltpu.make_async_copy(wo_hbm.bitcast(u32).at[rows], wo_b.at[rows],
                                     sems.at[SEM_WO + i])

    def w1_copy(c):
        return pltpu.make_async_copy(
            w1_hbm.at[:, :, pl.ds(_mult(c * 128, 128), 128)], yt.at[pl.ds(W1_AT + 8 * c, 8)],
            sems.at[SEM_W1 + c])

    def prologue(*stg):

        def start_chunk(g, m, first=False):
            src = w_hbm[m].bitcast(u32)
            for pair, par in itertools.product(range(4), range(2)):
                pltpu.make_async_copy(
                    src.at[:, 16 * par + 4 * g + pair, :],
                    stg[m].at[pl.ds((2 * pair + par) * HD, HD)],
                    sems.at[SEM_OUT + pair if first else SEM_W + 3 * g + m]).start()

        def wait_chunk(g, m):
            pltpu.make_async_copy(stg[m], stg[m], sems.at[SEM_W + 3 * g + m]).wait()

        def relayout(g, m, pair, i0, n):
            ev, od = (stg[m][pl.ds(_mult((2 * pair + par) * HD + i0, 8), n), :]
                      for par in range(2))
            h = 8 * g + 2 * pair
            words = wa.bitcast(u32)
            words[m * H + h, pl.ds(i0, n), :] = (ev & jnp.uint32(0xFFFF)) | (od << 16)
            words[m * H + h + 1, pl.ds(i0, n), :] = (ev >> 16) | (od & jnp.uint32(0xFFFF0000))

        def weights(g, m, pair):
            h = m * H + 8 * g + 2 * pair
            for t in range(D // 32 + 1):
                if t < D // 32:
                    for k in range(2):
                        relayout(g, m, pair, D // 4 * k + 8 * t, 8)
                if t > 0:
                    r = 16 * (t - 1)
                    _right_operands(lambda k, n: wa[h + n, pl.ds(HD * k + r, 16), :],
                                    w4t, 28 * m + 7 * pair, r)
                yield

        def norm_rows(r0, n):
            xv = _rows(xs, pl.ds(r0, n)).astype(f32)
            _set_rows(hbuf, pl.ds(r0, n), xv)
            return _ln(xv)

        def later_rows(r0):
            for r in range(0, XP, 16):
                xn = norm_rows(pl.multiple_of(r0 + r, 16), 16)
                for c in range(8):
                    xg[c, pl.ds(pl.multiple_of(HALO + r0 + r, 8), 16), :] = (
                        xn[:, 128 * c:128 * c + 128])
                yield

        x0_copy.start()
        start_chunk(0, 0, first=True)
        start_chunk(0, 1)
        start_chunk(0, 2)
        x_copy(0).start()
        zero = jnp.zeros((HALO, 128), f32)
        for c in range(8):
            xg[c, pl.ds(0, HALO), :] = zero
            xg[c, pl.ds(HALO + S, HALO), :] = zero
        x0_copy.wait()

        @pl.loop(0, P0 // 64)
        def _(i):
            a = [norm_rows(pl.multiple_of(P0 // 2 * k + 32 * i, 32), 32) for k in range(2)]
            for p in range(7):
                v = _enc(ENC_A[p], lambda k, n: a[k][:, HD * n:HD * n + HD])
                for c in range(4):
                    yt[8 * p + 4 * (i // 4) + c, pl.ds(pl.multiple_of(i % 4 * 32, 32), 32), :] = (
                        v[:, 128 * c:128 * c + 128].astype(bf16))

        @pl.loop(0, 4)
        def _(pair):
            both = stg[0].at[pl.ds(pl.multiple_of(pair * D, D), D)]
            pltpu.make_async_copy(both, both, sems.at[SEM_OUT + pair]).wait()
            _run(weights(0, 0, pair))

        def stage(g, m):
            m1 = (m + 1) % 3
            g1 = jnp.minimum(g + (1 if m == 2 else 0), 3)
            if m == 2:
                x_copy(g).wait()

            @pl.when(g < 3)
            def _():
                start_chunk(g + 1, m)
                if m == 2:
                    x_copy(g + 1).start()
            if m == 1:
                pl.when(g > 0)(lambda: wo_copy(g).start())

            @pl.when(g == 3)
            def _():
                if m == 0:
                    wo_copy(0).start()
                if m == 1:
                    for c in range(8):
                        w1_copy(c).start()
            n = 64
            acc = {}

            def dot(pair, r, p):
                res = _dot(
                    _operand(yt, [8 * p + 4 * (r // R) + k for k in range(4)],
                             pl.ds(r % R // 2, n // 2)),
                    _operand(w4t, [28 * m + 7 * pair + p], pl.ds(0, HD // 2)))

                def emit(i, j, v):
                    rings[m * 8 + 2 * pair + j][g, pl.ds(P0 // 2 * i + r, n), :] = v

                return _collect(acc, p, res, emit)

            dots = [functools.partial(dot, pair, r, p) for pair in range(4)
                    for r in range(0, P0 // 2, n) for p in ORDER]
            early = 72
            if m == 2:
                _interleave(dots[:early], functools.partial(_pace, xg, (0,), 8 * (g >> 10)),
                            (later_rows(P0 + g * XP), XP // 16), pieces=4)
            else:
                for d in dots[:early]:
                    d()
            pl.when(3 * g + m < 11)(functools.partial(wait_chunk, g1, m1))
            _interleave(dots[early:], functools.partial(_pace, wa, (3 * H,), 16 * (g >> 10)),
                        (itertools.chain(*[weights(g1, m1, pair) for pair in range(4)]),
                         4 * (D // 32 + 1)), pieces=4)

        @pl.loop(0, 4)
        def _(g):
            for m in range(3):
                stage(g, m)

    pl.run_scoped(
        prologue,
        pltpu.VMEM((8 * D // 2, DH), u32),
        pltpu.VMEM((8 * D // 2, DH), u32),
        pltpu.VMEM((8 * D // 2, DH), u32),
    )
    for i in range(4):
        wo_copy(i).wait()
    for c in range(8):
        w1_copy(c).wait()

    @pl.loop(0, 16)
    def _(i):
        c, q = i >> 2, i & 3
        for r in range(0, 128, 16):
            _right_operands(lambda k, n: yt[W1_AT + 16 * c + 8 * n + 4 * k + q, pl.ds(r, 16), :],
                            w1t, 7 * c, pl.multiple_of(128 * q + r, 16))

    def wrap(r):
        return jnp.where(r >= RING, r - RING, r)

    group = UNROLL * TOK

    def step(i, k, mem, tok, rp, ra, rw):
        ri = lax.broadcasted_iota(jnp.int32, (2 * L, 2 * L), 0)
        ci = lax.broadcasted_iota(jnp.int32, (2 * L, 2 * L), 1)
        same = (ri >= L) == (ci >= L)
        ri, ci = (jnp.where(v >= L, v - L, v) for v in (ri, ci))
        mask = same & ((ri < MEM) | (ri >= ci))
        fill = jnp.where(same, NEG, -jnp.inf)

        lhs = jnp.concatenate([mem, tok], axis=0).astype(bf16)
        rps = [pl.multiple_of(wrap(rp + r // SEG * SEG), SEG) + r % SEG
               for r in range(TOK * k, TOK * (k + 1), 8)]
        ra_ = pl.multiple_of(wrap(ra + SEG * k), SEG)
        rw_ = pl.multiple_of(rw, SEG) + TOK * k

        rb = pl.multiple_of(jnp.maximum(i - 1, 0) * group, SEG)
        if k == 0:
            _left_operands([_ln(_ln(_rows(hbuf, pl.ds(rb + group // 2 * q, group // 2))))
                            for q in range(2)], ubuf, slice(None))
        filled = {}

        def filler(products):
            def emit(q, j, v):
                xg[2 * k + j, pl.ds(HALO + rb + group // 2 * q, group // 2), :] = _gelu(v)

            for p in products:
                _collect(filled, p, _dot(_operand(ubuf, range(4 * p, 4 * p + 4)),
                                         _operand(w1t, [7 * k + p])), emit)

        mem_qkv = {}
        scores = {}
        o_mem = {}
        total = [None]

        def qkv(h):
            res = {}
            for m in range(3):
                r = _dot(lhs, _operand(wa, [m * H + h]))
                for q in range(3):
                    ring[m][h][pl.ds(rps[q], 8), :] = r[8 + 8 * q:16 + 8 * q]
                res[m] = r[:MEM]
            mem_qkv[h] = res

        def both(m, a):
            return jnp.concatenate(
                [v for h in (2 * a, 2 * a + 1)
                 for v in (mem_qkv[h][m], ring[m][h][pl.ds(ra_, SEG), :])],
                axis=0).astype(bf16)

        def qk(a):
            scores[a] = lax.dot_general(both(0, a), both(1, a), (((1,), (1,)), ((), ())),
                                        preferred_element_type=f32)

        def pv(a):
            sc = jnp.where(mask, scores.pop(a) * (DH ** -0.5), fill)
            mx = jnp.max(sc, axis=1, keepdims=True)
            e = jnp.exp(sc - mx)
            den = jnp.sum(e, axis=1, keepdims=True)
            inv = pl.reciprocal(den, approx=True)
            inv = inv * (2.0 - den * inv)
            o = _dot(e.astype(bf16), both(2, a)) * inv
            for q, h in enumerate((2 * a, 2 * a + 1)):
                q_r[h][pl.ds(ra_, SEG), :] = o[q * L + MEM:(q + 1) * L]
                o_mem[h] = o[q * L:q * L + MEM]

        def wo(h):
            lo = jnp.concatenate([o_mem.pop(h), q_r[h][pl.ds(rw_, TOK), :]],
                                 axis=0).astype(bf16)
            r = _dot(lo, _unpack(wo_b[pl.ds(h * DH // 2, DH // 2), :]))
            total[0] = r if total[0] is None else total[0] + r

        npair = H // 2
        for t in range(npair + LAG_WO):
            if t < npair:
                qkv(2 * t)
                qkv(2 * t + 1)
            if 0 <= t - LAG_QK < npair:
                qk(t - LAG_QK)
            if 0 <= t - LAG_PV < npair:
                pv(t - LAG_PV)
            if t == FILL_AT:
                filler(ORDER[:1])
            if t >= LAG_WO:
                wo(2 * (t - LAG_WO))
                wo(2 * (t - LAG_WO) + 1)
        filler(ORDER[1:])

        a = total[0]
        rows = pl.ds(pl.multiple_of(group * i, SEG) + TOK * k, TOK)
        _set_rows(hbuf, rows, _rows(hbuf, rows) + a[MEM:])
        return a[:MEM]

    def steps(i, carry):
        mem, rp, ra, rw = carry
        fetch(i)
        r0 = pl.multiple_of(HALO + P0 + group * i, SEG)
        toks = [jnp.concatenate([xg[c, pl.ds(r0 + TOK * k, TOK), :] for c in range(8)], axis=1)
                for k in range(UNROLL)]
        for k in range(UNROLL):
            mem = step(i, k, mem, toks[k], rp, ra, rw)
        return mem, wrap(rp + group), wrap(ra + UNROLL * SEG), wrap(rw + group)

    carry = lax.fori_loop(
        0, NSEG // UNROLL, steps,
        (mem0_ref[...].astype(f32), jnp.int32(P0), jnp.int32(0), jnp.int32(0)))
    return carry[3] - TOK * NSEG % RING


def _interleave(dots, pace, *work, pieces=8):
    for i, dot in enumerate(dots):
        res = dot()
        k = min(pieces, res.shape[0] // 16)
        for j in range(k):
            pace(res[:res.shape[0] // 16 * (j + 1) // k * 16])
            for gen, n in work:
                for _ in range(n * (i * k + j) // (k * len(dots)),
                               n * (i * k + j + 1) // (k * len(dots))):
                    next(gen)
    for gen, _ in work:
        _run(gen)


def _up_dot(yt, wa, mu, b, j, half, p):
    res = _dot(
        _operand(yt, [98 * b + 2 * p, 98 * b + 2 * p + 1], pl.ds(half * R // 4, R // 4)),
        _operand(wa, [13 * j + p // 4], pl.ds(128 * (p % 4), 128)))
    mu[p, pl.ds(0, R // 2), :] = res
    return res


def _mixer(zero, mu0, wa, xs, w4t, hbuf, yt, wo_b, xg, w1t, q_rings, w2t, ulast, lhs0, lhs1, hs0, hs1, *ybuf):
    lhs, hs = (lhs0, lhs1), (hs0, hs1)

    def encode_w3(g):
        for j, t in itertools.product(range(NJ), range(4)):
            def get(k, n):
                return yt[32 * j + 8 * n + 2 * k + (g >> 1),
                          pl.ds(pl.multiple_of(64 * (g & 1) + 16 * t, 16), 16), :].astype(f32)

            def emit(p, v):
                wa[13 * j + p // 4, pl.ds(pl.multiple_of(C4 * (p % 4) + 64 * g + 16 * t, 16), 16),
                   :] = v.astype(bf16)

            yield from _enc2(ENC_B, get, emit)

    def encode_w4(g):
        c = g >> 1
        for j, t in itertools.product(range(NJ), range(4)):
            r = pl.multiple_of(64 * (g & 1) + 16 * t, 16)

            def get(k, n):
                if 512 * j < S:
                    return xs[c, pl.ds(512 * j + 128 * k + r, 16), pl.ds(128 * n, 128)].astype(f32)
                return yt[32 * NJ + W4T * (2 * n + c) + 4 * j - S // R + k,
                          pl.ds(r, 16), :].astype(f32)

            def emit(p, v):
                w4t[2 * p + c, pl.ds(128 * j + r, 16), :] = v.astype(bf16)

            yield from _enc2(ENC_B, get, emit)

    def encode_w2(g):
        for t, c in itertools.product(range(8), range(4)):
            _right_operands(
                lambda k, n: yt[W2_AT + 8 * (4 * n + c) + 4 * k + g, pl.ds(16 * t, 16), :],
                w2t, 7 * c, pl.multiple_of(128 * g + 16 * t, 16))
            yield

    done = TOK * NSEG
    first = 4 * TOK * (NSEG // 4 - 1)

    def last_wo(g):
        n = 128
        for k, q in enumerate(q_rings):
            for r in range(0, P0, 64):
                lhs0[k, pl.ds(r, 64), :] = q[g, pl.ds((done + r) % RING, 64), :].astype(bf16)

        part = []

        def dot(r, c, k):
            w = wo_b[pl.ds(pl.multiple_of((2 * g + k) * 2 * DH, 2 * DH), 2 * DH),
                     pl.ds(128 * c, 128)]
            res = _dot(_operand(lhs0, range(4 * k, 4 * k + 4), pl.ds(r // 2, n // 2)), _unpack(w))
            if k == 0:
                part.append(res)
            else:
                hbuf[c // 4, pl.ds(done + r, n), pl.ds(128 * (c % 4), 128)] += part.pop() + res
            return res

        _interleave(
            [functools.partial(dot, r, c, k)
             for r in range(0, P0, n) for c in range(8) for k in range(2)],
            lambda res: [_pace(yt, (98 * NB,), zero, res), _pace(xs, (0,), S + zero, res)],
            (encode_w2(g), 32),
            (encode_w4(g), 28 * NJ), (encode_w3(g), 28 * NJ), pieces=8)

    pl.loop(0, H // 8)(last_wo)

    half = (S - first) // 2

    def mixer_norm(r0, n):
        for r in range(r0, r0 + n, 16):
            _left_operands([_ln(_ln(_rows(hbuf, pl.ds(first + half * i + r, 16))))
                            for i in range(2)], ulast, pl.ds(r, 16))
            yield

    def mixer_in(c):
        step = 64
        for r in range(0, half, step):
            n = min(step, half - r)
            acc = {}

            def emit(i, j, v):
                xg[2 * c + j, pl.ds(HALO + first + half * i + r, n), :] = _gelu(v)

            for p in ORDER:
                _collect(acc, p, _dot(
                    _operand(ulast, range(4 * p, 4 * p + 4), pl.ds(r // 2, n // 2)),
                    _operand(w1t, [7 * c + p])), emit)

    def shift(i, dst):
        for r, c in itertools.product(range(0, RB // 2, 16), range(4)):
            a = [[xg[4 * k + c, pl.ds(HALO + (-1, 1, -2, 2)[2 * k + c // 2]
                                      + i * RB + RB // 2 * q + r, 16), :]
                  for k in range(2)] for q in range(2)]
            for p in range(7):
                dst[p, pl.ds(RB // 2 * c + r, 16), :] = _enc(
                    ENC_A[p], lambda q, k: a[q][k]).astype(bf16)
            yield

    def mixer_out(src, dst):
        n = 128
        acc = {}

        def dot(r, c, p):
            words = src.bitcast(u32)
            a = jnp.concatenate([words[p, pl.ds((RB // 2 * k + r) // 2, n // 2), :]
                                 for k in range(4)], axis=1)
            res = _dot(_unpack(a), _operand(w2t, [7 * c + p]))

            def emit(i, j, v):
                dst[pl.ds(RB // 2 * i + r, n), pl.ds(HD * j + 128 * c, 128)] = v

            return _collect(acc, p, res, emit)

        return [functools.partial(dot, r, c, p)
                for r in range(0, RB // 2, n) for c in range(4) for p in ORDER]

    def residual(i, src, dst):
        late = []
        for t in range(0, RB, 8):
            rows = pl.ds(_mult(i * RB + t, 8), 8)
            hv = _rows(hbuf, rows)
            x1 = _ln(hv) + src[pl.ds(t, 8), :]
            late.append((rows, hv + x1, t, _ln(x1)))
            if len(late) > 2 or t == RB - 8:
                for rows, v, t0, y in late[:None if t == RB - 8 else 1]:
                    _set_rows(hbuf, rows, v)
                    dst[pl.ds(t0, 8), :] = y
                del late[0]
            yield

    def up_operands(i, src):
        per = 4 * R // RB
        for t, c in itertools.product(range(0, RB, 64), range(2)):
            def emit(p, v):
                yt[98 * (i // per) + 2 * p + c,
                   pl.ds(_mult(i % per * (RB // 4) + t // 4, 16), 16), :] = v.astype(bf16)

            yield from _enc2(ENC_A, lambda q, k: src[
                pl.ds(t + 16 * q, 16), pl.ds(C4 * k + 128 * c, 128)], emit)

    def job(i, par, extra=None):
        work, paced = [], []
        if not isinstance(i, int) or i + 1 < S // RB:
            work.append((shift(i + 1, lhs[1 - par]), RB // 8))
            paced.append((lhs[1 - par], (7,), zero))
        if extra is None:
            work.append((up_operands(i - 2, ybuf[par]), 14 * RB // 64))
            paced.append((yt, (98 * NB,), zero))
        else:
            work.append((mixer_norm(*extra), extra[1] // 16))
            paced.append((ulast, (0,), half + zero))
        if extra is None or i > 0:
            work.append((residual(i - 1, hs[1 - par], ybuf[1 - par]), RB // 8))
            paced.append((ybuf[1 - par], (), RB + zero))
        pl.loop(zero, 1)(lambda _: _interleave(
            mixer_out(lhs[par], hs[par]), lambda res: [_pace(*p, res) for p in paced], *work,
            pieces=8))

    cut = 240
    _run(shift(0, lhs[0]))
    job(0, 0, (0, cut))
    job(1, 1, (cut, half - cut))
    pl.loop(0, 4)(mixer_in)

    @pl.loop(1, 3)
    def _(i):
        job(2 * i, 0)
        job(2 * i + 1, 1)

    job(6, 0)
    job(7, 1)
    last = S // RB - 1
    _interleave(
        [functools.partial(_up_dot, yt, wa, mu0, 0, 0, 0, p) for p in range(49)],
        lambda res: [_pace(y, (), RB + zero, res) for y in ybuf],
        (up_operands(last - 1, ybuf[0]), 14 * RB // 64),
        (residual(last, hs[1], ybuf[1]), RB // 8), pieces=4)
    _run(up_operands(last, ybuf[1]))


def _mlp(zero, out_hbm, wa, xs, hbuf, w4t, yt, sems, mu0, tt0, tt1, mu1, md):
    tts, mu = (tt0, tt1), (mu0, mu1)
    hr = R // 2
    lag = 15

    def out_copy(b, n):
        rows = pl.ds(_mult(b * 4 * R, 4 * R), 4 * R)
        return pltpu.make_async_copy(xs.at[n, rows], out_hbm.at[rows, pl.ds(n * HD, HD)],
                                     sems.at[SEM_OUT + 2 * b + n])

    def up_dot(b, j, half, p):
        return _up_dot(yt, wa, mu[half], b, j, half, p)

    def up_sums(act):
        for half, t in itertools.product(range(2), range(hr // 8)):
            c = {}
            for g in ORDER:
                y = _dec(lambda k: mu[half][7 * g + k, pl.ds(8 * t, 8), :])
                for i1, n1, sign in DEC[g]:
                    for (i0, n0), m in y.items():
                        key = (2 * i1 + i0, 2 * n1 + n0)
                        _accumulate(c, key, m, sign)
                        if LAST[i1, n1] == g:
                            act[half, t, key] = _gelu(c.pop(key))
                yield

    def down_operands(act, tt, j):
        for half, t in itertools.product(range(2), range(hr // 16)):
            def emit(p, v):
                tt[NJ * p + j, pl.ds(half * hr + 16 * t, 16), :] = v.astype(bf16)

            yield from _enc2(ENC_A, lambda q, k: jnp.concatenate(
                [act[half, 2 * t, (q, k)], act[half, 2 * t + 1, (q, k)]], axis=0), emit)

    n_sums = 7 * 2 * (hr // 8)

    def up_vector_work(tt, j):
        act = {}
        a, b = up_sums(act), down_operands(act, tt, j)
        for i in range(n_sums + lag):
            if i < n_sums:
                next(a)
            if i >= lag and (i - lag) % 2 == 1:
                next(b)
            yield

    part = []

    def down_dot(tt, g, slot, i, lo, hi):
        p = 7 * g + i // 2
        res = _dot(_operand(tt, [NJ * p + q for q in range(lo, hi)]),
                   _operand(w4t, [14 * g + i], pl.ds(64 * lo, 64 * (hi - lo))))
        if hi < NJ:
            part.append(res)
        else:
            md[7 * slot + i // 2, :, pl.ds(128 * (i % 2), 128)] = part.pop() + res if lo else res
        return res

    def down_block(slot, t):
        c = _dec(lambda k: md[7 * slot + k, pl.ds(16 * t, 16), :])
        return jnp.concatenate(
            [jnp.concatenate([c[i0, 0], c[i0, 1]], axis=1) for i0 in range(2)], axis=0)

    def down_sums(b, g, slot):
        dst = []
        for w in range(2):
            i1 = n1 = sign = 0
            for q in range(7):
                e = DEC[q][w] if w < len(DEC[q]) else DEC[q][0][:2] + (0,)
                i1, n1, sign = (jnp.where(g == q, new, old)
                                for new, old in zip(e, (i1, n1, sign)))
            dst.append((b * 4 * R + 32 * i1, n1, sign.astype(f32)))
        for t in range(R // 16):
            m = down_block(slot, t)
            rows = [pl.ds(pl.multiple_of(d[0] + 64 * t, 32), 32) for d in dst]
            new = [hbuf[dst[0][1], rows[0], :] + m,
                   hbuf[dst[1][1], rows[1], :] + dst[1][2] * m]
            for w in (1, 0):
                hbuf[dst[w][1], rows[w], :] = new[w]
                xs[dst[w][1], rows[w], :] = new[w].astype(bf16)
            yield

    def step(b, par, up, down, j):
        slot = (7 * b + j) & 1
        dots = []
        if up:
            nb = jnp.minimum(b + (j + 1) // NJ, NB - 1)
            nj = jnp.where(j == NJ - 1, 0, j + 1)
            dots = ([(1, functools.partial(up_dot, b, j, 1, p)) for p in range(49)]
                    + [(1, functools.partial(up_dot, nb, nj, 0, p)) for p in range(49)])
            up_work = up_vector_work(tts[par], j)
        if down:
            cuts = (0, 4, NJ) if up else (0, NJ)
            for i in reversed(range(14)):
                dots[7 * i + 6:7 * i + 6] = [
                    (hi - lo, functools.partial(down_dot, tts[1 - par], j, slot, i, lo, hi))
                    for lo, hi in zip(cuts, cuts[1:])]
            down_work = down_sums(jnp.maximum(b - 1 - (j == 0), 0),
                                  jnp.where(j == 0, 6, j - 1), 1 - slot)
        total = sum(w for w, _ in dots)
        pos = n_up = done_up = done_down = 0
        for w, dot in dots:
            if down:
                goal = (pos + 14) * (R // 16) * 100 // (105 * total)
                for _ in range(done_down, goal):
                    next(down_work, None)
                done_down = max(done_down, goal)
            res = dot()
            k = min(w, 3)
            for i in range(k * up):
                piece = res[:res.shape[0] * (i + 1) // k]
                _pace(mu[done_up >= n_sums // 2], (49,), zero, piece)
                _pace(tts[par], (49 * NJ,), zero, piece)
                goal = (pos * k + w * (i + 1) + 4 * k) * (n_sums + lag) // (total * k)
                goal = (min(goal, n_sums // 2) if n_up + (w == 1) < 49
                        else max(goal, n_sums // 2))
                for _ in range(done_up, goal):
                    next(up_work, None)
                done_up = max(done_up, goal)
            pos += w
            n_up += w == 1
        if up:
            _run(up_work)
        if down:
            _run(down_work)
        if down:
            @pl.when((j == 0) & (b > 1))
            def _():
                for n in range(2):
                    out_copy(b - 2, n).start()

    md[pl.ds(0, 7)] = jnp.zeros((7, R, C4), f32)
    pl.loop(0, NJ)(functools.partial(step, 0, 0, True, False))

    @pl.loop(0, NB // 2)
    def _(i):
        pl.loop(0, NJ)(functools.partial(step, 2 * i + 1, 1, True, True))
        pl.loop(0, jnp.where(2 * i + 2 < NB, NJ, 0))(
            functools.partial(step, 2 * i + 2, 0, True, True))

    pl.loop(0, NJ)(functools.partial(step, NB, 0, False, True))
    out_copy(NB - 1, 1).start()
    pieces = []
    for t in range(R // 16):
        rows = pl.ds(S - 4 * R + 64 * t, 32)
        xs[0, rows, :] = (hbuf[0, rows, :] + down_block((7 * NB + 6) & 1, t)).astype(bf16)
        if t % 2:
            rows = pl.ds(S - 4 * R + 64 * (t - 1), 128)
            pieces.append(pltpu.make_async_copy(
                xs.at[0, rows], out_hbm.at[rows, pl.ds(0, HD)], sems.at[t // 2]))
            pieces[-1].start()
    for b, n in itertools.product(range(NB), range(2)):
        if (b, n) != (NB - 1, 0):
            out_copy(b, n).wait()
    for c in pieces:
        c.wait()


@jax.jit
def pallas_sequential_preLN__memory_aug_recurrent_mem_tr__mixer_s_mlp__prompt_kernel(
    A_x: jax.Array,
    A_mem0: jax.Array,
    A_Wq: jax.Array,
    A_Wk: jax.Array,
    A_Wv: jax.Array,
    A_Wo: jax.Array,
    A_seg_len: jax.Array,
    B_x: jax.Array,
    B_w1: jax.Array,
    B_w2: jax.Array,
    B_w3: jax.Array,
    B_w4: jax.Array,
):
    del A_seg_len, B_x
    hbm = pl.BlockSpec(memory_space=pl.ANY)
    vmem = pl.BlockSpec(memory_space=pltpu.VMEM)
    scratch = [
        pltpu.VMEM((3 * H + 1, D, DH), bf16),
        pltpu.VMEM((2, S + 32, HD), bf16),
        pltpu.VMEM((2, S, HD), f32),
        pltpu.VMEM((98, F // 4, 128), bf16),
        pltpu.VMEM((98 * NB + 1, R, 128), bf16),
        pltpu.VMEM((52, R // 2 + 8, 128), f32),
        pltpu.SemaphoreType.DMA((NSEM,)),
    ]
    out = pl.pallas_call(
        _kernel,
        out_shape=jax.ShapeDtypeStruct((S, D), A_x.dtype),
        in_specs=[hbm, vmem] + [hbm] * 9,
        out_specs=hbm,
        scratch_shapes=scratch,
        compiler_params=pltpu.CompilerParams(
            vmem_limit_bytes=127 * 1024 * 1024,
            flags={"XLA_TPU_EVENLY_DISTRIBUTE_CRITICAL_NODES": True}),
    )(A_x.reshape(S, D), A_mem0.reshape(MEM, D),
      A_Wq.reshape(D // 2, 2 * H, DH), A_Wk.reshape(D // 2, 2 * H, DH),
      A_Wv.reshape(D // 2, 2 * H, DH),
      A_Wo.reshape(H * DH, D), B_w1.reshape(D // R, R, D), B_w2.reshape(D // R, R, D),
      B_w3.reshape(D // R, R, F),
      B_w4.reshape(F // R, R, D), B_w4)
    return out.reshape(A_x.shape)
```

```python
import functools
import itertools

import jax
import jax.numpy as jnp
from jax import lax
import jax.experimental.pallas as pl
import jax.experimental.pallas.tpu as pltpu

S = 2048
D = 1024
H = 32
DH = 128
MEM = 8
SEG = 32
F = 3584
NSEG = S // SEG
L = MEM + SEG
TOK = 24
P0 = S - TOK * NSEG
RING = 576
XP = (S - P0) // 4
C4 = D // 4
HALO = 32
RB = 256
R = 128
NB = S // (4 * R)
NJ = F // 512
HD = D // 2
W1_AT, W2_AT = 64, 320
W4T = (F - S) // R
EPS = 1e-5
NEG = -1000000000.0

LAG_QK, LAG_PV, LAG_WO = 1, 3, 4
FILL_AT = 17
UNROLL = 4

bf16 = jnp.bfloat16
f32 = jnp.float32
u32 = jnp.uint32

SEM_X0, SEM_X, SEM_WO, SEM_W1, SEM_W2, SEM_OUT, SEM_W, SEM_W4, SEM_W3 = (
    0, 2, 10, 14, 22, 30, 38, 50, 66)
NSEM = SEM_W3 + 4 * NJ

ENC_A = (((0, 0, 1), (1, 1, 1)), ((1, 0, 1), (1, 1, 1)), ((0, 0, 1),), ((1, 1, 1),),
         ((0, 0, 1), (0, 1, 1)), ((1, 0, 1), (0, 0, -1)), ((0, 1, 1), (1, 1, -1)))
ENC_B = (((0, 0, 1), (1, 1, 1)), ((0, 0, 1),), ((0, 1, 1), (1, 1, -1)),
         ((1, 0, 1), (0, 0, -1)), ((1, 1, 1),), ((0, 0, 1), (0, 1, 1)),
         ((1, 0, 1), (1, 1, 1)))
DEC = (((0, 0, 1), (1, 1, 1)), ((1, 0, 1), (1, 1, -1)), ((0, 1, 1), (1, 1, 1)),
       ((0, 0, 1), (1, 0, 1)), ((0, 1, 1), (0, 0, -1)), ((1, 1, 1),), ((0, 0, 1),))
ORDER = (0, 1, 3, 2, 4, 5, 6)
LAST = {(1, 0): 3, (0, 1): 4, (1, 1): 5, (0, 0): 6}


def _enc(terms, get):
    v = get(*terms[0][:2])
    for i, j, sign in terms[1:]:
        v = v + get(i, j) if sign > 0 else v - get(i, j)
    return v


def _enc2(table, get, emit):
    for g in range(7):
        y = [[_enc(table[g], lambda i1, j1: get(2 * i1 + i0, 2 * j1 + j0))
              for j0 in range(2)] for i0 in range(2)]
        for k in range(7):
            emit(7 * g + k, _enc(table[k], lambda i0, j0: y[i0][j0]))
        yield


def _right_operands(get, dst, first, row):
    b = [[get(i, j).astype(f32) for j in range(2)] for i in range(2)]
    for p in range(7):
        dst[first + p, pl.ds(row, 16), :] = _enc(ENC_B[p], lambda i, j: b[i][j]).astype(bf16)


def _left_operands(halves, dst, rows):
    for p in range(7):
        v = _enc(ENC_A[p], lambda i, j: halves[i][:, HD * j:HD * j + HD])
        for c in range(4):
            dst[4 * p + c, rows, :] = v[:, 128 * c:128 * c + 128].astype(bf16)


def _collect(acc, p, res, emit):
    for i, j, sign in DEC[p]:
        _accumulate(acc, (i, j), res, sign)
        if LAST[i, j] == p:
            emit(i, j, acc.pop((i, j)))
    return res


def _accumulate(c, key, m, sign):
    c[key] = m if key not in c else (c[key] + m if sign > 0 else c[key] - m)


def _dec(get):
    c = {}
    for k in range(7):
        m = get(k)
        for i, j, sign in DEC[k]:
            _accumulate(c, (i, j), m, sign)
    return c


def _pace(ref, lead, row, result):
    n = 32 // ref.dtype.itemsize
    ref[(*lead, pl.ds(pl.multiple_of(row, n), n), pl.ds(0, 128))] = (
        result[-n:, :128].astype(ref.dtype))


def _run(gen):
    for _ in gen:
        pass


def _mult(i, n):
    return i if isinstance(i, int) else pl.multiple_of(i, n)


def _ln(x):
    m = jnp.mean(x, axis=-1, keepdims=True)
    d = x - m
    v = jnp.mean(d * d, axis=-1, keepdims=True)
    return d * lax.rsqrt(v + EPS)


def _gelu(x):
    c = 0.7978845608028654
    hx = 0.5 * x
    return hx + hx * jnp.tanh(x * (c + (c * 0.044715) * (x * x)))


def _unpack(x):
    return pltpu.bitcast(x, bf16)


def _operand(ref, blocks, rows=slice(None)):
    words = ref.bitcast(u32)
    return _unpack(jnp.concatenate([words[b, rows, :] for b in blocks], axis=1))


def _dot(a, b):
    return jnp.dot(a, b, preferred_element_type=f32)


def _rows(ref, rows):
    return jnp.concatenate([ref[0, rows, :], ref[1, rows, :]], axis=1)


def _set_rows(ref, rows, v):
    ref[0, rows, :] = v[:, :HD]
    ref[1, rows, :] = v[:, HD:]


def _kernel(*refs):
    out_hbm, wa, xs, hbuf, w4t, yt, mu0, sems = refs[11:]
    zero = pl.run_scoped(
        functools.partial(_attention_and_mixer, *refs),
        pltpu.VMEM((H * DH // 2, D), u32),
        pltpu.VMEM((8, S + 2 * HALO, 128), f32),
        pltpu.VMEM((28, 2 * TOK, 128), bf16),
        pltpu.VMEM((28, HD, 128), bf16),
        *[pltpu.VMEM((H // 8, RING, DH), f32)] * 8)
    pl.run_scoped(
        functools.partial(_mlp, zero, out_hbm, wa, xs, hbuf, w4t, yt, sems, mu0),
        *[pltpu.VMEM((49 * NJ + 1, R, 128), bf16)] * 2,
        pltpu.VMEM(mu0.shape, f32),
        pltpu.VMEM((14, R, C4), f32))


def _attention_and_mixer(x_hbm, mem0_ref, wq_hbm, wk_hbm, wv_hbm, wo_hbm, w1_hbm, w2_hbm,
                         w3_hbm, w4_hbm, w4a_hbm, out_hbm, wa, xs, hbuf, w4t, yt, mu0, sems,
                         wo_b, xg, ubuf, w1t, *q_rings):
    def w3_copy(c):
        return pltpu.make_async_copy(
            w3_hbm.at[:, :, pl.ds(_mult(c * 128, 128), 128)], yt.at[pl.ds(8 * c, 8)],
            sems.at[SEM_W3 + c])

    def w4_head_copy(c):
        return pltpu.make_async_copy(
            w4a_hbm.at[pl.ds(0, S), pl.ds(_mult(c * 128, 128), 128)],
            xs.at[c % 2, pl.ds(0, S), pl.ds(_mult(c // 2 * 128, 128), 128)], sems.at[SEM_W4 + c])

    def w4_tail_copy(c):
        return pltpu.make_async_copy(
            w4_hbm.at[pl.ds(S // R, W4T), :, pl.ds(_mult(c * 128, 128), 128)],
            yt.at[pl.ds(32 * NJ + W4T * c, W4T)], sems.at[SEM_W4 + 8 + c])

    def w2_copy(c):
        return pltpu.make_async_copy(
            w2_hbm.at[:, :, pl.ds(_mult(c * 128, 128), 128)], yt.at[pl.ds(W2_AT + 8 * c, 8)],
            sems.at[SEM_W2 + c])

    others = [f(c) for f in (w2_copy, w4_head_copy, w4_tail_copy) for c in range(8)]

    def fetch(i):
        @pl.loop(i, jnp.where(i < 8, i + 1, i))
        def _(c):
            for f in (w2_copy, w4_head_copy, w4_tail_copy):
                f(c).start()

            @pl.when(c < NJ)
            def _():
                for k in range(4):
                    w3_copy(4 * c + k).start()

    zero = pl.run_scoped(
        functools.partial(_attention, x_hbm, mem0_ref, (wq_hbm, wk_hbm, wv_hbm), wo_hbm,
                          w1_hbm, fetch, w4t, yt, wa, xs, hbuf, sems, wo_b, xg, ubuf, w1t, q_rings),
        *[pltpu.VMEM((H // 8, RING, DH), f32)] * 16)
    for c in others:
        c.wait()
    for c in range(4 * NJ):
        w3_copy(c).wait()
    pl.run_scoped(
        functools.partial(_mixer, zero, mu0, wa, xs, w4t, hbuf, yt, wo_b, xg, w1t, q_rings),
        pltpu.VMEM((28, HD, 128), bf16),
        pltpu.VMEM((28, P0 // 2 + 2 * TOK + 16, 128), bf16),
        *[pltpu.VMEM((8, P0, 128), bf16)] * 2, *[pltpu.VMEM((RB, D), f32)] * 2,
        *[pltpu.VMEM((RB + 8, D), f32)] * 2)
    return zero


def _attention(x_hbm, mem0_ref, w_hbm, wo_hbm, w1_hbm, fetch,
               w4t, yt, wa, xs, hbuf, sems, wo_b, xg, ubuf, w1t, q_rings, *kv_rings):
    rings = q_rings + kv_rings
    ring = [[rings[m * 8 + h % 8].at[h // 8] for h in range(H)] for m in range(3)]
    q_r, k_r, v_r = ring

    class x_rows:
        def __init__(self, rows, sem):
            self.copies = [
                pltpu.make_async_copy(x_hbm.at[rows, pl.ds(n * HD, HD)], xs.at[n, rows],
                                      sems.at[sem + n]) for n in range(2)]

        def start(self):
            for c in self.copies:
                c.start()

        def wait(self):
            for c in self.copies:
                c.wait()

    x0_copy = x_rows(pl.ds(0, P0), SEM_X0)

    def x_copy(g):
        return x_rows(pl.ds(_mult(P0 + g * XP, 128), XP), SEM_X + 2 * g)

    def wo_copy(i):
        rows = pl.ds(_mult(i * 512, 512), 512)
        return pltpu.make_async_copy(wo_hbm.bitcast(u32).at[rows], wo_b.at[rows],
                                     sems.at[SEM_WO + i])

    def w1_copy(c):
        return pltpu.make_async_copy(
            w1_hbm.at[:, :, pl.ds(_mult(c * 128, 128), 128)], yt.at[pl.ds(W1_AT + 8 * c, 8)],
            sems.at[SEM_W1 + c])

    def prologue(*stg):

        def start_chunk(g, m, first=False):
            src = w_hbm[m].bitcast(u32)
            for pair, par in itertools.product(range(4), range(2)):
                pltpu.make_async_copy(
                    src.at[:, 16 * par + 4 * g + pair, :],
                    stg[m].at[pl.ds((2 * pair + par) * HD, HD)],
                    sems.at[SEM_OUT + pair if first else SEM_W + 3 * g + m]).start()

        def wait_chunk(g, m):
            pltpu.make_async_copy(stg[m], stg[m], sems.at[SEM_W + 3 * g + m]).wait()

        def relayout(g, m, pair, i0, n):
            ev, od = (stg[m][pl.ds(_mult((2 * pair + par) * HD + i0, 8), n), :]
                      for par in range(2))
            h = 8 * g + 2 * pair
            words = wa.bitcast(u32)
            words[m * H + h, pl.ds(i0, n), :] = (ev & jnp.uint32(0xFFFF)) | (od << 16)
            words[m * H + h + 1, pl.ds(i0, n), :] = (ev >> 16) | (od & jnp.uint32(0xFFFF0000))

        def weights(g, m, pair):
            h = m * H + 8 * g + 2 * pair
            for t in range(D // 32 + 1):
                if t < D // 32:
                    for k in range(2):
                        relayout(g, m, pair, D // 4 * k + 8 * t, 8)
                if t > 0:
                    r = 16 * (t - 1)
                    _right_operands(lambda k, n: wa[h + n, pl.ds(HD * k + r, 16), :],
                                    w4t, 28 * m + 7 * pair, r)
                yield

        def norm_rows(r0, n):
            xv = _rows(xs, pl.ds(r0, n)).astype(f32)
            _set_rows(hbuf, pl.ds(r0, n), xv)
            return _ln(xv)

        def later_rows(r0):
            for r in range(0, XP, 16):
                xn = norm_rows(pl.multiple_of(r0 + r, 16), 16)
                for c in range(8):
                    xg[c, pl.ds(pl.multiple_of(HALO + r0 + r, 8), 16), :] = (
                        xn[:, 128 * c:128 * c + 128])
                yield

        x0_copy.start()
        start_chunk(0, 0, first=True)
        start_chunk(0, 1)
        start_chunk(0, 2)
        x_copy(0).start()
        zero = jnp.zeros((HALO, 128), f32)
        for c in range(8):
            xg[c, pl.ds(0, HALO), :] = zero
            xg[c, pl.ds(HALO + S, HALO), :] = zero
        x0_copy.wait()

        @pl.loop(0, P0 // 64)
        def _(i):
            a = [norm_rows(pl.multiple_of(P0 // 2 * k + 32 * i, 32), 32) for k in range(2)]
            for p in range(7):
                v = _enc(ENC_A[p], lambda k, n: a[k][:, HD * n:HD * n + HD])
                for c in range(4):
                    yt[8 * p + 4 * (i // 4) + c, pl.ds(pl.multiple_of(i % 4 * 32, 32), 32), :] = (
                        v[:, 128 * c:128 * c + 128].astype(bf16))

        @pl.loop(0, 4)
        def _(pair):
            both = stg[0].at[pl.ds(pl.multiple_of(pair * D, D), D)]
            pltpu.make_async_copy(both, both, sems.at[SEM_OUT + pair]).wait()
            _run(weights(0, 0, pair))

        def stage(g, m):
            m1 = (m + 1) % 3
            g1 = jnp.minimum(g + (1 if m == 2 else 0), 3)
            if m == 2:
                x_copy(g).wait()

            @pl.when(g < 3)
            def _():
                start_chunk(g + 1, m)
                if m == 2:
                    x_copy(g + 1).start()
            if m == 1:
                pl.when(g > 0)(lambda: wo_copy(g).start())

            @pl.when(g == 3)
            def _():
                if m == 0:
                    wo_copy(0).start()
                if m == 1:
                    for c in range(8):
                        w1_copy(c).start()
            n = 64
            acc = {}

            def dot(pair, r, p):
                res = _dot(
                    _operand(yt, [8 * p + 4 * (r // R) + k for k in range(4)],
                             pl.ds(r % R // 2, n // 2)),
                    _operand(w4t, [28 * m + 7 * pair + p], pl.ds(0, HD // 2)))

                def emit(i, j, v):
                    rings[m * 8 + 2 * pair + j][g, pl.ds(P0 // 2 * i + r, n), :] = v

                return _collect(acc, p, res, emit)

            dots = [functools.partial(dot, pair, r, p) for pair in range(4)
                    for r in range(0, P0 // 2, n) for p in ORDER]
            early = 72
            if m == 2:
                _interleave(dots[:early], functools.partial(_pace, xg, (0,), 8 * (g >> 10)),
                            (later_rows(P0 + g * XP), XP // 16), pieces=4)
            else:
                for d in dots[:early]:
                    d()
            pl.when(3 * g + m < 11)(functools.partial(wait_chunk, g1, m1))
            _interleave(dots[early:], functools.partial(_pace, wa, (3 * H,), 16 * (g >> 10)),
                        (itertools.chain(*[weights(g1, m1, pair) for pair in range(4)]),
                         4 * (D // 32 + 1)), pieces=4)

        @pl.loop(0, 4)
        def _(g):
            for m in range(3):
                stage(g, m)

    pl.run_scoped(
        prologue,
        pltpu.VMEM((8 * D // 2, DH), u32),
        pltpu.VMEM((8 * D // 2, DH), u32),
        pltpu.VMEM((8 * D // 2, DH), u32),
    )
    for i in range(4):
        wo_copy(i).wait()
    for c in range(8):
        w1_copy(c).wait()

    @pl.loop(0, 16)
    def _(i):
        c, q = i >> 2, i & 3
        for r in range(0, 128, 16):
            _right_operands(lambda k, n: yt[W1_AT + 16 * c + 8 * n + 4 * k + q, pl.ds(r, 16), :],
                            w1t, 7 * c, pl.multiple_of(128 * q + r, 16))

    def wrap(r):
        return jnp.where(r >= RING, r - RING, r)

    group = UNROLL * TOK

    def step(i, k, mem, tok, rp, ra, rw):
        ri = lax.broadcasted_iota(jnp.int32, (2 * L, 2 * L), 0)
        ci = lax.broadcasted_iota(jnp.int32, (2 * L, 2 * L), 1)
        same = (ri >= L) == (ci >= L)
        ri, ci = (jnp.where(v >= L, v - L, v) for v in (ri, ci))
        mask = same & ((ri < MEM) | (ri >= ci))
        fill = jnp.where(same, NEG, -jnp.inf)

        lhs = jnp.concatenate([mem, tok], axis=0).astype(bf16)
        rps = [pl.multiple_of(wrap(rp + r // SEG * SEG), SEG) + r % SEG
               for r in range(TOK * k, TOK * (k + 1), 8)]
        ra_ = pl.multiple_of(wrap(ra + SEG * k), SEG)
        rw_ = pl.multiple_of(rw, SEG) + TOK * k

        rb = pl.multiple_of(jnp.maximum(i - 1, 0) * group, SEG)
        if k == 0:
            _left_operands([_ln(_ln(_rows(hbuf, pl.ds(rb + group // 2 * q, group // 2))))
                            for q in range(2)], ubuf, slice(None))
        filled = {}

        def filler(products):
            def emit(q, j, v):
                xg[2 * k + j, pl.ds(HALO + rb + group // 2 * q, group // 2), :] = _gelu(v)

            for p in products:
                _collect(filled, p, _dot(_operand(ubuf, range(4 * p, 4 * p + 4)),
                                         _operand(w1t, [7 * k + p])), emit)

        mem_qkv = {}
        scores = {}
        o_mem = {}
        total = [None]

        def qkv(h):
            res = {}
            for m in range(3):
                r = _dot(lhs, _operand(wa, [m * H + h]))
                for q in range(3):
                    ring[m][h][pl.ds(rps[q], 8), :] = r[8 + 8 * q:16 + 8 * q]
                res[m] = r[:MEM]
            mem_qkv[h] = res

        def both(m, a):
            return jnp.concatenate(
                [v for h in (2 * a, 2 * a + 1)
                 for v in (mem_qkv[h][m], ring[m][h][pl.ds(ra_, SEG), :])],
                axis=0).astype(bf16)

        def qk(a):
            scores[a] = lax.dot_general(both(0, a), both(1, a), (((1,), (1,)), ((), ())),
                                        preferred_element_type=f32)

        def pv(a):
            sc = jnp.where(mask, scores.pop(a) * (DH ** -0.5), fill)
            mx = jnp.max(sc, axis=1, keepdims=True)
            e = jnp.exp(sc - mx)
            den = jnp.sum(e, axis=1, keepdims=True)
            inv = pl.reciprocal(den, approx=True)
            inv = inv * (2.0 - den * inv)
            o = _dot(e.astype(bf16), both(2, a)) * inv
            for q, h in enumerate((2 * a, 2 * a + 1)):
                q_r[h][pl.ds(ra_, SEG), :] = o[q * L + MEM:(q + 1) * L]
                o_mem[h] = o[q * L:q * L + MEM]

        def wo(h):
            lo = jnp.concatenate([o_mem.pop(h), q_r[h][pl.ds(rw_, TOK), :]],
                                 axis=0).astype(bf16)
            r = _dot(lo, _unpack(wo_b[pl.ds(h * DH // 2, DH // 2), :]))
            total[0] = r if total[0] is None else total[0] + r

        npair = H // 2
        for t in range(npair + LAG_WO):
            if t < npair:
                qkv(2 * t)
                qkv(2 * t + 1)
            if 0 <= t - LAG_QK < npair:
                qk(t - LAG_QK)
            if 0 <= t - LAG_PV < npair:
                pv(t - LAG_PV)
            if t == FILL_AT:
                filler(ORDER[:1])
            if t >= LAG_WO:
                wo(2 * (t - LAG_WO))
                wo(2 * (t - LAG_WO) + 1)
        filler(ORDER[1:])

        a = total[0]
        rows = pl.ds(pl.multiple_of(group * i, SEG) + TOK * k, TOK)
        _set_rows(hbuf, rows, _rows(hbuf, rows) + a[MEM:])
        return a[:MEM]

    def steps(i, carry):
        mem, rp, ra, rw = carry
        fetch(i)
        r0 = pl.multiple_of(HALO + P0 + group * i, SEG)
        toks = [jnp.concatenate([xg[c, pl.ds(r0 + TOK * k, TOK), :] for c in range(8)], axis=1)
                for k in range(UNROLL)]
        for k in range(UNROLL):
            mem = step(i, k, mem, toks[k], rp, ra, rw)
        return mem, wrap(rp + group), wrap(ra + UNROLL * SEG), wrap(rw + group)

    carry = lax.fori_loop(
        0, NSEG // UNROLL, steps,
        (mem0_ref[...].astype(f32), jnp.int32(P0), jnp.int32(0), jnp.int32(0)))
    return carry[3] - TOK * NSEG % RING


def _interleave(dots, pace, *work, pieces=8):
    for i, dot in enumerate(dots):
        res = dot()
        k = min(pieces, res.shape[0] // 16)
        for j in range(k):
            pace(res[:res.shape[0] // 16 * (j + 1) // k * 16])
            for gen, n in work:
                for _ in range(n * (i * k + j) // (k * len(dots)),
                               n * (i * k + j + 1) // (k * len(dots))):
                    next(gen)
    for gen, _ in work:
        _run(gen)


def _up_dot(yt, wa, mu, b, j, half, p):
    res = _dot(
        _operand(yt, [98 * b + 2 * p, 98 * b + 2 * p + 1], pl.ds(half * R // 4, R // 4)),
        _operand(wa, [13 * j + p // 4], pl.ds(128 * (p % 4), 128)))
    mu[p, pl.ds(0, R // 2), :] = res
    return res


def _mixer(zero, mu0, wa, xs, w4t, hbuf, yt, wo_b, xg, w1t, q_rings, w2t, ulast, lhs0, lhs1, hs0, hs1, *ybuf):
    lhs, hs = (lhs0, lhs1), (hs0, hs1)

    def encode_w3(g):
        for j, t in itertools.product(range(NJ), range(4)):
            def get(k, n):
                return yt[32 * j + 8 * n + 2 * k + (g >> 1),
                          pl.ds(pl.multiple_of(64 * (g & 1) + 16 * t, 16), 16), :].astype(f32)

            def emit(p, v):
                wa[13 * j + p // 4, pl.ds(pl.multiple_of(C4 * (p % 4) + 64 * g + 16 * t, 16), 16),
                   :] = v.astype(bf16)

            yield from _enc2(ENC_B, get, emit)

    def encode_w4(g):
        c = g >> 1
        for j, t in itertools.product(range(NJ), range(4)):
            r = pl.multiple_of(64 * (g & 1) + 16 * t, 16)

            def get(k, n):
                if 512 * j < S:
                    return xs[c, pl.ds(512 * j + 128 * k + r, 16), pl.ds(128 * n, 128)].astype(f32)
                return yt[32 * NJ + W4T * (2 * n + c) + 4 * j - S // R + k,
                          pl.ds(r, 16), :].astype(f32)

            def emit(p, v):
                w4t[2 * p + c, pl.ds(128 * j + r, 16), :] = v.astype(bf16)

            yield from _enc2(ENC_B, get, emit)

    def encode_w2(g):
        for t, c in itertools.product(range(8), range(4)):
            _right_operands(
                lambda k, n: yt[W2_AT + 8 * (4 * n + c) + 4 * k + g, pl.ds(16 * t, 16), :],
                w2t, 7 * c, pl.multiple_of(128 * g + 16 * t, 16))
            yield

    done = TOK * NSEG
    first = 4 * TOK * (NSEG // 4 - 1)

    def last_wo(g):
        n = 128
        for k, q in enumerate(q_rings):
            for r in range(0, P0, 64):
                lhs0[k, pl.ds(r, 64), :] = q[g, pl.ds((done + r) % RING, 64), :].astype(bf16)

        part = []

        def dot(r, c, k):
            w = wo_b[pl.ds(pl.multiple_of((2 * g + k) * 2 * DH, 2 * DH), 2 * DH),
                     pl.ds(128 * c, 128)]
            res = _dot(_operand(lhs0, range(4 * k, 4 * k + 4), pl.ds(r // 2, n // 2)), _unpack(w))
            if k == 0:
                part.append(res)
            else:
                hbuf[c // 4, pl.ds(done + r, n), pl.ds(128 * (c % 4), 128)] += part.pop() + res
            return res

        _interleave(
            [functools.partial(dot, r, c, k)
             for r in range(0, P0, n) for c in range(8) for k in range(2)],
            lambda res: [_pace(yt, (98 * NB,), zero, res), _pace(xs, (0,), S + zero, res)],
            (encode_w2(g), 32),
            (encode_w4(g), 28 * NJ), (encode_w3(g), 28 * NJ), pieces=8)

    pl.loop(0, H // 8)(last_wo)

    half = (S - first) // 2

    def mixer_norm(r0, n):
        for r in range(r0, r0 + n, 16):
            _left_operands([_ln(_ln(_rows(hbuf, pl.ds(first + half * i + r, 16))))
                            for i in range(2)], ulast, pl.ds(r, 16))
            yield

    def mixer_in(c):
        step = 64
        for r in range(0, half, step):
            n = min(step, half - r)
            acc = {}

            def emit(i, j, v):
                xg[2 * c + j, pl.ds(HALO + first + half * i + r, n), :] = _gelu(v)

            for p in ORDER:
                _collect(acc, p, _dot(
                    _operand(ulast, range(4 * p, 4 * p + 4), pl.ds(r // 2, n // 2)),
                    _operand(w1t, [7 * c + p])), emit)

    def shift(i, dst):
        for r, c in itertools.product(range(0, RB // 2, 16), range(4)):
            a = [[xg[4 * k + c, pl.ds(HALO + (-1, 1, -2, 2)[2 * k + c // 2]
                                      + i * RB + RB // 2 * q + r, 16), :]
                  for k in range(2)] for q in range(2)]
            for p in range(7):
                dst[p, pl.ds(RB // 2 * c + r, 16), :] = _enc(
                    ENC_A[p], lambda q, k: a[q][k]).astype(bf16)
            yield

    def mixer_out(src, dst):
        n = 128
        acc = {}

        def dot(r, c, p):
            words = src.bitcast(u32)
            a = jnp.concatenate([words[p, pl.ds((RB // 2 * k + r) // 2, n // 2), :]
                                 for k in range(4)], axis=1)
            res = _dot(_unpack(a), _operand(w2t, [7 * c + p]))

            def emit(i, j, v):
                dst[pl.ds(RB // 2 * i + r, n), pl.ds(HD * j + 128 * c, 128)] = v

            return _collect(acc, p, res, emit)

        return [functools.partial(dot, r, c, p)
                for r in range(0, RB // 2, n) for c in range(4) for p in ORDER]

    def residual(i, src, dst):
        late = []
        for t in range(0, RB, 8):
            rows = pl.ds(_mult(i * RB + t, 8), 8)
            hv = _rows(hbuf, rows)
            x1 = _ln(hv) + src[pl.ds(t, 8), :]
            late.append((rows, hv + x1, t, _ln(x1)))
            if len(late) > 2 or t == RB - 8:
                for rows, v, t0, y in late[:None if t == RB - 8 else 1]:
                    _set_rows(hbuf, rows, v)
                    dst[pl.ds(t0, 8), :] = y
                del late[0]
            yield

    def up_operands(i, src):
        per = 4 * R // RB
        for t, c in itertools.product(range(0, RB, 64), range(2)):
            def emit(p, v):
                yt[98 * (i // per) + 2 * p + c,
                   pl.ds(_mult(i % per * (RB // 4) + t // 4, 16), 16), :] = v.astype(bf16)

            yield from _enc2(ENC_A, lambda q, k: src[
                pl.ds(t + 16 * q, 16), pl.ds(C4 * k + 128 * c, 128)], emit)

    def job(i, par, extra=None):
        work, paced = [], []
        if not isinstance(i, int) or i + 1 < S // RB:
            work.append((shift(i + 1, lhs[1 - par]), RB // 8))
            paced.append((lhs[1 - par], (7,), zero))
        if extra is None:
            work.append((up_operands(i - 2, ybuf[par]), 14 * RB // 64))
            paced.append((yt, (98 * NB,), zero))
        else:
            work.append((mixer_norm(*extra), extra[1] // 16))
            paced.append((ulast, (0,), half + zero))
        if extra is None or i > 0:
            work.append((residual(i - 1, hs[1 - par], ybuf[1 - par]), RB // 8))
            paced.append((ybuf[1 - par], (), RB + zero))
        pl.loop(zero, 1)(lambda _: _interleave(
            mixer_out(lhs[par], hs[par]), lambda res: [_pace(*p, res) for p in paced], *work,
            pieces=8))

    cut = 240
    _run(shift(0, lhs[0]))
    job(0, 0, (0, cut))
    job(1, 1, (cut, half - cut))
    pl.loop(0, 4)(mixer_in)

    @pl.loop(1, 3)
    def _(i):
        job(2 * i, 0)
        job(2 * i + 1, 1)

    job(6, 0)
    job(7, 1)
    last = S // RB - 1
    _interleave(
        [functools.partial(_up_dot, yt, wa, mu0, 0, 0, 0, p) for p in range(49)],
        lambda res: [_pace(y, (), RB + zero, res) for y in ybuf],
        (up_operands(last - 1, ybuf[0]), 14 * RB // 64),
        (residual(last, hs[1], ybuf[1]), RB // 8), pieces=4)
    _run(up_operands(last, ybuf[1]))


def _mlp(zero, out_hbm, wa, xs, hbuf, w4t, yt, sems, mu0, tt0, tt1, mu1, md):
    tts, mu = (tt0, tt1), (mu0, mu1)
    hr = R // 2

    def out_copy(b, n):
        rows = pl.ds(_mult(b * 4 * R, 4 * R), 4 * R)
        return pltpu.make_async_copy(xs.at[n, rows], out_hbm.at[rows, pl.ds(n * HD, HD)],
                                     sems.at[SEM_OUT + 2 * b + n])

    def up_dot(b, j, half, p):
        return _up_dot(yt, wa, mu[half], b, j, half, p)

    def up_sums(act):
        for half, t in itertools.product(range(2), range(hr // 8)):
            c = {}
            for g in ORDER:
                y = _dec(lambda k: mu[half][7 * g + k, pl.ds(8 * t, 8), :])
                for i1, n1, sign in DEC[g]:
                    for (i0, n0), m in y.items():
                        key = (2 * i1 + i0, 2 * n1 + n0)
                        _accumulate(c, key, m, sign)
                        if LAST[i1, n1] == g:
                            act[half, t, key] = _gelu(c.pop(key))
                yield

    def down_operands(act, tt, j):
        for half, t in itertools.product(range(2), range(hr // 16)):
            def emit(p, v):
                tt[NJ * p + j, pl.ds(half * hr + 16 * t, 16), :] = v.astype(bf16)

            yield from _enc2(ENC_A, lambda q, k: jnp.concatenate(
                [act[half, 2 * t, (q, k)], act[half, 2 * t + 1, (q, k)]], axis=0), emit)

    n_sums = 7 * 2 * (hr // 8)

    def up_vector_work(tt, j, lag):
        act = {}
        a, b = up_sums(act), down_operands(act, tt, j)
        for i in range(n_sums + lag):
            if i < n_sums:
                next(a)
            if i >= lag and (i - lag) % 2 == 1:
                next(b)
            yield

    part = []

    def down_dot(tt, g, slot, i, lo, hi):
        p = 7 * g + i // 2
        res = _dot(_operand(tt, [NJ * p + q for q in range(lo, hi)]),
                   _operand(w4t, [14 * g + i], pl.ds(64 * lo, 64 * (hi - lo))))
        if hi < NJ:
            part.append(res)
        else:
            md[7 * slot + i // 2, :, pl.ds(128 * (i % 2), 128)] = part.pop() + res if lo else res
        return res

    def down_block(slot, t):
        c = _dec(lambda k: md[7 * slot + k, pl.ds(16 * t, 16), :])
        return jnp.concatenate(
            [jnp.concatenate([c[i0, 0], c[i0, 1]], axis=1) for i0 in range(2)], axis=0)

    def down_sums(b, g, slot):
        dst = []
        for w in range(2):
            i1 = n1 = sign = 0
            for q in range(7):
                e = DEC[q][w] if w < len(DEC[q]) else DEC[q][0][:2] + (0,)
                i1, n1, sign = (jnp.where(g == q, new, old)
                                for new, old in zip(e, (i1, n1, sign)))
            dst.append((b * 4 * R + 32 * i1, n1, sign.astype(f32)))
        for t in range(R // 16):
            m = down_block(slot, t)
            rows = [pl.ds(pl.multiple_of(d[0] + 64 * t, 32), 32) for d in dst]
            new = [hbuf[dst[0][1], rows[0], :] + m,
                   hbuf[dst[1][1], rows[1], :] + dst[1][2] * m]
            for w in (1, 0):
                hbuf[dst[w][1], rows[w], :] = new[w]
                xs[dst[w][1], rows[w], :] = new[w].astype(bf16)
            yield

    def step(b, par, up, down, j):
        slot = (7 * b + j) & 1
        lag, ahead = (15, 4) if down else (16, 2)
        dots = []
        if up:
            nb = jnp.minimum(b + (j + 1) // NJ, NB - 1)
            nj = jnp.where(j == NJ - 1, 0, j + 1)
            dots = ([(1, functools.partial(up_dot, b, j, 1, p)) for p in range(49)]
                    + [(1, functools.partial(up_dot, nb, nj, 0, p)) for p in range(49)])
            up_work = up_vector_work(tts[par], j, lag)
        if down:
            cuts = (0, 4, NJ) if up else (0, NJ)
            for i in reversed(range(14)):
                dots[7 * i + 6:7 * i + 6] = [
                    (hi - lo, functools.partial(down_dot, tts[1 - par], j, slot, i, lo, hi))
                    for lo, hi in zip(cuts, cuts[1:])]
            down_work = down_sums(jnp.maximum(b - 1 - (j == 0), 0),
                                  jnp.where(j == 0, 6, j - 1), 1 - slot)
        total = sum(w for w, _ in dots)
        pos = n_up = done_up = done_down = 0
        for w, dot in dots:
            if down:
                goal = (pos + 14) * (R // 16) * 100 // (105 * total)
                for _ in range(done_down, goal):
                    next(down_work, None)
                done_down = max(done_down, goal)
            res = dot()
            k = min(w, 3)
            for i in range(k * up):
                piece = res[:res.shape[0] * (i + 1) // k]
                if down or n_up % 2 == 0:
                    _pace(mu[done_up >= n_sums // 2], (49,), zero, piece)
                _pace(tts[par], (49 * NJ,), zero, piece)
                goal = (pos * k + w * (i + 1) + ahead * k) * (n_sums + lag) // (total * k)
                goal = (min(goal, n_sums // 2) if n_up + (w == 1) < 49
                        else max(goal, n_sums // 2))
                for _ in range(done_up, goal):
                    next(up_work, None)
                done_up = max(done_up, goal)
            pos += w
            n_up += w == 1
        if up:
            _run(up_work)
        if down:
            _run(down_work)
        if down:
            @pl.when((j == 0) & (b > 1))
            def _():
                for n in range(2):
                    out_copy(b - 2, n).start()

    md[pl.ds(0, 7)] = jnp.zeros((7, R, C4), f32)
    pl.loop(0, NJ)(functools.partial(step, 0, 0, True, False))

    @pl.loop(0, NB // 2)
    def _(i):
        pl.loop(0, NJ)(functools.partial(step, 2 * i + 1, 1, True, True))
        pl.loop(0, jnp.where(2 * i + 2 < NB, NJ, 0))(
            functools.partial(step, 2 * i + 2, 0, True, True))

    pl.loop(0, NJ)(functools.partial(step, NB, 0, False, True))
    out_copy(NB - 1, 1).start()
    pieces = []
    for t in range(R // 16):
        rows = pl.ds(S - 4 * R + 64 * t, 32)
        xs[0, rows, :] = (hbuf[0, rows, :] + down_block((7 * NB + 6) & 1, t)).astype(bf16)
        if t % 2:
            rows = pl.ds(S - 4 * R + 64 * (t - 1), 128)
            pieces.append(pltpu.make_async_copy(
                xs.at[0, rows], out_hbm.at[rows, pl.ds(0, HD)], sems.at[t // 2]))
            pieces[-1].start()
    for b, n in itertools.product(range(NB), range(2)):
        if (b, n) != (NB - 1, 0):
            out_copy(b, n).wait()
    for c in pieces:
        c.wait()


@jax.jit
def pallas_sequential_preLN__memory_aug_recurrent_mem_tr__mixer_s_mlp__prompt_kernel(
    A_x: jax.Array,
    A_mem0: jax.Array,
    A_Wq: jax.Array,
    A_Wk: jax.Array,
    A_Wv: jax.Array,
    A_Wo: jax.Array,
    A_seg_len: jax.Array,
    B_x: jax.Array,
    B_w1: jax.Array,
    B_w2: jax.Array,
    B_w3: jax.Array,
    B_w4: jax.Array,
):
    del A_seg_len, B_x
    hbm = pl.BlockSpec(memory_space=pl.ANY)
    vmem = pl.BlockSpec(memory_space=pltpu.VMEM)
    scratch = [
        pltpu.VMEM((3 * H + 1, D, DH), bf16),
        pltpu.VMEM((2, S + 32, HD), bf16),
        pltpu.VMEM((2, S, HD), f32),
        pltpu.VMEM((98, F // 4, 128), bf16),
        pltpu.VMEM((98 * NB + 1, R, 128), bf16),
        pltpu.VMEM((52, R // 2 + 8, 128), f32),
        pltpu.SemaphoreType.DMA((NSEM,)),
    ]
    out = pl.pallas_call(
        _kernel,
        out_shape=jax.ShapeDtypeStruct((S, D), A_x.dtype),
        in_specs=[hbm, vmem] + [hbm] * 9,
        out_specs=hbm,
        scratch_shapes=scratch,
        compiler_params=pltpu.CompilerParams(
            vmem_limit_bytes=127 * 1024 * 1024,
            flags={"XLA_TPU_EVENLY_DISTRIBUTE_CRITICAL_NODES": True}),
    )(A_x.reshape(S, D), A_mem0.reshape(MEM, D),
      A_Wq.reshape(D // 2, 2 * H, DH), A_Wk.reshape(D // 2, 2 * H, DH),
      A_Wv.reshape(D // 2, 2 * H, DH),
      A_Wo.reshape(H * DH, D), B_w1.reshape(D // R, R, D), B_w2.reshape(D // R, R, D),
      B_w3.reshape(D // R, R, F),
      B_w4.reshape(F // R, R, D), B_w4)
    return out.reshape(A_x.shape)
```

```python
import functools
import itertools

import jax
import jax.numpy as jnp
from jax import lax
import jax.experimental.pallas as pl
import jax.experimental.pallas.tpu as pltpu

S = 2048
D = 1024
H = 32
DH = 128
MEM = 8
SEG = 32
F = 3584
NSEG = S // SEG
L = MEM + SEG
TOK = 24
P0 = S - TOK * NSEG
RING = 576
XP = (S - P0) // 4
C4 = D // 4
HALO = 32
RB = 256
R = 128
NB = S // (4 * R)
NJ = F // 512
HD = D // 2
W1_AT, W2_AT = 64, 320
W4T = (F - S) // R
EPS = 1e-5
NEG = -1000000000.0

LAG_QK, LAG_PV, LAG_WO = 1, 3, 4
FILL_AT = 17
UNROLL = 4

bf16 = jnp.bfloat16
f32 = jnp.float32
u32 = jnp.uint32

SEM_X0, SEM_X, SEM_WO, SEM_W1, SEM_W2, SEM_OUT, SEM_W, SEM_W4, SEM_W3 = (
    0, 2, 10, 14, 22, 30, 38, 50, 66)
NSEM = SEM_W3 + 4 * NJ

ENC_A = (((0, 0, 1), (1, 1, 1)), ((1, 0, 1), (1, 1, 1)), ((0, 0, 1),), ((1, 1, 1),),
         ((0, 0, 1), (0, 1, 1)), ((1, 0, 1), (0, 0, -1)), ((0, 1, 1), (1, 1, -1)))
ENC_B = (((0, 0, 1), (1, 1, 1)), ((0, 0, 1),), ((0, 1, 1), (1, 1, -1)),
         ((1, 0, 1), (0, 0, -1)), ((1, 1, 1),), ((0, 0, 1), (0, 1, 1)),
         ((1, 0, 1), (1, 1, 1)))
DEC = (((0, 0, 1), (1, 1, 1)), ((1, 0, 1), (1, 1, -1)), ((0, 1, 1), (1, 1, 1)),
       ((0, 0, 1), (1, 0, 1)), ((0, 1, 1), (0, 0, -1)), ((1, 1, 1),), ((0, 0, 1),))
ORDER = (0, 1, 3, 2, 4, 5, 6)
LAST = {(1, 0): 3, (0, 1): 4, (1, 1): 5, (0, 0): 6}


def _enc(terms, get):
    v = get(*terms[0][:2])
    for i, j, sign in terms[1:]:
        v = v + get(i, j) if sign > 0 else v - get(i, j)
    return v


def _enc2(table, get, emit):
    for g in range(7):
        y = [[_enc(table[g], lambda i1, j1: get(2 * i1 + i0, 2 * j1 + j0))
              for j0 in range(2)] for i0 in range(2)]
        for k in range(7):
            emit(7 * g + k, _enc(table[k], lambda i0, j0: y[i0][j0]))
        yield


def _right_operands(get, dst, first, row):
    b = [[get(i, j).astype(f32) for j in range(2)] for i in range(2)]
    for p in range(7):
        dst[first + p, pl.ds(row, 16), :] = _enc(ENC_B[p], lambda i, j: b[i][j]).astype(bf16)


def _left_operands(halves, dst, rows):
    for p in range(7):
        v = _enc(ENC_A[p], lambda i, j: halves[i][:, HD * j:HD * j + HD])
        for c in range(4):
            dst[4 * p + c, rows, :] = v[:, 128 * c:128 * c + 128].astype(bf16)


def _collect(acc, p, res, emit):
    for i, j, sign in DEC[p]:
        _accumulate(acc, (i, j), res, sign)
        if LAST[i, j] == p:
            emit(i, j, acc.pop((i, j)))
    return res


def _accumulate(c, key, m, sign):
    c[key] = m if key not in c else (c[key] + m if sign > 0 else c[key] - m)


def _dec(get):
    c = {}
    for k in range(7):
        m = get(k)
        for i, j, sign in DEC[k]:
            _accumulate(c, (i, j), m, sign)
    return c


def _pace(ref, lead, row, result):
    n = 32 // ref.dtype.itemsize
    ref[(*lead, pl.ds(pl.multiple_of(row, n), n), pl.ds(0, 128))] = (
        result[-n:, :128].astype(ref.dtype))


def _run(gen):
    for _ in gen:
        pass


def _mult(i, n):
    return i if isinstance(i, int) else pl.multiple_of(i, n)


def _ln(x):
    m = jnp.mean(x, axis=-1, keepdims=True)
    d = x - m
    v = jnp.mean(d * d, axis=-1, keepdims=True)
    return d * lax.rsqrt(v + EPS)


def _gelu(x):
    c = 0.7978845608028654
    hx = 0.5 * x
    return hx + hx * jnp.tanh(x * (c + (c * 0.044715) * (x * x)))


def _unpack(x):
    return pltpu.bitcast(x, bf16)


def _operand(ref, blocks, rows=slice(None)):
    words = ref.bitcast(u32)
    return _unpack(jnp.concatenate([words[b, rows, :] for b in blocks], axis=1))


def _dot(a, b):
    return jnp.dot(a, b, preferred_element_type=f32)


def _rows(ref, rows):
    return jnp.concatenate([ref[0, rows, :], ref[1, rows, :]], axis=1)


def _set_rows(ref, rows, v):
    ref[0, rows, :] = v[:, :HD]
    ref[1, rows, :] = v[:, HD:]


def _kernel(*refs):
    out_hbm, wa, xs, hbuf, w4t, yt, mu0, sems = refs[11:]
    zero = pl.run_scoped(
        functools.partial(_attention_and_mixer, *refs),
        pltpu.VMEM((H * DH // 2, D), u32),
        pltpu.VMEM((8, S + 2 * HALO, 128), f32),
        pltpu.VMEM((28, 2 * TOK, 128), bf16),
        pltpu.VMEM((28, HD, 128), bf16),
        *[pltpu.VMEM((H // 8, RING, DH), f32)] * 8)
    pl.run_scoped(
        functools.partial(_mlp, zero, out_hbm, wa, xs, hbuf, w4t, yt, sems, mu0),
        *[pltpu.VMEM((49 * NJ + 1, R, 128), bf16)] * 2,
        pltpu.VMEM(mu0.shape, f32),
        pltpu.VMEM((14, R, C4), f32))


def _attention_and_mixer(x_hbm, mem0_ref, wq_hbm, wk_hbm, wv_hbm, wo_hbm, w1_hbm, w2_hbm,
                         w3_hbm, w4_hbm, w4a_hbm, out_hbm, wa, xs, hbuf, w4t, yt, mu0, sems,
                         wo_b, xg, ubuf, w1t, *q_rings):
    def w3_copy(c):
        return pltpu.make_async_copy(
            w3_hbm.at[:, :, pl.ds(_mult(c * 128, 128), 128)], yt.at[pl.ds(8 * c, 8)],
            sems.at[SEM_W3 + c])

    def w4_head_copy(c):
        return pltpu.make_async_copy(
            w4a_hbm.at[pl.ds(0, S), pl.ds(_mult(c * 128, 128), 128)],
            xs.at[c % 2, pl.ds(0, S), pl.ds(_mult(c // 2 * 128, 128), 128)], sems.at[SEM_W4 + c])

    def w4_tail_copy(c):
        return pltpu.make_async_copy(
            w4_hbm.at[pl.ds(S // R, W4T), :, pl.ds(_mult(c * 128, 128), 128)],
            yt.at[pl.ds(32 * NJ + W4T * c, W4T)], sems.at[SEM_W4 + 8 + c])

    def w2_copy(c):
        return pltpu.make_async_copy(
            w2_hbm.at[:, :, pl.ds(_mult(c * 128, 128), 128)], yt.at[pl.ds(W2_AT + 8 * c, 8)],
            sems.at[SEM_W2 + c])

    others = [f(c) for f in (w2_copy, w4_head_copy, w4_tail_copy) for c in range(8)]

    def fetch(i):
        @pl.loop(i, jnp.where(i < 8, i + 1, i))
        def _(c):
            for f in (w2_copy, w4_head_copy, w4_tail_copy):
                f(c).start()

            @pl.when(c < NJ)
            def _():
                for k in range(4):
                    w3_copy(4 * c + k).start()

    zero = pl.run_scoped(
        functools.partial(_attention, x_hbm, mem0_ref, (wq_hbm, wk_hbm, wv_hbm), wo_hbm,
                          w1_hbm, fetch, w4t, yt, wa, xs, hbuf, sems, wo_b, xg, ubuf, w1t, q_rings),
        *[pltpu.VMEM((H // 8, RING, DH), f32)] * 16)
    for c in others:
        c.wait()
    for c in range(4 * NJ):
        w3_copy(c).wait()
    pl.run_scoped(
        functools.partial(_mixer, zero, mu0, wa, xs, w4t, hbuf, yt, wo_b, xg, w1t, q_rings),
        pltpu.VMEM((28, HD, 128), bf16),
        pltpu.VMEM((28, P0 // 2 + 2 * TOK + 16, 128), bf16),
        *[pltpu.VMEM((8, P0, 128), bf16)] * 2, *[pltpu.VMEM((RB, D), f32)] * 2,
        *[pltpu.VMEM((RB + 8, D), f32)] * 2)
    return zero


def _attention(x_hbm, mem0_ref, w_hbm, wo_hbm, w1_hbm, fetch,
               w4t, yt, wa, xs, hbuf, sems, wo_b, xg, ubuf, w1t, q_rings, *kv_rings):
    rings = q_rings + kv_rings
    ring = [[rings[m * 8 + h % 8].at[h // 8] for h in range(H)] for m in range(3)]
    q_r, k_r, v_r = ring

    class x_rows:
        def __init__(self, rows, sem):
            self.copies = [
                pltpu.make_async_copy(x_hbm.at[rows, pl.ds(n * HD, HD)], xs.at[n, rows],
                                      sems.at[sem + n]) for n in range(2)]

        def start(self):
            for c in self.copies:
                c.start()

        def wait(self):
            for c in self.copies:
                c.wait()

    x0_copy = x_rows(pl.ds(0, P0), SEM_X0)

    def x_copy(g):
        return x_rows(pl.ds(_mult(P0 + g * XP, 128), XP), SEM_X + 2 * g)

    def wo_copy(i):
        rows = pl.ds(_mult(i * 512, 512), 512)
        return pltpu.make_async_copy(wo_hbm.bitcast(u32).at[rows], wo_b.at[rows],
                                     sems.at[SEM_WO + i])

    def w1_copy(c):
        return pltpu.make_async_copy(
            w1_hbm.at[:, :, pl.ds(_mult(c * 128, 128), 128)], yt.at[pl.ds(W1_AT + 8 * c, 8)],
            sems.at[SEM_W1 + c])

    def prologue(*stg):

        def start_chunk(g, m, first=False):
            src = w_hbm[m].bitcast(u32)
            for pair, par in itertools.product(range(4), range(2)):
                pltpu.make_async_copy(
                    src.at[:, 16 * par + 4 * g + pair, :],
                    stg[m].at[pl.ds((2 * pair + par) * HD, HD)],
                    sems.at[SEM_OUT + pair if first else SEM_W + 3 * g + m]).start()

        def wait_chunk(g, m):
            pltpu.make_async_copy(stg[m], stg[m], sems.at[SEM_W + 3 * g + m]).wait()

        def relayout(g, m, pair, i0, n):
            ev, od = (stg[m][pl.ds(_mult((2 * pair + par) * HD + i0, 8), n), :]
                      for par in range(2))
            h = 8 * g + 2 * pair
            words = wa.bitcast(u32)
            words[m * H + h, pl.ds(i0, n), :] = (ev & jnp.uint32(0xFFFF)) | (od << 16)
            words[m * H + h + 1, pl.ds(i0, n), :] = (ev >> 16) | (od & jnp.uint32(0xFFFF0000))

        def weights(g, m, pair):
            h = m * H + 8 * g + 2 * pair
            for t in range(D // 32 + 1):
                if t < D // 32:
                    for k in range(2):
                        relayout(g, m, pair, D // 4 * k + 8 * t, 8)
                if t > 0:
                    r = 16 * (t - 1)
                    _right_operands(lambda k, n: wa[h + n, pl.ds(HD * k + r, 16), :],
                                    w4t, 28 * m + 7 * pair, r)
                yield

        def norm_rows(r0, n):
            xv = _rows(xs, pl.ds(r0, n)).astype(f32)
            _set_rows(hbuf, pl.ds(r0, n), xv)
            return _ln(xv)

        def later_rows(r0):
            late = []
            for r in range(0, XP + 16, 16):
                if r < XP:
                    late.append(norm_rows(pl.multiple_of(r0 + r, 16), 16))
                yield
                if r == 0:
                    continue
                xn = late.pop(0)
                for c in range(8):
                    xg[c, pl.ds(pl.multiple_of(HALO + r0 + r - 16, 16), 16), :] = (
                        xn[:, 128 * c:128 * c + 128])
                    if c % 2:
                        yield

        x0_copy.start()
        start_chunk(0, 0, first=True)
        start_chunk(0, 1)
        start_chunk(0, 2)
        x_copy(0).start()
        zero = jnp.zeros((HALO, 128), f32)
        for c in range(8):
            xg[c, pl.ds(0, HALO), :] = zero
            xg[c, pl.ds(HALO + S, HALO), :] = zero
        x0_copy.wait()

        @pl.loop(0, P0 // 64)
        def _(i):
            a = [norm_rows(pl.multiple_of(P0 // 2 * k + 32 * i, 32), 32) for k in range(2)]
            for p in range(7):
                v = _enc(ENC_A[p], lambda k, n: a[k][:, HD * n:HD * n + HD])
                for c in range(4):
                    yt[8 * p + 4 * (i // 4) + c, pl.ds(pl.multiple_of(i % 4 * 32, 32), 32), :] = (
                        v[:, 128 * c:128 * c + 128].astype(bf16))

        @pl.loop(0, 4)
        def _(pair):
            both = stg[0].at[pl.ds(pl.multiple_of(pair * D, D), D)]
            pltpu.make_async_copy(both, both, sems.at[SEM_OUT + pair]).wait()
            _run(weights(0, 0, pair))

        def stage(g, m):
            m1 = (m + 1) % 3
            g1 = jnp.minimum(g + (1 if m == 2 else 0), 3)
            if m == 2:
                x_copy(g).wait()

            @pl.when(g < 3)
            def _():
                start_chunk(g + 1, m)
                if m == 2:
                    x_copy(g + 1).start()
            if m == 1:
                pl.when(g > 0)(lambda: wo_copy(g).start())

            @pl.when(g == 3)
            def _():
                if m == 0:
                    wo_copy(0).start()
                if m == 1:
                    for c in range(8):
                        w1_copy(c).start()
            n = 64
            acc = {}

            def dot(pair, r, p):
                res = _dot(
                    _operand(yt, [8 * p + 4 * (r // R) + k for k in range(4)],
                             pl.ds(r % R // 2, n // 2)),
                    _operand(w4t, [28 * m + 7 * pair + p], pl.ds(0, HD // 2)))

                def emit(i, j, v):
                    rings[m * 8 + 2 * pair + j][g, pl.ds(P0 // 2 * i + r, n), :] = v

                return _collect(acc, p, res, emit)

            dots = [functools.partial(dot, pair, r, p) for pair in range(4)
                    for r in range(0, P0 // 2, n) for p in ORDER]
            early = 72
            if m == 2:
                _interleave(dots[:early], functools.partial(_pace, xg, (0,), 8 * (g >> 10)),
                            (later_rows(P0 + g * XP), 5 * XP // 16 + 1), pieces=4)
            else:
                for d in dots[:early]:
                    d()
            pl.when(3 * g + m < 11)(functools.partial(wait_chunk, g1, m1))
            _interleave(dots[early:], functools.partial(_pace, wa, (3 * H,), 16 * (g >> 10)),
                        (itertools.chain(*[weights(g1, m1, pair) for pair in range(4)]),
                         4 * (D // 32 + 1)), pieces=4)

        @pl.loop(0, 4)
        def _(g):
            for m in range(3):
                stage(g, m)

    pl.run_scoped(
        prologue,
        pltpu.VMEM((8 * D // 2, DH), u32),
        pltpu.VMEM((8 * D // 2, DH), u32),
        pltpu.VMEM((8 * D // 2, DH), u32),
    )
    for i in range(4):
        wo_copy(i).wait()
    for c in range(8):
        w1_copy(c).wait()

    @pl.loop(0, 16)
    def _(i):
        c, q = i >> 2, i & 3
        for r in range(0, 128, 16):
            _right_operands(lambda k, n: yt[W1_AT + 16 * c + 8 * n + 4 * k + q, pl.ds(r, 16), :],
                            w1t, 7 * c, pl.multiple_of(128 * q + r, 16))

    def wrap(r):
        return jnp.where(r >= RING, r - RING, r)

    group = UNROLL * TOK

    def step(i, k, mem, tok, rp, ra, rw):
        ri = lax.broadcasted_iota(jnp.int32, (2 * L, 2 * L), 0)
        ci = lax.broadcasted_iota(jnp.int32, (2 * L, 2 * L), 1)
        same = (ri >= L) == (ci >= L)
        ri, ci = (jnp.where(v >= L, v - L, v) for v in (ri, ci))
        mask = same & ((ri < MEM) | (ri >= ci))
        fill = jnp.where(same, NEG, -jnp.inf)

        lhs = jnp.concatenate([mem, tok], axis=0).astype(bf16)
        rps = [pl.multiple_of(wrap(rp + r // SEG * SEG), SEG) + r % SEG
               for r in range(TOK * k, TOK * (k + 1), 8)]
        ra_ = pl.multiple_of(wrap(ra + SEG * k), SEG)
        rw_ = pl.multiple_of(rw, SEG) + TOK * k

        rb = pl.multiple_of(jnp.maximum(i - 1, 0) * group, SEG)
        if k == 0:
            _left_operands([_ln(_ln(_rows(hbuf, pl.ds(rb + group // 2 * q, group // 2))))
                            for q in range(2)], ubuf, slice(None))
        filled = {}

        def filler(products):
            def emit(q, j, v):
                xg[2 * k + j, pl.ds(HALO + rb + group // 2 * q, group // 2), :] = _gelu(v)

            for p in products:
                _collect(filled, p, _dot(_operand(ubuf, range(4 * p, 4 * p + 4)),
                                         _operand(w1t, [7 * k + p])), emit)

        mem_qkv = {}
        scores = {}
        o_mem = {}
        total = [None]

        def qkv(h):
            res = {}
            for m in range(3):
                r = _dot(lhs, _operand(wa, [m * H + h]))
                for q in range(3):
                    ring[m][h][pl.ds(rps[q], 8), :] = r[8 + 8 * q:16 + 8 * q]
                res[m] = r[:MEM]
            mem_qkv[h] = res

        def both(m, a):
            return jnp.concatenate(
                [v for h in (2 * a, 2 * a + 1)
                 for v in (mem_qkv[h][m], ring[m][h][pl.ds(ra_, SEG), :])],
                axis=0).astype(bf16)

        def qk(a):
            scores[a] = lax.dot_general(both(0, a), both(1, a), (((1,), (1,)), ((), ())),
                                        preferred_element_type=f32)

        def pv(a):
            sc = jnp.where(mask, scores.pop(a) * (DH ** -0.5), fill)
            mx = jnp.max(sc, axis=1, keepdims=True)
            e = jnp.exp(sc - mx)
            den = jnp.sum(e, axis=1, keepdims=True)
            inv = pl.reciprocal(den, approx=True)
            inv = inv * (2.0 - den * inv)
            o = _dot(e.astype(bf16), both(2, a)) * inv
            for q, h in enumerate((2 * a, 2 * a + 1)):
                q_r[h][pl.ds(ra_, SEG), :] = o[q * L + MEM:(q + 1) * L]
                o_mem[h] = o[q * L:q * L + MEM]

        def wo(h):
            lo = jnp.concatenate([o_mem.pop(h), q_r[h][pl.ds(rw_, TOK), :]],
                                 axis=0).astype(bf16)
            r = _dot(lo, _unpack(wo_b[pl.ds(h * DH // 2, DH // 2), :]))
            total[0] = r if total[0] is None else total[0] + r

        npair = H // 2
        for t in range(npair + LAG_WO):
            if t < npair:
                qkv(2 * t)
                qkv(2 * t + 1)
            if 0 <= t - LAG_QK < npair:
                qk(t - LAG_QK)
            if 0 <= t - LAG_PV < npair:
                pv(t - LAG_PV)
            if t == FILL_AT:
                filler(ORDER[:1])
            if t >= LAG_WO:
                wo(2 * (t - LAG_WO))
                wo(2 * (t - LAG_WO) + 1)
        filler(ORDER[1:])

        a = total[0]
        rows = pl.ds(pl.multiple_of(group * i, SEG) + TOK * k, TOK)
        _set_rows(hbuf, rows, _rows(hbuf, rows) + a[MEM:])
        return a[:MEM]

    def steps(i, carry):
        mem, rp, ra, rw = carry
        fetch(i)
        r0 = pl.multiple_of(HALO + P0 + group * i, SEG)
        toks = [jnp.concatenate([xg[c, pl.ds(r0 + TOK * k, TOK), :] for c in range(8)], axis=1)
                for k in range(UNROLL)]
        for k in range(UNROLL):
            mem = step(i, k, mem, toks[k], rp, ra, rw)
        return mem, wrap(rp + group), wrap(ra + UNROLL * SEG), wrap(rw + group)

    carry = lax.fori_loop(
        0, NSEG // UNROLL, steps,
        (mem0_ref[...].astype(f32), jnp.int32(P0), jnp.int32(0), jnp.int32(0)))
    return carry[3] - TOK * NSEG % RING


def _interleave(dots, pace, *work, pieces=8):
    for i, dot in enumerate(dots):
        res = dot()
        k = min(pieces, res.shape[0] // 16)
        for j in range(k):
            pace(res[:res.shape[0] // 16 * (j + 1) // k * 16])
            for gen, n in work:
                for _ in range(n * (i * k + j) // (k * len(dots)),
                               n * (i * k + j + 1) // (k * len(dots))):
                    next(gen)
    for gen, _ in work:
        _run(gen)


def _up_dot(yt, wa, mu, b, j, half, p):
    res = _dot(
        _operand(yt, [98 * b + 2 * p, 98 * b + 2 * p + 1], pl.ds(half * R // 4, R // 4)),
        _operand(wa, [13 * j + p // 4], pl.ds(128 * (p % 4), 128)))
    mu[p, pl.ds(0, R // 2), :] = res
    return res


def _mixer(zero, mu0, wa, xs, w4t, hbuf, yt, wo_b, xg, w1t, q_rings, w2t, ulast, lhs0, lhs1, hs0, hs1, *ybuf):
    lhs, hs = (lhs0, lhs1), (hs0, hs1)

    def encode_w3(g):
        for j, t in itertools.product(range(NJ), range(4)):
            def get(k, n):
                return yt[32 * j + 8 * n + 2 * k + (g >> 1),
                          pl.ds(pl.multiple_of(64 * (g & 1) + 16 * t, 16), 16), :].astype(f32)

            def emit(p, v):
                wa[13 * j + p // 4, pl.ds(pl.multiple_of(C4 * (p % 4) + 64 * g + 16 * t, 16), 16),
                   :] = v.astype(bf16)

            yield from _enc2(ENC_B, get, emit)

    def encode_w4(g):
        c = g >> 1
        for j, t in itertools.product(range(NJ), range(4)):
            r = pl.multiple_of(64 * (g & 1) + 16 * t, 16)

            def get(k, n):
                if 512 * j < S:
                    return xs[c, pl.ds(512 * j + 128 * k + r, 16), pl.ds(128 * n, 128)].astype(f32)
                return yt[32 * NJ + W4T * (2 * n + c) + 4 * j - S // R + k,
                          pl.ds(r, 16), :].astype(f32)

            def emit(p, v):
                w4t[2 * p + c, pl.ds(128 * j + r, 16), :] = v.astype(bf16)

            yield from _enc2(ENC_B, get, emit)

    def encode_w2(g):
        for t, c in itertools.product(range(8), range(4)):
            _right_operands(
                lambda k, n: yt[W2_AT + 8 * (4 * n + c) + 4 * k + g, pl.ds(16 * t, 16), :],
                w2t, 7 * c, pl.multiple_of(128 * g + 16 * t, 16))
            yield

    done = TOK * NSEG
    first = 4 * TOK * (NSEG // 4 - 1)

    def last_wo(g):
        n = 128
        for k, q in enumerate(q_rings):
            for r in range(0, P0, 64):
                lhs0[k, pl.ds(r, 64), :] = q[g, pl.ds((done + r) % RING, 64), :].astype(bf16)

        part = []

        def dot(r, c, k):
            w = wo_b[pl.ds(pl.multiple_of((2 * g + k) * 2 * DH, 2 * DH), 2 * DH),
                     pl.ds(128 * c, 128)]
            res = _dot(_operand(lhs0, range(4 * k, 4 * k + 4), pl.ds(r // 2, n // 2)), _unpack(w))
            if k == 0:
                part.append(res)
            else:
                hbuf[c // 4, pl.ds(done + r, n), pl.ds(128 * (c % 4), 128)] += part.pop() + res
            return res

        _interleave(
            [functools.partial(dot, r, c, k)
             for r in range(0, P0, n) for c in range(8) for k in range(2)],
            lambda res: [_pace(yt, (98 * NB,), zero, res), _pace(xs, (0,), S + zero, res)],
            (encode_w2(g), 32),
            (encode_w4(g), 28 * NJ), (encode_w3(g), 28 * NJ), pieces=8)

    pl.loop(0, H // 8)(last_wo)

    half = (S - first) // 2

    def mixer_norm(r0, n):
        for r in range(r0, r0 + n, 16):
            _left_operands([_ln(_ln(_rows(hbuf, pl.ds(first + half * i + r, 16))))
                            for i in range(2)], ulast, pl.ds(r, 16))
            yield

    def mixer_in(c):
        step = 64
        for r in range(0, half, step):
            n = min(step, half - r)
            acc = {}

            def emit(i, j, v):
                xg[2 * c + j, pl.ds(HALO + first + half * i + r, n), :] = _gelu(v)

            for p in ORDER:
                _collect(acc, p, _dot(
                    _operand(ulast, range(4 * p, 4 * p + 4), pl.ds(r // 2, n // 2)),
                    _operand(w1t, [7 * c + p])), emit)

    def shift(i, dst):
        for r, c in itertools.product(range(0, RB // 2, 16), range(4)):
            a = [[xg[4 * k + c, pl.ds(HALO + (-1, 1, -2, 2)[2 * k + c // 2]
                                      + i * RB + RB // 2 * q + r, 16), :]
                  for k in range(2)] for q in range(2)]
            for p in range(7):
                dst[p, pl.ds(RB // 2 * c + r, 16), :] = _enc(
                    ENC_A[p], lambda q, k: a[q][k]).astype(bf16)
            yield

    def mixer_out(src, dst):
        n = 128
        acc = {}

        def dot(r, c, p):
            words = src.bitcast(u32)
            a = jnp.concatenate([words[p, pl.ds((RB // 2 * k + r) // 2, n // 2), :]
                                 for k in range(4)], axis=1)
            res = _dot(_unpack(a), _operand(w2t, [7 * c + p]))

            def emit(i, j, v):
                dst[pl.ds(RB // 2 * i + r, n), pl.ds(HD * j + 128 * c, 128)] = v

            return _collect(acc, p, res, emit)

        return [functools.partial(dot, r, c, p)
                for r in range(0, RB // 2, n) for c in range(4) for p in ORDER]

    def residual(i, src, dst):
        late = []
        for t in range(0, RB, 8):
            rows = pl.ds(_mult(i * RB + t, 8), 8)
            hv = _rows(hbuf, rows)
            x1 = _ln(hv) + src[pl.ds(t, 8), :]
            late.append((rows, hv + x1, t, _ln(x1)))
            if len(late) > 2 or t == RB - 8:
                for rows, v, t0, y in late[:None if t == RB - 8 else 1]:
                    _set_rows(hbuf, rows, v)
                    dst[pl.ds(t0, 8), :] = y
                del late[0]
            yield

    def up_operands(i, src):
        per = 4 * R // RB
        for t, c in itertools.product(range(0, RB, 64), range(2)):
            def emit(p, v):
                yt[98 * (i // per) + 2 * p + c,
                   pl.ds(_mult(i % per * (RB // 4) + t // 4, 16), 16), :] = v.astype(bf16)

            yield from _enc2(ENC_A, lambda q, k: src[
                pl.ds(t + 16 * q, 16), pl.ds(C4 * k + 128 * c, 128)], emit)

    def job(i, par, extra=None):
        work, paced = [], []
        if not isinstance(i, int) or i + 1 < S // RB:
            work.append((shift(i + 1, lhs[1 - par]), RB // 8))
            paced.append((lhs[1 - par], (7,), zero))
        if extra is None:
            work.append((up_operands(i - 2, ybuf[par]), 14 * RB // 64))
            paced.append((yt, (98 * NB,), zero))
        else:
            work.append((mixer_norm(*extra), extra[1] // 16))
            paced.append((ulast, (0,), half + zero))
        if extra is None or i > 0:
            work.append((residual(i - 1, hs[1 - par], ybuf[1 - par]), RB // 8))
            paced.append((ybuf[1 - par], (), RB + zero))
        pl.loop(zero, 1)(lambda _: _interleave(
            mixer_out(lhs[par], hs[par]), lambda res: [_pace(*p, res) for p in paced], *work,
            pieces=8))

    cut = 240
    _run(shift(0, lhs[0]))
    job(0, 0, (0, cut))
    job(1, 1, (cut, half - cut))
    pl.loop(0, 4)(mixer_in)

    @pl.loop(1, 3)
    def _(i):
        job(2 * i, 0)
        job(2 * i + 1, 1)

    job(6, 0)
    job(7, 1)
    last = S // RB - 1
    _interleave(
        [functools.partial(_up_dot, yt, wa, mu0, 0, 0, 0, p) for p in range(49)],
        lambda res: [_pace(y, (), RB + zero, res) for y in ybuf],
        (up_operands(last - 1, ybuf[0]), 14 * RB // 64),
        (residual(last, hs[1], ybuf[1]), RB // 8), pieces=4)
    _run(up_operands(last, ybuf[1]))


def _mlp(zero, out_hbm, wa, xs, hbuf, w4t, yt, sems, mu0, tt0, tt1, mu1, md):
    tts, mu = (tt0, tt1), (mu0, mu1)
    hr = R // 2

    def out_copy(b, n):
        rows = pl.ds(_mult(b * 4 * R, 4 * R), 4 * R)
        return pltpu.make_async_copy(xs.at[n, rows], out_hbm.at[rows, pl.ds(n * HD, HD)],
                                     sems.at[SEM_OUT + 2 * b + n])

    def up_dot(b, j, half, p):
        return _up_dot(yt, wa, mu[half], b, j, half, p)

    def up_sums(act):
        for half, t in itertools.product(range(2), range(hr // 8)):
            c = {}
            for g in ORDER:
                y = _dec(lambda k: mu[half][7 * g + k, pl.ds(8 * t, 8), :])
                for i1, n1, sign in DEC[g]:
                    for (i0, n0), m in y.items():
                        key = (2 * i1 + i0, 2 * n1 + n0)
                        _accumulate(c, key, m, sign)
                        if LAST[i1, n1] == g:
                            act[half, t, key] = _gelu(c.pop(key))
                yield

    def down_operands(act, tt, j):
        for half, t in itertools.product(range(2), range(hr // 16)):
            def emit(p, v):
                tt[NJ * p + j, pl.ds(half * hr + 16 * t, 16), :] = v.astype(bf16)

            yield from _enc2(ENC_A, lambda q, k: jnp.concatenate(
                [act[half, 2 * t, (q, k)], act[half, 2 * t + 1, (q, k)]], axis=0), emit)

    n_sums = 7 * 2 * (hr // 8)

    def up_vector_work(tt, j, lag):
        act = {}
        a, b = up_sums(act), down_operands(act, tt, j)
        for i in range(n_sums + lag):
            if i < n_sums:
                next(a)
            if i >= lag and (i - lag) % 2 == 1:
                next(b)
            yield

    part = []

    def down_dot(tt, g, slot, i, lo, hi):
        p = 7 * g + i // 2
        res = _dot(_operand(tt, [NJ * p + q for q in range(lo, hi)]),
                   _operand(w4t, [14 * g + i], pl.ds(64 * lo, 64 * (hi - lo))))
        if hi < NJ:
            part.append(res)
        else:
            md[7 * slot + i // 2, :, pl.ds(128 * (i % 2), 128)] = part.pop() + res if lo else res
        return res

    def down_block(slot, t):
        c = _dec(lambda k: md[7 * slot + k, pl.ds(16 * t, 16), :])
        return jnp.concatenate(
            [jnp.concatenate([c[i0, 0], c[i0, 1]], axis=1) for i0 in range(2)], axis=0)

    def down_sums(b, g, slot):
        dst = []
        for w in range(2):
            i1 = n1 = sign = 0
            for q in range(7):
                e = DEC[q][w] if w < len(DEC[q]) else DEC[q][0][:2] + (0,)
                i1, n1, sign = (jnp.where(g == q, new, old)
                                for new, old in zip(e, (i1, n1, sign)))
            dst.append((b * 4 * R + 32 * i1, n1, sign.astype(f32)))
        for t in range(R // 16):
            m = down_block(slot, t)
            rows = [pl.ds(pl.multiple_of(d[0] + 64 * t, 32), 32) for d in dst]
            new = [hbuf[dst[0][1], rows[0], :] + m,
                   hbuf[dst[1][1], rows[1], :] + dst[1][2] * m]
            for w in (1, 0):
                hbuf[dst[w][1], rows[w], :] = new[w]
                xs[dst[w][1], rows[w], :] = new[w].astype(bf16)
            yield

    def step(b, par, up, down, j):
        slot = (7 * b + j) & 1
        lag, ahead = (15, 4) if down else (16, 2)
        dots = []
        if up:
            nb = jnp.minimum(b + (j + 1) // NJ, NB - 1)
            nj = jnp.where(j == NJ - 1, 0, j + 1)
            dots = ([(1, functools.partial(up_dot, b, j, 1, p)) for p in range(49)]
                    + [(1, functools.partial(up_dot, nb, nj, 0, p)) for p in range(49)])
            up_work = up_vector_work(tts[par], j, lag)
        if down:
            cuts = (0, 4, NJ) if up else (0, NJ)
            for i in reversed(range(14)):
                dots[7 * i + 6:7 * i + 6] = [
                    (hi - lo, functools.partial(down_dot, tts[1 - par], j, slot, i, lo, hi))
                    for lo, hi in zip(cuts, cuts[1:])]
            down_work = down_sums(jnp.maximum(b - 1 - (j == 0), 0),
                                  jnp.where(j == 0, 6, j - 1), 1 - slot)
        total = sum(w for w, _ in dots)
        pos = n_up = done_up = done_down = 0
        for w, dot in dots:
            if down:
                goal = (pos + 14) * (R // 16) * 100 // (105 * total)
                for _ in range(done_down, goal):
                    next(down_work, None)
                done_down = max(done_down, goal)
            res = dot()
            k = min(w, 3)
            for i in range(k * up):
                piece = res[:res.shape[0] * (i + 1) // k]
                if down or n_up % 2 == 0:
                    _pace(mu[done_up >= n_sums // 2], (49,), zero, piece)
                _pace(tts[par], (49 * NJ,), zero, piece)
                goal = (pos * k + w * (i + 1) + ahead * k) * (n_sums + lag) // (total * k)
                goal = (min(goal, n_sums // 2) if n_up + (w == 1) < 49
                        else max(goal, n_sums // 2))
                for _ in range(done_up, goal):
                    next(up_work, None)
                done_up = max(done_up, goal)
            pos += w
            n_up += w == 1
        if up:
            _run(up_work)
        if down:
            _run(down_work)
        if down:
            @pl.when((j == 0) & (b > 1))
            def _():
                for n in range(2):
                    out_copy(b - 2, n).start()

    md[pl.ds(0, 7)] = jnp.zeros((7, R, C4), f32)
    pl.loop(0, NJ)(functools.partial(step, 0, 0, True, False))

    @pl.loop(0, NB // 2)
    def _(i):
        pl.loop(0, NJ)(functools.partial(step, 2 * i + 1, 1, True, True))
        pl.loop(0, jnp.where(2 * i + 2 < NB, NJ, 0))(
            functools.partial(step, 2 * i + 2, 0, True, True))

    pl.loop(0, NJ)(functools.partial(step, NB, 0, False, True))
    out_copy(NB - 1, 1).start()
    pieces = []
    for t in range(R // 16):
        rows = pl.ds(S - 4 * R + 64 * t, 32)
        xs[0, rows, :] = (hbuf[0, rows, :] + down_block((7 * NB + 6) & 1, t)).astype(bf16)
        if t % 2:
            rows = pl.ds(S - 4 * R + 64 * (t - 1), 128)
            pieces.append(pltpu.make_async_copy(
                xs.at[0, rows], out_hbm.at[rows, pl.ds(0, HD)], sems.at[t // 2]))
            pieces[-1].start()
    for b, n in itertools.product(range(NB), range(2)):
        if (b, n) != (NB - 1, 0):
            out_copy(b, n).wait()
    for c in pieces:
        c.wait()


@jax.jit
def pallas_sequential_preLN__memory_aug_recurrent_mem_tr__mixer_s_mlp__prompt_kernel(
    A_x: jax.Array,
    A_mem0: jax.Array,
    A_Wq: jax.Array,
    A_Wk: jax.Array,
    A_Wv: jax.Array,
    A_Wo: jax.Array,
    A_seg_len: jax.Array,
    B_x: jax.Array,
    B_w1: jax.Array,
    B_w2: jax.Array,
    B_w3: jax.Array,
    B_w4: jax.Array,
):
    del A_seg_len, B_x
    hbm = pl.BlockSpec(memory_space=pl.ANY)
    vmem = pl.BlockSpec(memory_space=pltpu.VMEM)
    scratch = [
        pltpu.VMEM((3 * H + 1, D, DH), bf16),
        pltpu.VMEM((2, S + 32, HD), bf16),
        pltpu.VMEM((2, S, HD), f32),
        pltpu.VMEM((98, F // 4, 128), bf16),
        pltpu.VMEM((98 * NB + 1, R, 128), bf16),
        pltpu.VMEM((52, R // 2 + 8, 128), f32),
        pltpu.SemaphoreType.DMA((NSEM,)),
    ]
    out = pl.pallas_call(
        _kernel,
        out_shape=jax.ShapeDtypeStruct((S, D), A_x.dtype),
        in_specs=[hbm, vmem] + [hbm] * 9,
        out_specs=hbm,
        scratch_shapes=scratch,
        compiler_params=pltpu.CompilerParams(
            vmem_limit_bytes=127 * 1024 * 1024,
            flags={"XLA_TPU_EVENLY_DISTRIBUTE_CRITICAL_NODES": True}),
    )(A_x.reshape(S, D), A_mem0.reshape(MEM, D),
      A_Wq.reshape(D // 2, 2 * H, DH), A_Wk.reshape(D // 2, 2 * H, DH),
      A_Wv.reshape(D // 2, 2 * H, DH),
      A_Wo.reshape(H * DH, D), B_w1.reshape(D // R, R, D), B_w2.reshape(D // R, R, D),
      B_w3.reshape(D // R, R, F),
      B_w4.reshape(F // R, R, D), B_w4)
    return out.reshape(A_x.shape)
```

```python
import functools
import itertools

import jax
import jax.numpy as jnp
from jax import lax
import jax.experimental.pallas as pl
import jax.experimental.pallas.tpu as pltpu

S = 2048
D = 1024
H = 32
DH = 128
MEM = 8
SEG = 32
F = 3584
NSEG = S // SEG
L = MEM + SEG
TOK = 24
P0 = S - TOK * NSEG
RING = 576
XP = (S - P0) // 4
C4 = D // 4
HALO = 32
RB = 256
R = 128
NB = S // (4 * R)
NJ = F // 512
HD = D // 2
W1_AT, W2_AT = 64, 320
W4T = (F - S) // R
EPS = 1e-5
NEG = -1000000000.0

LAG_QK, LAG_PV, LAG_WO = 1, 3, 4
FILL_AT = 17
UNROLL = 4

bf16 = jnp.bfloat16
f32 = jnp.float32
u32 = jnp.uint32

SEM_X0, SEM_X, SEM_WO, SEM_W1, SEM_W2, SEM_OUT, SEM_W, SEM_W4, SEM_W3 = (
    0, 2, 10, 14, 22, 30, 38, 50, 66)
NSEM = SEM_W3 + 4 * NJ

ENC_A = (((0, 0, 1), (1, 1, 1)), ((1, 0, 1), (1, 1, 1)), ((0, 0, 1),), ((1, 1, 1),),
         ((0, 0, 1), (0, 1, 1)), ((1, 0, 1), (0, 0, -1)), ((0, 1, 1), (1, 1, -1)))
ENC_B = (((0, 0, 1), (1, 1, 1)), ((0, 0, 1),), ((0, 1, 1), (1, 1, -1)),
         ((1, 0, 1), (0, 0, -1)), ((1, 1, 1),), ((0, 0, 1), (0, 1, 1)),
         ((1, 0, 1), (1, 1, 1)))
DEC = (((0, 0, 1), (1, 1, 1)), ((1, 0, 1), (1, 1, -1)), ((0, 1, 1), (1, 1, 1)),
       ((0, 0, 1), (1, 0, 1)), ((0, 1, 1), (0, 0, -1)), ((1, 1, 1),), ((0, 0, 1),))
ORDER = (0, 1, 3, 2, 4, 5, 6)
LAST = {(1, 0): 3, (0, 1): 4, (1, 1): 5, (0, 0): 6}


def _enc(terms, get):
    v = get(*terms[0][:2])
    for i, j, sign in terms[1:]:
        v = v + get(i, j) if sign > 0 else v - get(i, j)
    return v


def _enc2(table, get, emit):
    for g in range(7):
        y = [[_enc(table[g], lambda i1, j1: get(2 * i1 + i0, 2 * j1 + j0))
              for j0 in range(2)] for i0 in range(2)]
        for k in range(7):
            emit(7 * g + k, _enc(table[k], lambda i0, j0: y[i0][j0]))
        yield


def _right_operands(get, dst, first, row):
    b = [[get(i, j).astype(f32) for j in range(2)] for i in range(2)]
    for p in range(7):
        dst[first + p, pl.ds(row, 16), :] = _enc(ENC_B[p], lambda i, j: b[i][j]).astype(bf16)


def _left_operands(halves, dst, rows):
    for p in range(7):
        v = _enc(ENC_A[p], lambda i, j: halves[i][:, HD * j:HD * j + HD])
        for c in range(4):
            dst[4 * p + c, rows, :] = v[:, 128 * c:128 * c + 128].astype(bf16)


def _collect(acc, p, res, emit):
    for i, j, sign in DEC[p]:
        _accumulate(acc, (i, j), res, sign)
        if LAST[i, j] == p:
            emit(i, j, acc.pop((i, j)))
    return res


def _accumulate(c, key, m, sign):
    c[key] = m if key not in c else (c[key] + m if sign > 0 else c[key] - m)


def _dec(get):
    c = {}
    for k in range(7):
        m = get(k)
        for i, j, sign in DEC[k]:
            _accumulate(c, (i, j), m, sign)
    return c


def _pace(ref, lead, row, result):
    n = 32 // ref.dtype.itemsize
    ref[(*lead, pl.ds(pl.multiple_of(row, n), n), pl.ds(0, 128))] = (
        result[-n:, :128].astype(ref.dtype))


def _run(gen):
    for _ in gen:
        pass


def _mult(i, n):
    return i if isinstance(i, int) else pl.multiple_of(i, n)


def _ln(x):
    m = jnp.mean(x, axis=-1, keepdims=True)
    d = x - m
    v = jnp.mean(d * d, axis=-1, keepdims=True)
    return d * lax.rsqrt(v + EPS)


def _gelu(x):
    c = 0.7978845608028654
    hx = 0.5 * x
    return hx + hx * jnp.tanh(x * (c + (c * 0.044715) * (x * x)))


def _unpack(x):
    return pltpu.bitcast(x, bf16)


def _operand(ref, blocks, rows=slice(None)):
    words = ref.bitcast(u32)
    return _unpack(jnp.concatenate([words[b, rows, :] for b in blocks], axis=1))


def _dot(a, b):
    return jnp.dot(a, b, preferred_element_type=f32)


def _rows(ref, rows):
    return jnp.concatenate([ref[0, rows, :], ref[1, rows, :]], axis=1)


def _set_rows(ref, rows, v):
    ref[0, rows, :] = v[:, :HD]
    ref[1, rows, :] = v[:, HD:]


def _kernel(*refs):
    out_hbm, wa, xs, hbuf, w4t, yt, mu0, sems = refs[11:]
    zero = pl.run_scoped(
        functools.partial(_attention_and_mixer, *refs),
        pltpu.VMEM((H * DH // 2, D), u32),
        pltpu.VMEM((8, S + 2 * HALO, 128), f32),
        pltpu.VMEM((28, 2 * TOK, 128), bf16),
        pltpu.VMEM((28, HD, 128), bf16),
        *[pltpu.VMEM((H // 8, RING, DH), f32)] * 8)
    pl.run_scoped(
        functools.partial(_mlp, zero, out_hbm, wa, xs, hbuf, w4t, yt, sems, mu0),
        *[pltpu.VMEM((49 * NJ + 1, R, 128), bf16)] * 2,
        pltpu.VMEM(mu0.shape, f32),
        pltpu.VMEM((14, R, C4), f32))


def _attention_and_mixer(x_hbm, mem0_ref, wq_hbm, wk_hbm, wv_hbm, wo_hbm, w1_hbm, w2_hbm,
                         w3_hbm, w4_hbm, w4a_hbm, out_hbm, wa, xs, hbuf, w4t, yt, mu0, sems,
                         wo_b, xg, ubuf, w1t, *q_rings):
    def w3_copy(c):
        return pltpu.make_async_copy(
            w3_hbm.at[:, :, pl.ds(_mult(c * 128, 128), 128)], yt.at[pl.ds(8 * c, 8)],
            sems.at[SEM_W3 + c])

    def w4_head_copy(c):
        return pltpu.make_async_copy(
            w4a_hbm.at[pl.ds(0, S), pl.ds(_mult(c * 128, 128), 128)],
            xs.at[c % 2, pl.ds(0, S), pl.ds(_mult(c // 2 * 128, 128), 128)], sems.at[SEM_W4 + c])

    def w4_tail_copy(c):
        return pltpu.make_async_copy(
            w4_hbm.at[pl.ds(S // R, W4T), :, pl.ds(_mult(c * 128, 128), 128)],
            yt.at[pl.ds(32 * NJ + W4T * c, W4T)], sems.at[SEM_W4 + 8 + c])

    def w2_copy(c):
        return pltpu.make_async_copy(
            w2_hbm.at[:, :, pl.ds(_mult(c * 128, 128), 128)], yt.at[pl.ds(W2_AT + 8 * c, 8)],
            sems.at[SEM_W2 + c])

    others = [f(c) for f in (w2_copy, w4_head_copy, w4_tail_copy) for c in range(8)]

    def fetch(i):
        @pl.loop(i, jnp.where(i < 8, i + 1, i))
        def _(c):
            for f in (w2_copy, w4_head_copy, w4_tail_copy):
                f(c).start()

            @pl.when(c < NJ)
            def _():
                for k in range(4):
                    w3_copy(4 * c + k).start()

    zero = pl.run_scoped(
        functools.partial(_attention, x_hbm, mem0_ref, (wq_hbm, wk_hbm, wv_hbm), wo_hbm,
                          w1_hbm, fetch, w4t, yt, wa, xs, hbuf, sems, wo_b, xg, ubuf, w1t, q_rings),
        *[pltpu.VMEM((H // 8, RING, DH), f32)] * 16)
    for c in others:
        c.wait()
    for c in range(4 * NJ):
        w3_copy(c).wait()
    pl.run_scoped(
        functools.partial(_mixer, zero, mu0, wa, xs, w4t, hbuf, yt, wo_b, xg, w1t, q_rings),
        pltpu.VMEM((28, HD, 128), bf16),
        pltpu.VMEM((28, P0 // 2 + 2 * TOK + 16, 128), bf16),
        *[pltpu.VMEM((8, P0, 128), bf16)] * 2, *[pltpu.VMEM((RB, D), f32)] * 2,
        *[pltpu.VMEM((RB + 8, D), f32)] * 2)
    return zero


def _attention(x_hbm, mem0_ref, w_hbm, wo_hbm, w1_hbm, fetch,
               w4t, yt, wa, xs, hbuf, sems, wo_b, xg, ubuf, w1t, q_rings, *kv_rings):
    rings = q_rings + kv_rings
    ring = [[rings[m * 8 + h % 8].at[h // 8] for h in range(H)] for m in range(3)]
    q_r, k_r, v_r = ring

    class x_rows:
        def __init__(self, rows, sem):
            self.copies = [
                pltpu.make_async_copy(x_hbm.at[rows, pl.ds(n * HD, HD)], xs.at[n, rows],
                                      sems.at[sem + n]) for n in range(2)]

        def start(self):
            for c in self.copies:
                c.start()

        def wait(self):
            for c in self.copies:
                c.wait()

    x0_copy = x_rows(pl.ds(0, P0), SEM_X0)

    def x_copy(g):
        return x_rows(pl.ds(_mult(P0 + g * XP, 128), XP), SEM_X + 2 * g)

    def wo_copy(i):
        rows = pl.ds(_mult(i * 512, 512), 512)
        return pltpu.make_async_copy(wo_hbm.bitcast(u32).at[rows], wo_b.at[rows],
                                     sems.at[SEM_WO + i])

    def w1_copy(c):
        return pltpu.make_async_copy(
            w1_hbm.at[:, :, pl.ds(_mult(c * 128, 128), 128)], yt.at[pl.ds(W1_AT + 8 * c, 8)],
            sems.at[SEM_W1 + c])

    def prologue(*stg):

        def start_chunk(g, m, first=False):
            src = w_hbm[m].bitcast(u32)
            for pair, par in itertools.product(range(4), range(2)):
                pltpu.make_async_copy(
                    src.at[:, 16 * par + 4 * g + pair, :],
                    stg[m].at[pl.ds((2 * pair + par) * HD, HD)],
                    sems.at[SEM_OUT + pair if first else SEM_W + 3 * g + m]).start()

        def wait_chunk(g, m):
            pltpu.make_async_copy(stg[m], stg[m], sems.at[SEM_W + 3 * g + m]).wait()

        def relayout(g, m, pair, i0, n):
            ev, od = (stg[m][pl.ds(_mult((2 * pair + par) * HD + i0, 8), n), :]
                      for par in range(2))
            h = 8 * g + 2 * pair
            words = wa.bitcast(u32)
            words[m * H + h, pl.ds(i0, n), :] = (ev & jnp.uint32(0xFFFF)) | (od << 16)
            words[m * H + h + 1, pl.ds(i0, n), :] = (ev >> 16) | (od & jnp.uint32(0xFFFF0000))

        def weights(g, m, pair):
            h = m * H + 8 * g + 2 * pair
            for t in range(D // 32 + 1):
                if t < D // 32:
                    for k in range(2):
                        relayout(g, m, pair, D // 4 * k + 8 * t, 8)
                if t > 0:
                    r = 16 * (t - 1)
                    _right_operands(lambda k, n: wa[h + n, pl.ds(HD * k + r, 16), :],
                                    w4t, 28 * m + 7 * pair, r)
                yield

        def norm_rows(r0, n):
            xv = _rows(xs, pl.ds(r0, n)).astype(f32)
            _set_rows(hbuf, pl.ds(r0, n), xv)
            return _ln(xv)

        def later_rows(r0):
            late = []
            for r in range(0, XP + 16, 16):
                if r < XP:
                    late.append(norm_rows(pl.multiple_of(r0 + r, 16), 16))
                yield
                if r == 0:
                    continue
                xn = late.pop(0)
                for c in range(8):
                    xg[c, pl.ds(pl.multiple_of(HALO + r0 + r - 16, 16), 16), :] = (
                        xn[:, 128 * c:128 * c + 128])
                    if c % 2:
                        yield

        x0_copy.start()
        start_chunk(0, 0, first=True)
        start_chunk(0, 1)
        start_chunk(0, 2)
        x_copy(0).start()
        zero = jnp.zeros((HALO, 128), f32)
        for c in range(8):
            xg[c, pl.ds(0, HALO), :] = zero
            xg[c, pl.ds(HALO + S, HALO), :] = zero
        x0_copy.wait()

        @pl.loop(0, P0 // 64)
        def _(i):
            a = [norm_rows(pl.multiple_of(P0 // 2 * k + 32 * i, 32), 32) for k in range(2)]
            for p in range(7):
                v = _enc(ENC_A[p], lambda k, n: a[k][:, HD * n:HD * n + HD])
                for c in range(4):
                    yt[8 * p + 4 * (i // 4) + c, pl.ds(pl.multiple_of(i % 4 * 32, 32), 32), :] = (
                        v[:, 128 * c:128 * c + 128].astype(bf16))

        @pl.loop(0, 4)
        def _(pair):
            both = stg[0].at[pl.ds(pl.multiple_of(pair * D, D), D)]
            pltpu.make_async_copy(both, both, sems.at[SEM_OUT + pair]).wait()
            _run(weights(0, 0, pair))

        def stage(g, m):
            m1 = (m + 1) % 3
            g1 = jnp.minimum(g + (1 if m == 2 else 0), 3)

            def copies():
                pl.when(3 * g + m < 11)(functools.partial(wait_chunk, g1, m1))
                if m == 1:
                    x_copy(g).wait()

                @pl.when(g < 3)
                def _():
                    start_chunk(g + 1, m)
                    if m == 2:
                        x_copy(g + 1).start()

                if m == 0:
                    pl.when(g > 0)(lambda: wo_copy(g).start())

                @pl.when(g == 3)
                def _():
                    if m == 0:
                        wo_copy(0).start()
                    if m == 1:
                        for c in range(8):
                            w1_copy(c).start()

            n = 64
            acc = {}

            def dot(pair, r, p, then=None):
                res = _dot(
                    _operand(yt, [8 * p + 4 * (r // R) + k for k in range(4)],
                             pl.ds(r % R // 2, n // 2)),
                    _operand(w4t, [28 * m + 7 * pair + p], pl.ds(0, HD // 2)))
                if then:
                    then()

                def emit(i, j, v):
                    rings[m * 8 + 2 * pair + j][g, pl.ds(P0 // 2 * i + r, n), :] = v

                return _collect(acc, p, res, emit)

            dots = [functools.partial(dot, pair, r, p) for pair in range(4)
                    for r in range(0, P0 // 2, n) for p in ORDER]
            early = (69, 55, 69)[m]
            dots[early] = functools.partial(dots[early], then=copies)
            if m == 2:
                _interleave(dots[:early], functools.partial(_pace, xg, (0,), 8 * (g >> 10)),
                            (later_rows(P0 + g * XP), 5 * XP // 16 + 1), pieces=4)
            else:
                for d in dots[:early]:
                    d()
            _interleave(dots[early:], functools.partial(_pace, wa, (3 * H,), 16 * (g >> 10)),
                        (itertools.chain(*[weights(g1, m1, pair) for pair in range(4)]),
                         4 * (D // 32 + 1)), pieces=4)

        @pl.loop(0, 4)
        def _(g):
            for m in range(3):
                stage(g, m)

    pl.run_scoped(
        prologue,
        pltpu.VMEM((8 * D // 2, DH), u32),
        pltpu.VMEM((8 * D // 2, DH), u32),
        pltpu.VMEM((8 * D // 2, DH), u32),
    )
    for i in range(4):
        wo_copy(i).wait()
    for c in range(8):
        w1_copy(c).wait()

    @pl.loop(0, 16)
    def _(i):
        c, q = i >> 2, i & 3
        for r in range(0, 128, 16):
            _right_operands(lambda k, n: yt[W1_AT + 16 * c + 8 * n + 4 * k + q, pl.ds(r, 16), :],
                            w1t, 7 * c, pl.multiple_of(128 * q + r, 16))

    def wrap(r):
        return jnp.where(r >= RING, r - RING, r)

    group = UNROLL * TOK

    def step(i, k, mem, tok, rp, ra, rw):
        ri = lax.broadcasted_iota(jnp.int32, (2 * L, 2 * L), 0)
        ci = lax.broadcasted_iota(jnp.int32, (2 * L, 2 * L), 1)
        same = (ri >= L) == (ci >= L)
        ri, ci = (jnp.where(v >= L, v - L, v) for v in (ri, ci))
        mask = same & ((ri < MEM) | (ri >= ci))
        fill = jnp.where(same, NEG, -jnp.inf)

        lhs = jnp.concatenate([mem, tok], axis=0).astype(bf16)
        rps = [pl.multiple_of(wrap(rp + r // SEG * SEG), SEG) + r % SEG
               for r in range(TOK * k, TOK * (k + 1), 8)]
        ra_ = pl.multiple_of(wrap(ra + SEG * k), SEG)
        rw_ = pl.multiple_of(rw, SEG) + TOK * k

        rb = pl.multiple_of(jnp.maximum(i - 1, 0) * group, SEG)
        if k == 0:
            _left_operands([_ln(_ln(_rows(hbuf, pl.ds(rb + group // 2 * q, group // 2))))
                            for q in range(2)], ubuf, slice(None))
        filled = {}

        def filler(products):
            def emit(q, j, v):
                xg[2 * k + j, pl.ds(HALO + rb + group // 2 * q, group // 2), :] = _gelu(v)

            for p in products:
                _collect(filled, p, _dot(_operand(ubuf, range(4 * p, 4 * p + 4)),
                                         _operand(w1t, [7 * k + p])), emit)

        mem_qkv = {}
        scores = {}
        o_mem = {}
        total = [None]

        def qkv(h):
            res = {}
            for m in range(3):
                r = _dot(lhs, _operand(wa, [m * H + h]))
                for q in range(3):
                    ring[m][h][pl.ds(rps[q], 8), :] = r[8 + 8 * q:16 + 8 * q]
                res[m] = r[:MEM]
            mem_qkv[h] = res

        def both(m, a):
            return jnp.concatenate(
                [v for h in (2 * a, 2 * a + 1)
                 for v in (mem_qkv[h][m], ring[m][h][pl.ds(ra_, SEG), :])],
                axis=0).astype(bf16)

        def qk(a):
            scores[a] = lax.dot_general(both(0, a), both(1, a), (((1,), (1,)), ((), ())),
                                        preferred_element_type=f32)

        def pv(a):
            sc = jnp.where(mask, scores.pop(a) * (DH ** -0.5), fill)
            mx = jnp.max(sc, axis=1, keepdims=True)
            e = jnp.exp(sc - mx)
            den = jnp.sum(e, axis=1, keepdims=True)
            inv = pl.reciprocal(den, approx=True)
            inv = inv * (2.0 - den * inv)
            o = _dot(e.astype(bf16), both(2, a)) * inv
            for q, h in enumerate((2 * a, 2 * a + 1)):
                q_r[h][pl.ds(ra_, SEG), :] = o[q * L + MEM:(q + 1) * L]
                o_mem[h] = o[q * L:q * L + MEM]

        def wo(h):
            lo = jnp.concatenate([o_mem.pop(h), q_r[h][pl.ds(rw_, TOK), :]],
                                 axis=0).astype(bf16)
            r = _dot(lo, _unpack(wo_b[pl.ds(h * DH // 2, DH // 2), :]))
            total[0] = r if total[0] is None else total[0] + r

        npair = H // 2
        for t in range(npair + LAG_WO):
            if t < npair:
                qkv(2 * t)
                qkv(2 * t + 1)
            if 0 <= t - LAG_QK < npair:
                qk(t - LAG_QK)
            if 0 <= t - LAG_PV < npair:
                pv(t - LAG_PV)
            if t == FILL_AT:
                filler(ORDER[:1])
            if t >= LAG_WO:
                wo(2 * (t - LAG_WO))
                wo(2 * (t - LAG_WO) + 1)
        filler(ORDER[1:])

        a = total[0]
        rows = pl.ds(pl.multiple_of(group * i, SEG) + TOK * k, TOK)
        _set_rows(hbuf, rows, _rows(hbuf, rows) + a[MEM:])
        return a[:MEM]

    def steps(i, carry):
        mem, rp, ra, rw = carry
        fetch(i)
        r0 = pl.multiple_of(HALO + P0 + group * i, SEG)
        toks = [jnp.concatenate([xg[c, pl.ds(r0 + TOK * k, TOK), :] for c in range(8)], axis=1)
                for k in range(UNROLL)]
        for k in range(UNROLL):
            mem = step(i, k, mem, toks[k], rp, ra, rw)
        return mem, wrap(rp + group), wrap(ra + UNROLL * SEG), wrap(rw + group)

    carry = lax.fori_loop(
        0, NSEG // UNROLL, steps,
        (mem0_ref[...].astype(f32), jnp.int32(P0), jnp.int32(0), jnp.int32(0)))
    return carry[3] - TOK * NSEG % RING


def _interleave(dots, pace, *work, pieces=8):
    for i, dot in enumerate(dots):
        res = dot()
        k = min(pieces, res.shape[0] // 16)
        for j in range(k):
            pace(res[:res.shape[0] // 16 * (j + 1) // k * 16])
            for gen, n in work:
                for _ in range(n * (i * k + j) // (k * len(dots)),
                               n * (i * k + j + 1) // (k * len(dots))):
                    next(gen)
    for gen, _ in work:
        _run(gen)


def _up_dot(yt, wa, mu, b, j, half, p):
    res = _dot(
        _operand(yt, [98 * b + 2 * p, 98 * b + 2 * p + 1], pl.ds(half * R // 4, R // 4)),
        _operand(wa, [13 * j + p // 4], pl.ds(128 * (p % 4), 128)))
    mu[p, pl.ds(0, R // 2), :] = res
    return res


def _mixer(zero, mu0, wa, xs, w4t, hbuf, yt, wo_b, xg, w1t, q_rings, w2t, ulast, lhs0, lhs1, hs0, hs1, *ybuf):
    lhs, hs = (lhs0, lhs1), (hs0, hs1)

    def encode_w3(g):
        for j, t in itertools.product(range(NJ), range(4)):
            def get(k, n):
                return yt[32 * j + 8 * n + 2 * k + (g >> 1),
                          pl.ds(pl.multiple_of(64 * (g & 1) + 16 * t, 16), 16), :].astype(f32)

            def emit(p, v):
                wa[13 * j + p // 4, pl.ds(pl.multiple_of(C4 * (p % 4) + 64 * g + 16 * t, 16), 16),
                   :] = v.astype(bf16)

            yield from _enc2(ENC_B, get, emit)

    def encode_w4(g):
        c = g >> 1
        for j, t in itertools.product(range(NJ), range(4)):
            r = pl.multiple_of(64 * (g & 1) + 16 * t, 16)

            def get(k, n):
                if 512 * j < S:
                    return xs[c, pl.ds(512 * j + 128 * k + r, 16), pl.ds(128 * n, 128)].astype(f32)
                return yt[32 * NJ + W4T * (2 * n + c) + 4 * j - S // R + k,
                          pl.ds(r, 16), :].astype(f32)

            def emit(p, v):
                w4t[2 * p + c, pl.ds(128 * j + r, 16), :] = v.astype(bf16)

            yield from _enc2(ENC_B, get, emit)

    def encode_w2(g):
        for t, c in itertools.product(range(8), range(4)):
            _right_operands(
                lambda k, n: yt[W2_AT + 8 * (4 * n + c) + 4 * k + g, pl.ds(16 * t, 16), :],
                w2t, 7 * c, pl.multiple_of(128 * g + 16 * t, 16))
            yield

    done = TOK * NSEG
    first = 4 * TOK * (NSEG // 4 - 1)

    def last_wo(g):
        n = 128
        for k, q in enumerate(q_rings):
            for r in range(0, P0, 64):
                lhs0[k, pl.ds(r, 64), :] = q[g, pl.ds((done + r) % RING, 64), :].astype(bf16)

        part = []

        def dot(r, c, k):
            w = wo_b[pl.ds(pl.multiple_of((2 * g + k) * 2 * DH, 2 * DH), 2 * DH),
                     pl.ds(128 * c, 128)]
            res = _dot(_operand(lhs0, range(4 * k, 4 * k + 4), pl.ds(r // 2, n // 2)), _unpack(w))
            if k == 0:
                part.append(res)
            else:
                hbuf[c // 4, pl.ds(done + r, n), pl.ds(128 * (c % 4), 128)] += part.pop() + res
            return res

        _interleave(
            [functools.partial(dot, r, c, k)
             for r in range(0, P0, n) for c in range(8) for k in range(2)],
            lambda res: [_pace(yt, (98 * NB,), zero, res), _pace(xs, (0,), S + zero, res)],
            (encode_w2(g), 32),
            (encode_w4(g), 28 * NJ), (encode_w3(g), 28 * NJ), pieces=8)

    pl.loop(0, H // 8)(last_wo)

    half = (S - first) // 2

    def mixer_norm(r0, n):
        for r in range(r0, r0 + n, 16):
            _left_operands([_ln(_ln(_rows(hbuf, pl.ds(first + half * i + r, 16))))
                            for i in range(2)], ulast, pl.ds(r, 16))
            yield

    def mixer_in(c):
        step = 64
        for r in range(0, half, step):
            n = min(step, half - r)
            acc = {}

            def emit(i, j, v):
                xg[2 * c + j, pl.ds(HALO + first + half * i + r, n), :] = _gelu(v)

            for p in ORDER:
                _collect(acc, p, _dot(
                    _operand(ulast, range(4 * p, 4 * p + 4), pl.ds(r // 2, n // 2)),
                    _operand(w1t, [7 * c + p])), emit)

    def shift(i, dst):
        for r, c in itertools.product(range(0, RB // 2, 16), range(4)):
            a = [[xg[4 * k + c, pl.ds(HALO + (-1, 1, -2, 2)[2 * k + c // 2]
                                      + i * RB + RB // 2 * q + r, 16), :]
                  for k in range(2)] for q in range(2)]
            for p in range(7):
                dst[p, pl.ds(RB // 2 * c + r, 16), :] = _enc(
                    ENC_A[p], lambda q, k: a[q][k]).astype(bf16)
            yield

    def mixer_out(src, dst):
        n = 128
        acc = {}

        def dot(r, c, p):
            words = src.bitcast(u32)
            a = jnp.concatenate([words[p, pl.ds((RB // 2 * k + r) // 2, n // 2), :]
                                 for k in range(4)], axis=1)
            res = _dot(_unpack(a), _operand(w2t, [7 * c + p]))

            def emit(i, j, v):
                dst[pl.ds(RB // 2 * i + r, n), pl.ds(HD * j + 128 * c, 128)] = v

            return _collect(acc, p, res, emit)

        return [functools.partial(dot, r, c, p)
                for r in range(0, RB // 2, n) for c in range(4) for p in ORDER]

    def residual(i, src, dst):
        late = []
        for t in range(0, RB, 8):
            rows = pl.ds(_mult(i * RB + t, 8), 8)
            hv = _rows(hbuf, rows)
            x1 = _ln(hv) + src[pl.ds(t, 8), :]
            late.append((rows, hv + x1, t, _ln(x1)))
            if len(late) > 2 or t == RB - 8:
                for rows, v, t0, y in late[:None if t == RB - 8 else 1]:
                    _set_rows(hbuf, rows, v)
                    dst[pl.ds(t0, 8), :] = y
                del late[0]
            yield

    def up_operands(i, src):
        per = 4 * R // RB
        for t, c in itertools.product(range(0, RB, 64), range(2)):
            def emit(p, v):
                yt[98 * (i // per) + 2 * p + c,
                   pl.ds(_mult(i % per * (RB // 4) + t // 4, 16), 16), :] = v.astype(bf16)

            yield from _enc2(ENC_A, lambda q, k: src[
                pl.ds(t + 16 * q, 16), pl.ds(C4 * k + 128 * c, 128)], emit)

    def job(i, par, extra=None):
        work, paced = [], []
        if not isinstance(i, int) or i + 1 < S // RB:
            work.append((shift(i + 1, lhs[1 - par]), RB // 8))
            paced.append((lhs[1 - par], (7,), zero))
        if extra is None:
            work.append((up_operands(i - 2, ybuf[par]), 14 * RB // 64))
            paced.append((yt, (98 * NB,), zero))
        else:
            work.append((mixer_norm(*extra), extra[1] // 16))
            paced.append((ulast, (0,), half + zero))
        if extra is None or i > 0:
            work.append((residual(i - 1, hs[1 - par], ybuf[1 - par]), RB // 8))
            paced.append((ybuf[1 - par], (), RB + zero))
        pl.loop(zero, 1)(lambda _: _interleave(
            mixer_out(lhs[par], hs[par]), lambda res: [_pace(*p, res) for p in paced], *work,
            pieces=8))

    cut = 240
    _run(shift(0, lhs[0]))
    job(0, 0, (0, cut))
    job(1, 1, (cut, half - cut))
    pl.loop(0, 4)(mixer_in)

    @pl.loop(1, 3)
    def _(i):
        job(2 * i, 0)
        job(2 * i + 1, 1)

    job(6, 0)
    job(7, 1)
    last = S // RB - 1
    _interleave(
        [functools.partial(_up_dot, yt, wa, mu0, 0, 0, 0, p) for p in range(49)],
        lambda res: [_pace(y, (), RB + zero, res) for y in ybuf],
        (up_operands(last - 1, ybuf[0]), 14 * RB // 64),
        (residual(last, hs[1], ybuf[1]), RB // 8), pieces=4)
    _run(up_operands(last, ybuf[1]))


def _mlp(zero, out_hbm, wa, xs, hbuf, w4t, yt, sems, mu0, tt0, tt1, mu1, md):
    tts, mu = (tt0, tt1), (mu0, mu1)
    hr = R // 2

    def out_copy(b, n):
        rows = pl.ds(_mult(b * 4 * R, 4 * R), 4 * R)
        return pltpu.make_async_copy(xs.at[n, rows], out_hbm.at[rows, pl.ds(n * HD, HD)],
                                     sems.at[SEM_OUT + 2 * b + n])

    def up_dot(b, j, half, p):
        return _up_dot(yt, wa, mu[half], b, j, half, p)

    def up_sums(act):
        for half, t in itertools.product(range(2), range(hr // 8)):
            c = {}
            for g in ORDER:
                y = _dec(lambda k: mu[half][7 * g + k, pl.ds(8 * t, 8), :])
                for i1, n1, sign in DEC[g]:
                    for (i0, n0), m in y.items():
                        key = (2 * i1 + i0, 2 * n1 + n0)
                        _accumulate(c, key, m, sign)
                        if LAST[i1, n1] == g:
                            act[half, t, key] = _gelu(c.pop(key))
                yield

    def down_operands(act, tt, j):
        for half, t in itertools.product(range(2), range(hr // 16)):
            def emit(p, v):
                tt[NJ * p + j, pl.ds(half * hr + 16 * t, 16), :] = v.astype(bf16)

            yield from _enc2(ENC_A, lambda q, k: jnp.concatenate(
                [act[half, 2 * t, (q, k)], act[half, 2 * t + 1, (q, k)]], axis=0), emit)

    n_sums = 7 * 2 * (hr // 8)

    def up_vector_work(tt, j, lag):
        act = {}
        a, b = up_sums(act), down_operands(act, tt, j)
        for i in range(n_sums + lag):
            if i < n_sums:
                next(a)
            if i >= lag and (i - lag) % 2 == 1:
                next(b)
            yield

    part = []

    def down_dot(tt, g, slot, i, lo, hi):
        p = 7 * g + i // 2
        res = _dot(_operand(tt, [NJ * p + q for q in range(lo, hi)]),
                   _operand(w4t, [14 * g + i], pl.ds(64 * lo, 64 * (hi - lo))))
        if hi < NJ:
            part.append(res)
        else:
            md[7 * slot + i // 2, :, pl.ds(128 * (i % 2), 128)] = part.pop() + res if lo else res
        return res

    def down_block(slot, t):
        c = _dec(lambda k: md[7 * slot + k, pl.ds(16 * t, 16), :])
        return jnp.concatenate(
            [jnp.concatenate([c[i0, 0], c[i0, 1]], axis=1) for i0 in range(2)], axis=0)

    def down_sums(b, g, slot):
        dst = []
        for w in range(2):
            i1 = n1 = sign = 0
            for q in range(7):
                e = DEC[q][w] if w < len(DEC[q]) else DEC[q][0][:2] + (0,)
                i1, n1, sign = (jnp.where(g == q, new, old)
                                for new, old in zip(e, (i1, n1, sign)))
            dst.append((b * 4 * R + 32 * i1, n1, sign.astype(f32)))
        for t in range(R // 16):
            m = down_block(slot, t)
            rows = [pl.ds(pl.multiple_of(d[0] + 64 * t, 32), 32) for d in dst]
            new = [hbuf[dst[0][1], rows[0], :] + m,
                   hbuf[dst[1][1], rows[1], :] + dst[1][2] * m]
            for w in (1, 0):
                hbuf[dst[w][1], rows[w], :] = new[w]
                xs[dst[w][1], rows[w], :] = new[w].astype(bf16)
            yield

    def step(b, par, up, down, j):
        slot = (7 * b + j) & 1
        lag, ahead = (15, 4) if down else (16, 2)
        dots = []
        if up:
            nb = jnp.minimum(b + (j + 1) // NJ, NB - 1)
            nj = jnp.where(j == NJ - 1, 0, j + 1)
            dots = ([(1, functools.partial(up_dot, b, j, 1, p)) for p in range(49)]
                    + [(1, functools.partial(up_dot, nb, nj, 0, p)) for p in range(49)])
            up_work = up_vector_work(tts[par], j, lag)
        if down:
            cuts = (0, 4, NJ) if up else (0, NJ)
            for i in reversed(range(14)):
                dots[7 * i + 6:7 * i + 6] = [
                    (hi - lo, functools.partial(down_dot, tts[1 - par], j, slot, i, lo, hi))
                    for lo, hi in zip(cuts, cuts[1:])]
            down_work = down_sums(jnp.maximum(b - 1 - (j == 0), 0),
                                  jnp.where(j == 0, 6, j - 1), 1 - slot)
        total = sum(w for w, _ in dots)
        pos = n_up = done_up = done_down = 0
        for w, dot in dots:
            if down:
                goal = (pos + 14) * (R // 16) * 100 // (105 * total)
                for _ in range(done_down, goal):
                    next(down_work, None)
                done_down = max(done_down, goal)
            res = dot()
            k = min(w, 3)
            for i in range(k * up):
                piece = res[:res.shape[0] * (i + 1) // k]
                if down or n_up % 2 == 0:
                    _pace(mu[done_up >= n_sums // 2], (49,), zero, piece)
                _pace(tts[par], (49 * NJ,), zero, piece)
                goal = (pos * k + w * (i + 1) + ahead * k) * (n_sums + lag) // (total * k)
                goal = (min(goal, n_sums // 2) if n_up + (w == 1) < 49
                        else max(goal, n_sums // 2))
                for _ in range(done_up, goal):
                    next(up_work, None)
                done_up = max(done_up, goal)
            pos += w
            n_up += w == 1
        if up:
            _run(up_work)
        if down:
            _run(down_work)
        if down:
            @pl.when((j == 0) & (b > 1))
            def _():
                for n in range(2):
                    out_copy(b - 2, n).start()

    md[pl.ds(0, 7)] = jnp.zeros((7, R, C4), f32)
    pl.loop(0, NJ)(functools.partial(step, 0, 0, True, False))

    @pl.loop(0, NB // 2)
    def _(i):
        pl.loop(0, NJ)(functools.partial(step, 2 * i + 1, 1, True, True))
        pl.loop(0, jnp.where(2 * i + 2 < NB, NJ, 0))(
            functools.partial(step, 2 * i + 2, 0, True, True))

    pl.loop(0, NJ)(functools.partial(step, NB, 0, False, True))
    out_copy(NB - 1, 1).start()
    pieces = []
    for t in range(R // 16):
        rows = pl.ds(S - 4 * R + 64 * t, 32)
        xs[0, rows, :] = (hbuf[0, rows, :] + down_block((7 * NB + 6) & 1, t)).astype(bf16)
        if t % 2:
            rows = pl.ds(S - 4 * R + 64 * (t - 1), 128)
            pieces.append(pltpu.make_async_copy(
                xs.at[0, rows], out_hbm.at[rows, pl.ds(0, HD)], sems.at[t // 2]))
            pieces[-1].start()
    for b, n in itertools.product(range(NB), range(2)):
        if (b, n) != (NB - 1, 0):
            out_copy(b, n).wait()
    for c in pieces:
        c.wait()


@jax.jit
def pallas_sequential_preLN__memory_aug_recurrent_mem_tr__mixer_s_mlp__prompt_kernel(
    A_x: jax.Array,
    A_mem0: jax.Array,
    A_Wq: jax.Array,
    A_Wk: jax.Array,
    A_Wv: jax.Array,
    A_Wo: jax.Array,
    A_seg_len: jax.Array,
    B_x: jax.Array,
    B_w1: jax.Array,
    B_w2: jax.Array,
    B_w3: jax.Array,
    B_w4: jax.Array,
):
    del A_seg_len, B_x
    hbm = pl.BlockSpec(memory_space=pl.ANY)
    vmem = pl.BlockSpec(memory_space=pltpu.VMEM)
    scratch = [
        pltpu.VMEM((3 * H + 1, D, DH), bf16),
        pltpu.VMEM((2, S + 32, HD), bf16),
        pltpu.VMEM((2, S, HD), f32),
        pltpu.VMEM((98, F // 4, 128), bf16),
        pltpu.VMEM((98 * NB + 1, R, 128), bf16),
        pltpu.VMEM((52, R // 2 + 8, 128), f32),
        pltpu.SemaphoreType.DMA((NSEM,)),
    ]
    out = pl.pallas_call(
        _kernel,
        out_shape=jax.ShapeDtypeStruct((S, D), A_x.dtype),
        in_specs=[hbm, vmem] + [hbm] * 9,
        out_specs=hbm,
        scratch_shapes=scratch,
        compiler_params=pltpu.CompilerParams(
            vmem_limit_bytes=128 * 1024 * 1024,
            flags={"XLA_TPU_EVENLY_DISTRIBUTE_CRITICAL_NODES": True}),
    )(A_x.reshape(S, D), A_mem0.reshape(MEM, D),
      A_Wq.reshape(D // 2, 2 * H, DH), A_Wk.reshape(D // 2, 2 * H, DH),
      A_Wv.reshape(D // 2, 2 * H, DH),
      A_Wo.reshape(H * DH, D), B_w1.reshape(D // R, R, D), B_w2.reshape(D // R, R, D),
      B_w3.reshape(D // R, R, F),
      B_w4.reshape(F // R, R, D), B_w4)
    return out.reshape(A_x.shape)
```

```python
import functools
import itertools

import jax
import jax.numpy as jnp
from jax import lax
import jax.experimental.pallas as pl
import jax.experimental.pallas.tpu as pltpu

S = 2048
D = 1024
H = 32
DH = 128
MEM = 8
SEG = 32
F = 3584
NSEG = S // SEG
L = MEM + SEG
TOK = 24
P0 = S - TOK * NSEG
RING = 576
XP = (S - P0) // 4
C4 = D // 4
HALO = 32
RB = 256
R = 128
NB = S // (4 * R)
NJ = F // 512
HD = D // 2
W1_AT, W2_AT = 64, 320
W4T = (F - S) // R
EPS = 1e-5
NEG = -1000000000.0

LAG_QK, LAG_PV, LAG_WO = 1, 3, 4
FILL_AT = 17
UNROLL = 4

bf16 = jnp.bfloat16
f32 = jnp.float32
u32 = jnp.uint32

SEM_X0, SEM_X, SEM_WO, SEM_W1, SEM_W2, SEM_OUT, SEM_W, SEM_W4, SEM_W3 = (
    0, 2, 10, 14, 22, 30, 38, 50, 66)
NSEM = SEM_W3 + 4 * NJ

ENC_A = (((0, 0, 1), (1, 1, 1)), ((1, 0, 1), (1, 1, 1)), ((0, 0, 1),), ((1, 1, 1),),
         ((0, 0, 1), (0, 1, 1)), ((1, 0, 1), (0, 0, -1)), ((0, 1, 1), (1, 1, -1)))
ENC_B = (((0, 0, 1), (1, 1, 1)), ((0, 0, 1),), ((0, 1, 1), (1, 1, -1)),
         ((1, 0, 1), (0, 0, -1)), ((1, 1, 1),), ((0, 0, 1), (0, 1, 1)),
         ((1, 0, 1), (1, 1, 1)))
DEC = (((0, 0, 1), (1, 1, 1)), ((1, 0, 1), (1, 1, -1)), ((0, 1, 1), (1, 1, 1)),
       ((0, 0, 1), (1, 0, 1)), ((0, 1, 1), (0, 0, -1)), ((1, 1, 1),), ((0, 0, 1),))
ORDER = (0, 1, 3, 2, 4, 5, 6)
LAST = {(1, 0): 3, (0, 1): 4, (1, 1): 5, (0, 0): 6}


def _enc(terms, get):
    v = get(*terms[0][:2])
    for i, j, sign in terms[1:]:
        v = v + get(i, j) if sign > 0 else v - get(i, j)
    return v


def _enc2(table, get, emit):
    for g in range(7):
        y = [[_enc(table[g], lambda i1, j1: get(2 * i1 + i0, 2 * j1 + j0))
              for j0 in range(2)] for i0 in range(2)]
        for k in range(7):
            emit(7 * g + k, _enc(table[k], lambda i0, j0: y[i0][j0]))
        yield


def _right_operands(get, dst, first, row):
    b = [[get(i, j).astype(f32) for j in range(2)] for i in range(2)]
    for p in range(7):
        dst[first + p, pl.ds(row, 16), :] = _enc(ENC_B[p], lambda i, j: b[i][j]).astype(bf16)


def _left_operands(halves, dst, rows):
    for p in range(7):
        v = _enc(ENC_A[p], lambda i, j: halves[i][:, HD * j:HD * j + HD])
        for c in range(4):
            dst[4 * p + c, rows, :] = v[:, 128 * c:128 * c + 128].astype(bf16)


def _collect(acc, p, res, emit):
    for i, j, sign in DEC[p]:
        _accumulate(acc, (i, j), res, sign)
        if LAST[i, j] == p:
            emit(i, j, acc.pop((i, j)))
    return res


def _accumulate(c, key, m, sign):
    c[key] = m if key not in c else (c[key] + m if sign > 0 else c[key] - m)


def _dec(get):
    c = {}
    for k in range(7):
        m = get(k)
        for i, j, sign in DEC[k]:
            _accumulate(c, (i, j), m, sign)
    return c


def _pace(ref, lead, row, result):
    n = 32 // ref.dtype.itemsize
    ref[(*lead, pl.ds(pl.multiple_of(row, n), n), pl.ds(0, 128))] = (
        result[-n:, :128].astype(ref.dtype))


def _run(gen):
    for _ in gen:
        pass


def _mult(i, n):
    return i if isinstance(i, int) else pl.multiple_of(i, n)


def _ln(x):
    m = jnp.mean(x, axis=-1, keepdims=True)
    d = x - m
    v = jnp.mean(d * d, axis=-1, keepdims=True)
    return d * lax.rsqrt(v + EPS)


def _gelu(x):
    c = 0.7978845608028654
    hx = 0.5 * x
    return hx + hx * jnp.tanh(x * (c + (c * 0.044715) * (x * x)))


def _unpack(x):
    return pltpu.bitcast(x, bf16)


def _operand(ref, blocks, rows=slice(None)):
    words = ref.bitcast(u32)
    return _unpack(jnp.concatenate([words[b, rows, :] for b in blocks], axis=1))


def _dot(a, b):
    return jnp.dot(a, b, preferred_element_type=f32)


def _rows(ref, rows):
    return jnp.concatenate([ref[0, rows, :], ref[1, rows, :]], axis=1)


def _set_rows(ref, rows, v):
    ref[0, rows, :] = v[:, :HD]
    ref[1, rows, :] = v[:, HD:]


def _kernel(*refs):
    out_hbm, wa, xs, hbuf, w4t, yt, mu0, sems = refs[11:]
    zero = pl.run_scoped(
        functools.partial(_attention_and_mixer, *refs),
        pltpu.VMEM((H * DH // 2, D), u32),
        pltpu.VMEM((8, S + 2 * HALO, 128), f32),
        pltpu.VMEM((28, 2 * TOK, 128), bf16),
        pltpu.VMEM((28, HD, 128), bf16),
        *[pltpu.VMEM((H // 8, RING, DH), f32)] * 8)
    pl.run_scoped(
        functools.partial(_mlp, zero, out_hbm, wa, xs, hbuf, w4t, yt, sems, mu0),
        *[pltpu.VMEM((49 * NJ + 1, R, 128), bf16)] * 2,
        pltpu.VMEM(mu0.shape, f32),
        pltpu.VMEM((14, R, C4), f32))


def _attention_and_mixer(x_hbm, mem0_ref, wq_hbm, wk_hbm, wv_hbm, wo_hbm, w1_hbm, w2_hbm,
                         w3_hbm, w4_hbm, w4a_hbm, out_hbm, wa, xs, hbuf, w4t, yt, mu0, sems,
                         wo_b, xg, ubuf, w1t, *q_rings):
    def w3_copy(c):
        return pltpu.make_async_copy(
            w3_hbm.at[:, :, pl.ds(_mult(c * 128, 128), 128)], yt.at[pl.ds(8 * c, 8)],
            sems.at[SEM_W3 + c])

    def w4_head_copy(c):
        return pltpu.make_async_copy(
            w4a_hbm.at[pl.ds(0, S), pl.ds(_mult(c * 128, 128), 128)],
            xs.at[c % 2, pl.ds(0, S), pl.ds(_mult(c // 2 * 128, 128), 128)], sems.at[SEM_W4 + c])

    def w4_tail_copy(c):
        return pltpu.make_async_copy(
            w4_hbm.at[pl.ds(S // R, W4T), :, pl.ds(_mult(c * 128, 128), 128)],
            yt.at[pl.ds(32 * NJ + W4T * c, W4T)], sems.at[SEM_W4 + 8 + c])

    def w2_copy(c):
        return pltpu.make_async_copy(
            w2_hbm.at[:, :, pl.ds(_mult(c * 128, 128), 128)], yt.at[pl.ds(W2_AT + 8 * c, 8)],
            sems.at[SEM_W2 + c])

    others = [f(c) for f in (w2_copy, w4_head_copy, w4_tail_copy) for c in range(8)]

    def fetch(i):
        @pl.loop(i, jnp.where(i < 8, i + 1, i))
        def _(c):
            for f in (w2_copy, w4_head_copy, w4_tail_copy):
                f(c).start()

            @pl.when(c < NJ)
            def _():
                for k in range(4):
                    w3_copy(4 * c + k).start()

    zero = pl.run_scoped(
        functools.partial(_attention, x_hbm, mem0_ref, (wq_hbm, wk_hbm, wv_hbm), wo_hbm,
                          w1_hbm, fetch, w4t, yt, wa, xs, hbuf, sems, wo_b, xg, ubuf, w1t, q_rings),
        *[pltpu.VMEM((H // 8, RING, DH), f32)] * 16)
    for c in others:
        c.wait()
    for c in range(4 * NJ):
        w3_copy(c).wait()
    pl.run_scoped(
        functools.partial(_mixer, zero, mu0, wa, xs, w4t, hbuf, yt, wo_b, xg, w1t, q_rings),
        pltpu.VMEM((28, HD, 128), bf16),
        pltpu.VMEM((28, P0 // 2 + 2 * TOK + 16, 128), bf16),
        *[pltpu.VMEM((8, P0, 128), bf16)] * 2, *[pltpu.VMEM((RB, D), f32)] * 2,
        *[pltpu.VMEM((RB + 8, D), f32)] * 2)
    return zero


def _attention(x_hbm, mem0_ref, w_hbm, wo_hbm, w1_hbm, fetch,
               w4t, yt, wa, xs, hbuf, sems, wo_b, xg, ubuf, w1t, q_rings, *kv_rings):
    rings = q_rings + kv_rings
    ring = [[rings[m * 8 + h % 8].at[h // 8] for h in range(H)] for m in range(3)]
    q_r, k_r, v_r = ring

    class x_rows:
        def __init__(self, rows, sem):
            self.copies = [
                pltpu.make_async_copy(x_hbm.at[rows, pl.ds(n * HD, HD)], xs.at[n, rows],
                                      sems.at[sem + n]) for n in range(2)]

        def start(self):
            for c in self.copies:
                c.start()

        def wait(self):
            for c in self.copies:
                c.wait()

    x0_copy = x_rows(pl.ds(0, P0), SEM_X0)

    def x_copy(g):
        return x_rows(pl.ds(_mult(P0 + g * XP, 128), XP), SEM_X + 2 * g)

    def wo_copy(i):
        rows = pl.ds(_mult(i * 512, 512), 512)
        return pltpu.make_async_copy(wo_hbm.bitcast(u32).at[rows], wo_b.at[rows],
                                     sems.at[SEM_WO + i])

    def w1_copy(c):
        return pltpu.make_async_copy(
            w1_hbm.at[:, :, pl.ds(_mult(c * 128, 128), 128)], yt.at[pl.ds(W1_AT + 8 * c, 8)],
            sems.at[SEM_W1 + c])

    def prologue(*stg):

        def start_chunk(g, m, first=False):
            src = w_hbm[m].bitcast(u32)
            for pair, par in itertools.product(range(4), range(2)):
                pltpu.make_async_copy(
                    src.at[:, 16 * par + 4 * g + pair, :],
                    stg[m].at[pl.ds((2 * pair + par) * HD, HD)],
                    sems.at[SEM_OUT + pair if first else SEM_W + 3 * g + m]).start()

        def wait_chunk(g, m):
            pltpu.make_async_copy(stg[m], stg[m], sems.at[SEM_W + 3 * g + m]).wait()

        def relayout(g, m, pair, i0, n):
            ev, od = (stg[m][pl.ds(_mult((2 * pair + par) * HD + i0, 8), n), :]
                      for par in range(2))
            h = 8 * g + 2 * pair
            words = wa.bitcast(u32)
            words[m * H + h, pl.ds(i0, n), :] = (ev & jnp.uint32(0xFFFF)) | (od << 16)
            words[m * H + h + 1, pl.ds(i0, n), :] = (ev >> 16) | (od & jnp.uint32(0xFFFF0000))

        def weights(g, m, pair):
            h = m * H + 8 * g + 2 * pair
            for t in range(D // 32 + 1):
                if t < D // 32:
                    for k in range(2):
                        relayout(g, m, pair, D // 4 * k + 8 * t, 8)
                if t > 0:
                    r = 16 * (t - 1)
                    _right_operands(lambda k, n: wa[h + n, pl.ds(HD * k + r, 16), :],
                                    w4t, 28 * m + 7 * pair, r)
                yield

        def norm_rows(r0, n):
            xv = _rows(xs, pl.ds(r0, n)).astype(f32)
            _set_rows(hbuf, pl.ds(r0, n), xv)
            return _ln(xv)

        def later_rows(r0):
            late = []
            for r in range(0, XP + 16, 16):
                if r < XP:
                    late.append(norm_rows(pl.multiple_of(r0 + r, 16), 16))
                yield
                if r == 0:
                    continue
                xn = late.pop(0)
                for c in range(8):
                    xg[c, pl.ds(pl.multiple_of(HALO + r0 + r - 16, 16), 16), :] = (
                        xn[:, 128 * c:128 * c + 128])
                    if c % 2:
                        yield

        x0_copy.start()
        start_chunk(0, 0, first=True)
        start_chunk(0, 1)
        start_chunk(0, 2)
        x_copy(0).start()
        zero = jnp.zeros((HALO, 128), f32)
        for c in range(8):
            xg[c, pl.ds(0, HALO), :] = zero
            xg[c, pl.ds(HALO + S, HALO), :] = zero
        x0_copy.wait()

        @pl.loop(0, P0 // 64)
        def _(i):
            a = [norm_rows(pl.multiple_of(P0 // 2 * k + 32 * i, 32), 32) for k in range(2)]
            for p in range(7):
                v = _enc(ENC_A[p], lambda k, n: a[k][:, HD * n:HD * n + HD])
                for c in range(4):
                    yt[8 * p + 4 * (i // 4) + c, pl.ds(pl.multiple_of(i % 4 * 32, 32), 32), :] = (
                        v[:, 128 * c:128 * c + 128].astype(bf16))

        @pl.loop(0, 4)
        def _(pair):
            both = stg[0].at[pl.ds(pl.multiple_of(pair * D, D), D)]
            pltpu.make_async_copy(both, both, sems.at[SEM_OUT + pair]).wait()
            _run(weights(0, 0, pair))

        def stage(g, m):
            m1 = (m + 1) % 3
            g1 = jnp.minimum(g + (1 if m == 2 else 0), 3)

            def copies():
                pl.when(3 * g + m < 11)(functools.partial(wait_chunk, g1, m1))
                if m == 1:
                    x_copy(g).wait()

                @pl.when(g < 3)
                def _():
                    start_chunk(g + 1, m)
                    if m == 2:
                        x_copy(g + 1).start()

                if m == 0:
                    pl.when(g > 0)(lambda: wo_copy(g).start())

                @pl.when(g == 3)
                def _():
                    if m == 0:
                        wo_copy(0).start()
                    if m == 1:
                        for c in range(8):
                            w1_copy(c).start()

            n = 64
            acc = {}

            def dot(pair, r, p, then=None):
                res = _dot(
                    _operand(yt, [8 * p + 4 * (r // R) + k for k in range(4)],
                             pl.ds(r % R // 2, n // 2)),
                    _operand(w4t, [28 * m + 7 * pair + p], pl.ds(0, HD // 2)))
                if then:
                    then()

                def emit(i, j, v):
                    rings[m * 8 + 2 * pair + j][g, pl.ds(P0 // 2 * i + r, n), :] = v

                return _collect(acc, p, res, emit)

            dots = [functools.partial(dot, pair, r, p) for pair in range(4)
                    for r in range(0, P0 // 2, n) for p in ORDER]
            early = (76, 55, 69)[m]
            dots[early] = functools.partial(dots[early], then=copies)
            if m == 2:
                _interleave(dots[:early], functools.partial(_pace, xg, (0,), 8 * (g >> 10)),
                            (later_rows(P0 + g * XP), 5 * XP // 16 + 1), pieces=4)
            else:
                for d in dots[:early]:
                    d()
            _interleave(dots[early:], functools.partial(_pace, wa, (3 * H,), 16 * (g >> 10)),
                        (itertools.chain(*[weights(g1, m1, pair) for pair in range(4)]),
                         4 * (D // 32 + 1)), pieces=4)

        @pl.loop(0, 4)
        def _(g):
            for m in range(3):
                stage(g, m)

    pl.run_scoped(
        prologue,
        pltpu.VMEM((8 * D // 2, DH), u32),
        pltpu.VMEM((8 * D // 2, DH), u32),
        pltpu.VMEM((8 * D // 2, DH), u32),
    )
    for i in range(4):
        wo_copy(i).wait()
    for c in range(8):
        w1_copy(c).wait()

    @pl.loop(0, 16)
    def _(i):
        c, q = i >> 2, i & 3
        for r in range(0, 128, 16):
            _right_operands(lambda k, n: yt[W1_AT + 16 * c + 8 * n + 4 * k + q, pl.ds(r, 16), :],
                            w1t, 7 * c, pl.multiple_of(128 * q + r, 16))

    def wrap(r):
        return jnp.where(r >= RING, r - RING, r)

    group = UNROLL * TOK

    def step(i, k, mem, tok, rp, ra, rw):
        ri = lax.broadcasted_iota(jnp.int32, (2 * L, 2 * L), 0)
        ci = lax.broadcasted_iota(jnp.int32, (2 * L, 2 * L), 1)
        same = (ri >= L) == (ci >= L)
        ri, ci = (jnp.where(v >= L, v - L, v) for v in (ri, ci))
        mask = same & ((ri < MEM) | (ri >= ci))
        fill = jnp.where(same, NEG, -jnp.inf)

        lhs = jnp.concatenate([mem, tok], axis=0).astype(bf16)
        rps = [pl.multiple_of(wrap(rp + r // SEG * SEG), SEG) + r % SEG
               for r in range(TOK * k, TOK * (k + 1), 8)]
        ra_ = pl.multiple_of(wrap(ra + SEG * k), SEG)
        rw_ = pl.multiple_of(rw, SEG) + TOK * k

        rb = pl.multiple_of(jnp.maximum(i - 1, 0) * group, SEG)
        if k == 0:
            _left_operands([_ln(_ln(_rows(hbuf, pl.ds(rb + group // 2 * q, group // 2))))
                            for q in range(2)], ubuf, slice(None))
        filled = {}

        def filler(products):
            def emit(q, j, v):
                xg[2 * k + j, pl.ds(HALO + rb + group // 2 * q, group // 2), :] = _gelu(v)

            for p in products:
                _collect(filled, p, _dot(_operand(ubuf, range(4 * p, 4 * p + 4)),
                                         _operand(w1t, [7 * k + p])), emit)

        mem_qkv = {}
        scores = {}
        o_mem = {}
        total = [None]

        def qkv(h):
            res = {}
            for m in range(3):
                r = _dot(lhs, _operand(wa, [m * H + h]))
                for q in range(3):
                    ring[m][h][pl.ds(rps[q], 8), :] = r[8 + 8 * q:16 + 8 * q]
                res[m] = r[:MEM]
            mem_qkv[h] = res

        def both(m, a):
            return jnp.concatenate(
                [v for h in (2 * a, 2 * a + 1)
                 for v in (mem_qkv[h][m], ring[m][h][pl.ds(ra_, SEG), :])],
                axis=0).astype(bf16)

        def qk(a):
            scores[a] = lax.dot_general(both(0, a), both(1, a), (((1,), (1,)), ((), ())),
                                        preferred_element_type=f32)

        def pv(a):
            sc = jnp.where(mask, scores.pop(a) * (DH ** -0.5), fill)
            mx = jnp.max(sc, axis=1, keepdims=True)
            e = jnp.exp(sc - mx)
            den = jnp.sum(e, axis=1, keepdims=True)
            inv = pl.reciprocal(den, approx=True)
            inv = inv * (2.0 - den * inv)
            o = _dot(e.astype(bf16), both(2, a)) * inv
            for q, h in enumerate((2 * a, 2 * a + 1)):
                q_r[h][pl.ds(ra_, SEG), :] = o[q * L + MEM:(q + 1) * L]
                o_mem[h] = o[q * L:q * L + MEM]

        def wo(h):
            lo = jnp.concatenate([o_mem.pop(h), q_r[h][pl.ds(rw_, TOK), :]],
                                 axis=0).astype(bf16)
            r = _dot(lo, _unpack(wo_b[pl.ds(h * DH // 2, DH // 2), :]))
            total[0] = r if total[0] is None else total[0] + r

        npair = H // 2
        for t in range(npair + LAG_WO):
            if t < npair:
                qkv(2 * t)
                qkv(2 * t + 1)
            if 0 <= t - LAG_QK < npair:
                qk(t - LAG_QK)
            if 0 <= t - LAG_PV < npair:
                pv(t - LAG_PV)
            if t == FILL_AT:
                filler(ORDER[:2])
            if t >= LAG_WO:
                wo(2 * (t - LAG_WO))
                wo(2 * (t - LAG_WO) + 1)
        filler(ORDER[2:])

        a = total[0]
        rows = pl.ds(pl.multiple_of(group * i, SEG) + TOK * k, TOK)
        _set_rows(hbuf, rows, _rows(hbuf, rows) + a[MEM:])
        return a[:MEM]

    def steps(i, carry):
        mem, rp, ra, rw = carry
        fetch(i)
        r0 = pl.multiple_of(HALO + P0 + group * i, SEG)
        toks = [jnp.concatenate([xg[c, pl.ds(r0 + TOK * k, TOK), :] for c in range(8)], axis=1)
                for k in range(UNROLL)]
        for k in range(UNROLL):
            mem = step(i, k, mem, toks[k], rp, ra, rw)
        return mem, wrap(rp + group), wrap(ra + UNROLL * SEG), wrap(rw + group)

    carry = lax.fori_loop(
        0, NSEG // UNROLL, steps,
        (mem0_ref[...].astype(f32), jnp.int32(P0), jnp.int32(0), jnp.int32(0)))
    return carry[3] - TOK * NSEG % RING


def _interleave(dots, pace, *work, pieces=8):
    for i, dot in enumerate(dots):
        res = dot()
        k = min(pieces, res.shape[0] // 16)
        for j in range(k):
            pace(res[:res.shape[0] // 16 * (j + 1) // k * 16])
            for gen, n in work:
                for _ in range(n * (i * k + j) // (k * len(dots)),
                               n * (i * k + j + 1) // (k * len(dots))):
                    next(gen)
    for gen, _ in work:
        _run(gen)


def _up_dot(yt, wa, mu, b, j, half, p):
    res = _dot(
        _operand(yt, [98 * b + 2 * p, 98 * b + 2 * p + 1], pl.ds(half * R // 4, R // 4)),
        _operand(wa, [13 * j + p // 4], pl.ds(128 * (p % 4), 128)))
    mu[p, pl.ds(0, R // 2), :] = res
    return res


def _mixer(zero, mu0, wa, xs, w4t, hbuf, yt, wo_b, xg, w1t, q_rings, w2t, ulast, lhs0, lhs1, hs0, hs1, *ybuf):
    lhs, hs = (lhs0, lhs1), (hs0, hs1)

    def encode_w3(g):
        for j, t in itertools.product(range(NJ), range(4)):
            def get(k, n):
                return yt[32 * j + 8 * n + 2 * k + (g >> 1),
                          pl.ds(pl.multiple_of(64 * (g & 1) + 16 * t, 16), 16), :].astype(f32)

            def emit(p, v):
                wa[13 * j + p // 4, pl.ds(pl.multiple_of(C4 * (p % 4) + 64 * g + 16 * t, 16), 16),
                   :] = v.astype(bf16)

            yield from _enc2(ENC_B, get, emit)

    def encode_w4(g):
        c = g >> 1
        for j, t in itertools.product(range(NJ), range(4)):
            r = pl.multiple_of(64 * (g & 1) + 16 * t, 16)

            def get(k, n):
                if 512 * j < S:
                    return xs[c, pl.ds(512 * j + 128 * k + r, 16), pl.ds(128 * n, 128)].astype(f32)
                return yt[32 * NJ + W4T * (2 * n + c) + 4 * j - S // R + k,
                          pl.ds(r, 16), :].astype(f32)

            def emit(p, v):
                w4t[2 * p + c, pl.ds(128 * j + r, 16), :] = v.astype(bf16)

            yield from _enc2(ENC_B, get, emit)

    def encode_w2(g):
        for t, c in itertools.product(range(8), range(4)):
            _right_operands(
                lambda k, n: yt[W2_AT + 8 * (4 * n + c) + 4 * k + g, pl.ds(16 * t, 16), :],
                w2t, 7 * c, pl.multiple_of(128 * g + 16 * t, 16))
            yield

    done = TOK * NSEG
    first = 4 * TOK * (NSEG // 4 - 1)

    def last_wo(g):
        n = 128
        for k, q in enumerate(q_rings):
            for r in range(0, P0, 64):
                lhs0[k, pl.ds(r, 64), :] = q[g, pl.ds((done + r) % RING, 64), :].astype(bf16)

        part = []

        def dot(r, c, k):
            w = wo_b[pl.ds(pl.multiple_of((2 * g + k) * 2 * DH, 2 * DH), 2 * DH),
                     pl.ds(128 * c, 128)]
            res = _dot(_operand(lhs0, range(4 * k, 4 * k + 4), pl.ds(r // 2, n // 2)), _unpack(w))
            if k == 0:
                part.append(res)
            else:
                hbuf[c // 4, pl.ds(done + r, n), pl.ds(128 * (c % 4), 128)] += part.pop() + res
            return res

        _interleave(
            [functools.partial(dot, r, c, k)
             for r in range(0, P0, n) for c in range(8) for k in range(2)],
            lambda res: [_pace(yt, (98 * NB,), zero, res), _pace(xs, (0,), S + zero, res)],
            (encode_w2(g), 32),
            (encode_w4(g), 28 * NJ), (encode_w3(g), 28 * NJ), pieces=8)

    pl.loop(0, H // 8)(last_wo)

    half = (S - first) // 2

    def mixer_norm(r0, n):
        for r in range(r0, r0 + n, 16):
            _left_operands([_ln(_ln(_rows(hbuf, pl.ds(first + half * i + r, 16))))
                            for i in range(2)], ulast, pl.ds(r, 16))
            yield

    def mixer_in(c):
        step = 64
        for r in range(0, half, step):
            n = min(step, half - r)
            acc = {}

            def emit(i, j, v):
                xg[2 * c + j, pl.ds(HALO + first + half * i + r, n), :] = _gelu(v)

            for p in ORDER:
                _collect(acc, p, _dot(
                    _operand(ulast, range(4 * p, 4 * p + 4), pl.ds(r // 2, n // 2)),
                    _operand(w1t, [7 * c + p])), emit)

    def shift(i, dst):
        for r, c in itertools.product(range(0, RB // 2, 16), range(4)):
            a = [[xg[4 * k + c, pl.ds(HALO + (-1, 1, -2, 2)[2 * k + c // 2]
                                      + i * RB + RB // 2 * q + r, 16), :]
                  for k in range(2)] for q in range(2)]
            for p in range(7):
                dst[p, pl.ds(RB // 2 * c + r, 16), :] = _enc(
                    ENC_A[p], lambda q, k: a[q][k]).astype(bf16)
            yield

    def mixer_out(src, dst):
        n = 128
        acc = {}

        def dot(r, c, p):
            words = src.bitcast(u32)
            a = jnp.concatenate([words[p, pl.ds((RB // 2 * k + r) // 2, n // 2), :]
                                 for k in range(4)], axis=1)
            res = _dot(_unpack(a), _operand(w2t, [7 * c + p]))

            def emit(i, j, v):
                dst[pl.ds(RB // 2 * i + r, n), pl.ds(HD * j + 128 * c, 128)] = v

            return _collect(acc, p, res, emit)

        return [functools.partial(dot, r, c, p)
                for r in range(0, RB // 2, n) for c in range(4) for p in ORDER]

    def residual(i, src, dst):
        late = []
        for t in range(0, RB, 8):
            rows = pl.ds(_mult(i * RB + t, 8), 8)
            hv = _rows(hbuf, rows)
            x1 = _ln(hv) + src[pl.ds(t, 8), :]
            late.append((rows, hv + x1, t, _ln(x1)))
            if len(late) > 2 or t == RB - 8:
                for rows, v, t0, y in late[:None if t == RB - 8 else 1]:
                    _set_rows(hbuf, rows, v)
                    dst[pl.ds(t0, 8), :] = y
                del late[0]
            yield

    def up_operands(i, src):
        per = 4 * R // RB
        for t, c in itertools.product(range(0, RB, 64), range(2)):
            def emit(p, v):
                yt[98 * (i // per) + 2 * p + c,
                   pl.ds(_mult(i % per * (RB // 4) + t // 4, 16), 16), :] = v.astype(bf16)

            yield from _enc2(ENC_A, lambda q, k: src[
                pl.ds(t + 16 * q, 16), pl.ds(C4 * k + 128 * c, 128)], emit)

    def job(i, par, extra=None):
        work, paced = [], []
        if not isinstance(i, int) or i + 1 < S // RB:
            work.append((shift(i + 1, lhs[1 - par]), RB // 8))
            paced.append((lhs[1 - par], (7,), zero))
        if extra is None:
            work.append((up_operands(i - 2, ybuf[par]), 14 * RB // 64))
            paced.append((yt, (98 * NB,), zero))
        else:
            work.append((mixer_norm(*extra), extra[1] // 16))
            paced.append((ulast, (0,), half + zero))
        if extra is None or i > 0:
            work.append((residual(i - 1, hs[1 - par], ybuf[1 - par]), RB // 8))
            paced.append((ybuf[1 - par], (), RB + zero))
        pl.loop(zero, 1)(lambda _: _interleave(
            mixer_out(lhs[par], hs[par]), lambda res: [_pace(*p, res) for p in paced], *work,
            pieces=8))

    cut = 240
    _run(shift(0, lhs[0]))
    job(0, 0, (0, cut))
    job(1, 1, (cut, half - cut))
    pl.loop(0, 4, unroll=4)(mixer_in)

    @pl.loop(1, 3)
    def _(i):
        job(2 * i, 0)
        job(2 * i + 1, 1)

    job(6, 0)
    job(7, 1)
    last = S // RB - 1
    _interleave(
        [functools.partial(_up_dot, yt, wa, mu0, 0, 0, 0, p) for p in range(49)],
        lambda res: [_pace(y, (), RB + zero, res) for y in ybuf],
        (up_operands(last - 1, ybuf[0]), 14 * RB // 64),
        (residual(last, hs[1], ybuf[1]), RB // 8), pieces=4)
    _run(up_operands(last, ybuf[1]))


def _mlp(zero, out_hbm, wa, xs, hbuf, w4t, yt, sems, mu0, tt0, tt1, mu1, md):
    tts, mu = (tt0, tt1), (mu0, mu1)
    hr = R // 2

    def out_copy(b, n):
        rows = pl.ds(_mult(b * 4 * R, 4 * R), 4 * R)
        return pltpu.make_async_copy(xs.at[n, rows], out_hbm.at[rows, pl.ds(n * HD, HD)],
                                     sems.at[SEM_OUT + 2 * b + n])

    def up_dot(b, j, half, p):
        return _up_dot(yt, wa, mu[half], b, j, half, p)

    def up_sums(act):
        for half, t in itertools.product(range(2), range(hr // 8)):
            c = {}
            for g in ORDER:
                y = _dec(lambda k: mu[half][7 * g + k, pl.ds(8 * t, 8), :])
                for i1, n1, sign in DEC[g]:
                    for (i0, n0), m in y.items():
                        key = (2 * i1 + i0, 2 * n1 + n0)
                        _accumulate(c, key, m, sign)
                        if LAST[i1, n1] == g:
                            act[half, t, key] = _gelu(c.pop(key))
                yield

    def down_operands(act, tt, j):
        for half, t in itertools.product(range(2), range(hr // 16)):
            def emit(p, v):
                tt[NJ * p + j, pl.ds(half * hr + 16 * t, 16), :] = v.astype(bf16)

            yield from _enc2(ENC_A, lambda q, k: jnp.concatenate(
                [act[half, 2 * t, (q, k)], act[half, 2 * t + 1, (q, k)]], axis=0), emit)

    n_sums = 7 * 2 * (hr // 8)

    def up_vector_work(tt, j, lag):
        act = {}
        a, b = up_sums(act), down_operands(act, tt, j)
        for i in range(n_sums + lag):
            if i < n_sums:
                next(a)
            if i >= lag and (i - lag) % 2 == 1:
                next(b)
            yield

    part = []

    def down_dot(tt, g, slot, i, lo, hi):
        p = 7 * g + i // 2
        res = _dot(_operand(tt, [NJ * p + q for q in range(lo, hi)]),
                   _operand(w4t, [14 * g + i], pl.ds(64 * lo, 64 * (hi - lo))))
        if hi < NJ:
            part.append(res)
        else:
            md[7 * slot + i // 2, :, pl.ds(128 * (i % 2), 128)] = part.pop() + res if lo else res
        return res

    def down_block(slot, t):
        c = _dec(lambda k: md[7 * slot + k, pl.ds(16 * t, 16), :])
        return jnp.concatenate(
            [jnp.concatenate([c[i0, 0], c[i0, 1]], axis=1) for i0 in range(2)], axis=0)

    def down_sums(b, g, slot):
        dst = []
        for w in range(2):
            i1 = n1 = sign = 0
            for q in range(7):
                e = DEC[q][w] if w < len(DEC[q]) else DEC[q][0][:2] + (0,)
                i1, n1, sign = (jnp.where(g == q, new, old)
                                for new, old in zip(e, (i1, n1, sign)))
            dst.append((b * 4 * R + 32 * i1, n1, sign.astype(f32)))
        for t in range(R // 16):
            m = down_block(slot, t)
            rows = [pl.ds(pl.multiple_of(d[0] + 64 * t, 32), 32) for d in dst]
            new = [hbuf[dst[0][1], rows[0], :] + m,
                   hbuf[dst[1][1], rows[1], :] + dst[1][2] * m]
            for w in (1, 0):
                hbuf[dst[w][1], rows[w], :] = new[w]
                xs[dst[w][1], rows[w], :] = new[w].astype(bf16)
            yield

    def step(b, par, up, down, j):
        slot = (7 * b + j) & 1
        lag, ahead = (15, 4) if down else (16, 2)
        dots = []
        if up:
            nb = jnp.minimum(b + (j + 1) // NJ, NB - 1)
            nj = jnp.where(j == NJ - 1, 0, j + 1)
            dots = ([(1, functools.partial(up_dot, b, j, 1, p)) for p in range(49)]
                    + [(1, functools.partial(up_dot, nb, nj, 0, p)) for p in range(49)])
            up_work = up_vector_work(tts[par], j, lag)
        if down:
            cuts = (0, 4, NJ) if up else (0, NJ)
            for i in reversed(range(14)):
                dots[7 * i + 6:7 * i + 6] = [
                    (hi - lo, functools.partial(down_dot, tts[1 - par], j, slot, i, lo, hi))
                    for lo, hi in zip(cuts, cuts[1:])]
            down_work = down_sums(jnp.maximum(b - 1 - (j == 0), 0),
                                  jnp.where(j == 0, 6, j - 1), 1 - slot)
        total = sum(w for w, _ in dots)
        pos = n_up = done_up = done_down = 0
        for w, dot in dots:
            if down:
                goal = (pos + 14) * (R // 16) * 100 // (105 * total)
                for _ in range(done_down, goal):
                    next(down_work, None)
                done_down = max(done_down, goal)
            res = dot()
            k = min(w, 3)
            for i in range(k * up):
                piece = res[:res.shape[0] * (i + 1) // k]
                if down or n_up % 2 == 0:
                    _pace(mu[done_up >= n_sums // 2], (49,), zero, piece)
                _pace(tts[par], (49 * NJ,), zero, piece)
                goal = (pos * k + w * (i + 1) + ahead * k) * (n_sums + lag) // (total * k)
                goal = (min(goal, n_sums // 2) if n_up + (w == 1) < 49
                        else max(goal, n_sums // 2))
                for _ in range(done_up, goal):
                    next(up_work, None)
                done_up = max(done_up, goal)
            pos += w
            n_up += w == 1
        if up:
            _run(up_work)
        if down:
            _run(down_work)
        if down:
            @pl.when((j == 0) & (b > 1))
            def _():
                for n in range(2):
                    out_copy(b - 2, n).start()

    md[pl.ds(0, 7)] = jnp.zeros((7, R, C4), f32)
    pl.loop(0, NJ)(functools.partial(step, 0, 0, True, False))

    @pl.loop(0, NB // 2)
    def _(i):
        pl.loop(0, NJ)(functools.partial(step, 2 * i + 1, 1, True, True))
        pl.loop(0, jnp.where(2 * i + 2 < NB, NJ, 0))(
            functools.partial(step, 2 * i + 2, 0, True, True))

    pl.loop(0, NJ)(functools.partial(step, NB, 0, False, True))
    out_copy(NB - 1, 1).start()
    pieces = []
    for t in range(R // 16):
        rows = pl.ds(S - 4 * R + 64 * t, 32)
        xs[0, rows, :] = (hbuf[0, rows, :] + down_block((7 * NB + 6) & 1, t)).astype(bf16)
        if t % 2:
            rows = pl.ds(S - 4 * R + 64 * (t - 1), 128)
            pieces.append(pltpu.make_async_copy(
                xs.at[0, rows], out_hbm.at[rows, pl.ds(0, HD)], sems.at[t // 2]))
            pieces[-1].start()
    for b, n in itertools.product(range(NB), range(2)):
        if (b, n) != (NB - 1, 0):
            out_copy(b, n).wait()
    for c in pieces:
        c.wait()


@jax.jit
def pallas_sequential_preLN__memory_aug_recurrent_mem_tr__mixer_s_mlp__prompt_kernel(
    A_x: jax.Array,
    A_mem0: jax.Array,
    A_Wq: jax.Array,
    A_Wk: jax.Array,
    A_Wv: jax.Array,
    A_Wo: jax.Array,
    A_seg_len: jax.Array,
    B_x: jax.Array,
    B_w1: jax.Array,
    B_w2: jax.Array,
    B_w3: jax.Array,
    B_w4: jax.Array,
):
    del A_seg_len, B_x
    hbm = pl.BlockSpec(memory_space=pl.ANY)
    vmem = pl.BlockSpec(memory_space=pltpu.VMEM)
    scratch = [
        pltpu.VMEM((3 * H + 1, D, DH), bf16),
        pltpu.VMEM((2, S + 32, HD), bf16),
        pltpu.VMEM((2, S, HD), f32),
        pltpu.VMEM((98, F // 4, 128), bf16),
        pltpu.VMEM((98 * NB + 1, R, 128), bf16),
        pltpu.VMEM((52, R // 2 + 8, 128), f32),
        pltpu.SemaphoreType.DMA((NSEM,)),
    ]
    out = pl.pallas_call(
        _kernel,
        out_shape=jax.ShapeDtypeStruct((S, D), A_x.dtype),
        in_specs=[hbm, vmem] + [hbm] * 9,
        out_specs=hbm,
        scratch_shapes=scratch,
        compiler_params=pltpu.CompilerParams(
            vmem_limit_bytes=128 * 1024 * 1024,
            flags={"XLA_TPU_EVENLY_DISTRIBUTE_CRITICAL_NODES": True}),
    )(A_x.reshape(S, D), A_mem0.reshape(MEM, D),
      A_Wq.reshape(D // 2, 2 * H, DH), A_Wk.reshape(D // 2, 2 * H, DH),
      A_Wv.reshape(D // 2, 2 * H, DH),
      A_Wo.reshape(H * DH, D), B_w1.reshape(D // R, R, D), B_w2.reshape(D // R, R, D),
      B_w3.reshape(D // R, R, F),
      B_w4.reshape(F // R, R, D), B_w4)
    return out.reshape(A_x.shape)
```
